```python
import jax
import jax.numpy as jnp

def _softmax(x, axis=-1):
    return jax.nn.softmax(x, axis=axis)

def _gelu(x):
    return jax.nn.gelu(x, approximate=True)

def _silu(x):
    return jax.nn.silu(x)

def _sigmoid(x):
    return jax.nn.sigmoid(x)

def _layernorm(x, axis=-1, eps=1e-05):
    m = jnp.mean(x, axis=axis, keepdims=True)
    v = jnp.var(x, axis=axis, keepdims=True)
    return (x - m) / jnp.sqrt(v + eps)

def _scatter_add(tgt, idx, src, axis=0):
    return tgt.at[idx].add(src)

def _segment_sum(src, seg, n):
    return jax.ops.segment_sum(src, seg, n)

class _Rng:

    def __init__(self, key):
        self._k = key

    def _next(self):
        self._k, sub = jax.random.split(self._k)
        return sub

    def normal(self, shape):
        return jax.random.normal(self._next(), shape, dtype=jnp.bfloat16)

    def randint(self, lo, hi, shape):
        return jax.random.randint(self._next(), shape, lo, hi, dtype=jnp.int32)

    def uniform(self, shape, lo=0.0, hi=1.0):
        return jax.random.uniform(self._next(), shape, jnp.bfloat16, lo, hi)

    def permutation(self, n):
        return jax.random.permutation(self._next(), n)
kernel_name = 'adaLN_cond__memory_aug_recurrent_mem_tr__moe_arch_mod__prompt'

def setup_inputs():
    _rng = _Rng(jax.random.key(int.from_bytes(__import__("os").urandom(4), "little")))
    _w = lambda a: (lambda t: t.astype(jnp.bfloat16) if jnp.issubdtype(t.dtype, jnp.floating) else t)(jnp.asarray(a))

    def _A_setup():
        B, S, Dm = (1, 2048, 1024)
        H, Dh = (32, 128)
        M, seg = (8, 32)
        seg = min(seg, S)
        S = S // seg * seg
        return {'x': _w((lambda *s: _rng.normal(s) * 0.05)(B, S, Dm)), 'mem0': _w((lambda *s: _rng.normal(s) * 0.05)(B, M, Dm)), 'Wq': _w((lambda *s: _rng.normal(s) * 0.05)(Dm, H, Dh) * Dm ** (-0.5)), 'Wk': _w((lambda *s: _rng.normal(s) * 0.05)(Dm, H, Dh) * Dm ** (-0.5)), 'Wv': _w((lambda *s: _rng.normal(s) * 0.05)(Dm, H, Dh) * Dm ** (-0.5)), 'Wo': _w((lambda *s: _rng.normal(s) * 0.05)(H, Dh, Dm) * (H * Dh) ** (-0.5)), 'seg_len': seg}
    _A_in = _A_setup()

    def _B_setup():
        B, S, D, F, C = (1, 2048, 1024, 3584, 2)
        return {'x': _w((lambda *s: _rng.normal(s) * 0.05)(B, S, D)), 'w_r': _w((lambda *s: _rng.normal(s) * 0.05)(D)), 'w_gate': _w((lambda *s: _rng.normal(s) * 0.05)(D, F)), 'w_up': _w((lambda *s: _rng.normal(s) * 0.05)(D, F)), 'w_down': _w((lambda *s: _rng.normal(s) * 0.05)(F, D))}
    _B_in = _B_setup()
    return {'A_x': _A_in['x'], 'A_mem0': _A_in['mem0'], 'A_Wq': _A_in['Wq'], 'A_Wk': _A_in['Wk'], 'A_Wv': _A_in['Wv'], 'A_Wo': _A_in['Wo'], 'A_seg_len': _A_in['seg_len'], 'B_x': _B_in['x'], 'B_w_r': _B_in['w_r'], 'B_w_gate': _B_in['w_gate'], 'B_w_up': _B_in['w_up'], 'B_w_down': _B_in['w_down'], 'c': _w((lambda *s: _rng.normal(s) * 0.05)(1, 1024)), 'w_mod': _w((lambda *s: _rng.normal(s) * 0.05)(1024, 6 * 1024) * 1024 ** (-0.5))}

def reference(A_x, A_mem0, A_Wq, A_Wk, A_Wv, A_Wo, A_seg_len, B_x, B_w_r, B_w_gate, B_w_up, B_w_down, c, w_mod):

    def _A_ref(x, mem0, Wq, Wk, Wv, Wo, seg_len):
        B, S, Dm = x.shape
        H, Dh = (Wq.shape[1], Wq.shape[2])
        M = mem0.shape[1]
        scale = Dh ** (-0.5)
        n_seg = S // seg_len
        L = M + seg_len
        idx = jnp.arange(L)
        mask = (idx[:, None] < M) | (idx[:, None] >= idx[None, :])
        mem = mem0
        outs = []
        for s in range(n_seg):
            xs = x[:, s * seg_len:(s + 1) * seg_len, :].copy()
            h = jnp.concatenate([mem, xs], axis=1)
            q = jnp.einsum('btd,dhe->bhte', h, Wq)
            k = jnp.einsum('btd,dhe->bhte', h, Wk)
            v = jnp.einsum('btd,dhe->bhte', h, Wv)
            scores = jnp.einsum('bhqe,bhke->bhqk', q, k) * scale
            scores = jnp.where(mask[None, None], scores, -1000000000.0)
            p = _softmax(scores, axis=-1)
            o = jnp.einsum('bhqk,bhke->bhqe', p, v)
            o = jnp.einsum('bhte,hed->btd', o, Wo)
            mem = o[:, :M, :].copy()
            outs.append(o[:, M:, :])
        return jnp.concatenate(outs, axis=1)

    def _B_ref(x, w_r, w_gate, w_up, w_down):
        B, S, D = x.shape
        C = 2
        r = x @ w_r
        idx = jnp.argsort(-r, axis=-1)[:, :C]
        idx_e = jnp.repeat(idx.reshape(B, C, 1), D, axis=2)
        x_sel = jnp.take_along_axis(x, idx_e, axis=1)
        g = _silu(x_sel @ w_gate)
        u = x_sel @ w_up
        y = g * u @ w_down
        r_sel = _sigmoid(jnp.take_along_axis(r, idx, axis=1))
        y = y * r_sel.reshape(B, C, 1)
        b_off = (jnp.arange(B) * S).reshape(B, 1)
        flat_idx = (idx + b_off).reshape(B * C)
        zero = (x * 0.0).reshape(B * S, D)
        upd = _scatter_add(zero, flat_idx, y.reshape(B * C, D), axis=0)
        return x + upd.reshape(B, S, D)
    x = A_x
    mod = (_silu(c) @ w_mod).reshape(c.shape[0], 6, 1, -1)
    sa, ca, ga, sb, cb, gb = (mod[:, 0].copy(), mod[:, 1].copy(), mod[:, 2].copy(), mod[:, 3].copy(), mod[:, 4].copy(), mod[:, 5].copy())
    h = _layernorm(x, axis=-1) * (1 + ca) + sa
    x = x + ga * _A_ref(h, A_mem0, A_Wq, A_Wk, A_Wv, A_Wo, A_seg_len)
    h = _layernorm(x, axis=-1) * (1 + cb) + sb
    x = x + gb * _B_ref(h, B_w_r, B_w_gate, B_w_up, B_w_down)
    return x
```

```python
import functools

import jax
import jax.numpy as jnp
from jax import lax
import jax.experimental.pallas as pl
import jax.experimental.pallas.tpu as pltpu

F32 = jnp.float32
BF16 = jnp.bfloat16

D = 1024
S = 2048
H = 32
DH = 128
M = 8
SEG = 32
NSEG = S // SEG
FF = 3584
NT = D // 128
XR = 24
R0 = S - XR * NSEG
RING = 576
ROFF = RING - R0
CH = 8
NCHUNK = 3 * H // CH
NSLOT = 4
PR = 2 * SEG + 2 * M
GH = 8
NG = H // GH
EPS = 1e-5
SCALE = DH ** -0.5
NEG_MASK = -1000000000.0


def _rb(x):
    return x.astype(BF16).astype(F32)


def _ln_mod(x, s1p, shift):
    mu = jnp.mean(x, axis=-1, keepdims=True)
    xc = x - mu
    var = jnp.mean(xc * xc, axis=-1, keepdims=True)
    sd = _rb(jnp.sqrt(_rb(_rb(var) + EPS)))
    n = _rb(_rb(x - _rb(mu)) * (1.0 / sd))
    return _rb(n * s1p) + shift


def _dot(a, b):
    return jnp.dot(a, b, preferred_element_type=F32)


def _kernel(x_hbm, mem0_ref, wq_hbm, wk_hbm, wv_hbm, wo_hbm, wr_ref, wg_hbm, wu_hbm, wd_hbm,
            c_ref, wmod_hbm, out_hbm,
            wqkv, wo_s, ring, obuf, xbuf, outbuf, rbuf, lhs, olhs, mqkv, ybuf, mod, mk,
            sem_x, sem_wo, sem_out):

    def lhs_val():
        return jnp.concatenate([lhs[k] for k in range(NT)], axis=1)

    def store_lhs_rows(r0, val):
        n = val.shape[0]
        vb = val.astype(BF16)
        for k in range(NT):
            lhs[k, r0:r0 + n, :] = vb[:, k * 128:(k + 1) * 128]

    def x_copy(i):
        lo, n = ((0, R0), (R0, S - R0))[i]
        return pltpu.make_async_copy(x_hbm.at[pl.ds(lo, n)], xbuf.at[pl.ds(lo, n)], sem_x.at[i])

    def wo_copy(j):
        return pltpu.make_async_copy(wo_hbm.at[:, pl.ds(j * 128, 128)], wo_s.at[j], sem_wo.at[j])

    def prologue(stage, wmod_s, h0, sem_st, sem_mod):
        w_hbms = (wq_hbm, wk_hbm, wv_hbm)

        def mod_copy(i):
            lo, n = ((0, 2 * D), (2 * D, 4 * D))[i]
            return pltpu.make_async_copy(wmod_hbm.at[:, pl.ds(lo, n)], wmod_s.at[:, pl.ds(lo, n)],
                                         sem_mod.at[i])

        def chunk_copy(mat, g, slot):
            return pltpu.make_async_copy(w_hbms[mat].at[:, pl.ds(g * CH, CH), :], stage.at[slot],
                                         sem_st.at[slot])

        def relayout(i, slot):
            for d0 in range(0, D, 16):
                v = stage[slot, d0:d0 + 16]
                wqkv[pl.ds(i * CH, CH), d0:d0 + 16, :] = jnp.swapaxes(v, 0, 1)

        mod_copy(0).start()
        x_copy(0).start()
        chunk_copy(0, 0, 0).start()
        chunk_copy(0, 1, 1).start()

        qi = lax.broadcasted_iota(jnp.int32, (PR, PR), 0)
        ki = lax.broadcasted_iota(jnp.int32, (PR, PR), 1)

        def head_of(i):
            return jnp.where(i < 2 * SEG, i // SEG, (i - 2 * SEG) // M)

        same = head_of(qi) == head_of(ki)
        vis = (qi >= 2 * SEG) | (ki >= 2 * SEG) | (qi >= ki)
        mk[...] = jnp.where(same, jnp.where(vis, 0.0, NEG_MASK), -jnp.inf).astype(F32)
        ybuf[...] = jnp.zeros_like(ybuf)

        cv = c_ref[...].astype(F32)
        sc = jnp.broadcast_to(_rb(cv * _rb(jax.nn.sigmoid(cv))), (M, D)).astype(BF16)

        def mod_part(lo, n):
            for j in range(lo, lo + n):
                v = _rb(_dot(sc, wmod_s[:, j * D:(j + 1) * D]))
                if j in (1, 4):
                    v = _rb(1.0 + v)
                mod[j] = v

        mod_copy(0).wait()
        mod_part(0, 2)
        chunk_copy(0, 2, 2).start()
        x_copy(0).wait()

        def ln_body(i, c):
            r = pl.multiple_of(i * 32, 32)
            hv = _ln_mod(xbuf[pl.ds(r, 32), :].astype(F32), mod[1, 0:1, :], mod[0, 0:1, :])
            hb = hv.astype(BF16)
            for k in range(NT):
                h0[k, pl.ds(r, 32), :] = hb[:, k * 128:(k + 1) * 128]
            return c

        lax.fori_loop(0, R0 // 32, ln_body, 0)
        chunk_copy(0, 0, 0).wait()
        relayout(0, 0)

        def chunk_body(i, c):
            nxt = i + NSLOT - 1
            for mat in range(3):
                @pl.when(jnp.logical_and(nxt < NCHUNK, nxt // (H // CH) == mat))
                def _():
                    g = pl.multiple_of((nxt % (H // CH)) * CH, CH)
                    pltpu.make_async_copy(w_hbms[mat].at[:, pl.ds(g, CH), :],
                                          stage.at[nxt % NSLOT], sem_st.at[nxt % NSLOT]).start()

            @pl.when(i == 1)
            def _():
                x_copy(1).start()

            @pl.when(i == 3)
            def _():
                mod_copy(1).start()

            @pl.when(i == 6)
            def _():
                for j in range(NT):
                    wo_copy(j).start()

            i1 = jnp.minimum(i + 1, NCHUNK - 1)
            slot1 = i1 % NSLOT

            @pl.when(i + 1 < NCHUNK)
            def _():
                chunk_copy(0, 0, slot1).wait()

            hv = jnp.concatenate([h0[k] for k in range(NT)], axis=1)
            ws = [wqkv[i * CH + hh] for hh in range(CH)]
            relayout(i1, slot1)
            for hh in range(CH):
                ring[i * CH + hh, ROFF:RING, :] = _dot(hv, ws[hh]).astype(BF16)
            return c

        lax.fori_loop(0, NCHUNK, chunk_body, 0)
        mod_copy(1).wait()
        mod_part(2, 4)

    pl.run_scoped(
        prologue,
        pltpu.VMEM((NSLOT, D, CH, 128), BF16),
        pltpu.VMEM((D, 6 * D), BF16),
        pltpu.VMEM((NT, R0, 128), BF16),
        pltpu.SemaphoreType.DMA((NSLOT,)),
        pltpu.SemaphoreType.DMA((2,)),
    )

    def ln1_rows(r):
        return _ln_mod(xbuf[pl.ds(r, XR), :].astype(F32), mod[1, 0:1, :], mod[0, 0:1, :])

    def post(r, n, y):
        x1 = _rb(xbuf[pl.ds(r, n), :].astype(F32) + _rb(mod[2, 0:1, :] * _rb(y)))
        xbuf[pl.ds(r, n), :] = x1.astype(BF16)
        h2 = _rb(_ln_mod(x1, mod[4, 0:1, :], mod[3, 0:1, :]))
        rbuf[pl.ds(r, n), :] = _rb(jnp.sum(h2 * wr_ref[...].astype(F32), axis=-1, keepdims=True))
        outbuf[pl.ds(r, n), :] = (x1 + _rb(mod[5, 0:1, :] * h2)).astype(BF16)

    def out_copy(r, n):
        return pltpu.make_async_copy(outbuf.at[pl.ds(r, n)], out_hbm.at[pl.ds(r, n)], sem_out.at[0])

    def main(wg_s, wu_s, wd_s, sem_f):
        def ffn_copies():
            cps = []
            for j in range(FF // 128):
                cps.append(pltpu.make_async_copy(wg_hbm.at[:, pl.ds(j * 128, 128)], wg_s.at[j],
                                                 sem_f.at[0]))
                cps.append(pltpu.make_async_copy(wu_hbm.at[:, pl.ds(j * 128, 128)], wu_s.at[j],
                                                 sem_f.at[1]))
            for j in range(NT):
                cps.append(pltpu.make_async_copy(wd_hbm.at[:, pl.ds(j * 128, 128)], wd_s.at[j],
                                                 sem_f.at[2]))
            return cps

        x_copy(1).wait()
        store_lhs_rows(0, ln1_rows(R0))
        store_lhs_rows(XR, mem0_ref[...].astype(F32))
        for j in range(NT):
            wo_copy(j).wait()
        for cp in ffn_copies():
            cp.start()

        def step(s, carry):
            @pl.when(s >= 2)
            def _():
                out_copy(pl.multiple_of((s - 2) * XR, 8), XR).start()

            wslot = pl.multiple_of((s * XR) % RING, 8)
            rslot = pl.multiple_of((s * SEG + ROFF) % RING, SEG)
            orow = pl.multiple_of(s * SEG, SEG)
            xrow = pl.multiple_of(s * XR, 8)

            def qkv(g):
                lv = lhs_val()
                for p in range(g * GH // 2, (g + 1) * GH // 2):
                    for mat in range(3):
                        for a in range(2):
                            hm = mat * H + 2 * p + a
                            y = _dot(lv, wqkv[hm]).astype(BF16)
                            ring[hm, pl.ds(wslot, XR), :] = y[0:XR]
                            mqkv[mat, p, a * M:(a + 1) * M, :] = y[XR:XR + M]

            def gather(mat, p):
                return jnp.concatenate(
                    [ring[mat * H + 2 * p, pl.ds(rslot, SEG), :],
                     ring[mat * H + 2 * p + 1, pl.ds(rslot, SEG), :],
                     mqkv[mat, p]], axis=0)

            def scores(g):
                res = []
                for p in range(g * GH // 2, (g + 1) * GH // 2):
                    sc = lax.dot_general(gather(0, p), gather(1, p), (((1,), (1,)), ((), ())),
                                         preferred_element_type=F32)
                    mv = mk[...]
                    sc = jnp.where(mv == 0.0, sc * SCALE, mv)
                    e = jnp.exp(sc - jnp.max(sc, axis=-1, keepdims=True))
                    inv = 1.0 / jnp.sum(e, axis=-1, keepdims=True)
                    res.append((e.astype(BF16), inv))
                return res

            def pv(g, probs):
                for i, p in enumerate(range(g * GH // 2, (g + 1) * GH // 2)):
                    e, inv = probs[i]
                    o = (_dot(e, gather(2, p)) * inv).astype(BF16)
                    for a in range(2):
                        h = 2 * p + a
                        obuf[h, pl.ds(orow, SEG), :] = o[a * SEG:(a + 1) * SEG]
                        olhs[h, XR:XR + M, :] = o[2 * SEG + a * M:2 * SEG + (a + 1) * M]
                        olhs[h, 0:XR, :] = obuf[h, pl.ds(xrow, XR), :]

            def oproj(g, acc):
                ov = jnp.concatenate([olhs[h] for h in range(g * GH, (g + 1) * GH)], axis=1)
                out = []
                for j in range(NT):
                    y = _dot(ov, wo_s[j, g * GH * DH:(g + 1) * GH * DH, :])
                    out.append(y if acc is None else acc[j] + y)
                return out

            probs = {}
            acc = None
            og = 0
            for g in range(NG + 2):
                if g < NG:
                    qkv(g)
                else:
                    acc = oproj(og, acc)
                    og += 1
                if g == 0:
                    post(pl.multiple_of(jnp.maximum(s - 1, 0) * XR, 8), XR, ybuf[...])
                if 1 <= g <= NG:
                    probs[g - 1] = scores(g - 1)
                if g >= 2:
                    pv(g - 2, probs.pop(g - 2))
                if g == NG - 1:
                    nrow = pl.multiple_of(jnp.minimum(R0 + (s + 1) * XR, S - XR), 8)
                    store_lhs_rows(0, ln1_rows(nrow))
            while og < NG:
                acc = oproj(og, acc)
                og += 1
            for j in range(NT):
                ybuf[:, j * 128:(j + 1) * 128] = acc[j][0:XR]
                lhs[j, XR:XR + M, :] = acc[j][XR:XR + M].astype(BF16)
            return carry

        lax.fori_loop(0, NSEG, step, 0)

        last = (NSEG - 1) * XR
        out_copy(last - XR, XR).start()
        post(last, XR, ybuf[...])
        out_copy(last, XR).start()

        EC = 128

        def ep_body(i, c):
            r = pl.multiple_of(NSEG * XR + i * EC, EC)
            ov = jnp.concatenate([obuf[h, pl.ds(r, EC), :] for h in range(H)], axis=1)
            y = jnp.concatenate([_dot(ov, wo_s[j]) for j in range(NT)], axis=1)
            post(r, EC, y)
            out_copy(r, EC).start()
            return c

        lax.fori_loop(0, R0 // EC, ep_body, 0)

        rv = rbuf[...]
        idx = lax.broadcasted_iota(jnp.int32, (S, 1), 0)
        m1 = jnp.max(rv, axis=0, keepdims=True)
        i1v = jnp.min(jnp.where(rv == m1, idx, S), axis=0, keepdims=True)
        rv2 = jnp.where(idx == i1v, -jnp.inf, rv)
        m2 = jnp.max(rv2, axis=0, keepdims=True)
        i2v = jnp.min(jnp.where(jnp.logical_and(rv2 == m2, idx != i1v), idx, S), axis=0,
                      keepdims=True)
        i1 = jnp.clip(i1v[0, 0], 0, S - 1)
        i2 = jnp.clip(i2v[0, 0], 0, S - 1)
        b1 = pl.multiple_of((i1 // 8) * 8, 8)
        b2 = pl.multiple_of((i2 // 8) * 8, 8)

        x1 = jnp.concatenate([xbuf[pl.ds(b1, 8), :].astype(F32),
                              xbuf[pl.ds(b2, 8), :].astype(F32)], axis=0)
        h2 = _rb(_ln_mod(x1, mod[4, 0:1, :], mod[3, 0:1, :]))
        rsel = jnp.concatenate([rbuf[pl.ds(b1, 8), :], rbuf[pl.ds(b2, 8), :]], axis=0)
        h2b = h2.astype(BF16)
        for cp in ffn_copies():
            cp.wait()
        acts = []
        for j in range(FF // 128):
            gt = _rb(_dot(h2b, wg_s[j]))
            gt = _rb(gt * _rb(jax.nn.sigmoid(gt)))
            ut = _rb(_dot(h2b, wu_s[j]))
            acts.append((gt * ut).astype(BF16))
        act = jnp.concatenate(acts, axis=1)
        y = _rb(jnp.concatenate([_dot(act, wd_s[j]) for j in range(NT)], axis=1))
        y = _rb(y * _rb(jax.nn.sigmoid(rsel)))
        row = lax.broadcasted_iota(jnp.int32, (2 * 8, 1), 0)
        grow = jnp.where(row < 8, b1 + row, b2 + row - 8)
        sel = jnp.logical_or(grow == i1, grow == i2)
        hb = _rb(h2 + jnp.where(sel, y, 0.0))
        fixed = (x1 + _rb(mod[5, 0:1, :] * hb)).astype(BF16)

        pltpu.make_async_copy(outbuf, out_hbm, sem_out.at[0]).wait()
        outbuf[pl.ds(b1, 8), :] = fixed[0:8]
        outbuf[pl.ds(b2, 8), :] = fixed[8:16]
        cp1 = pltpu.make_async_copy(outbuf.at[pl.ds(b1, 8)], out_hbm.at[pl.ds(b1, 8)], sem_out.at[0])
        cp2 = pltpu.make_async_copy(outbuf.at[pl.ds(b2, 8)], out_hbm.at[pl.ds(b2, 8)], sem_out.at[1])
        cp1.start()

        @pl.when(b1 != b2)
        def _():
            cp2.start()
            cp2.wait()

        cp1.wait()

    pl.run_scoped(
        main,
        pltpu.VMEM((FF // 128, D, 128), BF16),
        pltpu.VMEM((FF // 128, D, 128), BF16),
        pltpu.VMEM((NT, FF, 128), BF16),
        pltpu.SemaphoreType.DMA((3,)),
    )


@functools.partial(jax.jit, static_argnames=("A_seg_len",))
def pallas_adaLN_cond__memory_aug_recurrent_mem_tr__moe_arch_mod__prompt_kernel(
    A_x: jax.Array,
    A_mem0: jax.Array,
    A_Wq: jax.Array,
    A_Wk: jax.Array,
    A_Wv: jax.Array,
    A_Wo: jax.Array,
    A_seg_len,
    B_x: jax.Array,
    B_w_r: jax.Array,
    B_w_gate: jax.Array,
    B_w_up: jax.Array,
    B_w_down: jax.Array,
    c: jax.Array,
    w_mod: jax.Array,
):
    assert A_seg_len == SEG and A_x.shape == (1, S, D)
    del B_x
    hbm = pl.BlockSpec(memory_space=pl.ANY)
    vmem = pl.BlockSpec(memory_space=pltpu.VMEM)
    out = pl.pallas_call(
        _kernel,
        out_shape=jax.ShapeDtypeStruct((S, D), BF16),
        in_specs=[hbm, vmem, hbm, hbm, hbm, hbm, vmem, hbm, hbm, hbm, vmem, hbm],
        out_specs=hbm,
        scratch_shapes=[
            pltpu.VMEM((3 * H, D, DH), BF16),
            pltpu.VMEM((NT, H * DH, 128), BF16),
            pltpu.VMEM((3 * H, RING, DH), BF16),
            pltpu.VMEM((H, S, DH), BF16),
            pltpu.VMEM((S, D), BF16),
            pltpu.VMEM((S, D), BF16),
            pltpu.VMEM((S, 1), F32),
            pltpu.VMEM((NT, XR + M, 128), BF16),
            pltpu.VMEM((H, XR + M, DH), BF16),
            pltpu.VMEM((3, H // 2, 2 * M, DH), BF16),
            pltpu.VMEM((XR, D), F32),
            pltpu.VMEM((6, M, D), F32),
            pltpu.VMEM((PR, PR), F32),
            pltpu.SemaphoreType.DMA((2,)),
            pltpu.SemaphoreType.DMA((NT,)),
            pltpu.SemaphoreType.DMA((2,)),
        ],
        compiler_params=pltpu.CompilerParams(vmem_limit_bytes=120 * 1024 * 1024),
    )(A_x.reshape(S, D), A_mem0.reshape(M, D), A_Wq, A_Wk, A_Wv, A_Wo.reshape(H * DH, D),
      B_w_r.reshape(1, D), B_w_gate, B_w_up, B_w_down, c, w_mod)
    return out.reshape(1, S, D)
```

```python
import functools

import jax
import jax.numpy as jnp
from jax import lax
import jax.experimental.pallas as pl
import jax.experimental.pallas.tpu as pltpu

F32 = jnp.float32
BF16 = jnp.bfloat16
U32 = jnp.uint32

D = 1024
S = 2048
H = 32
DH = 128
M = 8
SEG = 32
NSEG = S // SEG
FF = 3584
NT = D // 128
XR = 24
R0 = S - XR * NSEG
RING = 576
ROFF = RING - R0
CH = 8
NCHUNK = 3 * H // CH
NSLOT = 4
PR = 2 * SEG + 2 * M
NP = H // 2
LAG_S = 1
LAG_PV = 3
T_POST = 0
T_LN = 3
HSPLIT = 24
RB = 32
LNB = 64
EC = 128
LOG2E = 1.4426950408889634
EPS = 1e-5
SCALE = DH ** -0.5
NEG_MASK = -1000000000.0


def _rb(x):
    return x.astype(BF16).astype(F32)


def _ln_mod(x, s1p, shift):
    mu = jnp.mean(x, axis=-1, keepdims=True)
    xc = x - mu
    var = jnp.mean(xc * xc, axis=-1, keepdims=True)
    sd = _rb(jnp.sqrt(_rb(_rb(var) + EPS)))
    n = _rb(_rb(x - _rb(mu)) * (1.0 / sd))
    return _rb(n * s1p) + shift


def _dot(a, b):
    return jnp.dot(a, b, preferred_element_type=F32)


def _recip(x):
    r = pl.reciprocal(x, approx=True)
    return r * (2.0 - x * r)


def _as_bf16(u):
    return pltpu.bitcast(u, BF16)


def _as_u32(b):
    return pltpu.bitcast(b, U32)


def _kernel(x_hbm, mem0_ref, wq_hbm, wk_hbm, wv_hbm, wo_hbm, wr_ref, wg_hbm, wu_hbm, wd_hbm,
            c_ref, wmod_hbm, out_hbm,
            wqkv, wo_s, ring, obuf, xo, lhs, olhs, mqkv, ybuf, mod, mk, topv, topi,
            sem_x, sem_out):

    def store_lhs_rows(slot, r0, val):
        n = val.shape[0]
        vb = val.astype(BF16)
        for k in range(NT):
            lhs[slot, k, r0:r0 + n, :] = vb[:, k * 128:(k + 1) * 128]

    def x_copy(i):
        lo, n = ((0, R0), (R0, S - R0))[i]
        return pltpu.make_async_copy(x_hbm.at[pl.ds(lo, n)], xo.at[pl.ds(lo, n)], sem_x.at[i])

    def prologue(stage, wo_raw, wmod_s, h0, tmp, sem_st, sem_mod, sem_wo):
        w_hbms = (wq_hbm, wk_hbm, wv_hbm)

        def mod_copy(i):
            lo, n = ((0, 2 * D), (2 * D, 4 * D))[i]
            return pltpu.make_async_copy(wmod_hbm.at[:, pl.ds(lo, n)], wmod_s.at[:, pl.ds(lo, n)],
                                         sem_mod.at[i])

        def chunk_copy(mat, g, slot):
            return pltpu.make_async_copy(w_hbms[mat].at[:, pl.ds(g * CH, CH), :], stage.at[slot],
                                         sem_st.at[slot])

        def wo_copy(j):
            return pltpu.make_async_copy(wo_hbm.at[:, pl.ds(j * 128, 128)], wo_raw.at[j],
                                         sem_wo.at[j])

        def relayout(i, slot, piece):
            for d0 in range(piece * 128, (piece + 1) * 128, RB):
                t0 = d0 * (CH // 2)
                v = stage[slot, d0:d0 + RB].reshape(RB * CH, 128)
                tmp[t0:t0 + RB * CH // 2, :] = _as_u32(v)
                for j in range(CH // 2):
                    w = tmp[pl.ds(t0 + j, RB, stride=CH // 2), :]
                    rows = pl.ds(d0 // 2, RB // 2)
                    wqkv[i * CH + 2 * j, rows, :] = _as_u32(w.astype(jnp.uint16))
                    wqkv[i * CH + 2 * j + 1, rows, :] = _as_u32((w >> 16).astype(jnp.uint16))

        mod_copy(0).start()
        x_copy(0).start()
        chunk_copy(0, 0, 0).start()
        chunk_copy(0, 1, 1).start()

        qi = lax.broadcasted_iota(jnp.int32, (PR, PR), 0)
        ki = lax.broadcasted_iota(jnp.int32, (PR, PR), 1)

        def head_of(i):
            return jnp.where(i < 2 * SEG, i // SEG, (i - 2 * SEG) // M)

        same = head_of(qi) == head_of(ki)
        vis = (qi >= 2 * SEG) | (ki >= 2 * SEG) | (qi >= ki)
        mk[...] = jnp.where(same, jnp.where(vis, 0.0, NEG_MASK * LOG2E), -jnp.inf).astype(F32)
        ybuf[...] = jnp.zeros_like(ybuf)
        topv[...] = jnp.full(topv.shape, -jnp.inf, F32)
        topi[...] = lax.broadcasted_iota(jnp.int32, topi.shape, 0)

        cv = c_ref[...].astype(F32)
        sc = jnp.broadcast_to(_rb(cv * _rb(jax.nn.sigmoid(cv))), (M, D)).astype(BF16)

        def mod_part(lo, n):
            for j in range(lo, lo + n):
                v = _rb(_dot(sc, wmod_s[:, j * D:(j + 1) * D]))
                if j in (1, 4):
                    v = _rb(1.0 + v)
                mod[j] = v

        mod_copy(0).wait()
        mod_part(0, 2)
        chunk_copy(0, 2, 2).start()
        x_copy(0).wait()

        def ln_body(i, c):
            for sub in range(LNB // 16):
                r = pl.multiple_of(i * LNB + sub * 16, 16)
                hv = _ln_mod(xo[pl.ds(r, 16), :].astype(F32), mod[1, 0:1, :], mod[0, 0:1, :])
                hb = hv.astype(BF16)
                r2 = pl.multiple_of(i * (LNB // 2) + sub * 8, 8)
                for k in range(NT):
                    h0[k, pl.ds(r2, 8), :] = _as_u32(hb[:, k * 128:(k + 1) * 128])
            return c

        lax.fori_loop(0, R0 // LNB, ln_body, 0)
        chunk_copy(0, 0, 0).wait()
        for piece in range(D // 128):
            relayout(0, 0, piece)

        def chunk_body(with_wo, i, c):
            nxt = i + NSLOT - 1
            for mat in range(3):
                @pl.when(jnp.logical_and(nxt < NCHUNK, nxt // (H // CH) == mat))
                def _():
                    g = pl.multiple_of((nxt % (H // CH)) * CH, CH)
                    pltpu.make_async_copy(w_hbms[mat].at[:, pl.ds(g, CH), :],
                                          stage.at[nxt % NSLOT], sem_st.at[nxt % NSLOT]).start()

            if not with_wo:
                @pl.when(i == 1)
                def _():
                    for j in range(NT):
                        wo_copy(j).start()
            else:
                @pl.when(i == NCHUNK - NT)
                def _():
                    x_copy(1).start()

                @pl.when(i == NCHUNK - NT + 2)
                def _():
                    mod_copy(1).start()

            i1 = jnp.minimum(i + 1, NCHUNK - 1)
            slot1 = i1 % NSLOT

            @pl.when(i + 1 < NCHUNK)
            def _():
                chunk_copy(0, 0, slot1).wait()

            if with_wo:
                jw = i - (NCHUNK - NT)
                pltpu.make_async_copy(wo_hbm.at[:, pl.ds(0, 128)], wo_raw.at[jw],
                                      sem_wo.at[jw]).wait()

            for hh in range(CH):
                hv = jnp.concatenate([_as_bf16(h0[k]) for k in range(NT)], axis=1)
                y = _dot(hv, _as_bf16(wqkv[i * CH + hh]))
                ring[i * CH + hh, ROFF:RING, :] = y.astype(BF16)
                if hh == 0:
                    relayout(i1, slot1, CH - 1)
                if hh < CH - 1:
                    relayout(i1, slot1, hh)
                    if with_wo:
                        for q in range(2 if hh == 0 else 1):
                            b = hh if q == 0 else CH - 1
                            n = H * DH // CH
                            wo_s[jw, b * n // 2:(b + 1) * n // 2, :] = _as_u32(
                                wo_raw[jw, b * n:(b + 1) * n, :])
            return c

        lax.fori_loop(0, NCHUNK - NT, functools.partial(chunk_body, False), 0)
        lax.fori_loop(NCHUNK - NT, NCHUNK, functools.partial(chunk_body, True), 0)
        mod_copy(1).wait()
        mod_part(2, 4)

    pl.run_scoped(
        prologue,
        pltpu.VMEM((NSLOT, D, CH, 128), BF16),
        pltpu.VMEM((NT, H * DH, 128), BF16),
        pltpu.VMEM((D, 6 * D), BF16),
        pltpu.VMEM((NT, R0 // 2, 128), U32),
        pltpu.VMEM((D * CH // 2, 128), U32),
        pltpu.SemaphoreType.DMA((NSLOT,)),
        pltpu.SemaphoreType.DMA((2,)),
        pltpu.SemaphoreType.DMA((NT,)),
    )

    def ln1_rows(r):
        return _ln_mod(xo[pl.ds(r, XR), :].astype(F32), mod[1, 0:1, :], mod[0, 0:1, :])

    def post(r, n, y, live=None):
        x1 = _rb(xo[pl.ds(r, n), :].astype(F32) + _rb(mod[2, 0:1, :] * _rb(y)))
        xo[pl.ds(r, n), :] = x1.astype(BF16)
        h2 = _rb(_ln_mod(x1, mod[4, 0:1, :], mod[3, 0:1, :]))
        xo[pl.ds(S + r, n), :] = (x1 + _rb(mod[5, 0:1, :] * h2)).astype(BF16)
        rv = _rb(jnp.sum(h2 * wr_ref[...].astype(F32), axis=-1, keepdims=True))
        if live is not None:
            rv = jnp.where(live, rv, -jnp.inf)
        m1, m2, i1, i2 = topv[0:8, :], topv[8:16, :], topi[0:8, :], topi[8:16, :]
        sub = lax.broadcasted_iota(jnp.int32, (8, 1), 0)
        for k in range(n // 8):
            v = rv[k * 8:(k + 1) * 8]
            idx = sub + (r + k * 8)
            g1 = v > m1
            g2 = v > m2
            m2 = jnp.where(g1, m1, jnp.where(g2, v, m2))
            i2 = jnp.where(g1, i1, jnp.where(g2, idx, i2))
            m1 = jnp.where(g1, v, m1)
            i1 = jnp.where(g1, idx, i1)
        topv[0:8, :] = m1
        topv[8:16, :] = m2
        topi[0:8, :] = i1
        topi[8:16, :] = i2

    def out_copy(r, n, k=0):
        return pltpu.make_async_copy(xo.at[pl.ds(S + r, n)], out_hbm.at[pl.ds(r, n)],
                                     sem_out.at[k])

    def main(wg_s, wu_s, wd_s, ye, sem_f):
        def ffn_copies():
            cps = []
            for j in range(FF // 128):
                cps.append(pltpu.make_async_copy(wg_hbm.at[:, pl.ds(j * 128, 128)], wg_s.at[j],
                                                 sem_f.at[0]))
                cps.append(pltpu.make_async_copy(wu_hbm.at[:, pl.ds(j * 128, 128)], wu_s.at[j],
                                                 sem_f.at[1]))
            for j in range(NT):
                cps.append(pltpu.make_async_copy(wd_hbm.at[:, pl.ds(j * 128, 128)], wd_s.at[j],
                                                 sem_f.at[2]))
            return cps

        x_copy(1).wait()
        store_lhs_rows(0, 0, ln1_rows(R0))
        store_lhs_rows(0, XR, mem0_ref[...].astype(F32))
        for cp in ffn_copies():
            cp.start()

        def step(s, carry):
            @pl.when(s >= 2)
            def _():
                out_copy(pl.multiple_of((s - 2) * XR, 8), XR).start()

            cur = s % 2
            nxt = 1 - cur
            wslot = pl.multiple_of((s * XR) % RING, 8)
            rslot = pl.multiple_of((s * SEG + ROFF) % RING, SEG)
            orow = pl.multiple_of(s * SEG, SEG)
            xrow = pl.multiple_of(s * XR, 8)
            pending = []

            def flush():
                for hm, y in pending:
                    ring[hm, pl.ds(wslot, XR), :] = y
                pending.clear()

            def qkv(p):
                lv = jnp.concatenate([lhs[cur, k] for k in range(NT)], axis=1)
                for mat in range(3):
                    for a in range(2):
                        hm = mat * H + 2 * p + a
                        y = _dot(lv, _as_bf16(wqkv[hm])).astype(BF16)
                        pending.append((hm, y[0:XR]))
                        mqkv[mat, p, a * M:(a + 1) * M, :] = y[XR:XR + M]

            def gather(mat, p):
                return jnp.concatenate(
                    [ring[mat * H + 2 * p, pl.ds(rslot, SEG), :],
                     ring[mat * H + 2 * p + 1, pl.ds(rslot, SEG), :],
                     mqkv[mat, p]], axis=0)

            probs = {}

            def scores(p):
                sc = lax.dot_general(gather(0, p), gather(1, p), (((1,), (1,)), ((), ())),
                                     preferred_element_type=F32)
                mv = mk[...]
                sc = jnp.where(mv == 0.0, sc * (SCALE * LOG2E), mv)
                e = jnp.exp2(sc - jnp.max(sc, axis=-1, keepdims=True))
                probs[p] = (e * _recip(jnp.sum(e, axis=-1, keepdims=True))).astype(BF16)

            def pv(p):
                o = _dot(probs.pop(p), gather(2, p)).astype(BF16)
                for a in range(2):
                    h = 2 * p + a
                    obuf[h, pl.ds(orow, SEG), :] = o[a * SEG:(a + 1) * SEG]
                    olhs[h, XR:XR + M, :] = o[2 * SEG + a * M:2 * SEG + (a + 1) * M]
                    olhs[h, 0:XR, :] = obuf[h, pl.ds(xrow, XR), :]

            def oproj(j, h0_, h1_):
                ov = jnp.concatenate([olhs[h] for h in range(h0_, h1_)], axis=1)
                return _dot(ov, _as_bf16(wo_s[j, h0_ * DH // 2:h1_ * DH // 2, :]))

            def attn(t):
                if 0 <= t - LAG_S < NP:
                    scores(t - LAG_S)
                if 0 <= t - LAG_PV < NP:
                    pv(t - LAG_PV)
                flush()

            for t in range(NP):
                qkv(t)
                attn(t)
                if t == T_POST:
                    post(pl.multiple_of(jnp.maximum(s - 1, 0) * XR, 8), XR, ybuf[...], s > 0)
                if t == T_LN:
                    nrow = pl.multiple_of(jnp.minimum(R0 + (s + 1) * XR, S - XR), 8)
                    store_lhs_rows(nxt, 0, ln1_rows(nrow))
            acc = []
            t = NP
            for j in range(NT):
                acc.append(oproj(j, 0, HSPLIT))
                if j % 2 == 1:
                    attn(t)
                    t += 1
            assert t - LAG_PV >= NP
            for j in range(NT):
                y = oproj(j, HSPLIT, H) + acc[j]
                ybuf[:, j * 128:(j + 1) * 128] = y[0:XR]
                lhs[nxt, j, XR:XR + M, :] = y[XR:XR + M].astype(BF16)
            return carry

        lax.fori_loop(0, NSEG, step, 0)

        def o_rows(r, n, mid=None):
            for j in range(NT):
                ov = jnp.concatenate([obuf[h, pl.ds(r, n), :] for h in range(H)], axis=1)
                yj = _dot(ov, _as_bf16(wo_s[j]))
                if mid is not None:
                    mid(j)
                ye[0:n, j * 128:(j + 1) * 128] = yj

        last = (NSEG - 1) * XR
        out_copy(last - XR, XR).start()
        post(last, XR, ybuf[...])
        out_copy(last, XR).start()

        def ep_body(i, c):
            r = pl.multiple_of(NSEG * XR + i * EC, EC)
            o_rows(r, EC)
            post(r, EC, ye[...])
            out_copy(r, EC).start()
            return c

        lax.fori_loop(0, R0 // EC, ep_body, 0)

        tv = topv[...]
        ti = topi[...]
        m1 = jnp.max(tv, axis=0, keepdims=True)
        i1v = jnp.min(jnp.where(tv == m1, ti, S), axis=0, keepdims=True)
        rest = ti != i1v
        m2 = jnp.max(jnp.where(rest, tv, -jnp.inf), axis=0, keepdims=True)
        i2v = jnp.min(jnp.where(jnp.logical_and(rest, tv == m2), ti, S), axis=0, keepdims=True)
        i1 = jnp.clip(i1v[0, 0], 0, S - 1)
        i2 = jnp.clip(i2v[0, 0], 0, S - 1)
        b1 = pl.multiple_of((i1 // 8) * 8, 8)
        b2 = pl.multiple_of((i2 // 8) * 8, 8)

        x1 = jnp.concatenate([xo[pl.ds(b1, 8), :].astype(F32),
                              xo[pl.ds(b2, 8), :].astype(F32)], axis=0)
        h2 = _rb(_ln_mod(x1, mod[4, 0:1, :], mod[3, 0:1, :]))
        h2b = h2.astype(BF16)
        row = lax.broadcasted_iota(jnp.int32, (2 * 8, 1), 0)
        grow = jnp.where(row < 8, b1 + row, b2 + row - 8)
        rsel = jnp.where(grow == i1, m1, m2)
        for cp in ffn_copies():
            cp.wait()
        acts = []
        for j in range(FF // 128):
            gt = _rb(_dot(h2b, wg_s[j]))
            gt = _rb(gt * _rb(jax.nn.sigmoid(gt)))
            ut = _rb(_dot(h2b, wu_s[j]))
            acts.append((gt * ut).astype(BF16))
        act = jnp.concatenate(acts, axis=1)
        y = _rb(jnp.concatenate([_dot(act, wd_s[j]) for j in range(NT)], axis=1))
        y = _rb(y * _rb(jax.nn.sigmoid(rsel)))
        sel = jnp.logical_or(grow == i1, grow == i2)
        hb = _rb(h2 + jnp.where(sel, y, 0.0))
        fixed = (x1 + _rb(mod[5, 0:1, :] * hb)).astype(BF16)

        out_copy(0, S).wait()
        xo[pl.ds(S + b1, 8), :] = fixed[0:8]
        xo[pl.ds(S + b2, 8), :] = fixed[8:16]
        out_copy(b1, 8, 0).start()

        @pl.when(b1 != b2)
        def _():
            out_copy(b2, 8, 1).start()
            out_copy(b2, 8, 1).wait()

        out_copy(b1, 8, 0).wait()

    pl.run_scoped(
        main,
        pltpu.VMEM((FF // 128, D, 128), BF16),
        pltpu.VMEM((FF // 128, D, 128), BF16),
        pltpu.VMEM((NT, FF, 128), BF16),
        pltpu.VMEM((EC, D), F32),
        pltpu.SemaphoreType.DMA((3,)),
    )


@functools.partial(jax.jit, static_argnames=("A_seg_len",))
def pallas_adaLN_cond__memory_aug_recurrent_mem_tr__moe_arch_mod__prompt_kernel(
    A_x: jax.Array,
    A_mem0: jax.Array,
    A_Wq: jax.Array,
    A_Wk: jax.Array,
    A_Wv: jax.Array,
    A_Wo: jax.Array,
    A_seg_len,
    B_x: jax.Array,
    B_w_r: jax.Array,
    B_w_gate: jax.Array,
    B_w_up: jax.Array,
    B_w_down: jax.Array,
    c: jax.Array,
    w_mod: jax.Array,
):
    assert A_seg_len == SEG and A_x.shape == (1, S, D)
    del B_x
    hbm = pl.BlockSpec(memory_space=pl.ANY)
    vmem = pl.BlockSpec(memory_space=pltpu.VMEM)
    out = pl.pallas_call(
        _kernel,
        out_shape=jax.ShapeDtypeStruct((S, D), BF16),
        in_specs=[hbm, vmem, hbm, hbm, hbm, hbm, vmem, hbm, hbm, hbm, vmem, hbm],
        out_specs=hbm,
        scratch_shapes=[
            pltpu.VMEM((3 * H, D // 2, DH), U32),
            pltpu.VMEM((NT, H * DH // 2, 128), U32),
            pltpu.VMEM((3 * H, RING, DH), BF16),
            pltpu.VMEM((H, S, DH), BF16),
            pltpu.VMEM((2 * S, D), BF16),
            pltpu.VMEM((2, NT, XR + M, 128), BF16),
            pltpu.VMEM((H, XR + M, DH), BF16),
            pltpu.VMEM((3, H // 2, 2 * M, DH), BF16),
            pltpu.VMEM((XR, D), F32),
            pltpu.VMEM((6, M, D), F32),
            pltpu.VMEM((PR, PR), F32),
            pltpu.VMEM((16, 1), F32),
            pltpu.VMEM((16, 1), jnp.int32),
            pltpu.SemaphoreType.DMA((2,)),
            pltpu.SemaphoreType.DMA((2,)),
        ],
        compiler_params=pltpu.CompilerParams(vmem_limit_bytes=120 * 1024 * 1024,
                                             disable_bounds_checks=True),
    )(A_x.reshape(S, D), A_mem0.reshape(M, D), A_Wq, A_Wk, A_Wv, A_Wo.reshape(H * DH, D),
      B_w_r.reshape(1, D), B_w_gate, B_w_up, B_w_down, c, w_mod)
    return out.reshape(1, S, D)
```

```python
import functools

import jax
import jax.numpy as jnp
from jax import lax
import jax.experimental.pallas as pl
import jax.experimental.pallas.tpu as pltpu

F32 = jnp.float32
BF16 = jnp.bfloat16
U32 = jnp.uint32

D = 1024
S = 2048
H = 32
DH = 128
M = 8
SEG = 32
NSEG = S // SEG
FF = 3584
NT = D // 128
XR = SEG - M
R0 = M * NSEG
CH = 8
NCHUNK = 3 * H // CH
NA = NCHUNK - NT
NSLOT = 4
PR = 2 * SEG + 2 * M
NP = H // 2
RB = 32
EC = 128
NEC = R0 // EC
PPI = (S // 8 - EC // 8) // NEC
LOG2E = 1.4426950408889634
EPS = 1e-5
SCALE = DH ** -0.5
NEG_MASK = -1000000000.0

PHASES = ("pro", "step", "epi")
POS_P = None
POS_S = 0
POS_P2 = 3
OJ_S = 1
OJ_P = 7
OMERGE = False
UNROLL = 2
LNU = 8
POST_SPLIT = (9, 9, 9, 9, 8, 8, 8, 0)


def _schedule():
    groups = [list(range(4 * g, 4 * g + 4)) for g in range(4)]
    ops = []
    for t in range(4):
        for i, p in enumerate(groups[t]):
            ops.append(("Q", p, p == 0))
            if i == POS_P and t >= 2:
                ops.extend(("P", q) for q in groups[t - 2])
            if i == POS_S and t >= 1:
                ops.extend(("S", q) for q in groups[t - 1])
            if i == POS_P2 and t >= 1:
                ops.extend(("P", q) for q in groups[t - 1])
    first = groups[0] + groups[1]
    for j in range(NT):
        ops.append(("O", j, first))
        if j == OJ_S:
            if POS_P is not None:
                ops.extend(("P", q) for q in groups[2])
            ops.extend(("S", q) for q in groups[3])
        if j == OJ_P:
            ops.extend(("P", q) for q in groups[3])
    if OMERGE:
        for j in range(NT):
            ops.append(("O", j, groups[2] + groups[3]))
            ops.append(("F", j))
    else:
        ops.extend(("O", j, groups[2]) for j in range(NT))
        for j in range(NT):
            ops.append(("O", j, groups[3]))
            ops.append(("F", j))
    return ops


def _rb(x):
    return x.astype(BF16).astype(F32)


def _recip(x):
    r = pl.reciprocal(x, approx=True)
    return r * (2.0 - x * r)


def _ln_mod(x, s1p, shift):
    xc = x - jnp.mean(x, axis=-1, keepdims=True)
    v = _rb(_rb(jnp.mean(xc * xc, axis=-1, keepdims=True)) + EPS)
    return xc * _recip(_rb(v * lax.rsqrt(v))) * s1p + shift


def _dot(a, b):
    return jnp.dot(a, b, preferred_element_type=F32)


def _as_bf16(u):
    return pltpu.bitcast(u, BF16)


def _as_u32(b):
    return pltpu.bitcast(b, U32)


def _kernel(x_hbm, mem0_ref, wq_hbm, wk_hbm, wv_hbm, wo_hbm, wr_ref, wg_hbm, wu_hbm, wd_hbm,
            c_ref, wmod_hbm, out_hbm,
            wqkv, hs, wo_s, pre, cur_s, olhs, odef, xbuf, ybuf, outs, lhs, mod, mk, topv, topi, sc_s,
            sem_x, sem_out):
    def x_copy(i):
        lo, n = ((XR, M), (0, XR))[i]
        return pltpu.make_async_copy(x_hbm.at[:, pl.ds(lo, n), :], xbuf.at[:, pl.ds(lo, n), :],
                                     sem_x.at[i])

    def mod_tile(wm, t):
        v = _rb(_dot(sc_s[...], wm))
        if t // NT in (1, 4):
            v = _rb(1.0 + v)
        mod[t // NT, :, (t % NT) * 128:(t % NT + 1) * 128] = v

    def ln1(x):
        x3 = x.astype(F32).reshape(x.shape[0] // 8, 8, D)
        return _ln_mod(x3, mod[1], mod[0]).reshape(x.shape[0], D).astype(BF16)

    def prologue(stage, wo_raw, wmod_s, h0, tmp, sem_st, sem_c0, sem_mod, sem_wo):
        w_hbms = (wq_hbm, wk_hbm, wv_hbm)

        def mod_copy(g):
            return pltpu.make_async_copy(wmod_hbm.at[:, pl.ds(g * 512, 512)], wmod_s.at[g],
                                         sem_mod.at[g])

        def chunk_copy(mat, g, slot):
            return pltpu.make_async_copy(w_hbms[mat].at[:, pl.ds(g * CH, CH), :], stage.at[slot],
                                         sem_st.at[slot])

        def c0_copy(q):
            rows = pl.ds(q * (D // 4), D // 4)
            return pltpu.make_async_copy(wq_hbm.at[rows, pl.ds(0, CH), :], stage.at[0, rows],
                                         sem_c0.at[q])

        def wo_copy(j, col):
            return pltpu.make_async_copy(wo_hbm.at[:, pl.ds(col, 128)], wo_raw.at[j], sem_wo.at[j])

        def relayout(i, slot, piece):
            for d0 in range(piece * 128, (piece + 1) * 128, RB):
                t0 = d0 * (CH // 2)
                v = stage[slot, d0:d0 + RB].reshape(RB * CH, 128)
                tmp[t0:t0 + RB * CH // 2, :] = _as_u32(v)
                for j in range(CH // 2):
                    w = tmp[pl.ds(t0 + j, RB, stride=CH // 2), :]
                    rows = pl.ds(d0 // 2, RB // 2)
                    wqkv[i * CH + 2 * j, rows, :] = _as_u32(w.astype(jnp.uint16))
                    wqkv[i * CH + 2 * j + 1, rows, :] = _as_u32((w >> 16).astype(jnp.uint16))

        for g in range(4):
            mod_copy(g).start()
        x_copy(0).start()
        for q in range(4):
            c0_copy(q).start()
        chunk_copy(0, 1, 1).start()
        chunk_copy(0, 2, 2).start()

        def decode(i):
            lo = i < 2 * SEG
            head = jnp.where(lo, i // SEG, (i - 2 * SEG) // M)
            is_mem = jnp.logical_and(lo, i % SEG >= XR)
            pos = jnp.where(lo, i % SEG, XR + i % M)
            return head, is_mem, pos

        qh, qm, qp = decode(lax.broadcasted_iota(jnp.int32, (PR, PR), 0))
        kh, km, kp = decode(lax.broadcasted_iota(jnp.int32, (PR, PR), 1))
        vis = qm | km | (qp >= kp)
        mk[...] = jnp.where(qh == kh, jnp.where(vis, 0.0, NEG_MASK * LOG2E), -jnp.inf).astype(F32)
        mod[6] = jnp.broadcast_to(wr_ref[...].astype(F32), (M, D))
        topv[...] = jnp.full(topv.shape, -jnp.inf, F32)
        topi[...] = lax.broadcasted_iota(jnp.int32, topi.shape, 0)
        cv = c_ref[...].astype(F32)
        sc_s[...] = jnp.broadcast_to(cv * _rb(jax.nn.sigmoid(cv)), (M, D)).astype(BF16)
        mb = mem0_ref[...]
        for k in range(NT):
            lhs[0, k, XR // 2:, :] = _as_u32(mb[:, k * 128:(k + 1) * 128])

        with jax.named_scope("p_mod"):
            for g in range(4):
                mod_copy(g).wait()
                for t in range(4):
                    mod_tile(wmod_s[g, :, t * 128:(t + 1) * 128], 4 * g + t)
        with jax.named_scope("p_xwait"):
            x_copy(0).wait()

        def ln_body(i, c):
            for u in range(LNU):
                q = (i * LNU + u) * 2
                hb = ln1(xbuf[pl.ds(q, 2), XR:, :].reshape(16, D))
                r2 = pl.multiple_of(q * 4, 8)
                for k in range(NT):
                    h0[k, pl.ds(r2, 8), :] = _as_u32(hb[:, k * 128:(k + 1) * 128])
            return c

        with jax.named_scope("p_ln"):
            lax.fori_loop(0, NSEG // (2 * LNU), ln_body, 0)
        with jax.named_scope("p_c0"):
            for q in range(4):
                c0_copy(q).wait()
                relayout(0, 0, 2 * q)
                relayout(0, 0, 2 * q + 1)

        def bulk(i, hh):
            hv = jnp.concatenate([_as_bf16(h0[k]) for k in range(NT)], axis=1)
            y = _dot(hv, _as_bf16(wqkv[i * CH + hh]))
            a = (hh % 2) * M
            pre[i * (CH // 2) + hh // 2, :, a:a + M, :] = y.reshape(NSEG, M, DH).astype(BF16)

        def start_chunk(nxt):
            for mat in range(3):
                @pl.when(jnp.logical_and(nxt < NCHUNK, nxt // (H // CH) == mat))
                def _():
                    g = pl.multiple_of((nxt % (H // CH)) * CH, CH)
                    pltpu.make_async_copy(w_hbms[mat].at[:, pl.ds(g, CH), :],
                                          stage.at[nxt % NSLOT], sem_st.at[nxt % NSLOT]).start()

        def body_a(i, c):
            start_chunk(i + NSLOT - 1)

            @pl.when(i == 0)
            def _():
                x_copy(1).start()

            @pl.when(i > 0)
            def _():
                wo_copy(i - 1, pl.multiple_of((i - 1) * 128, 128)).start()

            for hh in range(CH // 2):
                bulk(i, hh)
            chunk_copy(0, 0, (i + 1) % NSLOT).wait()
            for hh in range(CH // 2, CH):
                bulk(i, hh)
                for piece in ((0, 1, 2), (3, 4, 5), (6, 7), ())[hh - CH // 2]:
                    relayout(i + 1, (i + 1) % NSLOT, piece)
            return c

        def body_b(i, c):
            start_chunk(i + NSLOT - 1)

            @pl.when(i - 1 < NT)
            def _():
                wo_copy(i - 1, pl.multiple_of((i - 1) * 128, 128)).start()

            i1 = jnp.minimum(i + 1, NCHUNK - 1)
            slot1 = i1 % NSLOT

            @pl.when(i + 1 < NCHUNK)
            def _():
                chunk_copy(0, 0, slot1).wait()

            jw = i - NA
            wo_copy(jw, 0).wait()
            n = H * DH // CH
            for hh in range(CH):
                bulk(i, hh)
                for b in ((0, CH - 1) if hh == 0 else (hh,) if hh < CH - 1 else ()):
                    relayout(i1, slot1, b)
                    wo_s[jw, b * n // 2:(b + 1) * n // 2, :] = _as_u32(
                        wo_raw[jw, b * n:(b + 1) * n, :])
                    seg = jw * CH + b
                    hb = ln1(xbuf[seg, 0:XR, :])
                    for k in range(NT):
                        hs[seg, k] = _as_u32(hb[:, k * 128:(k + 1) * 128])
            return c

        with jax.named_scope("p_loopa"):
            lax.fori_loop(0, NA, body_a, 0)
        with jax.named_scope("p_xwait2"):
            x_copy(1).wait()
        with jax.named_scope("p_loopb"):
            lax.fori_loop(NA, NCHUNK, body_b, 0)

    if "pro" in PHASES: pl.run_scoped(
        prologue,
        pltpu.VMEM((NSLOT, D, CH, 128), BF16),
        pltpu.VMEM((NT, H * DH, 128), BF16),
        pltpu.VMEM((4, D, 512), BF16),
        pltpu.VMEM((NT, R0 // 2, 128), U32),
        pltpu.VMEM((D * CH // 2, 128), U32),
        pltpu.SemaphoreType.DMA((NSLOT,)),
        pltpu.SemaphoreType.DMA((4,)),
        pltpu.SemaphoreType.DMA((4,)),
        pltpu.SemaphoreType.DMA((NT,)),
    )

    def load_x_rows(slot, seg):
        for k in range(NT):
            lhs[slot, k, 0:XR // 2, :] = hs[seg, k]

    def post(seg, r):
        rows = pl.ds(r, 8)
        x1 = _rb(xbuf[seg, rows, :].astype(F32) + mod[2] * ybuf[seg, rows, :].astype(F32))
        xbuf[seg, rows, :] = x1.astype(BF16)
        h2 = _rb(_ln_mod(x1, mod[4], mod[3]))
        outs[seg, rows, :] = (x1 + mod[5] * h2).astype(BF16)
        v = _rb(jnp.sum(h2 * mod[6], axis=-1, keepdims=True))
        m1, m2, i1, i2 = topv[0:8, :], topv[8:16, :], topi[0:8, :], topi[8:16, :]
        idx = lax.broadcasted_iota(jnp.int32, (8, 1), 0) + (seg * SEG + r)
        g1 = (v > m1) | ((v == m1) & (idx < i1))
        g2 = (v > m2) | ((v == m2) & (idx < i2))
        topv[8:16, :] = jnp.where(g1, m1, jnp.where(g2, v, m2))
        topi[8:16, :] = jnp.where(g1, i1, jnp.where(g2, idx, i2))
        topv[0:8, :] = jnp.where(g1, v, m1)
        topi[0:8, :] = jnp.where(g1, idx, i1)

    def out_copy(g0, ng, r, n, k=0):
        return pltpu.make_async_copy(outs.at[pl.ds(g0, ng), pl.ds(r, n), :],
                                     out_hbm.at[pl.ds(g0, ng), pl.ds(r, n), :], sem_out.at[k])

    def main(wg_s, wu_s, wd_s, wmod_s, sem_f):
        def col_copy(src, dst, j, off, k):
            return pltpu.make_async_copy(src.at[:, pl.ds(pl.multiple_of((off + j) * 128, 128), 128)],
                                         dst.at[j], sem_f.at[k])

        late = ((wmod_hbm, wmod_s, 2 * NT, 4 * NT), (wg_hbm, wg_s, 0, FF // 128),
                (wu_hbm, wu_s, 0, FF // 128), (wd_hbm, wd_s, 0, NT))

        def wait_late(k):
            src, dst, off, n = late[k]
            for j in range(n):
                col_copy(src, dst, j, off, k).wait()

        if PHASES == ("pro",):
            return
        load_x_rows(0, 0)

        def step(s, cur):
            nxt = 1 - cur
            drow = pl.multiple_of(s * M, M)

            def lv(k0, k1):
                return jnp.concatenate([_as_bf16(lhs[cur, k]) for k in range(k0, k1)], axis=1)

            def qkv(p, split=False):
                part = {}
                if split:
                    for mat in range(3):
                        for a in range(2):
                            part[mat, a] = _dot(
                                lv(0, NT // 2), _as_bf16(wqkv[mat * H + 2 * p + a, :D // 4, :]))
                for mat in range(3):
                    for a in range(2):
                        hm = mat * H + 2 * p + a
                        if split:
                            y = _dot(lv(NT // 2, NT), _as_bf16(wqkv[hm, D // 4:, :])) + part[mat, a]
                        else:
                            y = _dot(lv(0, NT), _as_bf16(wqkv[hm]))
                        cur_s[hm] = _as_u32(y.astype(BF16))

            def gather(mat, p):
                hm = mat * H + 2 * p
                return jnp.concatenate(
                    [_as_bf16(cur_s[hm]), _as_bf16(cur_s[hm + 1]), pre[mat * NP + p, s]], axis=0)

            probs = {}

            def scores(p):
                sc = lax.dot_general(gather(0, p), gather(1, p), (((1,), (1,)), ((), ())),
                                     preferred_element_type=F32)
                mv = mk[...]
                sc = jnp.where(mv == 0.0, sc * (SCALE * LOG2E), mv)
                e = jnp.exp2(sc - jnp.max(sc, axis=-1, keepdims=True))
                probs[p] = (e.astype(BF16), _recip(jnp.sum(e, axis=-1, keepdims=True)))

            def pv(p):
                e, inv = probs.pop(p)
                o = (_dot(e, gather(2, p)) * inv).astype(BF16)
                for a in range(2):
                    h = 2 * p + a
                    olhs[h] = _as_u32(o[a * SEG:(a + 1) * SEG])
                    odef[h, pl.ds(drow, M), :] = o[2 * SEG + a * M:2 * SEG + (a + 1) * M]

            acc = [None] * NT

            def oproj(j, pairs):
                ov = jnp.concatenate([_as_bf16(olhs[2 * p + a]) for p in pairs for a in range(2)],
                                     axis=1)
                w = wo_s[j, pairs[0] * DH:(pairs[-1] + 1) * DH, :]
                y = _dot(ov, _as_bf16(w))
                acc[j] = y if acc[j] is None else y + acc[j]

            def fin(j):
                yb = acc[j].astype(BF16)
                ybuf[s, 0:XR, j * 128:(j + 1) * 128] = yb[0:XR]
                lhs[nxt, j, XR // 2:, :] = _as_u32(yb[XR:])

            load_x_rows(nxt, jnp.minimum(s + 1, NSEG - 1))
            ops = dict(Q=qkv, S=scores, P=pv, O=oproj, F=fin)
            for op in _schedule():
                ops[op[0]](*op[1:])

        def steps(i, carry):
            for k, (src, dst, off, n) in enumerate(late):
                @pl.when(i < n)
                def _():
                    col_copy(src, dst, i, off, k).start()

            for u in range(UNROLL):
                step(i * UNROLL + u, u % 2)
            return carry

        if "step" in PHASES: lax.fori_loop(0, NSEG // UNROLL, steps, 0)
        if "epi" not in PHASES:
            for k in range(4):
                wait_late(k)
            return

        wait_late(0)
        for t in range(4 * NT):
            mod_tile(wmod_s[t], 2 * NT + t)

        gpi = PPI // (XR // 8)

        def ep_body(i, c):
            @pl.when(i > 0)
            def _():
                out_copy((i - 1) * gpi, gpi, 0, XR).start()

            r = pl.multiple_of(i * EC, EC)
            g0 = i * (EC // M)
            u = 0
            for j in range(NT):
                ov = jnp.concatenate([odef[h, pl.ds(r, EC), :] for h in range(H)], axis=1)
                yj = _dot(ov, _as_bf16(wo_s[j]))
                ybuf[pl.ds(g0, EC // M), XR:, j * 128:(j + 1) * 128] = (
                    yj.reshape(EC // M, M, 128).astype(BF16))
                for _ in range(POST_SPLIT[j]):
                    t = i * PPI + u
                    early = t < NSEG * (XR // 8)
                    seg = jnp.where(early, t // (XR // 8), t - NSEG * (XR // 8))
                    post(seg, pl.multiple_of(jnp.where(early, (t % (XR // 8)) * 8, XR), 8))
                    u += 1
            assert u == PPI
            return c

        lax.fori_loop(0, NEC, ep_body, 0)
        done = (NEC - 1) * gpi
        tail = NSEG - EC // M
        out_copy(done, NSEG - done, 0, XR).start()
        out_copy(0, tail, XR, M).start()
        for g in range(tail, NSEG):
            post(g, XR)
        out_copy(tail, NSEG - tail, XR, M).start()

        tv = topv[...]
        ti = topi[...]
        m1 = jnp.max(tv, axis=0, keepdims=True)
        i1v = jnp.min(jnp.where(tv == m1, ti, S), axis=0, keepdims=True)
        rest = ti != i1v
        m2 = jnp.max(jnp.where(rest, tv, -jnp.inf), axis=0, keepdims=True)
        i2v = jnp.min(jnp.where(jnp.logical_and(rest, tv == m2), ti, S), axis=0, keepdims=True)
        i1 = jnp.clip(i1v[0, 0], 0, S - 1)
        i2 = jnp.clip(i2v[0, 0], 0, S - 1)
        g1, g2 = i1 // SEG, i2 // SEG
        b1 = pl.multiple_of((i1 % SEG) // 8 * 8, 8)
        b2 = pl.multiple_of((i2 % SEG) // 8 * 8, 8)

        x1 = jnp.stack([xbuf[g1, pl.ds(b1, 8), :].astype(F32),
                        xbuf[g2, pl.ds(b2, 8), :].astype(F32)])
        h2 = _rb(_ln_mod(x1, mod[4], mod[3])).reshape(16, D)
        x1 = x1.reshape(16, D)
        h2b = h2.astype(BF16)
        row = lax.broadcasted_iota(jnp.int32, (16, 1), 0)
        grow = jnp.where(row < 8, g1 * SEG + b1 + row, g2 * SEG + b2 + row - 8)
        rsel = jnp.where(grow == i1, m1, m2)
        for k in range(1, 4):
            wait_late(k)
        acts = []
        for j in range(FF // 128):
            gt = _rb(_dot(h2b, wg_s[j]))
            gt = _rb(gt * _rb(jax.nn.sigmoid(gt)))
            ut = _rb(_dot(h2b, wu_s[j]))
            acts.append((gt * ut).astype(BF16))
        act = jnp.concatenate(acts, axis=1)
        y = _rb(jnp.concatenate([_dot(act, wd_s[j]) for j in range(NT)], axis=1))
        y = _rb(y * _rb(jax.nn.sigmoid(rsel)))
        sel = jnp.logical_or(grow == i1, grow == i2)
        hb = _rb(h2 + jnp.where(sel, y, 0.0))
        fixed = (x1 + mod[5, 0:1, :] * hb).astype(BF16)

        out_copy(0, NSEG, 0, SEG).wait()
        outs[g1, pl.ds(b1, 8), :] = fixed[0:8]
        outs[g2, pl.ds(b2, 8), :] = fixed[8:16]
        out_copy(g1, 1, b1, 8, 0).start()

        @pl.when(i1 // 8 != i2 // 8)
        def _():
            out_copy(g2, 1, b2, 8, 1).start()
            out_copy(g2, 1, b2, 8, 1).wait()

        out_copy(g1, 1, b1, 8, 0).wait()

    pl.run_scoped(
        main,
        pltpu.VMEM((FF // 128, D, 128), BF16),
        pltpu.VMEM((FF // 128, D, 128), BF16),
        pltpu.VMEM((NT, FF, 128), BF16),
        pltpu.VMEM((4 * NT, D, 128), BF16),
        pltpu.SemaphoreType.DMA((4,)),
    )


@functools.partial(jax.jit, static_argnames=("A_seg_len",))
def pallas_adaLN_cond__memory_aug_recurrent_mem_tr__moe_arch_mod__prompt_kernel(
    A_x: jax.Array,
    A_mem0: jax.Array,
    A_Wq: jax.Array,
    A_Wk: jax.Array,
    A_Wv: jax.Array,
    A_Wo: jax.Array,
    A_seg_len,
    B_x: jax.Array,
    B_w_r: jax.Array,
    B_w_gate: jax.Array,
    B_w_up: jax.Array,
    B_w_down: jax.Array,
    c: jax.Array,
    w_mod: jax.Array,
):
    assert A_seg_len == SEG and A_x.shape == (1, S, D)
    del B_x
    hbm = pl.BlockSpec(memory_space=pl.ANY)
    vmem = pl.BlockSpec(memory_space=pltpu.VMEM)
    out = pl.pallas_call(
        _kernel,
        out_shape=jax.ShapeDtypeStruct((NSEG, SEG, D), BF16),
        in_specs=[hbm, vmem, hbm, hbm, hbm, hbm, vmem, hbm, hbm, hbm, vmem, hbm],
        out_specs=hbm,
        scratch_shapes=[
            pltpu.VMEM((3 * H, D // 2, DH), U32),
            pltpu.VMEM((NSEG, NT, XR // 2, 128), U32),
            pltpu.VMEM((NT, H * DH // 2, 128), U32),
            pltpu.VMEM((3 * NP, NSEG, 2 * M, DH), BF16),
            pltpu.VMEM((3 * H, SEG // 2, DH), U32),
            pltpu.VMEM((H, SEG // 2, DH), U32),
            pltpu.VMEM((H, R0, DH), BF16),
            pltpu.VMEM((NSEG, SEG, D), BF16),
            pltpu.VMEM((NSEG, SEG, D), BF16),
            pltpu.VMEM((NSEG, SEG, D), BF16),
            pltpu.VMEM((2, NT, SEG // 2, 128), U32),
            pltpu.VMEM((7, M, D), F32),
            pltpu.VMEM((PR, PR), F32),
            pltpu.VMEM((16, 1), F32),
            pltpu.VMEM((16, 1), jnp.int32),
            pltpu.VMEM((M, D), BF16),
            pltpu.SemaphoreType.DMA((2,)),
            pltpu.SemaphoreType.DMA((2,)),
        ],
        compiler_params=pltpu.CompilerParams(vmem_limit_bytes=120 * 1024 * 1024,
                                             disable_bounds_checks=True),
    )(A_x.reshape(NSEG, SEG, D), A_mem0.reshape(M, D), A_Wq, A_Wk, A_Wv, A_Wo.reshape(H * DH, D),
      B_w_r.reshape(1, D), B_w_gate, B_w_up, B_w_down, c, w_mod)
    return out.reshape(1, S, D)
```

```python
import functools

import jax
import jax.numpy as jnp
from jax import lax
import jax.experimental.pallas as pl
import jax.experimental.pallas.tpu as pltpu

F32 = jnp.float32
BF16 = jnp.bfloat16
U32 = jnp.uint32

D = 1024
S = 2048
H = 32
DH = 128
M = 8
SEG = 32
NSEG = S // SEG
FF = 3584
NT = D // 128
XR = SEG - M
R0 = M * NSEG
CH = 8
NCHUNK = 3 * H // CH
NA = NCHUNK - NT
NSLOT = 4
PR = 2 * SEG + 2 * M
NP = H // 2
RB = 16
EC = 128
NEC = R0 // EC
PPI = (S // 8 - EC // 8) // NEC
LOG2E = 1.4426950408889634
EPS = 1e-5
SCALE = DH ** -0.5
NEG_MASK = -1000000000.0

PHASES = ("pro", "step", "epi")
POS_P = None
POS_S = 0
POS_P2 = 3
OJ_S = 1
OJ_P = 7
OMERGE = False
UNROLL = 2
EKH = 4
E_SPAN = 6
E_NREL = 1
PIN_OUT = True
NREL = 4
WOB = 128
JOB_SPAN = 3
JOB_END = 4
MB = 128
ZROW = 0
ZLAG = 0
A_SPLIT = ((0, 1, 2), (3, 4, 5), (6, 7), ())
B_SPLIT = ((0,), (1,), (2,), (3,), (4,), (5,), (6,), (7,))
L_SPLIT = ((0, 1), (2,), (3,), (4,), (5,), (6,), (7,), ())
LNU = 8
POST_SPLIT = (9, 9, 9, 9, 8, 8, 8, 0)


def _schedule():
    groups = [list(range(4 * g, 4 * g + 4)) for g in range(4)]
    ops = []
    for t in range(4):
        for i, p in enumerate(groups[t]):
            ops.append(("Q", p, p == 0))
            if i == POS_P and t >= 2:
                ops.extend(("P", q) for q in groups[t - 2])
            if i == POS_S and t >= 1:
                ops.extend(("S", q) for q in groups[t - 1])
            if i == POS_P2 and t >= 1:
                ops.extend(("P", q) for q in groups[t - 1])
    first = groups[0] + groups[1]
    for j in range(NT):
        ops.append(("O", j, first))
        if j == OJ_S:
            if POS_P is not None:
                ops.extend(("P", q) for q in groups[2])
            ops.extend(("S", q) for q in groups[3])
        if j == OJ_P:
            ops.extend(("P", q) for q in groups[3])
    if OMERGE:
        for j in range(NT):
            ops.append(("O", j, groups[2] + groups[3]))
            ops.append(("F", j))
    else:
        ops.extend(("O", j, groups[2]) for j in range(NT))
        for j in range(NT):
            ops.append(("O", j, groups[3]))
            ops.append(("F", j))
    return ops


def _rb(x):
    return x.astype(BF16).astype(F32)


def _recip(x):
    r = pl.reciprocal(x, approx=True)
    return r * (2.0 - x * r)


def _ln_mod(x, s1p, shift, zero=None):
    xm = x if zero is None else jnp.concatenate([x[..., :128] + zero, x[..., 128:]], axis=-1)
    xc = x - jnp.mean(xm, axis=-1, keepdims=True)
    v = _rb(_rb(jnp.mean(xc * xc, axis=-1, keepdims=True)) + EPS)
    return xc * _recip(_rb(v * lax.rsqrt(v))) * s1p + shift


def _dot(a, b):
    return jnp.dot(a, b, preferred_element_type=F32)


def _as_bf16(u):
    return pltpu.bitcast(u, BF16)


def _as_u32(b):
    return pltpu.bitcast(b, U32)


def _kernel(x_hbm, mem0_ref, wq_hbm, wk_hbm, wv_hbm, wo_hbm, wr_ref, wg_hbm, wu_hbm, wd_hbm,
            c_ref, wmod_hbm, out_hbm,
            wqkv, hs, wo_s, pre, cur_s, olhs, odef, xbuf, ybuf, outs, lhs, mod, mk, topv, topi, sc_s, zero_s,
            sem, sem_out):
    def x_copy(i):
        lo, n = ((XR, M), (0, XR))[i]
        return pltpu.make_async_copy(x_hbm.at[:, pl.ds(lo, n), :], xbuf.at[:, pl.ds(lo, n), :],
                                     sem.at[i])

    def mod_tile(wm, t):
        v = _rb(_dot(sc_s[...], wm))
        if t // NT in (1, 4):
            v = _rb(1.0 + v)
        mod[t // NT, :, (t % NT) * 128:(t % NT + 1) * 128] = v

    def ln1(x, zero=None):
        x3 = x.astype(F32).reshape(x.shape[0] // 8, 8, D)
        zf = None if zero is None else pltpu.bitcast(zero, F32)
        return _ln_mod(x3, mod[1], mod[0], zf).reshape(x.shape[0], D).astype(BF16)

    def zero_after(y):
        return (y if y.dtype == U32 else pltpu.bitcast(y, U32)) & zero_s[...]

    def or_tile(u, z):
        if z is None:
            return u
        return (u.reshape(u.shape[0] // 8, 8, 128) | z).reshape(u.shape)

    def prologue(stage, wo_raw, wmod_s, h0, tmp):
        w_hbms = (wq_hbm, wk_hbm, wv_hbm)

        def mod_copy(g):
            return pltpu.make_async_copy(wmod_hbm.at[:, pl.ds(g * 512, 512)], wmod_s.at[g],
                                         sem.at[2 + g])

        def chunk_copy(mat, g, slot):
            return pltpu.make_async_copy(w_hbms[mat].at[:, pl.ds(g * CH, CH), :], stage.at[slot],
                                         sem.at[10 + slot])

        def c0_copy(q):
            rows = pl.ds(q * (D // 4), D // 4)
            return pltpu.make_async_copy(wq_hbm.at[rows, pl.ds(0, CH), :], stage.at[0, rows],
                                         sem.at[6 + q])

        def wo_copy(j, col):
            return pltpu.make_async_copy(wo_hbm.at[:, pl.ds(col, 128)], wo_raw.at[j],
                                         sem.at[10 + NSLOT + j])

        def relayout(i, slot, lo, hi, z=None):
            for d0 in range(lo, hi, RB):
                t0 = d0 * (CH // 2)
                v = stage[slot, d0:d0 + RB].reshape(RB * CH, 128)
                tmp[t0:t0 + RB * CH // 2, :] = or_tile(_as_u32(v), z)
                for j in range(CH // 2):
                    w = tmp[pl.ds(t0 + j, RB, stride=CH // 2), :]
                    rows = pl.ds(d0 // 2, RB // 2)
                    wqkv[i * CH + 2 * j, rows, :] = _as_u32(w.astype(jnp.uint16))
                    wqkv[i * CH + 2 * j + 1, rows, :] = _as_u32((w >> 16).astype(jnp.uint16))

        for g in range(4):
            mod_copy(g).start()
        x_copy(0).start()
        for q in range(4):
            c0_copy(q).start()
        chunk_copy(0, 1, 1).start()
        chunk_copy(0, 2, 2).start()

        def decode(i):
            lo = i < 2 * SEG
            head = jnp.where(lo, i // SEG, (i - 2 * SEG) // M)
            is_mem = jnp.logical_and(lo, i % SEG >= XR)
            pos = jnp.where(lo, i % SEG, XR + i % M)
            return head, is_mem, pos

        qh, qm, qp = decode(lax.broadcasted_iota(jnp.int32, (PR, PR), 0))
        kh, km, kp = decode(lax.broadcasted_iota(jnp.int32, (PR, PR), 1))
        vis = qm | km | (qp >= kp)
        mk[...] = jnp.where(qh == kh, jnp.where(vis, 0.0, NEG_MASK * LOG2E), -jnp.inf).astype(F32)
        mod[6] = jnp.broadcast_to(wr_ref[...].astype(F32), (M, D))
        zero_s[...] = jnp.zeros(zero_s.shape, U32)
        topv[...] = jnp.full(topv.shape, -jnp.inf, F32)
        topi[...] = lax.broadcasted_iota(jnp.int32, topi.shape, 0)
        cv = c_ref[...].astype(F32)
        sc_s[...] = jnp.broadcast_to(cv * _rb(jax.nn.sigmoid(cv)), (M, D)).astype(BF16)
        mb = mem0_ref[...]
        for k in range(NT):
            lhs[0, k, XR // 2:, :] = _as_u32(mb[:, k * 128:(k + 1) * 128])

        with jax.named_scope("p_mod"):
            for g in range(4):
                mod_copy(g).wait()
                for t in range(4):
                    mod_tile(wmod_s[g, :, t * 128:(t + 1) * 128], 4 * g + t)
        with jax.named_scope("p_xwait"):
            x_copy(0).wait()

        def ln_body(i, c):
            for u in range(LNU):
                q = (i * LNU + u) * 2
                hb = ln1(xbuf[pl.ds(q, 2), XR:, :].reshape(16, D))
                r2 = pl.multiple_of(q * 4, 8)
                for k in range(NT):
                    h0[k, pl.ds(r2, 8), :] = _as_u32(hb[:, k * 128:(k + 1) * 128])
            return c

        with jax.named_scope("p_ln"):
            lax.fori_loop(0, NSEG // (2 * LNU), ln_body, 0)
        with jax.named_scope("p_c0"):
            for q in range(4):
                c0_copy(q).wait()
                relayout(0, 0, q * (D // 4), (q + 1) * (D // 4))

        def bulk(i, heads, jobs):
            n = 0
            due = {}
            for hh in heads:
                a = (hh % 2) * M
                for r in range(0, R0, MB):
                    ts = [h0[k, r // 2:(r + MB) // 2, :] for k in range(NT)]
                    for z in due.pop(n, ()):
                        ts[0] = jnp.concatenate([ts[0][0:8] | z, ts[0][8:]], axis=0)
                    hv = jnp.concatenate([_as_bf16(t) for t in ts], axis=1)
                    y = _dot(hv, _as_bf16(wqkv[i * CH + hh]))
                    pre[i * (CH // 2) + hh // 2, r // M:(r + MB) // M, a:a + M, :] = (
                        y.reshape(MB // M, M, DH).astype(BF16))
                    for u in range(NREL):
                        for job in jobs.get(n * NREL + u, ()):
                            zr = u * (MB - 8) // max(NREL - 1, 1) // 8 * 8
                            res = job(zero_after(y[zr:zr + 8]))
                            if res is not None and JOB_SPAN:
                                due.setdefault(n + JOB_SPAN, []).append(zero_after(res))
                    n += 1

        def start_chunk(nxt):
            for mat in range(3):
                @pl.when(jnp.logical_and(nxt < NCHUNK, nxt // (H // CH) == mat))
                def _():
                    g = pl.multiple_of((nxt % (H // CH)) * CH, CH)
                    pltpu.make_async_copy(w_hbms[mat].at[:, pl.ds(g, CH), :],
                                          stage.at[nxt % NSLOT], sem.at[10 + nxt % NSLOT]).start()

        def body_a(i, c):
            start_chunk(i + NSLOT - 1)

            @pl.when(i == 0)
            def _():
                x_copy(1).start()

            @pl.when(i > 0)
            def _():
                wo_copy(i - 1, pl.multiple_of((i - 1) * 128, 128)).start()

            bulk(i, range(CH // 2), {})
            chunk_copy(0, 0, (i + 1) % NSLOT).wait()
            nrel = ((CH // 2) * (R0 // MB) - 1) * NREL
            jobs = {}
            for b in range(D // RB):
                jobs.setdefault(b * nrel // (D // RB), []).append(
                    functools.partial(relayout, i + 1, (i + 1) % NSLOT, b * RB, (b + 1) * RB))
            bulk(i, range(CH // 2, CH), jobs)
            return c

        def body_b(i, c):
            start_chunk(i + NSLOT - 1)

            @pl.when(i - 1 < NT)
            def _():
                wo_copy(i - 1, pl.multiple_of((i - 1) * 128, 128)).start()

            slot1 = (i + 1) % NSLOT

            @pl.when(i + 1 < NCHUNK)
            def _():
                chunk_copy(0, 0, slot1).wait()

            jw = i - NA
            wo_copy(jw, 0).wait()
            n = WOB

            def wo_job(b, z):
                wo_s[jw, b * n // 2:(b + 1) * n // 2, :] = or_tile(
                    _as_u32(wo_raw[jw, b * n:(b + 1) * n, :]), z)

            def ln_job(b, z):
                seg = jw * CH + b // 3
                r = (b % 3) * 8
                hb = ln1(xbuf[seg, r:r + 8, :], z)
                u = [_as_u32(hb[:, k * 128:(k + 1) * 128]) for k in range(NT)]
                for k in range(NT):
                    hs[seg, k, r // 2:r // 2 + 4, :] = u[k]
                res = jnp.concatenate(u[0:2], axis=0)
                for k in range(2, NT, 2):
                    res = res | jnp.concatenate(u[k:k + 2], axis=0)
                return res

            nrel = (CH * (R0 // MB) - 1) * NREL
            nln = (CH * (R0 // MB) - JOB_SPAN) * NREL
            jobs = {}
            for b in range(3 * CH):
                jobs.setdefault(b * nln // (3 * CH), []).append(functools.partial(ln_job, b))
            for b in range(D // RB):
                jobs.setdefault(b * nrel // (D // RB), []).append(
                    functools.partial(relayout, i + 1, slot1, b * RB, (b + 1) * RB))
            for b in range(H * DH // n):
                jobs.setdefault((2 * b + 1) * nrel // (2 * H * DH // n), []).append(
                    functools.partial(wo_job, b))
            bulk(i, range(CH), jobs)
            return c

        with jax.named_scope("p_loopa"):
            lax.fori_loop(0, NA, body_a, 0)
        with jax.named_scope("p_xwait2"):
            x_copy(1).wait()
        with jax.named_scope("p_loopb"):
            lax.fori_loop(NA, NCHUNK, body_b, 0)

    if "pro" in PHASES: pl.run_scoped(
        prologue,
        pltpu.VMEM((NSLOT, D, CH, 128), BF16),
        pltpu.VMEM((NT, H * DH, 128), BF16),
        pltpu.VMEM((4, D, 512), BF16),
        pltpu.VMEM((NT, R0 // 2, 128), U32),
        pltpu.VMEM((D * CH // 2, 128), U32),
    )

    def load_x_rows(slot, seg):
        for k in range(NT):
            lhs[slot, k, 0:XR // 2, :] = hs[seg, k]

    def post(seg, r, z=None):
        rows = pl.ds(r, 8)
        t = mod[2] * ybuf[seg, rows, :].astype(F32)
        if z is not None:
            t = t + jnp.concatenate([pltpu.bitcast(z, F32)] * NT, axis=1)
        x1 = _rb(xbuf[seg, rows, :].astype(F32) + t)
        xbuf[seg, rows, :] = x1.astype(BF16)
        h2 = _rb(_ln_mod(x1, mod[4], mod[3]))
        o = x1 + mod[5] * h2
        outs[seg, rows, :] = o.astype(BF16)
        v = _rb(jnp.sum(h2 * mod[6], axis=-1, keepdims=True))
        m1, m2, i1, i2 = topv[0:8, :], topv[8:16, :], topi[0:8, :], topi[8:16, :]
        idx = lax.broadcasted_iota(jnp.int32, (8, 1), 0) + (seg * SEG + r)
        g1 = (v > m1) | ((v == m1) & (idx < i1))
        g2 = (v > m2) | ((v == m2) & (idx < i2))
        topv[8:16, :] = jnp.where(g1, m1, jnp.where(g2, v, m2))
        topi[8:16, :] = jnp.where(g1, i1, jnp.where(g2, idx, i2))
        topv[0:8, :] = jnp.where(g1, v, m1)
        topi[0:8, :] = jnp.where(g1, idx, i1)
        if z is not None:
            res = pltpu.bitcast(jnp.broadcast_to(v, (8, 128)), U32)
            if PIN_OUT:
                for k in range(NT):
                    res = res | pltpu.bitcast(o[:, k * 128:(k + 1) * 128], U32)
            return res

    def out_copy(g0, ng, r, n, k=0):
        return pltpu.make_async_copy(outs.at[pl.ds(g0, ng), pl.ds(r, n), :],
                                     out_hbm.at[pl.ds(g0, ng), pl.ds(r, n), :], sem_out.at[k])

    def main(wg_s, wu_s, wd_s, wmod_s, sem_f):
        def col_copy(src, dst, j, off, k):
            return pltpu.make_async_copy(src.at[:, pl.ds(pl.multiple_of((off + j) * 128, 128), 128)],
                                         dst.at[j], sem_f.at[k])

        late = ((wmod_hbm, wmod_s, 2 * NT, 4 * NT), (wg_hbm, wg_s, 0, FF // 128),
                (wu_hbm, wu_s, 0, FF // 128), (wd_hbm, wd_s, 0, NT))

        def wait_late(k):
            src, dst, off, n = late[k]
            for j in range(n):
                col_copy(src, dst, j, off, k).wait()

        if PHASES == ("pro",):
            return
        load_x_rows(0, 0)

        def step(s, cur):
            nxt = 1 - cur
            drow = pl.multiple_of(s * M, M)

            def lv(k0, k1):
                return jnp.concatenate([_as_bf16(lhs[cur, k]) for k in range(k0, k1)], axis=1)

            def qkv(p, split=False):
                part = {}
                if split:
                    for mat in range(3):
                        for a in range(2):
                            part[mat, a] = _dot(
                                lv(0, NT // 2), _as_bf16(wqkv[mat * H + 2 * p + a, :D // 4, :]))
                for mat in range(3):
                    for a in range(2):
                        hm = mat * H + 2 * p + a
                        if split:
                            y = _dot(lv(NT // 2, NT), _as_bf16(wqkv[hm, D // 4:, :])) + part[mat, a]
                        else:
                            y = _dot(lv(0, NT), _as_bf16(wqkv[hm]))
                        cur_s[hm] = _as_u32(y.astype(BF16))

            def gather(mat, p):
                hm = mat * H + 2 * p
                return jnp.concatenate(
                    [_as_bf16(cur_s[hm]), _as_bf16(cur_s[hm + 1]), pre[mat * NP + p, s]], axis=0)

            probs = {}

            def scores(p):
                sc = lax.dot_general(gather(0, p), gather(1, p), (((1,), (1,)), ((), ())),
                                     preferred_element_type=F32)
                mv = mk[...]
                sc = jnp.where(mv == 0.0, sc * (SCALE * LOG2E), mv)
                e = jnp.exp2(sc - jnp.max(sc, axis=-1, keepdims=True))
                probs[p] = (e.astype(BF16), _recip(jnp.sum(e, axis=-1, keepdims=True)))

            def pv(p):
                e, inv = probs.pop(p)
                o = (_dot(e, gather(2, p)) * inv).astype(BF16)
                for a in range(2):
                    h = 2 * p + a
                    olhs[h] = _as_u32(o[a * SEG:(a + 1) * SEG])
                    odef[h, pl.ds(drow, M), :] = o[2 * SEG + a * M:2 * SEG + (a + 1) * M]

            acc = [None] * NT

            def oproj(j, pairs):
                ov = jnp.concatenate([_as_bf16(olhs[2 * p + a]) for p in pairs for a in range(2)],
                                     axis=1)
                w = wo_s[j, pairs[0] * DH:(pairs[-1] + 1) * DH, :]
                y = _dot(ov, _as_bf16(w))
                acc[j] = y if acc[j] is None else y + acc[j]

            def fin(j):
                yb = acc[j].astype(BF16)
                ybuf[s, 0:XR, j * 128:(j + 1) * 128] = yb[0:XR]
                lhs[nxt, j, XR // 2:, :] = _as_u32(yb[XR:])

            load_x_rows(nxt, jnp.minimum(s + 1, NSEG - 1))
            ops = dict(Q=qkv, S=scores, P=pv, O=oproj, F=fin)
            for op in _schedule():
                ops[op[0]](*op[1:])

        def steps(i, carry):
            for k, (src, dst, off, n) in enumerate(late):
                @pl.when(i < n)
                def _():
                    col_copy(src, dst, i, off, k).start()

            for u in range(UNROLL):
                step(i * UNROLL + u, u % 2)
            return carry

        if "step" in PHASES: lax.fori_loop(0, NSEG // UNROLL, steps, 0)
        if "epi" not in PHASES:
            for k in range(4):
                wait_late(k)
            return

        wait_late(0)
        for t in range(4 * NT):
            mod_tile(wmod_s[t], 2 * NT + t)

        gpi = PPI // (XR // 8)

        def ep_body(i, c):
            @pl.when(i > 0)
            def _():
                out_copy((i - 1) * gpi, gpi, 0, XR).start()

            r = pl.multiple_of(i * EC, EC)
            g0 = i * (EC // M)
            nk = H // EKH
            nrel = (NT * nk - E_SPAN) * E_NREL
            jobs = {}
            for u in range(PPI):
                jobs.setdefault(u * nrel // PPI, []).append(u)
            due = {}
            n = 0
            for j in range(NT):
                y = None
                for kk in range(nk):
                    ts = [odef[h, pl.ds(r, EC), :] for h in range(kk * EKH, (kk + 1) * EKH)]
                    for z in due.pop(n, ()):
                        ts[0] = jnp.concatenate(
                            [_as_bf16(_as_u32(ts[0][0:16]) | z), ts[0][16:]], axis=0)
                    w = wo_s[j, kk * EKH * DH // 2:(kk + 1) * EKH * DH // 2, :]
                    yp = _dot(jnp.concatenate(ts, axis=1), _as_bf16(w))
                    y = yp if y is None else yp + y
                    if kk == nk - 1:
                        ybuf[pl.ds(g0, EC // M), XR:, j * 128:(j + 1) * 128] = (
                            y.reshape(EC // M, M, 128).astype(BF16))
                    for q in range(E_NREL):
                        for u in jobs.get(n * E_NREL + q, ()):
                            zr = q * (EC - 8) // max(E_NREL - 1, 1) // 8 * 8
                            t = i * PPI + u
                            early = t < NSEG * (XR // 8)
                            seg = jnp.where(early, t // (XR // 8), t - NSEG * (XR // 8))
                            row = pl.multiple_of(jnp.where(early, (t % (XR // 8)) * 8, XR), 8)
                            res = post(seg, row, zero_after(y[zr:zr + 8]))
                            due.setdefault(n + E_SPAN, []).append(zero_after(res))
                    n += 1
            return c

        lax.fori_loop(0, NEC, ep_body, 0)
        done = (NEC - 1) * gpi
        tail = NSEG - EC // M
        out_copy(done, NSEG - done, 0, XR).start()
        out_copy(0, tail, XR, M).start()
        for g in range(tail, NSEG):
            post(g, XR)
        out_copy(tail, NSEG - tail, XR, M).start()

        tv = topv[...]
        ti = topi[...]
        m1 = jnp.max(tv, axis=0, keepdims=True)
        i1v = jnp.min(jnp.where(tv == m1, ti, S), axis=0, keepdims=True)
        rest = ti != i1v
        m2 = jnp.max(jnp.where(rest, tv, -jnp.inf), axis=0, keepdims=True)
        i2v = jnp.min(jnp.where(jnp.logical_and(rest, tv == m2), ti, S), axis=0, keepdims=True)
        i1 = jnp.clip(i1v[0, 0], 0, S - 1)
        i2 = jnp.clip(i2v[0, 0], 0, S - 1)
        g1, g2 = i1 // SEG, i2 // SEG
        b1 = pl.multiple_of((i1 % SEG) // 8 * 8, 8)
        b2 = pl.multiple_of((i2 % SEG) // 8 * 8, 8)

        x1 = jnp.stack([xbuf[g1, pl.ds(b1, 8), :].astype(F32),
                        xbuf[g2, pl.ds(b2, 8), :].astype(F32)])
        h2 = _rb(_ln_mod(x1, mod[4], mod[3])).reshape(16, D)
        x1 = x1.reshape(16, D)
        h2b = h2.astype(BF16)
        row = lax.broadcasted_iota(jnp.int32, (16, 1), 0)
        grow = jnp.where(row < 8, g1 * SEG + b1 + row, g2 * SEG + b2 + row - 8)
        rsel = jnp.where(grow == i1, m1, m2)
        for k in range(1, 4):
            wait_late(k)
        acts = []
        for j in range(FF // 128):
            gt = _rb(_dot(h2b, wg_s[j]))
            gt = _rb(gt * _rb(jax.nn.sigmoid(gt)))
            ut = _rb(_dot(h2b, wu_s[j]))
            acts.append((gt * ut).astype(BF16))
        act = jnp.concatenate(acts, axis=1)
        y = _rb(jnp.concatenate([_dot(act, wd_s[j]) for j in range(NT)], axis=1))
        y = _rb(y * _rb(jax.nn.sigmoid(rsel)))
        sel = jnp.logical_or(grow == i1, grow == i2)
        hb = _rb(h2 + jnp.where(sel, y, 0.0))
        fixed = (x1 + mod[5, 0:1, :] * hb).astype(BF16)

        out_copy(0, NSEG, 0, SEG).wait()
        outs[g1, pl.ds(b1, 8), :] = fixed[0:8]
        outs[g2, pl.ds(b2, 8), :] = fixed[8:16]
        out_copy(g1, 1, b1, 8, 0).start()

        @pl.when(i1 // 8 != i2 // 8)
        def _():
            out_copy(g2, 1, b2, 8, 1).start()
            out_copy(g2, 1, b2, 8, 1).wait()

        out_copy(g1, 1, b1, 8, 0).wait()

    pl.run_scoped(
        main,
        pltpu.VMEM((FF // 128, D, 128), BF16),
        pltpu.VMEM((FF // 128, D, 128), BF16),
        pltpu.VMEM((NT, FF, 128), BF16),
        pltpu.VMEM((4 * NT, D, 128), BF16),
        pltpu.SemaphoreType.DMA((4,)),
    )


@functools.partial(jax.jit, static_argnames=("A_seg_len",))
def pallas_adaLN_cond__memory_aug_recurrent_mem_tr__moe_arch_mod__prompt_kernel(
    A_x: jax.Array,
    A_mem0: jax.Array,
    A_Wq: jax.Array,
    A_Wk: jax.Array,
    A_Wv: jax.Array,
    A_Wo: jax.Array,
    A_seg_len,
    B_x: jax.Array,
    B_w_r: jax.Array,
    B_w_gate: jax.Array,
    B_w_up: jax.Array,
    B_w_down: jax.Array,
    c: jax.Array,
    w_mod: jax.Array,
):
    assert A_seg_len == SEG and A_x.shape == (1, S, D)
    del B_x
    hbm = pl.BlockSpec(memory_space=pl.ANY)
    vmem = pl.BlockSpec(memory_space=pltpu.VMEM)
    out = pl.pallas_call(
        _kernel,
        out_shape=jax.ShapeDtypeStruct((NSEG, SEG, D), BF16),
        in_specs=[hbm, vmem, hbm, hbm, hbm, hbm, vmem, hbm, hbm, hbm, vmem, hbm],
        out_specs=hbm,
        scratch_shapes=[
            pltpu.VMEM((3 * H + CH, D // 2, DH), U32),
            pltpu.VMEM((NSEG, NT, XR // 2, 128), U32),
            pltpu.VMEM((NT, H * DH // 2, 128), U32),
            pltpu.VMEM((3 * NP, NSEG, 2 * M, DH), BF16),
            pltpu.VMEM((3 * H, SEG // 2, DH), U32),
            pltpu.VMEM((H, SEG // 2, DH), U32),
            pltpu.VMEM((H, R0, DH), BF16),
            pltpu.VMEM((NSEG, SEG, D), BF16),
            pltpu.VMEM((NSEG, SEG, D), BF16),
            pltpu.VMEM((NSEG, SEG, D), BF16),
            pltpu.VMEM((2, NT, SEG // 2, 128), U32),
            pltpu.VMEM((7, M, D), F32),
            pltpu.VMEM((PR, PR), F32),
            pltpu.VMEM((16, 1), F32),
            pltpu.VMEM((16, 1), jnp.int32),
            pltpu.VMEM((M, D), BF16),
            pltpu.VMEM((8, 128), U32),
            pltpu.SemaphoreType.DMA((10 + NSLOT + NT,)),
            pltpu.SemaphoreType.DMA((2,)),
        ],
        compiler_params=pltpu.CompilerParams(vmem_limit_bytes=120 * 1024 * 1024,
                                             disable_bounds_checks=True),
    )(A_x.reshape(NSEG, SEG, D), A_mem0.reshape(M, D), A_Wq, A_Wk, A_Wv, A_Wo.reshape(H * DH, D),
      B_w_r.reshape(1, D), B_w_gate, B_w_up, B_w_down, c, w_mod)
    return out.reshape(1, S, D)
```

```python
import functools

import jax
import jax.numpy as jnp
from jax import lax
import jax.experimental.pallas as pl
import jax.experimental.pallas.tpu as pltpu

F32 = jnp.float32
BF16 = jnp.bfloat16
U32 = jnp.uint32

D = 1024
S = 2048
H = 32
DH = 128
M = 8
SEG = 32
NSEG = S // SEG
FF = 3584
NT = D // 128
XR = SEG - M
R0 = M * NSEG
CH = 8
NCHUNK = 3 * H // CH
NA = NCHUNK - NT
NSLOT = 4
PR = 2 * SEG + 2 * M
NP = H // 2
RB = 16
EC = 128
NEC = R0 // EC
PPI = (S // 8 - EC // 8) // NEC
LOG2E = 1.4426950408889634
EPS = 1e-5
SCALE = DH ** -0.5
NEG_MASK = -1000000000.0

PHASES = ("pro", "step", "epi")
POS_P = None
POS_S = 0
POS_P2 = 3
OJ_S = 1
OJ_P = 7
OMERGE = False
UNROLL = 2
SWAP = False
PADS = (0, 0, 0)
RLAG = 2
EKH = 4
E_SPAN = 6
E_NREL = 1
PIN_OUT = True
NREL = 4
WOB = 128
JOB_SPAN = 3
JOB_END = 4
MB = 128
ZROW = 0
ZLAG = 0
A_SPLIT = ((0, 1, 2), (3, 4, 5), (6, 7), ())
B_SPLIT = ((0,), (1,), (2,), (3,), (4,), (5,), (6,), (7,))
L_SPLIT = ((0, 1), (2,), (3,), (4,), (5,), (6,), (7,), ())
LNU = 8
POST_SPLIT = (9, 9, 9, 9, 8, 8, 8, 0)


def _schedule():
    groups = [list(range(4 * g, 4 * g + 4)) for g in range(4)]
    ops = []
    for t in range(4):
        for i, p in enumerate(groups[t]):
            ops.append(("Q", p, p == 0))
            if i == POS_P and t >= 2:
                ops.extend(("P", q) for q in groups[t - 2])
            if i == POS_S and t >= 1:
                ops.extend(("S", q) for q in groups[t - 1])
            if i == POS_P2 and t >= 1:
                ops.extend(("P", q) for q in groups[t - 1])
    first = groups[0] + groups[1]
    for j in range(NT):
        ops.append(("O", j, first))
        if j == OJ_S:
            if POS_P is not None:
                ops.extend(("P", q) for q in groups[2])
            ops.extend(("S", q) for q in groups[3])
        if j == OJ_P:
            ops.extend(("P", q) for q in groups[3])
    if OMERGE:
        for j in range(NT):
            ops.append(("O", j, groups[2] + groups[3]))
            ops.append(("F", j))
    else:
        ops.extend(("O", j, groups[2]) for j in range(NT))
        for j in range(NT):
            ops.append(("O", j, groups[3]))
            ops.append(("F", j))
    return ops


def _rb(x):
    return x.astype(BF16).astype(F32)


def _recip(x):
    r = pl.reciprocal(x, approx=True)
    return r * (2.0 - x * r)


def _ln_mod(x, s1p, shift, zero=None):
    xm = x if zero is None else jnp.concatenate([x[..., :128] + zero, x[..., 128:]], axis=-1)
    xc = x - jnp.mean(xm, axis=-1, keepdims=True)
    v = _rb(_rb(jnp.mean(xc * xc, axis=-1, keepdims=True)) + EPS)
    return xc * _recip(_rb(v * lax.rsqrt(v))) * s1p + shift


def _dot(a, b):
    return jnp.dot(a, b, preferred_element_type=F32)


def _as_bf16(u):
    return pltpu.bitcast(u, BF16)


def _as_u32(b):
    return pltpu.bitcast(b, U32)


def _kernel(x_hbm, mem0_ref, wq_hbm, wk_hbm, wv_hbm, wo_hbm, wr_ref, wg_hbm, wu_hbm, wd_hbm,
            c_ref, wmod_hbm, out_hbm,
            wqkv, hs, wo_s, pre, cur_s, olhs, odef, xbuf, ybuf, outs, lhs, mod, mk, topv, topi, sc_s, zero_s,
            sem, sem_out):
    def x_copy(i):
        lo, n = ((XR, M), (0, XR))[i]
        return pltpu.make_async_copy(x_hbm.at[:, pl.ds(lo, n), :], xbuf.at[:, pl.ds(lo, n), :],
                                     sem.at[i])

    def mod_tile(wm, t):
        v = _rb(_dot(sc_s[...], wm))
        if t // NT in (1, 4):
            v = _rb(1.0 + v)
        mod[t // NT, :, (t % NT) * 128:(t % NT + 1) * 128] = v

    def ln1(x, zero=None):
        x3 = x.astype(F32).reshape(x.shape[0] // 8, 8, D)
        zf = None if zero is None else pltpu.bitcast(zero, F32)
        return _ln_mod(x3, mod[1], mod[0], zf).reshape(x.shape[0], D).astype(BF16)

    def zero_after(y):
        return (y if y.dtype == U32 else pltpu.bitcast(y, U32)) & zero_s[0:8, :]

    def or_tile(u, z):
        if z is None:
            return u
        return (u.reshape(u.shape[0] // 8, 8, 128) | z).reshape(u.shape)

    def prologue(stage, wo_raw, wmod_s, h0, tmp):
        w_hbms = (wq_hbm, wk_hbm, wv_hbm)

        def mod_copy(g):
            return pltpu.make_async_copy(wmod_hbm.at[:, pl.ds(g * 512, 512)], wmod_s.at[g],
                                         sem.at[2 + g])

        def chunk_copy(mat, g, slot):
            return pltpu.make_async_copy(w_hbms[mat].at[:, pl.ds(g * CH, CH), :], stage.at[slot],
                                         sem.at[10 + slot])

        def c0_copy(q):
            rows = pl.ds(q * (D // 4), D // 4)
            return pltpu.make_async_copy(wq_hbm.at[rows, pl.ds(0, CH), :], stage.at[0, rows],
                                         sem.at[6 + q])

        def wo_copy(j, col):
            return pltpu.make_async_copy(wo_hbm.at[:, pl.ds(col, 128)], wo_raw.at[j],
                                         sem.at[10 + NSLOT + j])

        def relayout1(slot, d0, z=None):
            t0 = d0 * (CH // 2)
            v = stage[slot, d0:d0 + RB].reshape(RB * CH, 128)
            tmp[t0:t0 + RB * CH // 2, :] = or_tile(_as_u32(v), z)

        def relayout2(i, d0, z=None):
            t0 = d0 * (CH // 2)
            for j in range(CH // 2):
                w = or_tile(tmp[pl.ds(t0 + j, RB, stride=CH // 2), :], z)
                rows = pl.ds(d0 // 2, RB // 2)
                wqkv[i * CH + 2 * j, rows, :] = _as_u32(w.astype(jnp.uint16))
                wqkv[i * CH + 2 * j + 1, rows, :] = _as_u32((w >> 16).astype(jnp.uint16))

        def relayout_swap(i, slot, d0, z):
            v = stage[slot, d0:d0 + 16].reshape(16 * CH, 128)
            v = _as_bf16(or_tile(_as_u32(v), z)).reshape(16, CH, 128)
            wqkv[pl.ds(i * CH, CH), d0 // 2:d0 // 2 + 8, :] = _as_u32(jnp.swapaxes(v, 0, 1))

        def relayout_jobs(jobs, nrel, i, slot):
            if SWAP:
                for b in range(D // 16):
                    jobs.setdefault(b * nrel // (D // 16), []).append(
                        functools.partial(relayout_swap, i, slot, b * 16))
                return
            nb = D // RB
            for b in range(nb + RLAG):
                t = b * nrel // (nb + RLAG)
                if b >= RLAG:
                    jobs.setdefault(t, []).append(functools.partial(relayout2, i, (b - RLAG) * RB))
                if b < nb:
                    jobs.setdefault(t, []).append(functools.partial(relayout1, slot, b * RB))

        for g in range(4):
            mod_copy(g).start()
        x_copy(0).start()
        for q in range(4):
            c0_copy(q).start()
        chunk_copy(0, 1, 1).start()
        chunk_copy(0, 2, 2).start()

        def decode(i):
            lo = i < 2 * SEG
            head = jnp.where(lo, i // SEG, (i - 2 * SEG) // M)
            is_mem = jnp.logical_and(lo, i % SEG >= XR)
            pos = jnp.where(lo, i % SEG, XR + i % M)
            return head, is_mem, pos

        qh, qm, qp = decode(lax.broadcasted_iota(jnp.int32, (PR, PR), 0))
        kh, km, kp = decode(lax.broadcasted_iota(jnp.int32, (PR, PR), 1))
        vis = qm | km | (qp >= kp)
        mk[...] = jnp.where(qh == kh, jnp.where(vis, 0.0, NEG_MASK * LOG2E), -jnp.inf).astype(F32)
        mod[6] = jnp.broadcast_to(wr_ref[...].astype(F32).reshape(1, D), (M, D))
        zero_s[...] = jnp.zeros(zero_s.shape, U32)
        topv[...] = jnp.full(topv.shape, -jnp.inf, F32)
        topi[...] = lax.broadcasted_iota(jnp.int32, topi.shape, 0)
        cv = c_ref[...].astype(F32)
        sc_s[...] = jnp.broadcast_to(cv * _rb(jax.nn.sigmoid(cv)), (M, D)).astype(BF16)
        mb = mem0_ref[...]
        for k in range(NT):
            lhs[0, k, XR // 2:, :] = _as_u32(mb[:, k * 128:(k + 1) * 128])

        with jax.named_scope("p_mod"):
            for g in range(4):
                mod_copy(g).wait()
                for t in range(4):
                    mod_tile(wmod_s[g, :, t * 128:(t + 1) * 128], 4 * g + t)
        with jax.named_scope("p_xwait"):
            x_copy(0).wait()

        def ln_body(i, c):
            for u in range(LNU):
                q = (i * LNU + u) * 2
                hb = ln1(xbuf[pl.ds(q, 2), XR:, :].reshape(16, D))
                r2 = pl.multiple_of(q * 4, 8)
                for k in range(NT):
                    h0[k, pl.ds(r2, 8), :] = _as_u32(hb[:, k * 128:(k + 1) * 128])
            return c

        with jax.named_scope("p_ln"):
            lax.fori_loop(0, NSEG // (2 * LNU), ln_body, 0)
        with jax.named_scope("p_c0"):
            for q in range(4):
                c0_copy(q).wait()
                for d0 in range(q * (D // 4), (q + 1) * (D // 4), RB):
                    relayout1(0, d0)
                for d0 in range(q * (D // 4), (q + 1) * (D // 4), RB):
                    relayout2(0, d0)

        def bulk(i, heads, jobs):
            n = 0
            due = {}
            for hh in heads:
                a = (hh % 2) * M
                for r in range(0, R0, MB):
                    ts = [h0[k, r // 2:(r + MB) // 2, :] for k in range(NT)]
                    for z in due.pop(n, ()):
                        ts[0] = jnp.concatenate([ts[0][0:8] | z, ts[0][8:]], axis=0)
                    hv = jnp.concatenate([_as_bf16(t) for t in ts], axis=1)
                    y = _dot(hv, _as_bf16(wqkv[i * CH + hh]))
                    pre[i * (CH // 2) + hh // 2, r // M:(r + MB) // M, a:a + M, :] = (
                        y.reshape(MB // M, M, DH).astype(BF16))
                    for u in range(NREL):
                        for job in jobs.get(n * NREL + u, ()):
                            zr = u * (MB - 8) // max(NREL - 1, 1) // 8 * 8
                            res = job(zero_after(y[zr:zr + 8]))
                            if res is not None and JOB_SPAN:
                                due.setdefault(n + JOB_SPAN, []).append(zero_after(res))
                    n += 1

        def start_chunk(nxt):
            for mat in range(3):
                @pl.when(jnp.logical_and(nxt < NCHUNK, nxt // (H // CH) == mat))
                def _():
                    g = pl.multiple_of((nxt % (H // CH)) * CH, CH)
                    pltpu.make_async_copy(w_hbms[mat].at[:, pl.ds(g, CH), :],
                                          stage.at[nxt % NSLOT], sem.at[10 + nxt % NSLOT]).start()

        def body_a(i, c):
            start_chunk(i + NSLOT - 1)

            @pl.when(i == 0)
            def _():
                x_copy(1).start()

            @pl.when(i > 0)
            def _():
                wo_copy(i - 1, pl.multiple_of((i - 1) * 128, 128)).start()

            bulk(i, range(CH // 2), {})
            chunk_copy(0, 0, (i + 1) % NSLOT).wait()
            nrel = ((CH // 2) * (R0 // MB) - 1) * NREL
            jobs = {}
            relayout_jobs(jobs, nrel, i + 1, (i + 1) % NSLOT)
            bulk(i, range(CH // 2, CH), jobs)
            return c

        def body_b(i, c):
            start_chunk(i + NSLOT - 1)

            @pl.when(i - 1 < NT)
            def _():
                wo_copy(i - 1, pl.multiple_of((i - 1) * 128, 128)).start()

            slot1 = (i + 1) % NSLOT

            @pl.when(i + 1 < NCHUNK)
            def _():
                chunk_copy(0, 0, slot1).wait()

            jw = i - NA
            wo_copy(jw, 0).wait()
            n = WOB

            def wo_job(b, z):
                wo_s[jw, b * n // 2:(b + 1) * n // 2, :] = or_tile(
                    _as_u32(wo_raw[jw, b * n:(b + 1) * n, :]), z)

            def ln_job(b, z):
                seg = jw * CH + b // 3
                r = (b % 3) * 8
                hb = ln1(xbuf[seg, r:r + 8, :], z)
                u = [_as_u32(hb[:, k * 128:(k + 1) * 128]) for k in range(NT)]
                for k in range(NT):
                    hs[seg, k, r // 2:r // 2 + 4, :] = u[k]
                res = jnp.concatenate(u[0:2], axis=0)
                for k in range(2, NT, 2):
                    res = res | jnp.concatenate(u[k:k + 2], axis=0)
                return res

            nrel = (CH * (R0 // MB) - 1) * NREL
            nln = (CH * (R0 // MB) - JOB_SPAN) * NREL
            jobs = {}
            for b in range(3 * CH):
                jobs.setdefault(b * nln // (3 * CH), []).append(functools.partial(ln_job, b))
            relayout_jobs(jobs, nrel, i + 1, slot1)
            for b in range(H * DH // n):
                jobs.setdefault((2 * b + 1) * nrel // (2 * H * DH // n), []).append(
                    functools.partial(wo_job, b))
            bulk(i, range(CH), jobs)
            return c

        with jax.named_scope("p_loopa"):
            lax.fori_loop(0, NA, body_a, 0)
        with jax.named_scope("p_xwait2"):
            x_copy(1).wait()
        with jax.named_scope("p_loopb"):
            lax.fori_loop(NA, NCHUNK, body_b, 0)

    if "pro" in PHASES: pl.run_scoped(
        prologue,
        pltpu.VMEM((NSLOT, D, CH, 128), BF16),
        pltpu.VMEM((NT, H * DH, 128), BF16),
        pltpu.VMEM((4, D, 512), BF16),
        pltpu.VMEM((NT, R0 // 2 + PADS[0], 128), U32),
        pltpu.VMEM((D * CH // 2 + PADS[1], 128), U32),
    )

    def load_x_rows(slot, seg):
        for k in range(NT):
            lhs[slot, k, 0:XR // 2, :] = hs[seg, k]

    def post(seg, r, z=None):
        rows = pl.ds(r, 8)
        t = mod[2] * ybuf[seg, rows, :].astype(F32)
        if z is not None:
            t = t + jnp.concatenate([pltpu.bitcast(z, F32)] * NT, axis=1)
        x1 = _rb(xbuf[seg, rows, :].astype(F32) + t)
        xbuf[seg, rows, :] = x1.astype(BF16)
        h2 = _rb(_ln_mod(x1, mod[4], mod[3]))
        o = x1 + mod[5] * h2
        outs[seg, rows, :] = o.astype(BF16)
        v = _rb(jnp.sum(h2 * mod[6], axis=-1, keepdims=True))
        m1, m2, i1, i2 = topv[0:8, :], topv[8:16, :], topi[0:8, :], topi[8:16, :]
        idx = lax.broadcasted_iota(jnp.int32, (8, 1), 0) + (seg * SEG + r)
        g1 = (v > m1) | ((v == m1) & (idx < i1))
        g2 = (v > m2) | ((v == m2) & (idx < i2))
        topv[8:16, :] = jnp.where(g1, m1, jnp.where(g2, v, m2))
        topi[8:16, :] = jnp.where(g1, i1, jnp.where(g2, idx, i2))
        topv[0:8, :] = jnp.where(g1, v, m1)
        topi[0:8, :] = jnp.where(g1, idx, i1)
        if z is not None:
            res = pltpu.bitcast(jnp.broadcast_to(v, (8, 128)), U32)
            if PIN_OUT:
                for k in range(NT):
                    res = res | pltpu.bitcast(o[:, k * 128:(k + 1) * 128], U32)
            return res

    def out_copy(g0, ng, r, n, k=0):
        return pltpu.make_async_copy(outs.at[pl.ds(g0, ng), pl.ds(r, n), :],
                                     out_hbm.at[pl.ds(g0, ng), pl.ds(r, n), :], sem_out.at[k])

    def main(wg_s, wu_s, wd_s, wmod_s, sem_f):
        def col_copy(src, dst, j, off, k):
            return pltpu.make_async_copy(src.at[:, pl.ds(pl.multiple_of((off + j) * 128, 128), 128)],
                                         dst.at[j], sem_f.at[k])

        late = ((wmod_hbm, wmod_s, 2 * NT, 4 * NT), (wg_hbm, wg_s, 0, FF // 128),
                (wu_hbm, wu_s, 0, FF // 128), (wd_hbm, wd_s, 0, NT))

        def wait_late(k):
            src, dst, off, n = late[k]
            for j in range(n):
                col_copy(src, dst, j, off, k).wait()

        if PHASES == ("pro",):
            return
        load_x_rows(0, 0)

        def step(s, cur):
            nxt = (cur + 1) % UNROLL
            drow = pl.multiple_of(s * M, M)

            def lv(k0, k1):
                return jnp.concatenate([_as_bf16(lhs[cur, k]) for k in range(k0, k1)], axis=1)

            def qkv(p, split=False):
                part = {}
                if split:
                    for mat in range(3):
                        for a in range(2):
                            part[mat, a] = _dot(
                                lv(0, NT // 2), _as_bf16(wqkv[mat * H + 2 * p + a, :D // 4, :]))
                for mat in range(3):
                    for a in range(2):
                        hm = mat * H + 2 * p + a
                        if split:
                            y = _dot(lv(NT // 2, NT), _as_bf16(wqkv[hm, D // 4:, :])) + part[mat, a]
                        else:
                            y = _dot(lv(0, NT), _as_bf16(wqkv[hm]))
                        cur_s[hm] = y.astype(BF16)

            def gather(mat, p):
                hm = mat * H + 2 * p
                return jnp.concatenate([cur_s[hm], cur_s[hm + 1], pre[mat * NP + p, s]], axis=0)

            probs = {}

            def scores(p):
                sc = lax.dot_general(gather(0, p), gather(1, p), (((1,), (1,)), ((), ())),
                                     preferred_element_type=F32)
                mv = mk[...]
                sc = jnp.where(mv == 0.0, sc * (SCALE * LOG2E), mv)
                e = jnp.exp2(sc - jnp.max(sc, axis=-1, keepdims=True))
                probs[p] = (e.astype(BF16), _recip(jnp.sum(e, axis=-1, keepdims=True)))

            def pv(p):
                e, inv = probs.pop(p)
                o = (_dot(e, gather(2, p)) * inv).astype(BF16)
                for a in range(2):
                    h = 2 * p + a
                    olhs[h] = _as_u32(o[a * SEG:(a + 1) * SEG])
                    odef[h, pl.ds(drow, M), :] = o[2 * SEG + a * M:2 * SEG + (a + 1) * M]

            acc = [None] * NT

            def oproj(j, pairs):
                ov = jnp.concatenate([_as_bf16(olhs[2 * p + a]) for p in pairs for a in range(2)],
                                     axis=1)
                w = wo_s[j, pairs[0] * DH:(pairs[-1] + 1) * DH, :]
                y = _dot(ov, _as_bf16(w))
                acc[j] = y if acc[j] is None else y + acc[j]

            def fin(j):
                yb = acc[j].astype(BF16)
                ybuf[s, 0:XR, j * 128:(j + 1) * 128] = yb[0:XR]
                lhs[nxt, j, XR // 2:, :] = _as_u32(yb[XR:])

            load_x_rows(nxt, jnp.minimum(s + 1, NSEG - 1))
            ops = dict(Q=qkv, S=scores, P=pv, O=oproj, F=fin)
            for op in _schedule():
                ops[op[0]](*op[1:])

        def steps(i, carry):
            for u in range(UNROLL // 2):
                t = i * (UNROLL // 2) + u
                for k, (src, dst, off, n) in enumerate(late):
                    @pl.when(t < n)
                    def _():
                        col_copy(src, dst, t, off, k).start()

            for u in range(UNROLL):
                step(i * UNROLL + u, u)
            return carry

        with jax.named_scope("m_steps"):
            if "step" in PHASES: lax.fori_loop(0, NSEG // UNROLL, steps, 0)
        if "epi" not in PHASES:
            for k in range(4):
                wait_late(k)
            return

        with jax.named_scope("e_mod"):
            wait_late(0)
            for t in range(4 * NT):
                mod_tile(wmod_s[t], 2 * NT + t)

        gpi = PPI // (XR // 8)

        def ep_body(i, c):
            @pl.when(i > 0)
            def _():
                out_copy((i - 1) * gpi, gpi, 0, XR).start()

            r = pl.multiple_of(i * EC, EC)
            g0 = i * (EC // M)
            nk = H // EKH
            nrel = (NT * nk - E_SPAN) * E_NREL
            jobs = {}
            for u in range(PPI):
                jobs.setdefault(u * nrel // PPI, []).append(u)
            due = {}
            n = 0
            for j in range(NT):
                y = None
                for kk in range(nk):
                    ts = [odef[h, pl.ds(r, EC), :] for h in range(kk * EKH, (kk + 1) * EKH)]
                    for z in due.pop(n, ()):
                        ts[0] = jnp.concatenate(
                            [_as_bf16(_as_u32(ts[0][0:16]) | z), ts[0][16:]], axis=0)
                    w = wo_s[j, kk * EKH * DH // 2:(kk + 1) * EKH * DH // 2, :]
                    yp = _dot(jnp.concatenate(ts, axis=1), _as_bf16(w))
                    y = yp if y is None else yp + y
                    if kk == nk - 1:
                        ybuf[pl.ds(g0, EC // M), XR:, j * 128:(j + 1) * 128] = (
                            y.reshape(EC // M, M, 128).astype(BF16))
                    for q in range(E_NREL):
                        for u in jobs.get(n * E_NREL + q, ()):
                            zr = q * (EC - 8) // max(E_NREL - 1, 1) // 8 * 8
                            t = i * PPI + u
                            early = t < NSEG * (XR // 8)
                            seg = jnp.where(early, t // (XR // 8), t - NSEG * (XR // 8))
                            row = pl.multiple_of(jnp.where(early, (t % (XR // 8)) * 8, XR), 8)
                            res = post(seg, row, zero_after(y[zr:zr + 8]))
                            due.setdefault(n + E_SPAN, []).append(zero_after(res))
                    n += 1
            return c

        with jax.named_scope("e_loop"):
            lax.fori_loop(0, NEC, ep_body, 0)
        done = (NEC - 1) * gpi
        tail = NSEG - EC // M
        out_copy(done, NSEG - done, 0, XR).start()
        out_copy(0, tail, XR, M).start()
        for g in range(tail, NSEG):
            post(g, XR)
        out_copy(tail, NSEG - tail, XR, M).start()

        tv = topv[...]
        ti = topi[...]
        m1 = jnp.max(tv, axis=0, keepdims=True)
        i1v = jnp.min(jnp.where(tv == m1, ti, S), axis=0, keepdims=True)
        rest = ti != i1v
        m2 = jnp.max(jnp.where(rest, tv, -jnp.inf), axis=0, keepdims=True)
        i2v = jnp.min(jnp.where(jnp.logical_and(rest, tv == m2), ti, S), axis=0, keepdims=True)
        i1 = jnp.clip(i1v[0, 0], 0, S - 1)
        i2 = jnp.clip(i2v[0, 0], 0, S - 1)
        g1, g2 = i1 // SEG, i2 // SEG
        b1 = pl.multiple_of((i1 % SEG) // 8 * 8, 8)
        b2 = pl.multiple_of((i2 % SEG) // 8 * 8, 8)

        x1 = jnp.stack([xbuf[g1, pl.ds(b1, 8), :].astype(F32),
                        xbuf[g2, pl.ds(b2, 8), :].astype(F32)])
        h2 = _rb(_ln_mod(x1, mod[4], mod[3])).reshape(16, D)
        x1 = x1.reshape(16, D)
        h2b = h2.astype(BF16)
        row = lax.broadcasted_iota(jnp.int32, (16, 1), 0)
        grow = jnp.where(row < 8, g1 * SEG + b1 + row, g2 * SEG + b2 + row - 8)
        rsel = jnp.where(grow == i1, m1, m2)
        with jax.named_scope("e_ffnwait"):
            for k in range(1, 4):
                wait_late(k)
        acts = []
        for j in range(FF // 128):
            gt = _rb(_dot(h2b, wg_s[j]))
            gt = _rb(gt * _rb(jax.nn.sigmoid(gt)))
            ut = _rb(_dot(h2b, wu_s[j]))
            acts.append((gt * ut).astype(BF16))
        act = jnp.concatenate(acts, axis=1)
        y = _rb(jnp.concatenate([_dot(act, wd_s[j]) for j in range(NT)], axis=1))
        y = _rb(y * _rb(jax.nn.sigmoid(rsel)))
        sel = jnp.logical_or(grow == i1, grow == i2)
        hb = _rb(h2 + jnp.where(sel, y, 0.0))
        fixed = (x1 + mod[5, 0:1, :] * hb).astype(BF16)

        with jax.named_scope("e_outwait"):
            out_copy(0, NSEG, 0, SEG).wait()
        outs[g1, pl.ds(b1, 8), :] = fixed[0:8]
        outs[g2, pl.ds(b2, 8), :] = fixed[8:16]
        out_copy(g1, 1, b1, 8, 0).start()

        @pl.when(i1 // 8 != i2 // 8)
        def _():
            out_copy(g2, 1, b2, 8, 1).start()
            out_copy(g2, 1, b2, 8, 1).wait()

        out_copy(g1, 1, b1, 8, 0).wait()

    pl.run_scoped(
        main,
        pltpu.VMEM((FF // 128, D, 128), BF16),
        pltpu.VMEM((FF // 128, D, 128), BF16),
        pltpu.VMEM((NT, FF, 128), BF16),
        pltpu.VMEM((4 * NT, D, 128), BF16),
        pltpu.SemaphoreType.DMA((4,)),
    )


@functools.partial(jax.jit, static_argnames=("A_seg_len",))
def pallas_adaLN_cond__memory_aug_recurrent_mem_tr__moe_arch_mod__prompt_kernel(
    A_x: jax.Array,
    A_mem0: jax.Array,
    A_Wq: jax.Array,
    A_Wk: jax.Array,
    A_Wv: jax.Array,
    A_Wo: jax.Array,
    A_seg_len,
    B_x: jax.Array,
    B_w_r: jax.Array,
    B_w_gate: jax.Array,
    B_w_up: jax.Array,
    B_w_down: jax.Array,
    c: jax.Array,
    w_mod: jax.Array,
):
    assert A_seg_len == SEG and A_x.shape == (1, S, D)
    del B_x
    hbm = pl.BlockSpec(memory_space=pl.ANY)
    vmem = pl.BlockSpec(memory_space=pltpu.VMEM)
    out = pl.pallas_call(
        _kernel,
        out_shape=jax.ShapeDtypeStruct((NSEG, SEG, D), BF16),
        in_specs=[hbm, vmem, hbm, hbm, hbm, hbm, vmem, hbm, hbm, hbm, vmem, hbm],
        out_specs=hbm,
        scratch_shapes=[
            pltpu.VMEM((3 * H + CH, D // 2, DH), U32),
            pltpu.VMEM((NSEG, NT, XR // 2, 128), U32),
            pltpu.VMEM((NT, H * DH // 2, 128), U32),
            pltpu.VMEM((3 * NP, NSEG, 2 * M, DH), BF16),
            pltpu.VMEM((3 * H, SEG, DH), BF16),
            pltpu.VMEM((H, SEG // 2, DH), U32),
            pltpu.VMEM((H, R0, DH), BF16),
            pltpu.VMEM((NSEG, SEG, D), BF16),
            pltpu.VMEM((NSEG, SEG, D), BF16),
            pltpu.VMEM((NSEG, SEG, D), BF16),
            pltpu.VMEM((UNROLL, NT, SEG // 2, 128), U32),
            pltpu.VMEM((7, M, D), F32),
            pltpu.VMEM((PR, PR), F32),
            pltpu.VMEM((16, 1), F32),
            pltpu.VMEM((16, 1), jnp.int32),
            pltpu.VMEM((M, D), BF16),
            pltpu.VMEM((8 + PADS[2], 128), U32),
            pltpu.SemaphoreType.DMA((10 + NSLOT + NT,)),
            pltpu.SemaphoreType.DMA((2,)),
        ],
        compiler_params=pltpu.CompilerParams(vmem_limit_bytes=120 * 1024 * 1024,
                                             disable_bounds_checks=True),
    )(A_x.reshape(NSEG, SEG, D), A_mem0.reshape(M, D), A_Wq, A_Wk, A_Wv, A_Wo.reshape(H * DH, D),
      B_w_r, B_w_gate, B_w_up, B_w_down, c, w_mod)
    return out.reshape(1, S, D)
```

```python
import functools

import jax
import jax.numpy as jnp
from jax import lax
import jax.experimental.pallas as pl
import jax.experimental.pallas.tpu as pltpu

F32 = jnp.float32
BF16 = jnp.bfloat16
U32 = jnp.uint32

D = 1024
S = 2048
H = 32
DH = 128
M = 8
SEG = 32
NSEG = S // SEG
FF = 3584
NT = D // 128
XR = SEG - M
R0 = M * NSEG
CH = 8
NCHUNK = 3 * H // CH
NSLOT = 4
PR = 2 * SEG + 2 * M
NP = H // 2
EC = 128
NEC = R0 // EC
PPI = (S // 8 - EC // 8) // NEC
LOG2E = 1.4426950408889634
EPS = 1e-5
SCALE = DH ** -0.5
NEG_MASK = -1000000000.0

PHASES = ("pro", "step", "epi")
UNROLL = 4
MB = 128
RB = 16
RB2 = 64
NREL = 4
JOB_SPAN = 3
LNU = 8
EKH = 4
E_SPAN = 6
PADS = (0, 0, 0)
MOD_POS = 1
R1_END = 11
R2_0 = (3, 14)
LN_RANGE = (0, 29)
WO_RANGE = (12, 31)


def _schedule(with_mod):
    groups = [list(range(4 * g, 4 * g + 4)) for g in range(4)]
    ops = []
    for t in range(4):
        for i, p in enumerate(groups[t]):
            ops.append(("Q", p, p == 0))
            if i == 0 and t >= 1:
                ops.extend(("S", q) for q in groups[t - 1])
            if i == 3 and t >= 1:
                ops.extend(("P", q) for q in groups[t - 1])
                if with_mod and t == MOD_POS:
                    ops.append(("M",))
    first = groups[0] + groups[1]
    for j in range(NT):
        ops.append(("O", j, first))
        if j == 1:
            ops.extend(("S", q) for q in groups[3])
    ops.extend(("P", q) for q in groups[3])
    ops.extend(("O", j, groups[2]) for j in range(NT))
    for j in range(NT):
        ops.append(("O", j, groups[3]))
        ops.append(("F", j))
    return ops


def _rb(x):
    return x.astype(BF16).astype(F32)


def _recip(x):
    r = pl.reciprocal(x, approx=True)
    return r * (2.0 - x * r)


def _ln_mod(x, s1p, shift, zero=None):
    xm = x if zero is None else jnp.concatenate([x[..., :128] + zero, x[..., 128:]], axis=-1)
    xc = x - jnp.mean(xm, axis=-1, keepdims=True)
    v = _rb(_rb(jnp.mean(xc * xc, axis=-1, keepdims=True)) + EPS)
    return xc * _recip(_rb(v * lax.rsqrt(v))) * s1p + shift


def _dot(a, b):
    return jnp.dot(a, b, preferred_element_type=F32)


def _as_bf16(u):
    return pltpu.bitcast(u, BF16)


def _as_u32(b):
    return pltpu.bitcast(b, U32)


def _spread(jobs, fns, lo, hi):
    for n, fn in enumerate(fns):
        jobs.setdefault(lo + n * (hi - lo) // len(fns), []).append(fn)


def _kernel(x_hbm, mem0_ref, wq_hbm, wk_hbm, wv_hbm, wo_hbm, wr_ref, wg_hbm, wu_hbm, wd_hbm,
            c_ref, wmod_hbm, out_hbm,
            wqkv, hs, wo_s, pre, cur_s, olhs, odef, xbuf, ybuf, hbuf, outs, lhs, wm_s, mod, mk,
            topv, topi, sc_s, zero_s, sem_m, sem_out):
    mt = 4 * NT * UNROLL // NSEG

    def modv(j):
        return jnp.concatenate([mod[j * NT + k] for k in range(NT)], axis=1)

    def mod_tile(wm, t):
        v = _rb(_dot(sc_s[...], wm))
        mod[t] = jnp.where(jnp.logical_or(t // NT == 1, t // NT == 4), _rb(1.0 + v), v)

    def wm_copy(it, u):
        col = pl.multiple_of((2 * NT + it * mt + u) * 128, 128)
        return pltpu.make_async_copy(wmod_hbm.at[:, pl.ds(col, 128)], wm_s.at[it % 3, u],
                                     sem_m.at[it % 3])

    def ln1(x, zero=None):
        x3 = x.astype(F32).reshape(x.shape[0] // 8, 8, D)
        zf = None if zero is None else pltpu.bitcast(zero, F32)
        return _ln_mod(x3, modv(1), modv(0), zf).reshape(x.shape[0], D).astype(BF16)

    def zero_after(y):
        return (y if y.dtype == U32 else pltpu.bitcast(y, U32)) & zero_s[0:8, :]

    def or_tile(u, z):
        if z is None:
            return u
        return (u.reshape(u.shape[0] // 8, 8, 128) | z).reshape(u.shape)

    def prologue(stage, wo_raw, wmod_s, h0, tmp, sem):
        w_hbms = (wq_hbm, wk_hbm, wv_hbm)
        wob = H * DH // NT

        def x_copy(i):
            lo, n = ((XR, M), (0, XR))[i]
            return pltpu.make_async_copy(x_hbm.at[:, pl.ds(lo, n), :], xbuf.at[:, pl.ds(lo, n), :],
                                         sem.at[i])

        def mod_copy(g):
            return pltpu.make_async_copy(wmod_hbm.at[:, pl.ds(pl.multiple_of(g * 512, 512), 512)],
                                         wmod_s.at[g], sem.at[2 + g])

        def c0_copy(q):
            rows = pl.ds(q * (D // 4), D // 4)
            return pltpu.make_async_copy(wq_hbm.at[rows, pl.ds(0, CH), :], stage.at[0, rows],
                                         sem.at[6 + q])

        def chunk_copy(mat, g, slot):
            return pltpu.make_async_copy(w_hbms[mat].at[:, pl.ds(g, CH), :], stage.at[slot],
                                         sem.at[10 + slot])

        def wo_copy(j):
            return pltpu.make_async_copy(wo_hbm.at[pl.ds(pl.multiple_of(j * wob, wob), wob)],
                                         wo_raw.at[j], sem.at[10 + NSLOT + j])

        def relayout1(src, t0, z=None):
            v = src.reshape(RB * CH, 128)
            tmp[t0:t0 + RB * CH // 2, :] = or_tile(_as_u32(v), z)

        def relayout2(m0, j, t0, rows, z=None):
            w = or_tile(tmp[pl.ds(t0 + j, RB2, stride=CH // 2), :], z)
            wqkv[m0 + 2 * j, rows, :] = _as_u32(w.astype(jnp.uint16))
            wqkv[m0 + 2 * j + 1, rows, :] = _as_u32((w >> 16).astype(jnp.uint16))

        for g in range(4):
            mod_copy(g).start()
        x_copy(0).start()
        for q in range(4):
            c0_copy(q).start()
        for g in range(1, NSLOT):
            chunk_copy(0, g * CH, g).start()
        x_copy(1).start()

        def decode(i):
            lo = i < 2 * SEG
            head = jnp.where(lo, i // SEG, (i - 2 * SEG) // M)
            is_mem = jnp.logical_and(lo, i % SEG >= XR)
            pos = jnp.where(lo, i % SEG, XR + i % M)
            return head, is_mem, pos

        qh, qm, qp = decode(lax.broadcasted_iota(jnp.int32, (PR, PR), 0))
        kh, km, kp = decode(lax.broadcasted_iota(jnp.int32, (PR, PR), 1))
        vis = qm | km | (qp >= kp)
        mk[...] = jnp.where(qh == kh, jnp.where(vis, 0.0, NEG_MASK * LOG2E), -jnp.inf).astype(F32)
        wr = jnp.broadcast_to(wr_ref[...].astype(F32).reshape(1, D), (M, D))
        for k in range(NT):
            mod[6 * NT + k] = wr[:, k * 128:(k + 1) * 128]
        zero_s[...] = jnp.zeros(zero_s.shape, U32)
        topv[...] = jnp.full(topv.shape, -jnp.inf, F32)
        topi[...] = lax.broadcasted_iota(jnp.int32, topi.shape, 0)
        cv = c_ref[...].astype(F32)
        sc_s[...] = jnp.broadcast_to(cv * _rb(jax.nn.sigmoid(cv)), (M, D)).astype(BF16)
        mb = mem0_ref[...]
        for k in range(NT):
            lhs[0, k, XR // 2:, :] = _as_u32(mb[:, k * 128:(k + 1) * 128])

        def zero_body(i, c):
            wo_raw[NT, pl.ds(pl.multiple_of(i * 32, 32), 32), :] = jnp.zeros((32, D), BF16)
            return c

        lax.fori_loop(0, wob // 32, zero_body, 0)

        def mod_body(g, c):
            mod_copy(g).wait()
            for t in range(4):
                mod_tile(wmod_s[g, :, t * 128:(t + 1) * 128], 4 * g + t)
            return c

        with jax.named_scope("p_mod"):
            lax.fori_loop(0, 4, mod_body, 0)
        x_copy(0).wait()

        def ln_body(i, c):
            for u in range(LNU):
                q = (i * LNU + u) * 2
                hb = ln1(xbuf[pl.ds(q, 2), XR:, :].reshape(16, D))
                r2 = pl.multiple_of(q * 4, 8)
                for k in range(NT):
                    h0[k, pl.ds(r2, 8), :] = _as_u32(hb[:, k * 128:(k + 1) * 128])
            return c

        with jax.named_scope("p_ln"):
            lax.fori_loop(0, NSEG // (2 * LNU), ln_body, 0)

        def c0_body(q, c):
            c0_copy(q).wait()
            for d0 in range(0, D // 4, RB):
                relayout1(stage[0, pl.ds(q * (D // 4) + d0, RB)], d0 * CH // 2)
            for d0 in range(0, D // 4, RB2):
                rows = pl.ds(pl.multiple_of(q * (D // 8) + d0 // 2, 8), RB2 // 2)
                for j in range(CH // 2):
                    relayout2(0, j, d0 * CH // 2, rows)
            return c

        with jax.named_scope("p_c0"):
            lax.fori_loop(0, 4, c0_body, 0)

        def bulk(p0, npairs, jobs):
            n = 0
            due = {}
            for hh in range(2 * npairs):
                a = (hh % 2) * M
                for r in range(0, R0, MB):
                    ts = [h0[k, r // 2:(r + MB) // 2, :] for k in range(NT)]
                    for z in due.pop(n, ()):
                        ts[0] = jnp.concatenate([ts[0][0:8] | z, ts[0][8:]], axis=0)
                    hv = jnp.concatenate([_as_bf16(t) for t in ts], axis=1)
                    y = _dot(hv, _as_bf16(wqkv[2 * p0 + hh]))
                    pre[p0 + hh // 2, r // M:(r + MB) // M, a:a + M, :] = (
                        y.reshape(MB // M, M, DH).astype(BF16))
                    for u in range(NREL):
                        for job in jobs.get(n * NREL + u, ()):
                            zr = u * (MB - 8) // (NREL - 1) // 8 * 8
                            res = job(zero_after(y[zr:zr + 8]))
                            if res is not None:
                                due.setdefault(n + JOB_SPAN, []).append(zero_after(res))
                    n += 1
            assert not due

        nlate = NCHUNK - 1 - NT

        def rot_body(i, c):
            slot = (i + 1) % NSLOT
            chunk_copy(0, 0, slot).wait()

            @pl.when(i == nlate)
            def _():
                x_copy(1).wait()

            @pl.when(i >= nlate)
            def _():
                wo_copy(i - nlate).wait()

            nxt = i + NSLOT
            for mat in range(3):
                @pl.when(jnp.logical_and(nxt < NCHUNK, nxt // (H // CH) == mat))
                def _():
                    chunk_copy(mat, pl.multiple_of((nxt % (H // CH)) * CH, CH), nxt % NSLOT).start()

            @pl.when(i < NT)
            def _():
                wo_copy(i).start()

            live = i >= nlate
            jw = jnp.where(live, i - nlate, NT)
            p0 = i * (CH // 2) + CH // 4
            m1 = 2 * p0 + CH // 2

            def wo_job(b, z):
                v = wo_raw[jw, b * 16:(b + 1) * 16, :]
                rows = pl.ds(pl.multiple_of(jw * (wob // 2) + b * 8, 8), 8)
                for j in range(NT):
                    wo_s[j, rows, :] = _as_u32(v[:, j * 128:(j + 1) * 128]) | z

            def ln_job(b, z):
                r = (b % 3) * 8
                src = jnp.where(live, (i - nlate) * CH + b // 3, 0)
                hb = ln1(xbuf[src, pl.ds(pl.multiple_of(jnp.where(live, r, XR), 8), 8), :], z)
                u = [_as_u32(hb[:, k * 128:(k + 1) * 128]) for k in range(NT)]
                dst = jnp.where(live, src, NSEG)
                for k in range(NT):
                    hs[dst, k, r // 2:r // 2 + 4, :] = u[k]
                res = jnp.concatenate(u[0:2], axis=0)
                for k in range(2, NT, 2):
                    res = res | jnp.concatenate(u[k:k + 2], axis=0)
                return res

            def r1_job(d0, z):
                relayout1(stage[slot, d0:d0 + RB], d0 * CH // 2, z)

            def r2_jobs(j):
                return [functools.partial(relayout2, m1, j, d0 * CH // 2,
                                          pl.ds(d0 // 2, RB2 // 2)) for d0 in range(0, D, RB2)]

            jobs = {}
            _spread(jobs, [functools.partial(r1_job, d0) for d0 in range(0, D, RB)],
                    0, R1_END * NREL)
            _spread(jobs, r2_jobs(0), R2_0[0] * NREL, R2_0[1] * NREL)
            _spread(jobs, r2_jobs(1) + r2_jobs(2) + r2_jobs(3), R2_0[1] * NREL, 31 * NREL)
            _spread(jobs, [functools.partial(ln_job, b) for b in range(3 * CH)],
                    LN_RANGE[0] * NREL, LN_RANGE[1] * NREL)
            _spread(jobs, [functools.partial(wo_job, b) for b in range(wob // 16)],
                    WO_RANGE[0] * NREL, WO_RANGE[1] * NREL)
            bulk(p0, CH // 2, jobs)
            return c

        def outer(k, c):
            bulk(k * (3 * NP - CH // 4), CH // 4, {})

            @pl.when(k == 0)
            def _():
                with jax.named_scope("p_rot"):
                    lax.fori_loop(0, NCHUNK - 1, rot_body, 0)
                for it in range(2):
                    for u in range(mt):
                        wm_copy(it, u).start()

            return c

        with jax.named_scope("p_bulk"):
            lax.fori_loop(0, 2, outer, 0)

    if "pro" in PHASES: pl.run_scoped(
        prologue,
        pltpu.VMEM((NSLOT, D, CH, 128), BF16),
        pltpu.VMEM((NT + 1, H * DH // NT, D), BF16),
        pltpu.VMEM((4, D, 512), BF16),
        pltpu.VMEM((NT, R0 // 2 + PADS[0], 128), U32),
        pltpu.VMEM((D * CH // 2 + PADS[1], 128), U32),
        pltpu.SemaphoreType.DMA((10 + NSLOT + NT,)),
    )

    def load_x_rows(slot, seg):
        for k in range(NT):
            lhs[slot, k, 0:XR // 2, :] = hs[seg, k]

    def post(seg, r, z=None):
        rows = pl.ds(r, 8)
        t = modv(2) * ybuf[seg, rows, :].astype(F32)
        if z is not None:
            t = t + jnp.concatenate([pltpu.bitcast(z, F32)] * NT, axis=1)
        x1 = _rb(xbuf[seg, rows, :].astype(F32) + t)
        xbuf[seg, rows, :] = x1.astype(BF16)
        h2b = _ln_mod(x1, modv(4), modv(3)).astype(BF16)
        hbuf[seg, rows, :] = h2b
        h2 = h2b.astype(F32)
        o = x1 + modv(5) * h2
        outs[seg, rows, :] = o.astype(BF16)
        v = _rb(jnp.sum(h2 * modv(6), axis=-1, keepdims=True))
        m1, m2, i1, i2 = topv[0:8, :], topv[8:16, :], topi[0:8, :], topi[8:16, :]
        idx = lax.broadcasted_iota(jnp.int32, (8, 1), 0) + (seg * SEG + r)
        g1 = (v > m1) | ((v == m1) & (idx < i1))
        g2 = (v > m2) | ((v == m2) & (idx < i2))
        topv[8:16, :] = jnp.where(g1, m1, jnp.where(g2, v, m2))
        topi[8:16, :] = jnp.where(g1, i1, jnp.where(g2, idx, i2))
        topv[0:8, :] = jnp.where(g1, v, m1)
        topi[0:8, :] = jnp.where(g1, idx, i1)
        if z is not None:
            res = pltpu.bitcast(jnp.broadcast_to(v, (8, 128)), U32)
            for k in range(NT):
                res = res | pltpu.bitcast(o[:, k * 128:(k + 1) * 128], U32)
            return res

    def out_copy(g0, ng, r, n, k=0):
        return pltpu.make_async_copy(outs.at[pl.ds(g0, ng), pl.ds(r, n), :],
                                     out_hbm.at[pl.ds(g0, ng), pl.ds(r, n), :], sem_out.at[k])

    def main(wg_s, wu_s, wd_s, sem_f):
        late = ((wg_hbm, wg_s, FF // 128), (wu_hbm, wu_s, FF // 128), (wd_hbm, wd_s, NT))

        def col_copy(k, j):
            return pltpu.make_async_copy(
                late[k][0].at[:, pl.ds(pl.multiple_of(j * 128, 128), 128)], late[k][1].at[j],
                sem_f.at[k])

        load_x_rows(0, 0)

        def step(it, cur):
            s = it * UNROLL + cur
            nxt = (cur + 1) % UNROLL
            drow = pl.multiple_of(s * M, M)

            def lv(k0, k1):
                return jnp.concatenate([_as_bf16(lhs[cur, k]) for k in range(k0, k1)], axis=1)

            def qkv(p, split=False):
                part = {}
                if split:
                    for mat in range(3):
                        for a in range(2):
                            part[mat, a] = _dot(
                                lv(0, NT // 2), _as_bf16(wqkv[mat * H + 2 * p + a, :D // 4, :]))
                for mat in range(3):
                    for a in range(2):
                        hm = mat * H + 2 * p + a
                        if split:
                            y = _dot(lv(NT // 2, NT), _as_bf16(wqkv[hm, D // 4:, :])) + part[mat, a]
                        else:
                            y = _dot(lv(0, NT), _as_bf16(wqkv[hm]))
                        cur_s[hm] = y.astype(BF16)

            def gather(mat, p):
                hm = mat * H + 2 * p
                return jnp.concatenate([cur_s[hm], cur_s[hm + 1], pre[mat * NP + p, s]], axis=0)

            probs = {}

            def scores(p):
                sc = lax.dot_general(gather(0, p), gather(1, p), (((1,), (1,)), ((), ())),
                                     preferred_element_type=F32)
                mv = mk[...]
                sc = jnp.where(mv == 0.0, sc * (SCALE * LOG2E), mv)
                e = jnp.exp2(sc - jnp.max(sc, axis=-1, keepdims=True))
                probs[p] = (e.astype(BF16), _recip(jnp.sum(e, axis=-1, keepdims=True)))

            def pv(p):
                e, inv = probs.pop(p)
                o = (_dot(e, gather(2, p)) * inv).astype(BF16)
                for a in range(2):
                    h = 2 * p + a
                    olhs[h] = _as_u32(o[a * SEG:(a + 1) * SEG])
                    odef[h, pl.ds(drow, M), :] = o[2 * SEG + a * M:2 * SEG + (a + 1) * M]

            acc = [None] * NT

            def oproj(j, pairs):
                ov = jnp.concatenate([_as_bf16(olhs[2 * p + a]) for p in pairs for a in range(2)],
                                     axis=1)
                w = wo_s[j, pairs[0] * DH:(pairs[-1] + 1) * DH, :]
                y = _dot(ov, _as_bf16(w))
                acc[j] = y if acc[j] is None else y + acc[j]

            def fin(j):
                yb = acc[j].astype(BF16)
                ybuf[s, 0:XR, j * 128:(j + 1) * 128] = yb[0:XR]
                lhs[nxt, j, XR // 2:, :] = _as_u32(yb[XR:])

            def late_mod():
                u = cur // 2
                mod_tile(wm_s[it % 3, u], 2 * NT + it * mt + u)

            load_x_rows(nxt, jnp.minimum(s + 1, NSEG - 1))
            ops = dict(Q=qkv, S=scores, P=pv, O=oproj, F=fin, M=late_mod)
            for op in _schedule(cur % 2 == 1):
                ops[op[0]](*op[1:])

        def steps(it, carry):
            if "pro" in PHASES:
                for u in range(mt):
                    wm_copy(it, u).wait()

                @pl.when(it + 2 < NSEG // UNROLL)
                def _():
                    for u in range(mt):
                        wm_copy(it + 2, u).start()

            for u in range(UNROLL // 2):
                t = it * (UNROLL // 2) + u
                for k in range(3):
                    @pl.when(t < late[k][2])
                    def _():
                        col_copy(k, t).start()

            for u in range(UNROLL):
                step(it, u)
            return carry

        with jax.named_scope("m_steps"):
            if "step" in PHASES: lax.fori_loop(0, NSEG // UNROLL, steps, 0)
        for k in range(3):
            for j in range(late[k][2]):
                col_copy(k, j).wait()
        if "epi" not in PHASES:
            return

        gpi = PPI // (XR // 8)

        def ep_body(i, c):
            @pl.when(i > 0)
            def _():
                out_copy((i - 1) * gpi, gpi, 0, XR).start()

            r = pl.multiple_of(i * EC, EC)
            g0 = i * (EC // M)
            nk = H // EKH
            jobs = {}
            _spread(jobs, list(range(PPI)), 0, NT * nk - E_SPAN)
            due = {}
            n = 0
            for j in range(NT):
                y = None
                for kk in range(nk):
                    ts = [odef[h, pl.ds(r, EC), :] for h in range(kk * EKH, (kk + 1) * EKH)]
                    for z in due.pop(n, ()):
                        ts[0] = jnp.concatenate(
                            [_as_bf16(_as_u32(ts[0][0:16]) | z), ts[0][16:]], axis=0)
                    w = wo_s[j, kk * EKH * DH // 2:(kk + 1) * EKH * DH // 2, :]
                    yp = _dot(jnp.concatenate(ts, axis=1), _as_bf16(w))
                    y = yp if y is None else yp + y
                    if kk == nk - 1:
                        ybuf[pl.ds(g0, EC // M), XR:, j * 128:(j + 1) * 128] = (
                            y.reshape(EC // M, M, 128).astype(BF16))
                    for u in jobs.get(n, ()):
                        t = i * PPI + u
                        early = t < NSEG * (XR // 8)
                        seg = jnp.where(early, t // (XR // 8), t - NSEG * (XR // 8))
                        row = pl.multiple_of(jnp.where(early, (t % (XR // 8)) * 8, XR), 8)
                        res = post(seg, row, zero_after(y[0:8]))
                        due.setdefault(n + E_SPAN, []).append(zero_after(res))
                    n += 1
            return c

        with jax.named_scope("e_loop"):
            lax.fori_loop(0, NEC, ep_body, 0)
        done = (NEC - 1) * gpi
        tail = NSEG - EC // M
        out_copy(done, NSEG - done, 0, XR).start()
        out_copy(0, tail, XR, M).start()
        for g in range(tail, NSEG):
            post(g, XR)
        out_copy(tail, NSEG - tail, XR, M).start()

        tv = topv[...]
        ti = topi[...]
        m1 = jnp.max(tv, axis=0, keepdims=True)
        i1v = jnp.min(jnp.where(tv == m1, ti, S), axis=0, keepdims=True)
        rest = ti != i1v
        m2 = jnp.max(jnp.where(rest, tv, -jnp.inf), axis=0, keepdims=True)
        i2v = jnp.min(jnp.where(jnp.logical_and(rest, tv == m2), ti, S), axis=0, keepdims=True)
        i1 = jnp.clip(i1v[0, 0], 0, S - 1)
        i2 = jnp.clip(i2v[0, 0], 0, S - 1)
        g1, g2 = i1 // SEG, i2 // SEG
        b1 = pl.multiple_of((i1 % SEG) // 8 * 8, 8)
        b2 = pl.multiple_of((i2 % SEG) // 8 * 8, 8)

        def two_blocks(ref):
            return jnp.concatenate([ref[g1, pl.ds(b1, 8), :].astype(F32),
                                    ref[g2, pl.ds(b2, 8), :].astype(F32)], axis=0)

        x1 = two_blocks(xbuf)
        h2 = two_blocks(hbuf)
        h2b = h2.astype(BF16)
        row = lax.broadcasted_iota(jnp.int32, (16, 1), 0)
        grow = jnp.where(row < 8, g1 * SEG + b1 + row, g2 * SEG + b2 + row - 8)
        rsel = jnp.where(grow == i1, m1, m2)
        acts = []
        for j in range(FF // 128):
            gt = _rb(_dot(h2b, wg_s[j]))
            gt = _rb(gt * _rb(jax.nn.sigmoid(gt)))
            ut = _rb(_dot(h2b, wu_s[j]))
            acts.append((gt * ut).astype(BF16))
        act = jnp.concatenate(acts, axis=1)
        y = _rb(jnp.concatenate([_dot(act, wd_s[j]) for j in range(NT)], axis=1))
        y = _rb(y * _rb(jax.nn.sigmoid(rsel)))
        sel = jnp.logical_or(grow == i1, grow == i2)
        hb = _rb(h2 + jnp.where(sel, y, 0.0))
        fixed = (x1 + jnp.concatenate([modv(5)] * 2, axis=0) * hb).astype(BF16)

        with jax.named_scope("e_outwait"):
            out_copy(0, NSEG, 0, SEG).wait()
        outs[g1, pl.ds(b1, 8), :] = fixed[0:8]
        outs[g2, pl.ds(b2, 8), :] = fixed[8:16]
        out_copy(g1, 1, b1, 8, 0).start()

        @pl.when(i1 // 8 != i2 // 8)
        def _():
            out_copy(g2, 1, b2, 8, 1).start()
            out_copy(g2, 1, b2, 8, 1).wait()

        out_copy(g1, 1, b1, 8, 0).wait()

    pl.run_scoped(
        main,
        pltpu.VMEM((FF // 128, D, 128), BF16),
        pltpu.VMEM((FF // 128, D, 128), BF16),
        pltpu.VMEM((NT, FF, 128), BF16),
        pltpu.SemaphoreType.DMA((3,)),
    )


@functools.partial(jax.jit, static_argnames=("A_seg_len",))
def pallas_adaLN_cond__memory_aug_recurrent_mem_tr__moe_arch_mod__prompt_kernel(
    A_x: jax.Array,
    A_mem0: jax.Array,
    A_Wq: jax.Array,
    A_Wk: jax.Array,
    A_Wv: jax.Array,
    A_Wo: jax.Array,
    A_seg_len,
    B_x: jax.Array,
    B_w_r: jax.Array,
    B_w_gate: jax.Array,
    B_w_up: jax.Array,
    B_w_down: jax.Array,
    c: jax.Array,
    w_mod: jax.Array,
):
    assert A_seg_len == SEG and A_x.shape == (1, S, D)
    del B_x
    hbm = pl.BlockSpec(memory_space=pl.ANY)
    vmem = pl.BlockSpec(memory_space=pltpu.VMEM)
    out = pl.pallas_call(
        _kernel,
        out_shape=jax.ShapeDtypeStruct((NSEG, SEG, D), BF16),
        in_specs=[hbm, vmem, hbm, hbm, hbm, hbm, vmem, hbm, hbm, hbm, vmem, hbm],
        out_specs=hbm,
        scratch_shapes=[
            pltpu.VMEM((3 * H, D // 2, DH), U32),
            pltpu.VMEM((NSEG + 1, NT, XR // 2, 128), U32),
            pltpu.VMEM((NT, (H * DH + H * DH // NT) // 2, 128), U32),
            pltpu.VMEM((3 * NP, NSEG, 2 * M, DH), BF16),
            pltpu.VMEM((3 * H, SEG, DH), BF16),
            pltpu.VMEM((H, SEG // 2, DH), U32),
            pltpu.VMEM((H, R0, DH), BF16),
            pltpu.VMEM((NSEG, SEG, D), BF16),
            pltpu.VMEM((NSEG, SEG, D), BF16),
            pltpu.VMEM((NSEG, SEG, D), BF16),
            pltpu.VMEM((NSEG, SEG, D), BF16),
            pltpu.VMEM((UNROLL, NT, SEG // 2, 128), U32),
            pltpu.VMEM((3, 4 * NT * UNROLL // NSEG, D, 128), BF16),
            pltpu.VMEM((7 * NT, M, 128), F32),
            pltpu.VMEM((PR, PR), F32),
            pltpu.VMEM((16, 1), F32),
            pltpu.VMEM((16, 1), jnp.int32),
            pltpu.VMEM((M, D), BF16),
            pltpu.VMEM((8 + PADS[2], 128), U32),
            pltpu.SemaphoreType.DMA((3,)),
            pltpu.SemaphoreType.DMA((2,)),
        ],
        compiler_params=pltpu.CompilerParams(vmem_limit_bytes=120 * 1024 * 1024,
                                             disable_bounds_checks=True),
    )(A_x.reshape(NSEG, SEG, D), A_mem0.reshape(M, D), A_Wq, A_Wk, A_Wv, A_Wo.reshape(H * DH, D),
      B_w_r, B_w_gate, B_w_up, B_w_down, c, w_mod)
    return out.reshape(1, S, D)
```

```python
import functools

import jax
import jax.numpy as jnp
from jax import lax
import jax.experimental.pallas as pl
import jax.experimental.pallas.tpu as pltpu

F32 = jnp.float32
BF16 = jnp.bfloat16
U32 = jnp.uint32

D = 1024
S = 2048
H = 32
DH = 128
M = 8
SEG = 32
NSEG = S // SEG
FF = 3584
NT = D // 128
XR = SEG - M
R0 = M * NSEG
CH = 8
NCHUNK = 3 * H // CH
NSLOT = 4
PR = 2 * SEG + 2 * M
NP = H // 2
EC = 128
NEC = R0 // EC
PPI = (S // 8 - EC // 8) // NEC
LOG2E = 1.4426950408889634
EPS = 1e-5
SCALE = DH ** -0.5
NEG_MASK = -1000000000.0

PHASES = ("pro", "step", "epi")
UNROLL = 4
MB = 128
RB = 16
RB2 = 64
NREL = 4
JOB_SPAN = 3
LNU = 8
EKH = 4
E_SPAN = 6
PADS = (0, 0, 0)
MODS = ((-1, 4), (1, 4))
TOK_S = 9
TOK_P = None
TOK_STAG = 2
NORM_PRE = True
R1_END = 11
R2_0 = (3, 14)
LN_RANGE = (0, 29)
WO_RANGE = (12, 31)


def _schedule(mods):
    groups = [list(range(4 * g, 4 * g + 4)) for g in range(4)]
    ops = []

    def mod_at(pos):
        ops.extend(("M", u) for (u, q) in mods if q == pos)

    for t in range(4):
        for i, p in enumerate(groups[t]):
            ops.append(("Q", p, p == 0))
            if i == 0 and t >= 1:
                ops.extend(("S", q) for q in groups[t - 1])
                mod_at(10 + t)
            if i == 3 and t >= 1:
                ops.extend(("P", q) for q in groups[t - 1])
                mod_at(t)
    first = groups[0] + groups[1]
    for j in range(NT):
        ops.append(("O", j, first))
        if j == 1:
            ops.extend(("S", q) for q in groups[3])
            mod_at(14)
    ops.extend(("P", q) for q in groups[3])
    mod_at(4)
    ops.extend(("O", j, groups[2]) for j in range(NT))
    for j in range(NT):
        ops.append(("O", j, groups[3]))
        ops.append(("F", j))
    mod_at(5)
    return ops


def _rb(x):
    return x.astype(BF16).astype(F32)


def _recip(x):
    r = pl.reciprocal(x, approx=True)
    return r * (2.0 - x * r)


def _ln_mod(x, s1p, shift, zero=None):
    xm = x if zero is None else jnp.concatenate([x[..., :128] + zero, x[..., 128:]], axis=-1)
    xc = x - jnp.mean(xm, axis=-1, keepdims=True)
    v = _rb(_rb(jnp.mean(xc * xc, axis=-1, keepdims=True)) + EPS)
    return xc * _recip(_rb(v * lax.rsqrt(v))) * s1p + shift


def _dot(a, b):
    return jnp.dot(a, b, preferred_element_type=F32)


def _as_bf16(u):
    return pltpu.bitcast(u, BF16)


def _as_u32(b):
    return pltpu.bitcast(b, U32)


def _spread(jobs, fns, lo, hi):
    for n, fn in enumerate(fns):
        jobs.setdefault(lo + n * (hi - lo) // len(fns), []).append(fn)


def _kernel(x_hbm, mem0_ref, wq_hbm, wk_hbm, wv_hbm, wo_hbm, wr_ref, wg_hbm, wu_hbm, wd_hbm,
            c_ref, wmod_hbm, out_hbm,
            wqkv, hs, wo_s, pre, cur_s, olhs, odef, xbuf, ybuf, hbuf, outs, lhs, wm_s, mod, mk,
            topv, topi, sc_s, zero_s, sem_m, sem_out):
    mt = 4 * NT * UNROLL // NSEG

    def modv(j):
        return jnp.concatenate([mod[j * NT + k] for k in range(NT)], axis=1)

    def mod_tile(wm, t):
        v = _rb(_dot(sc_s[...], wm))
        mod[t] = jnp.where(jnp.logical_or(t // NT == 1, t // NT == 4), _rb(1.0 + v), v)

    def wm_copy(it, u):
        col = pl.multiple_of((2 * NT + it * mt + u) * 128, 128)
        return pltpu.make_async_copy(wmod_hbm.at[:, pl.ds(col, 128)], wm_s.at[it & 3, u],
                                     sem_m.at[it & 3])

    def ln1(x, zero=None):
        x3 = x.astype(F32).reshape(x.shape[0] // 8, 8, D)
        zf = None if zero is None else pltpu.bitcast(zero, F32)
        return _ln_mod(x3, modv(1), modv(0), zf).reshape(x.shape[0], D).astype(BF16)

    def zero_after(y):
        return (y if y.dtype == U32 else pltpu.bitcast(y, U32)) & zero_s[0:8, :]

    def or_tile(u, z):
        if z is None:
            return u
        return (u.reshape(u.shape[0] // 8, 8, 128) | z).reshape(u.shape)

    def prologue(stage, wo_raw, wmod_s, h0, tmp, sem):
        w_hbms = (wq_hbm, wk_hbm, wv_hbm)
        wob = H * DH // NT

        def x_copy(i):
            lo, n = ((XR, M), (0, XR))[i]
            return pltpu.make_async_copy(x_hbm.at[:, pl.ds(lo, n), :], xbuf.at[:, pl.ds(lo, n), :],
                                         sem.at[i])

        def mod_copy(g):
            return pltpu.make_async_copy(wmod_hbm.at[:, pl.ds(pl.multiple_of(g * 512, 512), 512)],
                                         wmod_s.at[g], sem.at[2 + g])

        def c0_copy(q):
            rows = pl.ds(q * (D // 4), D // 4)
            return pltpu.make_async_copy(wq_hbm.at[rows, pl.ds(0, CH), :], stage.at[0, rows],
                                         sem.at[6 + q])

        def chunk_copy(mat, g, slot):
            return pltpu.make_async_copy(w_hbms[mat].at[:, pl.ds(g, CH), :], stage.at[slot],
                                         sem.at[10 + slot])

        def wo_copy(j):
            return pltpu.make_async_copy(wo_hbm.at[pl.ds(pl.multiple_of(j * wob, wob), wob)],
                                         wo_raw.at[j], sem.at[10 + NSLOT + j])

        def relayout1(src, t0, z=None):
            v = src.reshape(RB * CH, 128)
            tmp[t0:t0 + RB * CH // 2, :] = or_tile(_as_u32(v), z)

        def relayout2(m0, j, t0, rows, z=None):
            w = or_tile(tmp[pl.ds(t0 + j, RB2, stride=CH // 2), :], z)
            wqkv[m0 + 2 * j, rows, :] = _as_u32(w.astype(jnp.uint16))
            wqkv[m0 + 2 * j + 1, rows, :] = _as_u32((w >> 16).astype(jnp.uint16))

        for g in range(4):
            mod_copy(g).start()
        x_copy(0).start()
        for q in range(4):
            c0_copy(q).start()
        for g in range(1, NSLOT):
            chunk_copy(0, g * CH, g).start()
        x_copy(1).start()

        def decode(i):
            lo = i < 2 * SEG
            head = jnp.where(lo, i // SEG, (i - 2 * SEG) // M)
            is_mem = jnp.logical_and(lo, i % SEG >= XR)
            pos = jnp.where(lo, i % SEG, XR + i % M)
            return head, is_mem, pos

        qh, qm, qp = decode(lax.broadcasted_iota(jnp.int32, (PR, PR), 0))
        kh, km, kp = decode(lax.broadcasted_iota(jnp.int32, (PR, PR), 1))
        vis = qm | km | (qp >= kp)
        mk[...] = jnp.where(qh == kh, jnp.where(vis, 0.0, NEG_MASK * LOG2E), -jnp.inf).astype(F32)
        wr = jnp.broadcast_to(wr_ref[...].astype(F32).reshape(1, D), (M, D))
        for k in range(NT):
            mod[6 * NT + k] = wr[:, k * 128:(k + 1) * 128]
        zero_s[...] = jnp.zeros(zero_s.shape, U32)
        topv[...] = jnp.full(topv.shape, -jnp.inf, F32)
        topi[...] = lax.broadcasted_iota(jnp.int32, topi.shape, 0)
        cv = c_ref[...].astype(F32)
        sc_s[...] = jnp.broadcast_to(cv * _rb(jax.nn.sigmoid(cv)), (M, D)).astype(BF16)
        mb = mem0_ref[...]
        for k in range(NT):
            lhs[0, k, XR // 2:, :] = _as_u32(mb[:, k * 128:(k + 1) * 128])

        def zero_body(i, c):
            wo_raw[NT, pl.ds(pl.multiple_of(i * 32, 32), 32), :] = jnp.zeros((32, D), BF16)
            return c

        lax.fori_loop(0, wob // 32, zero_body, 0)

        def mod_body(g, c):
            mod_copy(g).wait()
            for t in range(4):
                mod_tile(wmod_s[g, :, t * 128:(t + 1) * 128], 4 * g + t)
            return c

        with jax.named_scope("p_mod"):
            lax.fori_loop(0, 4, mod_body, 0)
        x_copy(0).wait()

        def ln_body(i, c):
            for u in range(LNU):
                q = (i * LNU + u) * 2
                hb = ln1(xbuf[pl.ds(q, 2), XR:, :].reshape(16, D))
                r2 = pl.multiple_of(q * 4, 8)
                for k in range(NT):
                    h0[k, pl.ds(r2, 8), :] = _as_u32(hb[:, k * 128:(k + 1) * 128])
            return c

        with jax.named_scope("p_ln"):
            lax.fori_loop(0, NSEG // (2 * LNU), ln_body, 0)

        def c0_body(q, c):
            c0_copy(q).wait()
            for d0 in range(0, D // 4, RB):
                relayout1(stage[0, pl.ds(q * (D // 4) + d0, RB)], d0 * CH // 2)
            for d0 in range(0, D // 4, RB2):
                rows = pl.ds(pl.multiple_of(q * (D // 8) + d0 // 2, 8), RB2 // 2)
                for j in range(CH // 2):
                    relayout2(0, j, d0 * CH // 2, rows)
            return c

        with jax.named_scope("p_c0"):
            lax.fori_loop(0, 4, c0_body, 0)

        def bulk(p0, npairs, jobs):
            n = 0
            due = {}
            for hh in range(2 * npairs):
                a = (hh % 2) * M
                for r in range(0, R0, MB):
                    ts = [h0[k, r // 2:(r + MB) // 2, :] for k in range(NT)]
                    for z in due.pop(n, ()):
                        ts[0] = jnp.concatenate([ts[0][0:8] | z, ts[0][8:]], axis=0)
                    hv = jnp.concatenate([_as_bf16(t) for t in ts], axis=1)
                    y = _dot(hv, _as_bf16(wqkv[2 * p0 + hh]))
                    pre[p0 + hh // 2, r // M:(r + MB) // M, a:a + M, :] = (
                        y.reshape(MB // M, M, DH).astype(BF16))
                    for u in range(NREL):
                        for job in jobs.get(n * NREL + u, ()):
                            zr = u * (MB - 8) // (NREL - 1) // 8 * 8
                            res = job(zero_after(y[zr:zr + 8]))
                            if res is not None:
                                due.setdefault(n + JOB_SPAN, []).append(zero_after(res))
                    n += 1
            assert not due

        nlate = NCHUNK - 1 - NT

        def rot_body(i, c):
            slot = (i + 1) % NSLOT
            chunk_copy(0, 0, slot).wait()

            @pl.when(i == nlate)
            def _():
                x_copy(1).wait()

            @pl.when(i >= nlate)
            def _():
                wo_copy(i - nlate).wait()

            nxt = i + NSLOT
            for mat in range(3):
                @pl.when(jnp.logical_and(nxt < NCHUNK, nxt // (H // CH) == mat))
                def _():
                    chunk_copy(mat, pl.multiple_of((nxt % (H // CH)) * CH, CH), nxt % NSLOT).start()

            @pl.when(i < NT)
            def _():
                wo_copy(i).start()

            live = i >= nlate
            jw = jnp.where(live, i - nlate, NT)
            p0 = i * (CH // 2) + CH // 4
            m1 = 2 * p0 + CH // 2

            def wo_job(b, z):
                v = wo_raw[jw, b * 16:(b + 1) * 16, :]
                rows = pl.ds(pl.multiple_of(jw * (wob // 2) + b * 8, 8), 8)
                for j in range(NT):
                    wo_s[j, rows, :] = _as_u32(v[:, j * 128:(j + 1) * 128]) | z

            def ln_job(b, z):
                r = (b % 3) * 8
                src = jnp.where(live, (i - nlate) * CH + b // 3, 0)
                hb = ln1(xbuf[src, pl.ds(pl.multiple_of(jnp.where(live, r, XR), 8), 8), :], z)
                u = [_as_u32(hb[:, k * 128:(k + 1) * 128]) for k in range(NT)]
                dst = jnp.where(live, src, NSEG)
                for k in range(NT):
                    hs[dst, k, r // 2:r // 2 + 4, :] = u[k]
                res = jnp.concatenate(u[0:2], axis=0)
                for k in range(2, NT, 2):
                    res = res | jnp.concatenate(u[k:k + 2], axis=0)
                return res

            def r1_job(d0, z):
                relayout1(stage[slot, d0:d0 + RB], d0 * CH // 2, z)

            def r2_jobs(j):
                return [functools.partial(relayout2, m1, j, d0 * CH // 2,
                                          pl.ds(d0 // 2, RB2 // 2)) for d0 in range(0, D, RB2)]

            jobs = {}
            _spread(jobs, [functools.partial(r1_job, d0) for d0 in range(0, D, RB)],
                    0, R1_END * NREL)
            _spread(jobs, r2_jobs(0), R2_0[0] * NREL, R2_0[1] * NREL)
            _spread(jobs, r2_jobs(1) + r2_jobs(2) + r2_jobs(3), R2_0[1] * NREL, 31 * NREL)
            _spread(jobs, [functools.partial(ln_job, b) for b in range(3 * CH)],
                    LN_RANGE[0] * NREL, LN_RANGE[1] * NREL)
            _spread(jobs, [functools.partial(wo_job, b) for b in range(wob // 16)],
                    WO_RANGE[0] * NREL, WO_RANGE[1] * NREL)
            bulk(p0, CH // 2, jobs)
            return c

        def outer(k, c):
            bulk(k * (3 * NP - CH // 4), CH // 4, {})

            @pl.when(k == 0)
            def _():
                with jax.named_scope("p_rot"):
                    lax.fori_loop(0, NCHUNK - 1, rot_body, 0)
                for it in range(2):
                    for u in range(mt):
                        wm_copy(it, u).start()

            return c

        with jax.named_scope("p_bulk"):
            lax.fori_loop(0, 2, outer, 0)

    if "pro" in PHASES: pl.run_scoped(
        prologue,
        pltpu.VMEM((NSLOT, D, CH, 128), BF16),
        pltpu.VMEM((NT + 1, H * DH // NT, D), BF16),
        pltpu.VMEM((4, D, 512), BF16),
        pltpu.VMEM((NT, R0 // 2 + PADS[0], 128), U32),
        pltpu.VMEM((D * CH // 2 + PADS[1], 128), U32),
        pltpu.SemaphoreType.DMA((10 + NSLOT + NT,)),
    )

    def load_x_rows(slot, seg):
        for k in range(NT):
            lhs[slot, k, 0:XR // 2, :] = hs[seg, k]

    def post(seg, r, z=None):
        rows = pl.ds(r, 8)
        t = modv(2) * ybuf[seg, rows, :].astype(F32)
        if z is not None:
            t = t + jnp.concatenate([pltpu.bitcast(z, F32)] * NT, axis=1)
        x1 = _rb(xbuf[seg, rows, :].astype(F32) + t)
        xbuf[seg, rows, :] = x1.astype(BF16)
        h2b = _ln_mod(x1, modv(4), modv(3)).astype(BF16)
        hbuf[seg, rows, :] = h2b
        h2 = h2b.astype(F32)
        o = x1 + modv(5) * h2
        outs[seg, rows, :] = o.astype(BF16)
        v = _rb(jnp.sum(h2 * modv(6), axis=-1, keepdims=True))
        m1, m2, i1, i2 = topv[0:8, :], topv[8:16, :], topi[0:8, :], topi[8:16, :]
        idx = lax.broadcasted_iota(jnp.int32, (8, 1), 0) + (seg * SEG + r)
        g1 = (v > m1) | ((v == m1) & (idx < i1))
        g2 = (v > m2) | ((v == m2) & (idx < i2))
        topv[8:16, :] = jnp.where(g1, m1, jnp.where(g2, v, m2))
        topi[8:16, :] = jnp.where(g1, i1, jnp.where(g2, idx, i2))
        topv[0:8, :] = jnp.where(g1, v, m1)
        topi[0:8, :] = jnp.where(g1, idx, i1)
        if z is not None:
            res = pltpu.bitcast(jnp.broadcast_to(v, (8, 128)), U32)
            for k in range(NT):
                res = res | pltpu.bitcast(o[:, k * 128:(k + 1) * 128], U32)
            return res

    def out_copy(g0, ng, r, n, k=0):
        return pltpu.make_async_copy(outs.at[pl.ds(g0, ng), pl.ds(r, n), :],
                                     out_hbm.at[pl.ds(g0, ng), pl.ds(r, n), :], sem_out.at[k])

    def main(wg_s, wu_s, wd_s, sem_f):
        late = ((wg_hbm, wg_s, FF // 128), (wu_hbm, wu_s, FF // 128), (wd_hbm, wd_s, NT))

        def col_copy(k, j):
            return pltpu.make_async_copy(
                late[k][0].at[:, pl.ds(pl.multiple_of(j * 128, 128), 128)], late[k][1].at[j],
                sem_f.at[k])

        load_x_rows(0, 0)

        def step(it, cur, state):
            s = it * UNROLL + cur
            nxt = (cur + 1) % UNROLL
            drow = pl.multiple_of(s * M, M)

            def pay(t, cost):
                now = state.get("now", 0)
                due = state.setdefault("due", [])
                for z in [z for (d, z) in due if d <= now]:
                    t = jnp.concatenate([t[0:8] | z, t[8:]], axis=0)
                state["due"] = [(d, z) for (d, z) in due if d > now]
                state["now"] = now + cost
                return t

            def owe(lag, p, tiles):
                z = tiles[0]
                for t in tiles[1:]:
                    z = z | t
                state.setdefault("due", []).append(
                    (state.get("now", 0) + lag + (p % 4) * TOK_STAG, zero_after(z)))

            def lv(k0, k1):
                ts = [lhs[cur, k] for k in range(k0, k1)]
                ts[0] = pay(ts[0], (k1 - k0) / NT)
                return jnp.concatenate([_as_bf16(t) for t in ts], axis=1)

            def qkv(p, split=False):
                part = {}
                if split:
                    for mat in range(3):
                        for a in range(2):
                            part[mat, a] = _dot(
                                lv(0, NT // 2), _as_bf16(wqkv[mat * H + 2 * p + a, :D // 4, :]))
                for mat in range(3):
                    for a in range(2):
                        hm = mat * H + 2 * p + a
                        if split:
                            y = _dot(lv(NT // 2, NT), _as_bf16(wqkv[hm, D // 4:, :])) + part[mat, a]
                        else:
                            y = _dot(lv(0, NT), _as_bf16(wqkv[hm]))
                        cur_s[hm] = y.astype(BF16)

            def gather(mat, p):
                hm = mat * H + 2 * p
                return jnp.concatenate([cur_s[hm], cur_s[hm + 1], pre[mat * NP + p, s]], axis=0)

            probs = {}

            def scores(p):
                sc = lax.dot_general(gather(0, p), gather(1, p), (((1,), (1,)), ((), ())),
                                     preferred_element_type=F32)
                mv = mk[...]
                sc = jnp.where(mv == 0.0, sc * (SCALE * LOG2E), mv)
                e = jnp.exp2(sc - jnp.max(sc, axis=-1, keepdims=True))
                inv = _recip(jnp.sum(e, axis=-1, keepdims=True))
                if NORM_PRE:
                    e = e * inv
                    if TOK_S is not None:
                        eu = pltpu.bitcast(e, U32)
                        z = eu[0:8]
                        for k in range(1, PR // 8):
                            z = z | eu[k * 8:(k + 1) * 8]
                        owe(TOK_S, p, [jnp.concatenate([z, jnp.zeros((8, 128 - PR), U32)], axis=1)])
                    probs[p] = (e.astype(BF16), None)
                else:
                    if TOK_S is not None:
                        iu = pltpu.bitcast(jnp.broadcast_to(inv, (PR, 128)), U32)
                        owe(TOK_S, p, [iu[k * 8:(k + 1) * 8] for k in range(PR // 8)])
                    probs[p] = (e.astype(BF16), inv)

            def pv(p):
                e, inv = probs.pop(p)
                o = _dot(e, gather(2, p))
                if inv is not None:
                    o = o * inv
                o = o.astype(BF16)
                if TOK_P is not None:
                    ou = _as_u32(o)
                    owe(TOK_P, p, [ou[k * 8:(k + 1) * 8] for k in range(PR // 16)])
                for a in range(2):
                    h = 2 * p + a
                    olhs[h] = _as_u32(o[a * SEG:(a + 1) * SEG])
                    odef[h, pl.ds(drow, M), :] = o[2 * SEG + a * M:2 * SEG + (a + 1) * M]

            acc = [None] * NT

            def oproj(j, pairs):
                ts = [olhs[2 * p + a] for p in pairs for a in range(2)]
                ts[0] = pay(ts[0], len(pairs) / 4)
                ov = jnp.concatenate([_as_bf16(t) for t in ts], axis=1)
                w = wo_s[j, pairs[0] * DH:(pairs[-1] + 1) * DH, :]
                y = _dot(ov, _as_bf16(w))
                acc[j] = y if acc[j] is None else y + acc[j]

            def fin(j):
                yb = acc[j].astype(BF16)
                ybuf[s, 0:XR, j * 128:(j + 1) * 128] = yb[0:XR]
                lhs[nxt, j, XR // 2:, :] = _as_u32(yb[XR:])

            def late_mod(u):
                mod_tile(wm_s[it & 3, u], 2 * NT + it * mt + u)

            load_x_rows(nxt, jnp.minimum(s + 1, NSEG - 1))
            ops = dict(Q=qkv, S=scores, P=pv, O=oproj, F=fin, M=late_mod)
            for op in _schedule([(u, q) for u, (c_, q) in enumerate(MODS[:mt]) if c_ % UNROLL == cur]):
                ops[op[0]](*op[1:])

        def steps(it, carry):
            if "pro" in PHASES:
                pltpu.make_async_copy(wm_s.at[it & 3], wm_s.at[it & 3], sem_m.at[it & 3]).wait()

                @pl.when(it + 2 < NSEG // UNROLL)
                def _():
                    for u in range(mt):
                        wm_copy(it + 2, u).start()

            for u in range(UNROLL // 2):
                t = it * (UNROLL // 2) + u
                for k in range(3):
                    @pl.when(t < late[k][2])
                    def _():
                        col_copy(k, t).start()

            state = {}
            for u in range(UNROLL):
                step(it, u, state)
            return carry

        with jax.named_scope("m_steps"):
            if "step" in PHASES: lax.fori_loop(0, NSEG // UNROLL, steps, 0)
        for k in range(3):
            for j in range(late[k][2]):
                col_copy(k, j).wait()
        if "epi" not in PHASES:
            return

        gpi = PPI // (XR // 8)

        def ep_body(i, c):
            @pl.when(i > 0)
            def _():
                out_copy((i - 1) * gpi, gpi, 0, XR).start()

            r = pl.multiple_of(i * EC, EC)
            g0 = i * (EC // M)
            nk = H // EKH
            jobs = {}
            _spread(jobs, list(range(PPI)), 0, NT * nk - E_SPAN)
            due = {}
            n = 0
            for j in range(NT):
                y = None
                for kk in range(nk):
                    ts = [odef[h, pl.ds(r, EC), :] for h in range(kk * EKH, (kk + 1) * EKH)]
                    for z in due.pop(n, ()):
                        ts[0] = jnp.concatenate(
                            [_as_bf16(_as_u32(ts[0][0:16]) | z), ts[0][16:]], axis=0)
                    w = wo_s[j, kk * EKH * DH // 2:(kk + 1) * EKH * DH // 2, :]
                    yp = _dot(jnp.concatenate(ts, axis=1), _as_bf16(w))
                    y = yp if y is None else yp + y
                    if kk == nk - 1:
                        ybuf[pl.ds(g0, EC // M), XR:, j * 128:(j + 1) * 128] = (
                            y.reshape(EC // M, M, 128).astype(BF16))
                    for u in jobs.get(n, ()):
                        t = i * PPI + u
                        early = t < NSEG * (XR // 8)
                        seg = jnp.where(early, t // (XR // 8), t - NSEG * (XR // 8))
                        row = pl.multiple_of(jnp.where(early, (t % (XR // 8)) * 8, XR), 8)
                        res = post(seg, row, zero_after(y[0:8]))
                        due.setdefault(n + E_SPAN, []).append(zero_after(res))
                    n += 1
            return c

        with jax.named_scope("e_loop"):
            lax.fori_loop(0, NEC, ep_body, 0)
        done = (NEC - 1) * gpi
        tail = NSEG - EC // M
        out_copy(done, NSEG - done, 0, XR).start()
        out_copy(0, tail, XR, M).start()
        for g in range(tail, NSEG):
            post(g, XR)
        out_copy(tail, NSEG - tail, XR, M).start()

        tv = topv[...]
        ti = topi[...]
        m1 = jnp.max(tv, axis=0, keepdims=True)
        i1v = jnp.min(jnp.where(tv == m1, ti, S), axis=0, keepdims=True)
        rest = ti != i1v
        m2 = jnp.max(jnp.where(rest, tv, -jnp.inf), axis=0, keepdims=True)
        i2v = jnp.min(jnp.where(jnp.logical_and(rest, tv == m2), ti, S), axis=0, keepdims=True)
        i1 = jnp.clip(i1v[0, 0], 0, S - 1)
        i2 = jnp.clip(i2v[0, 0], 0, S - 1)
        g1, g2 = i1 // SEG, i2 // SEG
        b1 = pl.multiple_of((i1 % SEG) // 8 * 8, 8)
        b2 = pl.multiple_of((i2 % SEG) // 8 * 8, 8)

        def two_blocks(ref):
            return jnp.concatenate([ref[g1, pl.ds(b1, 8), :].astype(F32),
                                    ref[g2, pl.ds(b2, 8), :].astype(F32)], axis=0)

        x1 = two_blocks(xbuf)
        h2 = two_blocks(hbuf)
        h2b = h2.astype(BF16)
        row = lax.broadcasted_iota(jnp.int32, (16, 1), 0)
        grow = jnp.where(row < 8, g1 * SEG + b1 + row, g2 * SEG + b2 + row - 8)
        rsel = jnp.where(grow == i1, m1, m2)
        acts = []
        for j in range(FF // 128):
            gt = _rb(_dot(h2b, wg_s[j]))
            gt = _rb(gt * _rb(jax.nn.sigmoid(gt)))
            ut = _rb(_dot(h2b, wu_s[j]))
            acts.append((gt * ut).astype(BF16))
        act = jnp.concatenate(acts, axis=1)
        y = _rb(jnp.concatenate([_dot(act, wd_s[j]) for j in range(NT)], axis=1))
        y = _rb(y * _rb(jax.nn.sigmoid(rsel)))
        sel = jnp.logical_or(grow == i1, grow == i2)
        hb = _rb(h2 + jnp.where(sel, y, 0.0))
        fixed = (x1 + jnp.concatenate([modv(5)] * 2, axis=0) * hb).astype(BF16)

        with jax.named_scope("e_outwait"):
            out_copy(0, NSEG, 0, SEG).wait()
        outs[g1, pl.ds(b1, 8), :] = fixed[0:8]
        outs[g2, pl.ds(b2, 8), :] = fixed[8:16]
        out_copy(g1, 1, b1, 8, 0).start()

        @pl.when(i1 // 8 != i2 // 8)
        def _():
            out_copy(g2, 1, b2, 8, 1).start()
            out_copy(g2, 1, b2, 8, 1).wait()

        out_copy(g1, 1, b1, 8, 0).wait()

    pl.run_scoped(
        main,
        pltpu.VMEM((FF // 128, D, 128), BF16),
        pltpu.VMEM((FF // 128, D, 128), BF16),
        pltpu.VMEM((NT, FF, 128), BF16),
        pltpu.SemaphoreType.DMA((3,)),
    )


@functools.partial(jax.jit, static_argnames=("A_seg_len",))
def pallas_adaLN_cond__memory_aug_recurrent_mem_tr__moe_arch_mod__prompt_kernel(
    A_x: jax.Array,
    A_mem0: jax.Array,
    A_Wq: jax.Array,
    A_Wk: jax.Array,
    A_Wv: jax.Array,
    A_Wo: jax.Array,
    A_seg_len,
    B_x: jax.Array,
    B_w_r: jax.Array,
    B_w_gate: jax.Array,
    B_w_up: jax.Array,
    B_w_down: jax.Array,
    c: jax.Array,
    w_mod: jax.Array,
):
    assert A_seg_len == SEG and A_x.shape == (1, S, D)
    del B_x
    hbm = pl.BlockSpec(memory_space=pl.ANY)
    vmem = pl.BlockSpec(memory_space=pltpu.VMEM)
    out = pl.pallas_call(
        _kernel,
        out_shape=jax.ShapeDtypeStruct((NSEG, SEG, D), BF16),
        in_specs=[hbm, vmem, hbm, hbm, hbm, hbm, vmem, hbm, hbm, hbm, vmem, hbm],
        out_specs=hbm,
        scratch_shapes=[
            pltpu.VMEM((3 * H, D // 2, DH), U32),
            pltpu.VMEM((NSEG + 1, NT, XR // 2, 128), U32),
            pltpu.VMEM((NT, (H * DH + H * DH // NT) // 2, 128), U32),
            pltpu.VMEM((3 * NP, NSEG, 2 * M, DH), BF16),
            pltpu.VMEM((3 * H, SEG, DH), BF16),
            pltpu.VMEM((H, SEG // 2, DH), U32),
            pltpu.VMEM((H, R0, DH), BF16),
            pltpu.VMEM((NSEG, SEG, D), BF16),
            pltpu.VMEM((NSEG, SEG, D), BF16),
            pltpu.VMEM((NSEG, SEG, D), BF16),
            pltpu.VMEM((NSEG, SEG, D), BF16),
            pltpu.VMEM((UNROLL, NT, SEG // 2, 128), U32),
            pltpu.VMEM((4, 4 * NT * UNROLL // NSEG, D, 128), BF16),
            pltpu.VMEM((7 * NT, M, 128), F32),
            pltpu.VMEM((PR, PR), F32),
            pltpu.VMEM((16, 1), F32),
            pltpu.VMEM((16, 1), jnp.int32),
            pltpu.VMEM((M, D), BF16),
            pltpu.VMEM((8 + PADS[2], 128), U32),
            pltpu.SemaphoreType.DMA((4,)),
            pltpu.SemaphoreType.DMA((2,)),
        ],
        compiler_params=pltpu.CompilerParams(vmem_limit_bytes=120 * 1024 * 1024,
                                             disable_bounds_checks=True),
    )(A_x.reshape(NSEG, SEG, D), A_mem0.reshape(M, D), A_Wq, A_Wk, A_Wv, A_Wo.reshape(H * DH, D),
      B_w_r, B_w_gate, B_w_up, B_w_down, c, w_mod)
    return out.reshape(1, S, D)
```

```python
import functools

import jax
import jax.numpy as jnp
from jax import lax
import jax.experimental.pallas as pl
import jax.experimental.pallas.tpu as pltpu

F32 = jnp.float32
BF16 = jnp.bfloat16
U32 = jnp.uint32

D = 1024
S = 2048
H = 32
DH = 128
M = 8
SEG = 32
NSEG = S // SEG
FF = 3584
NT = D // 128
XR = SEG - M
R0 = M * NSEG
CH = 8
NCHUNK = 3 * H // CH
NSLOT = 4
PR = 2 * SEG + 2 * M
NP = H // 2
EC = 128
NEC = R0 // EC
LOG2E = 1.4426950408889634
EPS = 1e-5
SCALE = DH ** -0.5
NEG_MASK = -1000000000.0

PHASES = ("pro", "step", "epi")
UNROLL = 4
MB = 128
RB = 16
RB2 = 64
NREL = 4
JOB_SPAN = 3
LNU = 8
EKH = 4
E_SPAN = 6
ZIN = "all"
PIN_OUT = False
EBLK = (128,)
PADS = (0, 0, 0)
MODS = ((-1, 4), (1, 4))
TOK_S = 9
TOK_P = None
TOK_STAG = 2
NORM_PRE = True
R1_END = 11
R2_0 = (3, 14)
LN_RANGE = (0, 29)
WO_RANGE = (12, 31)


def _schedule(mods):
    groups = [list(range(4 * g, 4 * g + 4)) for g in range(4)]
    ops = []

    def mod_at(pos):
        ops.extend(("M", u) for (u, q) in mods if q == pos)

    for t in range(4):
        for i, p in enumerate(groups[t]):
            ops.append(("Q", p, p == 0))
            if i == 0 and t >= 1:
                ops.extend(("S", q) for q in groups[t - 1])
                mod_at(10 + t)
            if i == 3 and t >= 1:
                ops.extend(("P", q) for q in groups[t - 1])
                mod_at(t)
    first = groups[0] + groups[1]
    for j in range(NT):
        ops.append(("O", j, first))
        if j == 1:
            ops.extend(("S", q) for q in groups[3])
            mod_at(14)
    ops.extend(("P", q) for q in groups[3])
    mod_at(4)
    ops.extend(("O", j, groups[2]) for j in range(NT))
    for j in range(NT):
        ops.append(("O", j, groups[3]))
        ops.append(("F", j))
    mod_at(5)
    return ops


def _rb(x):
    return x.astype(BF16).astype(F32)


def _recip(x):
    r = pl.reciprocal(x, approx=True)
    return r * (2.0 - x * r)


def _ln_mod(x, s1p, shift, zero=None):
    xm = x if zero is None else jnp.concatenate([x[..., :128] + zero, x[..., 128:]], axis=-1)
    xc = x - jnp.mean(xm, axis=-1, keepdims=True)
    v = _rb(_rb(jnp.mean(xc * xc, axis=-1, keepdims=True)) + EPS)
    return xc * _recip(_rb(v * lax.rsqrt(v))) * s1p + shift


def _dot(a, b):
    return jnp.dot(a, b, preferred_element_type=F32)


def _as_bf16(u):
    return pltpu.bitcast(u, BF16)


def _as_u32(b):
    return pltpu.bitcast(b, U32)


def _cumsum(xs):
    out, r = [], 0
    for x in xs:
        out.append(r)
        r += x
    return out


def _spread(jobs, fns, lo, hi):
    for n, fn in enumerate(fns):
        jobs.setdefault(lo + n * (hi - lo) // len(fns), []).append(fn)


def _kernel(x_hbm, mem0_hbm, wq_hbm, wk_hbm, wv_hbm, wo_hbm, wr_hbm, wg_hbm, wu_hbm, wd_hbm,
            c_hbm, wmod_hbm, out_hbm,
            wqkv, hs, wo_s, pre, cur_s, olhs, odef, xbuf, ybuf, hbuf, outs, lhs, wm_s, mod, mk,
            top, sc_s, zero_s, sem_m, sem_out):
    mt = 4 * NT * UNROLL // NSEG

    def modv(j):
        return jnp.concatenate([mod[j * NT + k] for k in range(NT)], axis=1)

    def mod_tile(wm, t):
        v = _rb(_dot(sc_s[...], wm))
        mod[t] = jnp.where(jnp.logical_or(t // NT == 1, t // NT == 4), _rb(1.0 + v), v)

    def wm_copy(it, u):
        col = pl.multiple_of((2 * NT + it * mt + u) * 128, 128)
        return pltpu.make_async_copy(wmod_hbm.at[:, pl.ds(col, 128)], wm_s.at[it & 3, u],
                                     sem_m.at[it & 3])

    def ln1(x, zero=None):
        x3 = x.astype(F32).reshape(x.shape[0] // 8, 8, D)
        zf = None if zero is None else pltpu.bitcast(zero, F32)
        return _ln_mod(x3, modv(1), modv(0), zf).reshape(x.shape[0], D).astype(BF16)

    def zero_after(y):
        return (y if y.dtype == U32 else pltpu.bitcast(y, U32)) & zero_s[0:8, :]

    def or_tile(u, z):
        if z is None:
            return u
        return (u.reshape(u.shape[0] // 8, 8, 128) | z).reshape(u.shape)

    def prologue(stage, wo_raw, wmod_s, h0, tmp, mem0_ref, wr_ref, c_ref, sem):
        w_hbms = (wq_hbm, wk_hbm, wv_hbm)
        wob = H * DH // NT

        def x_copy(i):
            lo, n = ((XR, M), (0, XR))[i]
            return pltpu.make_async_copy(x_hbm.at[:, pl.ds(lo, n), :], xbuf.at[:, pl.ds(lo, n), :],
                                         sem.at[i])

        def mod_copy(g):
            return pltpu.make_async_copy(wmod_hbm.at[:, pl.ds(pl.multiple_of(g * 512, 512), 512)],
                                         wmod_s.at[g], sem.at[2 + g])

        def c0_copy(q):
            rows = pl.ds(q * (D // 4), D // 4)
            return pltpu.make_async_copy(wq_hbm.at[rows, pl.ds(0, CH), :], stage.at[0, rows],
                                         sem.at[6 + q])

        def chunk_copy(mat, g, slot):
            return pltpu.make_async_copy(w_hbms[mat].at[:, pl.ds(g, CH), :], stage.at[slot],
                                         sem.at[10 + slot])

        def wo_copy(j):
            return pltpu.make_async_copy(wo_hbm.at[pl.ds(pl.multiple_of(j * wob, wob), wob)],
                                         wo_raw.at[j], sem.at[10 + NSLOT + j])

        def relayout1(src, t0, z=None):
            v = src.reshape(RB * CH, 128)
            tmp[t0:t0 + RB * CH // 2, :] = or_tile(_as_u32(v), z)

        def relayout2(m0, j, t0, rows, z=None):
            w = or_tile(tmp[pl.ds(t0 + j, RB2, stride=CH // 2), :], z)
            wqkv[m0 + 2 * j, rows, :] = _as_u32(w.astype(jnp.uint16))
            wqkv[m0 + 2 * j + 1, rows, :] = _as_u32((w >> 16).astype(jnp.uint16))

        small = [pltpu.make_async_copy(src, dst, sem.at[10 + NSLOT + NT])
                 for src, dst in ((c_hbm, c_ref), (mem0_hbm, mem0_ref), (wr_hbm, wr_ref))]
        for cp in small:
            cp.start()
        for g in range(4):
            mod_copy(g).start()
        x_copy(0).start()
        for q in range(4):
            c0_copy(q).start()
        for g in range(1, NSLOT):
            chunk_copy(0, g * CH, g).start()
        x_copy(1).start()

        def decode(i):
            lo = i < 2 * SEG
            head = jnp.where(lo, i // SEG, (i - 2 * SEG) // M)
            is_mem = jnp.logical_and(lo, i % SEG >= XR)
            pos = jnp.where(lo, i % SEG, XR + i % M)
            return head, is_mem, pos

        qh, qm, qp = decode(lax.broadcasted_iota(jnp.int32, (PR, PR), 0))
        kh, km, kp = decode(lax.broadcasted_iota(jnp.int32, (PR, PR), 1))
        vis = qm | km | (qp >= kp)
        mk[...] = jnp.where(qh == kh, jnp.where(vis, 0.0, NEG_MASK * LOG2E), -jnp.inf).astype(F32)
        for cp in small:
            cp.wait()
        wr = jnp.broadcast_to(wr_ref[...].astype(F32).reshape(1, D), (M, D))
        for k in range(NT):
            mod[6 * NT + k] = wr[:, k * 128:(k + 1) * 128]
        zero_s[...] = jnp.zeros(zero_s.shape, U32)
        top[...] = jnp.full(top.shape, jnp.iinfo(jnp.int32).min, jnp.int32)
        cv = c_ref[...].astype(F32)
        sc_s[...] = jnp.broadcast_to(cv * _rb(jax.nn.sigmoid(cv)), (M, D)).astype(BF16)
        mb = mem0_ref[...]
        for k in range(NT):
            lhs[0, k, XR // 2:, :] = _as_u32(mb[:, k * 128:(k + 1) * 128])

        def zero_body(i, c):
            wo_raw[NT, pl.ds(pl.multiple_of(i * 32, 32), 32), :] = jnp.zeros((32, D), BF16)
            return c

        lax.fori_loop(0, wob // 32, zero_body, 0)

        def mod_body(g, c):
            mod_copy(g).wait()
            for t in range(4):
                mod_tile(wmod_s[g, :, t * 128:(t + 1) * 128], 4 * g + t)
            return c

        with jax.named_scope("p_mod"):
            lax.fori_loop(0, 4, mod_body, 0)
        x_copy(0).wait()

        def ln_body(i, c):
            for u in range(LNU):
                q = (i * LNU + u) * 2
                hb = ln1(xbuf[pl.ds(q, 2), XR:, :].reshape(16, D))
                r2 = pl.multiple_of(q * 4, 8)
                for k in range(NT):
                    h0[k, pl.ds(r2, 8), :] = _as_u32(hb[:, k * 128:(k + 1) * 128])
            return c

        with jax.named_scope("p_ln"):
            lax.fori_loop(0, NSEG // (2 * LNU), ln_body, 0)

        def c0_body(q, c):
            c0_copy(q).wait()
            for d0 in range(0, D // 4, RB):
                relayout1(stage[0, pl.ds(q * (D // 4) + d0, RB)], d0 * CH // 2)
            for d0 in range(0, D // 4, RB2):
                rows = pl.ds(pl.multiple_of(q * (D // 8) + d0 // 2, 8), RB2 // 2)
                for j in range(CH // 2):
                    relayout2(0, j, d0 * CH // 2, rows)
            return c

        with jax.named_scope("p_c0"):
            lax.fori_loop(0, 4, c0_body, 0)

        def bulk(p0, npairs, jobs):
            n = 0
            due = {}
            for hh in range(2 * npairs):
                a = (hh % 2) * M
                for r in range(0, R0, MB):
                    ts = [h0[k, r // 2:(r + MB) // 2, :] for k in range(NT)]
                    for z in due.pop(n, ()):
                        ts[0] = jnp.concatenate([ts[0][0:8] | z, ts[0][8:]], axis=0)
                    hv = jnp.concatenate([_as_bf16(t) for t in ts], axis=1)
                    y = _dot(hv, _as_bf16(wqkv[2 * p0 + hh]))
                    pre[p0 + hh // 2, r // M:(r + MB) // M, a:a + M, :] = (
                        y.reshape(MB // M, M, DH).astype(BF16))
                    for u in range(NREL):
                        for job in jobs.get(n * NREL + u, ()):
                            zr = u * (MB - 8) // (NREL - 1) // 8 * 8
                            res = job(zero_after(y[zr:zr + 8]))
                            if res is not None:
                                due.setdefault(n + JOB_SPAN, []).append(zero_after(res))
                    n += 1
            assert not due

        nlate = NCHUNK - 1 - NT

        def rot_body(i, c):
            slot = (i + 1) & (NSLOT - 1)
            chunk_copy(0, 0, slot).wait()

            @pl.when(i == nlate)
            def _():
                x_copy(1).wait()

            @pl.when(i >= nlate)
            def _():
                wo_copy(i - nlate).wait()

            nxt = i + NSLOT
            for mat in range(1, 3):
                @pl.when((nxt >> 2) == mat)
                def _():
                    chunk_copy(mat, pl.multiple_of((nxt & 3) * CH, CH), nxt & (NSLOT - 1)).start()

            @pl.when(i < NT)
            def _():
                wo_copy(i).start()

            live = i >= nlate
            jw = jnp.where(live, i - nlate, NT)
            p0 = i * (CH // 2) + CH // 4
            m1 = 2 * p0 + CH // 2

            def wo_job(b, z):
                v = wo_raw[jw, b * 16:(b + 1) * 16, :]
                rows = pl.ds(pl.multiple_of(jw * (wob // 2) + b * 8, 8), 8)
                for j in range(NT):
                    wo_s[j, rows, :] = _as_u32(v[:, j * 128:(j + 1) * 128]) | z

            def ln_job(b, z):
                r = (b % 3) * 8
                src = jnp.where(live, (i - nlate) * CH + b // 3, 0)
                hb = ln1(xbuf[src, pl.ds(pl.multiple_of(jnp.where(live, r, XR), 8), 8), :], z)
                u = [_as_u32(hb[:, k * 128:(k + 1) * 128]) for k in range(NT)]
                dst = jnp.where(live, src, NSEG)
                for k in range(NT):
                    hs[dst, k, r // 2:r // 2 + 4, :] = u[k]
                res = jnp.concatenate(u[0:2], axis=0)
                for k in range(2, NT, 2):
                    res = res | jnp.concatenate(u[k:k + 2], axis=0)
                return res

            def r1_job(d0, z):
                relayout1(stage[slot, d0:d0 + RB], d0 * CH // 2, z)

            def r2_jobs(j):
                return [functools.partial(relayout2, m1, j, d0 * CH // 2,
                                          pl.ds(d0 // 2, RB2 // 2)) for d0 in range(0, D, RB2)]

            jobs = {}
            _spread(jobs, [functools.partial(r1_job, d0) for d0 in range(0, D, RB)],
                    0, R1_END * NREL)
            _spread(jobs, r2_jobs(0), R2_0[0] * NREL, R2_0[1] * NREL)
            _spread(jobs, r2_jobs(1) + r2_jobs(2) + r2_jobs(3), R2_0[1] * NREL, 31 * NREL)
            _spread(jobs, [functools.partial(ln_job, b) for b in range(3 * CH)],
                    LN_RANGE[0] * NREL, LN_RANGE[1] * NREL)
            _spread(jobs, [functools.partial(wo_job, b) for b in range(wob // 16)],
                    WO_RANGE[0] * NREL, WO_RANGE[1] * NREL)
            bulk(p0, CH // 2, jobs)
            return c

        def outer(k, c):
            bulk(k * (3 * NP - CH // 4), CH // 4, {})

            @pl.when(k == 0)
            def _():
                with jax.named_scope("p_rot"):
                    lax.fori_loop(0, NCHUNK - 1, rot_body, 0)
                for it in range(2):
                    for u in range(mt):
                        wm_copy(it, u).start()

            return c

        with jax.named_scope("p_bulk"):
            lax.fori_loop(0, 2, outer, 0)

    if "pro" in PHASES: pl.run_scoped(
        prologue,
        pltpu.VMEM((NSLOT, D, CH, 128), BF16),
        pltpu.VMEM((NT + 1, H * DH // NT, D), BF16),
        pltpu.VMEM((4, D, 512), BF16),
        pltpu.VMEM((NT, R0 // 2 + PADS[0], 128), U32),
        pltpu.VMEM((D * CH // 2 + PADS[1], 128), U32),
        pltpu.VMEM((M, D), BF16),
        pltpu.VMEM((D,), BF16),
        pltpu.VMEM((1, D), BF16),
        pltpu.SemaphoreType.DMA((11 + NSLOT + NT,)),
    )

    def load_x_rows(slot, seg):
        for k in range(NT):
            lhs[slot, k, 0:XR // 2, :] = hs[seg, k]

    def post(seg, r, z=None):
        if z is not None and ZIN == "scalar":
            seg = seg + pltpu.bitcast(z, jnp.int32)[0, 0]
        rows = pl.ds(r, 8)
        t = modv(2) * ybuf[seg, rows, :].astype(F32)
        if z is not None and ZIN == "all":
            t = t + jnp.concatenate([pltpu.bitcast(z, F32)] * NT, axis=1)
        x1 = xbuf[seg, rows, :].astype(F32) + t
        h2 = _ln_mod(x1, modv(4), modv(3),
                     pltpu.bitcast(z, F32) if z is not None and ZIN == "mean" else None)
        hbuf[seg, rows, :] = h2.astype(BF16)
        o = x1 + modv(5) * h2
        outs[seg, rows, :] = o.astype(BF16)
        v = _rb(jnp.sum(h2 * modv(6), axis=-1, keepdims=True))
        b = pltpu.bitcast(jnp.where(v != v, -jnp.inf, v + 0.0), jnp.int32)
        low = (S - 1 - seg * SEG - r) - lax.broadcasted_iota(jnp.int32, (8, 1), 0)
        key = (b ^ ((b >> 31) & 0x7FFF0000)) | low
        m1, m2 = top[0:8, :], top[8:16, :]
        top[8:16, :] = jnp.maximum(m2, jnp.minimum(m1, key))
        top[0:8, :] = jnp.maximum(m1, key)
        if z is not None:
            res = pltpu.bitcast(jnp.broadcast_to(v, (8, 128)), U32)
            if PIN_OUT:
                for k in range(NT):
                    res = res | pltpu.bitcast(o[:, k * 128:(k + 1) * 128], U32)
            return res

    def out_copy(g0, ng, r, n, k=0):
        return pltpu.make_async_copy(outs.at[pl.ds(g0, ng), pl.ds(r, n), :],
                                     out_hbm.at[pl.ds(g0, ng), pl.ds(r, n), :], sem_out.at[k])

    def main(wg_s, wu_s, wd_s, sem_f):
        late = ((wg_hbm, wg_s, FF // 128), (wu_hbm, wu_s, FF // 128), (wd_hbm, wd_s, NT))

        def col_copy(k, j):
            return pltpu.make_async_copy(
                late[k][0].at[:, pl.ds(pl.multiple_of(j * 128, 128), 128)], late[k][1].at[j],
                sem_f.at[k])

        load_x_rows(0, 0)

        def step(it, cur, state):
            s = it * UNROLL + cur
            nxt = (cur + 1) % UNROLL

            def pay(t, cost):
                now = state.get("now", 0)
                due = state.setdefault("due", [])
                for z in [z for (d, z) in due if d <= now]:
                    t = jnp.concatenate([t[0:8] | z, t[8:]], axis=0)
                state["due"] = [(d, z) for (d, z) in due if d > now]
                state["now"] = now + cost
                return t

            def owe(lag, p, tiles):
                z = tiles[0]
                for t in tiles[1:]:
                    z = z | t
                state.setdefault("due", []).append(
                    (state.get("now", 0) + lag + (p % 4) * TOK_STAG, zero_after(z)))

            def lv(k0, k1):
                ts = [lhs[cur, k] for k in range(k0, k1)]
                ts[0] = pay(ts[0], (k1 - k0) / NT)
                return jnp.concatenate([_as_bf16(t) for t in ts], axis=1)

            def qkv(p, split=False):
                part = {}
                if split:
                    for mat in range(3):
                        for a in range(2):
                            part[mat, a] = _dot(
                                lv(0, NT // 2), _as_bf16(wqkv[mat * H + 2 * p + a, :D // 4, :]))
                for mat in range(3):
                    for a in range(2):
                        hm = mat * H + 2 * p + a
                        if split:
                            y = _dot(lv(NT // 2, NT), _as_bf16(wqkv[hm, D // 4:, :])) + part[mat, a]
                        else:
                            y = _dot(lv(0, NT), _as_bf16(wqkv[hm]))
                        cur_s[hm] = y.astype(BF16)

            def gather(mat, p):
                hm = mat * H + 2 * p
                return jnp.concatenate([cur_s[hm], cur_s[hm + 1], pre[mat * NP + p, s]], axis=0)

            probs = {}

            def scores(p):
                sc = lax.dot_general(gather(0, p), gather(1, p), (((1,), (1,)), ((), ())),
                                     preferred_element_type=F32)
                mv = mk[...]
                sc = jnp.where(mv == 0.0, sc * (SCALE * LOG2E), mv)
                e = jnp.exp2(sc - jnp.max(sc, axis=-1, keepdims=True))
                inv = _recip(jnp.sum(e, axis=-1, keepdims=True))
                if NORM_PRE:
                    e = e * inv
                    if TOK_S is not None:
                        eu = pltpu.bitcast(e, U32)
                        z = eu[0:8]
                        for k in range(1, PR // 8):
                            z = z | eu[k * 8:(k + 1) * 8]
                        owe(TOK_S, p, [jnp.concatenate([z, jnp.zeros((8, 128 - PR), U32)], axis=1)])
                    probs[p] = (e.astype(BF16), None)
                else:
                    if TOK_S is not None:
                        iu = pltpu.bitcast(jnp.broadcast_to(inv, (PR, 128)), U32)
                        owe(TOK_S, p, [iu[k * 8:(k + 1) * 8] for k in range(PR // 8)])
                    probs[p] = (e.astype(BF16), inv)

            def pv(p):
                e, inv = probs.pop(p)
                o = _dot(e, gather(2, p))
                if inv is not None:
                    o = o * inv
                o = o.astype(BF16)
                if TOK_P is not None:
                    ou = _as_u32(o)
                    owe(TOK_P, p, [ou[k * 8:(k + 1) * 8] for k in range(PR // 16)])
                for a in range(2):
                    h = 2 * p + a
                    olhs[h] = _as_u32(o[a * SEG:(a + 1) * SEG])
                    odef[h, it, cur * 4:(cur + 1) * 4, :] = _as_u32(
                        o[2 * SEG + a * M:2 * SEG + (a + 1) * M])

            acc = [None] * NT

            def oproj(j, pairs):
                ts = [olhs[2 * p + a] for p in pairs for a in range(2)]
                ts[0] = pay(ts[0], len(pairs) / 4)
                ov = jnp.concatenate([_as_bf16(t) for t in ts], axis=1)
                w = wo_s[j, pairs[0] * DH:(pairs[-1] + 1) * DH, :]
                y = _dot(ov, _as_bf16(w))
                acc[j] = y if acc[j] is None else y + acc[j]

            def fin(j):
                yb = acc[j].astype(BF16)
                ybuf[s, 0:XR, j * 128:(j + 1) * 128] = yb[0:XR]
                lhs[nxt, j, XR // 2:, :] = _as_u32(yb[XR:])

            def late_mod(u):
                mod_tile(wm_s[it & 3, u], 2 * NT + it * mt + u)

            load_x_rows(nxt, jnp.minimum(s + 1, NSEG - 1))
            ops = dict(Q=qkv, S=scores, P=pv, O=oproj, F=fin, M=late_mod)
            for op in _schedule([(u, q) for u, (c_, q) in enumerate(MODS[:mt]) if c_ % UNROLL == cur]):
                ops[op[0]](*op[1:])

        def steps(it, carry):
            if "pro" in PHASES:
                pltpu.make_async_copy(wm_s.at[it & 3], wm_s.at[it & 3], sem_m.at[it & 3]).wait()

                @pl.when(it + 2 < NSEG // UNROLL)
                def _():
                    for u in range(mt):
                        wm_copy(it + 2, u).start()

            for u in range(UNROLL // 2):
                t = it * (UNROLL // 2) + u
                for k in range(3):
                    @pl.when(t < late[k][2])
                    def _():
                        col_copy(k, t).start()

            state = {}
            for u in range(UNROLL):
                step(it, u, state)
            return carry

        with jax.named_scope("m_steps"):
            if "step" in PHASES: lax.fori_loop(0, NSEG // UNROLL, steps, 0)
        for k in range(3):
            for j in range(late[k][2]):
                col_copy(k, j).wait()
        if "epi" not in PHASES:
            return

        ntail = EBLK[-1] // M
        ppi = (S // 8 - ntail) // NEC
        gpi = ppi // (XR // 8)
        gb_ = UNROLL * M

        def ep_body(i, c):
            @pl.when(i > 0)
            def _():
                out_copy((i - 1) * gpi, gpi, 0, XR).start()

            subs = []
            r0 = 0
            for nr in EBLK:
                kh = EKH * EC // nr if EC % nr == 0 else EKH
                for j in range(NT):
                    for h0_ in range(0, H, kh):
                        subs.append((r0, nr, j, h0_, kh))
                r0 += nr
            tot = sum(nr * kh for (_, nr, _, _, kh) in subs)
            span = E_SPAN * EC * EKH
            rel = [u * (tot - span) // ppi for u in range(ppi)]
            ready = {}
            due = []
            now = 0
            u = 0
            y = None
            for (r0, nr, j, h0_, kh) in subs:
                blk = pl.ds(i * (EC // gb_) + r0 // gb_, nr // gb_)
                ts = [odef[h, blk].reshape(nr // 2, DH) for h in range(h0_, h0_ + kh)]
                for z in [z for (d, z) in due if d <= now]:
                    ts[0] = jnp.concatenate([ts[0][0:8] | z, ts[0][8:]], axis=0)
                due = [(d, z) for (d, z) in due if d > now]
                w = wo_s[j, h0_ * DH // 2:(h0_ + kh) * DH // 2, :]
                yp = _dot(jnp.concatenate([_as_bf16(t) for t in ts], axis=1), _as_bf16(w))
                y = yp if h0_ == 0 else yp + y
                if h0_ + kh == H:
                    ybuf[pl.ds(i * (EC // M) + r0 // M, nr // M), XR:, j * 128:(j + 1) * 128] = (
                        y.reshape(nr // M, M, 128).astype(BF16))
                    if j == NT - 1:
                        ready[r0] = True
                start = now
                now += nr * kh
                while u < ppi and rel[u] < now:
                    d = (NEC - 1) * ppi + u - NSEG * (XR // 8) - (NEC - 1) * (EC // M)
                    if d >= 0 and sum(n for r, n in zip(_cumsum(EBLK), EBLK) if r in ready) <= d * M:
                        break
                    t = i * ppi + u
                    early = t < NSEG * (XR // 8)
                    seg = jnp.where(early, t // (XR // 8), t - NSEG * (XR // 8))
                    row = pl.multiple_of(jnp.where(early, (t % (XR // 8)) * 8, XR), 8)
                    res = post(seg, row, zero_after(y[0:8]))
                    due.append((start + span, zero_after(res)))
                    u += 1
            assert u == ppi
            return c

        with jax.named_scope("e_loop"):
            lax.fori_loop(0, NEC, ep_body, 0)
        done = (NEC - 1) * gpi
        tail = NSEG - ntail
        out_copy(done, NSEG - done, 0, XR).start()
        out_copy(0, tail, XR, M).start()
        for g in range(tail, NSEG):
            post(g, XR)
        out_copy(tail, NSEG - tail, XR, M).start()

        tk = top[...]
        k1 = jnp.max(tk[0:8], axis=0, keepdims=True)
        k2 = jnp.max(jnp.where(tk == k1, jnp.iinfo(jnp.int32).min, tk), axis=0, keepdims=True)
        i1 = (S - 1) - (k1[0, 0] & (S - 1))
        i2 = (S - 1) - (k2[0, 0] & (S - 1))
        g1, g2 = i1 >> 5, i2 >> 5
        b1 = pl.multiple_of(i1 & 24, 8)
        b2 = pl.multiple_of(i2 & 24, 8)

        def two_blocks(ref):
            return jnp.concatenate([ref[g1, pl.ds(b1, 8), :].astype(F32),
                                    ref[g2, pl.ds(b2, 8), :].astype(F32)], axis=0)

        h2b = two_blocks(hbuf).astype(BF16)
        row = lax.broadcasted_iota(jnp.int32, (16, 1), 0)
        grow = jnp.where(row < 8, g1 * SEG + b1 + row, g2 * SEG + b2 + row - 8)
        ks = jnp.where(grow == i1, k1, k2)
        rsel = pltpu.bitcast((ks ^ ((ks >> 31) & 0x7FFF0000)) & -65536, F32)
        acts = []
        for j in range(FF // 128):
            gt = _rb(_dot(h2b, wg_s[j]))
            gt = _rb(gt * _rb(jax.nn.sigmoid(gt)))
            ut = _rb(_dot(h2b, wu_s[j]))
            acts.append((gt * ut).astype(BF16))
        act = jnp.concatenate(acts, axis=1)
        y = _rb(jnp.concatenate([_dot(act, wd_s[j]) for j in range(NT)], axis=1))
        y = _rb(y * _rb(jax.nn.sigmoid(rsel)))
        sel = jnp.logical_or(grow == i1, grow == i2)
        upd = jnp.concatenate([modv(5)] * 2, axis=0) * y
        fixed = (two_blocks(outs) + jnp.where(sel, upd, 0.0)).astype(BF16)

        with jax.named_scope("e_outwait"):
            out_copy(0, NSEG, 0, SEG).wait()
        outs[g1, pl.ds(b1, 8), :] = fixed[0:8]
        outs[g2, pl.ds(b2, 8), :] = fixed[8:16]
        out_copy(g1, 1, b1, 8, 0).start()

        @pl.when((i1 >> 3) != (i2 >> 3))
        def _():
            out_copy(g2, 1, b2, 8, 1).start()
            out_copy(g2, 1, b2, 8, 1).wait()

        out_copy(g1, 1, b1, 8, 0).wait()

    pl.run_scoped(
        main,
        pltpu.VMEM((FF // 128, D, 128), BF16),
        pltpu.VMEM((FF // 128, D, 128), BF16),
        pltpu.VMEM((NT, FF, 128), BF16),
        pltpu.SemaphoreType.DMA((3,)),
    )


@functools.partial(jax.jit, static_argnames=("A_seg_len",))
def pallas_adaLN_cond__memory_aug_recurrent_mem_tr__moe_arch_mod__prompt_kernel(
    A_x: jax.Array,
    A_mem0: jax.Array,
    A_Wq: jax.Array,
    A_Wk: jax.Array,
    A_Wv: jax.Array,
    A_Wo: jax.Array,
    A_seg_len,
    B_x: jax.Array,
    B_w_r: jax.Array,
    B_w_gate: jax.Array,
    B_w_up: jax.Array,
    B_w_down: jax.Array,
    c: jax.Array,
    w_mod: jax.Array,
):
    assert A_seg_len == SEG and A_x.shape == (1, S, D)
    del B_x
    hbm = pl.BlockSpec(memory_space=pl.ANY)
    out = pl.pallas_call(
        _kernel,
        out_shape=jax.ShapeDtypeStruct((NSEG, SEG, D), BF16),
        in_specs=[hbm] * 12,
        out_specs=hbm,
        scratch_shapes=[
            pltpu.VMEM((3 * H, D // 2, DH), U32),
            pltpu.VMEM((NSEG + 1, NT, XR // 2, 128), U32),
            pltpu.VMEM((NT, (H * DH + H * DH // NT) // 2, 128), U32),
            pltpu.VMEM((3 * NP, NSEG, 2 * M, DH), BF16),
            pltpu.VMEM((3 * H, SEG, DH), BF16),
            pltpu.VMEM((H, SEG // 2, DH), U32),
            pltpu.VMEM((H, NSEG // UNROLL, UNROLL * M // 2, DH), U32),
            pltpu.VMEM((NSEG, SEG, D), BF16),
            pltpu.VMEM((NSEG, SEG, D), BF16),
            pltpu.VMEM((NSEG, SEG, D), BF16),
            pltpu.VMEM((NSEG, SEG, D), BF16),
            pltpu.VMEM((UNROLL, NT, SEG // 2, 128), U32),
            pltpu.VMEM((4, 4 * NT * UNROLL // NSEG, D, 128), BF16),
            pltpu.VMEM((7 * NT, M, 128), F32),
            pltpu.VMEM((PR, PR), F32),
            pltpu.VMEM((16, 1), jnp.int32),
            pltpu.VMEM((M, D), BF16),
            pltpu.VMEM((8 + PADS[2], 128), U32),
            pltpu.SemaphoreType.DMA((4,)),
            pltpu.SemaphoreType.DMA((2,)),
        ],
        compiler_params=pltpu.CompilerParams(vmem_limit_bytes=120 * 1024 * 1024,
                                             disable_bounds_checks=True),
    )(A_x.reshape(NSEG, SEG, D), A_mem0.reshape(M, D), A_Wq, A_Wk, A_Wv, A_Wo.reshape(H * DH, D),
      B_w_r, B_w_gate, B_w_up, B_w_down, c, w_mod)
    return out.reshape(1, S, D)
```

```python
import functools

import jax
import jax.numpy as jnp
from jax import lax
import jax.experimental.pallas as pl
import jax.experimental.pallas.tpu as pltpu

F32 = jnp.float32
BF16 = jnp.bfloat16
U32 = jnp.uint32

D = 1024
S = 2048
H = 32
DH = 128
M = 8
SEG = 32
NSEG = S // SEG
FF = 3584
NT = D // 128
XR = SEG - M
R0 = M * NSEG
CH = 8
KQ = D // 4
NCHUNK = 3 * D // KQ
NSLOT = 4
PR = 2 * SEG + 2 * M
NP = H // 2
EC = 128
NEC = R0 // EC
LOG2E = 1.4426950408889634
EPS = 1e-5
SCALE = DH ** -0.5
NEG_MASK = -1000000000.0

PHASES = ("pro", "step", "epi")
UNROLL = 4
FB = 32
MOD_SPLIT = True
R_AT = ((0, 3, 6), (6, 9, 13), (14, 18, 22), (22, 26, 30))
RB = 16
RB2 = 64
NREL = 8
JOB_SPAN = 12
LNU = 16
EKH = 4
E_SPAN = 6
ZIN = "all"
PIN_OUT = False
EBLK = (128,)
PADS = (0, 0, 0)
MODS = ((-1, 4), (1, 4))
TOK_S = 9
TOK_P = None
TOK_STAG = 2
NORM_PRE = True
R1_END = 11
R2_0 = (3, 14)
LN_RANGE = (0, 29)
WO_RANGE = (12, 31)


def _schedule(mods):
    groups = [list(range(4 * g, 4 * g + 4)) for g in range(4)]
    ops = []

    def mod_at(pos):
        ops.extend(("M", u) for (u, q) in mods if q == pos)

    for t in range(4):
        for i, p in enumerate(groups[t]):
            ops.append(("Q", p, p == 0))
            if i == 0 and t >= 1:
                ops.extend(("S", q) for q in groups[t - 1])
                mod_at(10 + t)
            if i == 3 and t >= 1:
                ops.extend(("P", q) for q in groups[t - 1])
                mod_at(t)
    first = groups[0] + groups[1]
    for j in range(NT):
        ops.append(("O", j, first))
        if j == 1:
            ops.extend(("S", q) for q in groups[3])
            mod_at(14)
    ops.extend(("P", q) for q in groups[3])
    mod_at(4)
    ops.extend(("O", j, groups[2]) for j in range(NT))
    for j in range(NT):
        ops.append(("O", j, groups[3]))
        ops.append(("F", j))
    mod_at(5)
    return ops


def _rb(x):
    return x.astype(BF16).astype(F32)


def _recip(x):
    r = pl.reciprocal(x, approx=True)
    return r * (2.0 - x * r)


def _ln(x, zero=None):
    xm = x if zero is None else jnp.concatenate([x[..., :128] + zero, x[..., 128:]], axis=-1)
    xc = x - jnp.mean(xm, axis=-1, keepdims=True)
    v = _rb(_rb(jnp.mean(xc * xc, axis=-1, keepdims=True)) + EPS)
    return xc * _recip(_rb(v * lax.rsqrt(v)))


def _ln_mod(x, s1p, shift, zero=None):
    return _ln(x, zero) * s1p + shift


def _dot(a, b):
    return jnp.dot(a, b, preferred_element_type=F32)


def _as_bf16(u):
    return pltpu.bitcast(u, BF16)


def _as_u32(b):
    return pltpu.bitcast(b, U32)


def _cumsum(xs):
    out, r = [], 0
    for x in xs:
        out.append(r)
        r += x
    return out


def _spread(jobs, fns, lo, hi):
    for n, fn in enumerate(fns):
        jobs.setdefault(lo + n * (hi - lo) // len(fns), []).append(fn)


def _kernel(x_hbm, mem0_hbm, wq_hbm, wk_hbm, wv_hbm, wo_hbm, wr_hbm, wg_hbm, wu_hbm, wd_hbm,
            c_hbm, wmod_hbm, out_hbm,
            wqkv, hs, wo_s, pre, cur_s, olhs, odef, xbuf, lhs, wm_s, mod, mk,
            top, sc_s, zero_s, sem_m, sem_out):
    mt = 4 * NT * UNROLL // NSEG

    def modv(j):
        return jnp.concatenate([mod[j * NT + k] for k in range(NT)], axis=1)

    def mod_tile(wm, t):
        v = _rb(_dot(sc_s[...], wm))
        mod[t] = jnp.where(jnp.logical_or(t // NT == 1, t // NT == 4), _rb(1.0 + v), v)

    def wm_copy(it, u):
        col = pl.multiple_of((2 * NT + it * mt + u) * 128, 128)
        return pltpu.make_async_copy(wmod_hbm.at[:, pl.ds(col, 128)], wm_s.at[it & 3, u],
                                     sem_m.at[it & 3])

    def ln1(x, zero=None):
        x3 = x.astype(F32).reshape(x.shape[0] // 8, 8, D)
        zf = None if zero is None else pltpu.bitcast(zero, F32)
        return _ln_mod(x3, modv(1), modv(0), zf).reshape(x.shape[0], D).astype(BF16)

    def zero_after(y):
        return (y if y.dtype == U32 else pltpu.bitcast(y, U32)) & zero_s[0:8, :]

    def or_tile(u, z):
        if z is None:
            return u
        return (u.reshape(u.shape[0] // 8, 8, 128) | z).reshape(u.shape)

    def prologue(stage, wo_raw, wmod_s, nrm, ha, hb, tmp, mem0_ref, wr_ref, c_ref, sem):
        w_hbms = (wq_hbm, wk_hbm, wv_hbm)
        wob = H * DH // NT
        S_X, S_C0, S_ST, S_WO, S_MOD, S_SM = 0, 2, 6, 6 + NSLOT, 6 + NSLOT + NT, 6 + NSLOT + 2 * NT

        def x_copy(i):
            lo, n = ((XR, M), (0, XR))[i]
            return pltpu.make_async_copy(x_hbm.at[:, pl.ds(lo, n), :], xbuf.at[:, pl.ds(lo, n), :],
                                         sem.at[S_X + i])

        def mod_copies(k):
            return [pltpu.make_async_copy(wmod_hbm.at[:, pl.ds(v * D + k * 128, 128)],
                                          wmod_s.at[k, v], sem.at[S_MOD + k]) for v in range(2)]

        def chunk_copy(mat, d0, g, slot, k):
            return pltpu.make_async_copy(w_hbms[mat].at[pl.ds(d0, KQ), pl.ds(g * CH, CH), :],
                                         stage.at[slot, g], sem.at[k])

        def wo_copy(j):
            return pltpu.make_async_copy(wo_hbm.at[pl.ds(pl.multiple_of(j * wob, wob), wob)],
                                         wo_raw.at[j], sem.at[S_WO + j])

        def relayout1(src, t0, z=None):
            v = src.reshape(RB * CH, 128)
            tmp[t0:t0 + RB * CH // 2, :] = or_tile(_as_u32(v), z)

        def relayout2(c, h0_, t0, d0, z=None):
            w = or_tile(tmp[pl.ds(t0, RB2, stride=CH // 2), :], z)
            rows = pl.ds(d0 // 2, RB2 // 2)
            wqkv[c, h0_, rows, :] = _as_u32(w.astype(jnp.uint16))
            wqkv[c, h0_ + 1, rows, :] = _as_u32((w >> 16).astype(jnp.uint16))

        def mod_pair(k):
            for v in range(2):
                mod_tile(wmod_s[k, v], v * NT + k)

        def fill(dst, q, t, r, z=None):
            k = 2 * q + t
            sh = mod[k] if z is None else mod[k] + pltpu.bitcast(z, F32)
            v = nrm[k, r:r + FB, :].reshape(FB // 8, 8, 128) * mod[NT + k] + sh
            dst[t, r // 2:(r + FB) // 2, :] = _as_u32(v.reshape(FB, 128).astype(BF16))

        small = [pltpu.make_async_copy(src, dst, sem.at[S_SM])
                 for src, dst in ((c_hbm, c_ref), (mem0_hbm, mem0_ref), (wr_hbm, wr_ref))]
        for cp in small:
            cp.start()
        x_copy(0).start()
        for cp in mod_copies(0) + mod_copies(1):
            cp.start()
        for g in range(4):
            chunk_copy(0, 0, g, 0, S_C0 + g).start()
        for c in range(1, NSLOT):
            for g in range(4):
                chunk_copy(c % 3, (c // 3) * KQ, g, c, S_ST + c).start()
            for cp in mod_copies(2 * c) + mod_copies(2 * c + 1):
                cp.start()

        def decode(i):
            lo = i < 2 * SEG
            head = jnp.where(lo, i // SEG, (i - 2 * SEG) // M)
            is_mem = jnp.logical_and(lo, i % SEG >= XR)
            pos = jnp.where(lo, i % SEG, XR + i % M)
            return head, is_mem, pos

        qh, qm, qp = decode(lax.broadcasted_iota(jnp.int32, (PR, PR), 0))
        kh, km, kp = decode(lax.broadcasted_iota(jnp.int32, (PR, PR), 1))
        vis = qm | km | (qp >= kp)
        mk[...] = jnp.where(qh == kh, jnp.where(vis, 0.0, NEG_MASK * LOG2E), -jnp.inf).astype(F32)
        mod[0:2 * NT] = jnp.zeros((2 * NT, M, 128), F32)
        zero_s[...] = jnp.zeros(zero_s.shape, U32)
        top[...] = jnp.full(top.shape, jnp.iinfo(jnp.int32).min, jnp.int32)
        for cp in small:
            cp.wait()
        wr = jnp.broadcast_to(wr_ref[...].astype(F32).reshape(1, D), (M, D))
        for k in range(NT):
            mod[6 * NT + k] = wr[:, k * 128:(k + 1) * 128]
        cv = c_ref[...].astype(F32)
        sc_s[...] = jnp.broadcast_to(cv * _rb(jax.nn.sigmoid(cv)), (M, D)).astype(BF16)
        mb = mem0_ref[...]
        for k in range(NT):
            lhs[0, k, XR // 2:, :] = _as_u32(mb[:, k * 128:(k + 1) * 128])

        def zero_body(i, c):
            wo_raw[NT, pl.ds(pl.multiple_of(i * 32, 32), 32), :] = jnp.zeros((32, D), BF16)
            return c

        lax.fori_loop(0, wob // 32, zero_body, 0)
        x_copy(0).wait()

        def ln_body(i, c):
            for u in range(LNU):
                q = i * LNU + u
                v = _ln(xbuf[q, XR:, :].astype(F32))
                for k in range(NT):
                    nrm[k, pl.ds(pl.multiple_of(q * 8, 8), 8), :] = v[:, k * 128:(k + 1) * 128]
            return c

        with jax.named_scope("p_ln"):
            lax.fori_loop(0, NSEG // LNU, ln_body, 0)

        def mod_body(k, c):
            pltpu.make_async_copy(wmod_s.at[k], wmod_s.at[k], sem.at[S_MOD + k]).wait()
            mod_pair(k)
            for r in range(0, R0, FB):
                fill(ha, 0, k, r)
            return c

        with jax.named_scope("p_mod"):
            lax.fori_loop(0, 2, mod_body, 0)

        def c0_body(g, c):
            chunk_copy(0, 0, 0, 0, S_C0 + g).wait()
            for d0 in range(0, KQ, RB):
                relayout1(stage[0, g, d0:d0 + RB], d0 * CH // 2)
            for j in range(CH // 2):
                for d0 in range(0, KQ, RB2):
                    relayout2(0, g * CH + 2 * j, d0 * CH // 2 + j, d0)
            return c

        with jax.named_scope("p_c0"):
            lax.fori_loop(0, 4, c0_body, 0)

        def bulk(units, jobs, inserts):
            due = {}
            blk = R0 // NREL
            for n, (hq, c, h0_, pi, first) in enumerate(units):
                t0 = hq[0]
                parts = []
                for u in range(NREL):
                    part = t0[u * blk // 2:(u + 1) * blk // 2]
                    for z in due.pop(n * NREL + u, ()):
                        part = jnp.concatenate([part[0:8] | z, part[8:]], axis=0)
                    parts.append(part)
                hv = jnp.concatenate([_as_bf16(jnp.concatenate(parts, axis=0)), _as_bf16(hq[1])],
                                     axis=1)
                w = jnp.concatenate([_as_bf16(wqkv[c, h0_]), _as_bf16(wqkv[c, h0_ + 1])], axis=1)
                y = _dot(hv, w)
                for a in range(2):
                    old = jnp.where(first, 0.0, pre[pi, :, a * M:(a + 1) * M, :])
                    pre[pi, :, a * M:(a + 1) * M, :] = (
                        y[:, a * DH:(a + 1) * DH].reshape(NSEG, M, DH) + old)
                for fn in inserts.get(n, ()):
                    fn()
                for u in range(NREL):
                    for job in jobs.get(n * NREL + u, ()):
                        res = job(zero_after(y[u * blk:u * blk + 8, 0:128]))
                        if res is not None:
                            t = max(n * NREL + u + JOB_SPAN, (n + 1) * NREL)
                            due.setdefault(t, []).append(zero_after(res))
            assert not due

        HP = NP // 2
        WO0 = NCHUNK - 1 - NT
        LN0 = NT - 2
        SPI = -(-NSEG // (NCHUNK - 1 - LN0))

        def rot_body(i, c):
            slot = (i + 1) & (NSLOT - 1)
            pltpu.make_async_copy(stage.at[slot], stage.at[slot], sem.at[S_ST + slot]).wait()
            km = jnp.minimum(i + 1, NT - 1)

            @pl.when(jnp.logical_and(i >= 1, i + 1 < NT))
            def _():
                pltpu.make_async_copy(wmod_s.at[km], wmod_s.at[km], sem.at[S_MOD + km]).wait()

            @pl.when(i == LN0)
            def _():
                x_copy(1).wait()

            @pl.when(i >= WO0)
            def _():
                wo_copy(i - WO0).wait()

            nxt = i + NSLOT
            qn = (nxt * 43) >> 7
            for mat in range(3):
                @pl.when(jnp.logical_and(nxt < NCHUNK, nxt - 3 * qn == mat))
                def _():
                    for g in range(4):
                        chunk_copy(mat, qn * KQ, g, nxt & (NSLOT - 1),
                                   S_ST + (nxt & (NSLOT - 1))).start()

            @pl.when(i < NT)
            def _():
                wo_copy(i).start()

            @pl.when(i == 1)
            def _():
                x_copy(1).start()

            q0 = (i * 43) >> 7
            q1 = ((i + 1) * 43) >> 7
            units = ([(ha, i, H // 2 + 2 * n, (i - 3 * q0) * NP + HP + n, q0 == 0)
                      for n in range(HP)]
                     + [(hb, i + 1, 2 * n, (i + 1 - 3 * q1) * NP + n, q1 == 0) for n in range(HP)])
            jw = jnp.where(i >= WO0, i - WO0, NT)

            def wo_job(b, z):
                v = wo_raw[jw, b * 16:(b + 1) * 16, :]
                rows = pl.ds(pl.multiple_of(jw * (wob // 2) + b * 8, 8), 8)
                for j in range(NT):
                    wo_s[j, rows, :] = _as_u32(v[:, j * 128:(j + 1) * 128]) | z

            def ln_job(b, z):
                r = (b % 3) * 8
                seg = (i - LN0) * SPI + b // 3
                live = jnp.logical_and(i >= LN0, seg < NSEG)
                src = jnp.where(live, seg, 0)
                hv = ln1(xbuf[src, pl.ds(pl.multiple_of(jnp.where(live, r, XR), 8), 8), :], z)
                u = [_as_u32(hv[:, k * 128:(k + 1) * 128]) for k in range(NT)]
                dst = jnp.where(live, seg, NSEG)
                for k in range(NT):
                    hs[dst, k, r // 2:r // 2 + 4, :] = u[k]
                res = jnp.concatenate(u[0:2], axis=0)
                for k in range(2, NT, 2):
                    res = res | jnp.concatenate(u[k:k + 2], axis=0)
                return res

            def r1_job(g, d0, z):
                relayout1(stage[slot, g, d0:d0 + RB], (g * KQ + d0) * CH // 2, z)

            def copy_job(t, r, z):
                ha[t, r:r + 32, :] = or_tile(hb[t, r:r + 32, :], z)

            P = functools.partial
            nr = 2 * HP * NREL
            jobs = {}
            for g in range(4):
                lo, mid, hi = (x * NREL // 2 for x in R_AT[g])
                _spread(jobs, [P(r1_job, g, d0) for d0 in range(0, KQ, RB)], lo, mid)
                _spread(jobs, [P(relayout2, i + 1, g * CH + 2 * j, (g * KQ + d0) * CH // 2 + j, d0)
                               for j in range(CH // 2) for d0 in range(0, KQ, RB2)], mid, hi)
            _spread(jobs, [P(fill, hb, q1, t, r) for t in range(2) for r in range(0, R0, FB)],
                    2 * NREL, (HP - 1) * NREL)
            _spread(jobs, [P(copy_job, t, r) for t in range(2) for r in range(0, R0 // 2, 32)],
                    HP * NREL, nr - NREL)
            _spread(jobs, [P(ln_job, b) for b in range(3 * SPI)], NREL, nr - NREL - JOB_SPAN // 2)
            _spread(jobs, [P(wo_job, b) for b in range(wob // 16)], 0, nr - NREL)
            bulk(units, jobs, {0: [P(mod_tile, wmod_s[km, 0], km)],
                               1: [P(mod_tile, wmod_s[km, 1], NT + km)]} if MOD_SPLIT else
                 {0: [P(mod_pair, km)]})
            return c

        def outer(k, c):
            cc = k * (NCHUNK - 1)
            bulk([(ha, cc, k * (H // 2) + 2 * n, k * (3 * NP - HP) + n, k == 0)
                  for n in range(HP)], {}, {})

            @pl.when(k == 0)
            def _():
                with jax.named_scope("p_rot"):
                    lax.fori_loop(0, NCHUNK - 1, rot_body, 0)
                for it in range(2):
                    for u in range(mt):
                        wm_copy(it, u).start()

            return c

        with jax.named_scope("p_bulk"):
            lax.fori_loop(0, 2, outer, 0)

    if "pro" in PHASES: pl.run_scoped(
        prologue,
        pltpu.VMEM((NSLOT, H // CH, KQ, CH, 128), BF16),
        pltpu.VMEM((NT + 1, H * DH // NT, D), BF16),
        pltpu.VMEM((NT, 2, D, 128), BF16),
        pltpu.VMEM((NT, R0, 128), F32),
        pltpu.VMEM((2, R0 // 2 + PADS[0], 128), U32),
        pltpu.VMEM((2, R0 // 2 + PADS[0], 128), U32),
        pltpu.VMEM((D * CH // 2 + PADS[1], 128), U32),
        pltpu.VMEM((M, D), BF16),
        pltpu.VMEM((D,), BF16),
        pltpu.VMEM((1, D), BF16),
        pltpu.SemaphoreType.DMA((7 + NSLOT + 2 * NT,)),
    )

    def main(wg_s, wu_s, wd_s, ybuf, hbuf, outs, sem_f):
        def load_x_rows(slot, seg):
            for k in range(NT):
                lhs[slot, k, 0:XR // 2, :] = hs[seg, k]

        def post(seg, r, z=None):
            if z is not None and ZIN == "scalar":
                seg = seg + pltpu.bitcast(z, jnp.int32)[0, 0]
            rows = pl.ds(r, 8)
            t = modv(2) * ybuf[seg, rows, :].astype(F32)
            if z is not None and ZIN == "all":
                t = t + jnp.concatenate([pltpu.bitcast(z, F32)] * NT, axis=1)
            x1 = xbuf[seg, rows, :].astype(F32) + t
            h2 = _ln_mod(x1, modv(4), modv(3),
                         pltpu.bitcast(z, F32) if z is not None and ZIN == "mean" else None)
            hbuf[seg, rows, :] = h2.astype(BF16)
            o = x1 + modv(5) * h2
            outs[seg, rows, :] = o.astype(BF16)
            v = _rb(jnp.sum(h2 * modv(6), axis=-1, keepdims=True))
            b = pltpu.bitcast(jnp.where(v != v, -jnp.inf, v + 0.0), jnp.int32)
            low = (S - 1 - seg * SEG - r) - lax.broadcasted_iota(jnp.int32, (8, 1), 0)
            key = (b ^ ((b >> 31) & 0x7FFF0000)) | low
            m1, m2 = top[0:8, :], top[8:16, :]
            top[8:16, :] = jnp.maximum(m2, jnp.minimum(m1, key))
            top[0:8, :] = jnp.maximum(m1, key)
            if z is not None:
                res = pltpu.bitcast(jnp.broadcast_to(v, (8, 128)), U32)
                if PIN_OUT:
                    for k in range(NT):
                        res = res | pltpu.bitcast(o[:, k * 128:(k + 1) * 128], U32)
                return res

        def out_copy(g0, ng, r, n, k=0):
            return pltpu.make_async_copy(outs.at[pl.ds(g0, ng), pl.ds(r, n), :],
                                         out_hbm.at[pl.ds(g0, ng), pl.ds(r, n), :], sem_out.at[k])

        late = ((wg_hbm, wg_s, FF // 128), (wu_hbm, wu_s, FF // 128), (wd_hbm, wd_s, NT))

        def col_copy(k, j):
            return pltpu.make_async_copy(
                late[k][0].at[:, pl.ds(pl.multiple_of(j * 128, 128), 128)], late[k][1].at[j],
                sem_f.at[k])

        load_x_rows(0, 0)

        def step(it, cur, state):
            s = it * UNROLL + cur
            nxt = (cur + 1) % UNROLL

            def pay(t, cost):
                now = state.get("now", 0)
                due = state.setdefault("due", [])
                for z in [z for (d, z) in due if d <= now]:
                    t = jnp.concatenate([t[0:8] | z, t[8:]], axis=0)
                state["due"] = [(d, z) for (d, z) in due if d > now]
                state["now"] = now + cost
                return t

            def owe(lag, p, tiles):
                z = tiles[0]
                for t in tiles[1:]:
                    z = z | t
                state.setdefault("due", []).append(
                    (state.get("now", 0) + lag + (p % 4) * TOK_STAG, zero_after(z)))

            def lv(k0, k1):
                ts = [lhs[cur, k] for k in range(k0, k1)]
                ts[0] = pay(ts[0], (k1 - k0) / NT)
                return jnp.concatenate([_as_bf16(t) for t in ts], axis=1)

            def wmat(mat, h, q0, q1):
                return _as_bf16(jnp.concatenate([wqkv[3 * q + mat, h] for q in range(q0, q1)],
                                                axis=0))

            def qkv(p, split=False):
                part = {}
                if split:
                    for mat in range(3):
                        for a in range(2):
                            part[mat, a] = _dot(lv(0, NT // 2), wmat(mat, 2 * p + a, 0, 2))
                for mat in range(3):
                    for a in range(2):
                        hm = mat * H + 2 * p + a
                        if split:
                            y = _dot(lv(NT // 2, NT), wmat(mat, 2 * p + a, 2, 4)) + part[mat, a]
                        else:
                            y = _dot(lv(0, NT), wmat(mat, 2 * p + a, 0, 4))
                        cur_s[hm] = y.astype(BF16)

            def gather(mat, p):
                hm = mat * H + 2 * p
                return jnp.concatenate(
                    [cur_s[hm], cur_s[hm + 1], pre[mat * NP + p, s].astype(BF16)], axis=0)

            probs = {}

            def scores(p):
                sc = lax.dot_general(gather(0, p), gather(1, p), (((1,), (1,)), ((), ())),
                                     preferred_element_type=F32)
                mv = mk[...]
                sc = jnp.where(mv == 0.0, sc * (SCALE * LOG2E), mv)
                e = jnp.exp2(sc - jnp.max(sc, axis=-1, keepdims=True))
                inv = _recip(jnp.sum(e, axis=-1, keepdims=True))
                if NORM_PRE:
                    e = e * inv
                    if TOK_S is not None:
                        eu = pltpu.bitcast(e, U32)
                        z = eu[0:8]
                        for k in range(1, PR // 8):
                            z = z | eu[k * 8:(k + 1) * 8]
                        owe(TOK_S, p, [jnp.concatenate([z, jnp.zeros((8, 128 - PR), U32)], axis=1)])
                    probs[p] = (e.astype(BF16), None)
                else:
                    if TOK_S is not None:
                        iu = pltpu.bitcast(jnp.broadcast_to(inv, (PR, 128)), U32)
                        owe(TOK_S, p, [iu[k * 8:(k + 1) * 8] for k in range(PR // 8)])
                    probs[p] = (e.astype(BF16), inv)

            def pv(p):
                e, inv = probs.pop(p)
                o = _dot(e, gather(2, p))
                if inv is not None:
                    o = o * inv
                o = o.astype(BF16)
                if TOK_P is not None:
                    ou = _as_u32(o)
                    owe(TOK_P, p, [ou[k * 8:(k + 1) * 8] for k in range(PR // 16)])
                for a in range(2):
                    h = 2 * p + a
                    olhs[h] = _as_u32(o[a * SEG:(a + 1) * SEG])
                    odef[h, it, cur * 4:(cur + 1) * 4, :] = _as_u32(
                        o[2 * SEG + a * M:2 * SEG + (a + 1) * M])

            acc = [None] * NT

            def oproj(j, pairs):
                ts = [olhs[2 * p + a] for p in pairs for a in range(2)]
                ts[0] = pay(ts[0], len(pairs) / 4)
                ov = jnp.concatenate([_as_bf16(t) for t in ts], axis=1)
                w = wo_s[j, pairs[0] * DH:(pairs[-1] + 1) * DH, :]
                y = _dot(ov, _as_bf16(w))
                acc[j] = y if acc[j] is None else y + acc[j]

            def fin(j):
                yb = acc[j].astype(BF16)
                ybuf[s, 0:XR, j * 128:(j + 1) * 128] = yb[0:XR]
                lhs[nxt, j, XR // 2:, :] = _as_u32(yb[XR:])

            def late_mod(u):
                mod_tile(wm_s[it & 3, u], 2 * NT + it * mt + u)

            load_x_rows(nxt, jnp.minimum(s + 1, NSEG - 1))
            ops = dict(Q=qkv, S=scores, P=pv, O=oproj, F=fin, M=late_mod)
            for op in _schedule([(u, q) for u, (c_, q) in enumerate(MODS[:mt]) if c_ % UNROLL == cur]):
                ops[op[0]](*op[1:])

        def steps(it, carry):
            if "pro" in PHASES:
                pltpu.make_async_copy(wm_s.at[it & 3], wm_s.at[it & 3], sem_m.at[it & 3]).wait()

                @pl.when(it + 2 < NSEG // UNROLL)
                def _():
                    for u in range(mt):
                        wm_copy(it + 2, u).start()

            for u in range(UNROLL // 2):
                t = it * (UNROLL // 2) + u
                for k in range(3):
                    @pl.when(t < late[k][2])
                    def _():
                        col_copy(k, t).start()

            state = {}
            for u in range(UNROLL):
                step(it, u, state)
            return carry

        with jax.named_scope("m_steps"):
            if "step" in PHASES: lax.fori_loop(0, NSEG // UNROLL, steps, 0)
        for k in range(3):
            for j in range(late[k][2]):
                col_copy(k, j).wait()
        if "epi" not in PHASES:
            return

        ntail = EBLK[-1] // M
        ppi = (S // 8 - ntail) // NEC
        gpi = ppi // (XR // 8)
        gb_ = UNROLL * M

        def ep_body(i, c):
            @pl.when(i > 0)
            def _():
                out_copy((i - 1) * gpi, gpi, 0, XR).start()

            subs = []
            r0 = 0
            for nr in EBLK:
                kh = EKH * EC // nr if EC % nr == 0 else EKH
                for j in range(NT):
                    for h0_ in range(0, H, kh):
                        subs.append((r0, nr, j, h0_, kh))
                r0 += nr
            tot = sum(nr * kh for (_, nr, _, _, kh) in subs)
            span = E_SPAN * EC * EKH
            rel = [u * (tot - span) // ppi for u in range(ppi)]
            ready = {}
            due = []
            now = 0
            u = 0
            y = None
            for (r0, nr, j, h0_, kh) in subs:
                blk = pl.ds(i * (EC // gb_) + r0 // gb_, nr // gb_)
                ts = [odef[h, blk].reshape(nr // 2, DH) for h in range(h0_, h0_ + kh)]
                for z in [z for (d, z) in due if d <= now]:
                    ts[0] = jnp.concatenate([ts[0][0:8] | z, ts[0][8:]], axis=0)
                due = [(d, z) for (d, z) in due if d > now]
                w = wo_s[j, h0_ * DH // 2:(h0_ + kh) * DH // 2, :]
                yp = _dot(jnp.concatenate([_as_bf16(t) for t in ts], axis=1), _as_bf16(w))
                y = yp if h0_ == 0 else yp + y
                if h0_ + kh == H:
                    ybuf[pl.ds(i * (EC // M) + r0 // M, nr // M), XR:, j * 128:(j + 1) * 128] = (
                        y.reshape(nr // M, M, 128).astype(BF16))
                    if j == NT - 1:
                        ready[r0] = True
                start = now
                now += nr * kh
                while u < ppi and rel[u] < now:
                    d = (NEC - 1) * ppi + u - NSEG * (XR // 8) - (NEC - 1) * (EC // M)
                    if d >= 0 and sum(n for r, n in zip(_cumsum(EBLK), EBLK) if r in ready) <= d * M:
                        break
                    t = i * ppi + u
                    early = t < NSEG * (XR // 8)
                    seg = jnp.where(early, t // (XR // 8), t - NSEG * (XR // 8))
                    row = pl.multiple_of(jnp.where(early, (t % (XR // 8)) * 8, XR), 8)
                    res = post(seg, row, zero_after(y[0:8]))
                    due.append((start + span, zero_after(res)))
                    u += 1
            assert u == ppi
            return c

        with jax.named_scope("e_loop"):
            lax.fori_loop(0, NEC, ep_body, 0)
        done = (NEC - 1) * gpi
        tail = NSEG - ntail
        out_copy(done, NSEG - done, 0, XR).start()
        out_copy(0, tail, XR, M).start()
        for g in range(tail, NSEG):
            post(g, XR)
        out_copy(tail, NSEG - tail, XR, M).start()

        tk = top[...]
        k1 = jnp.max(tk[0:8], axis=0, keepdims=True)
        k2 = jnp.max(jnp.where(tk == k1, jnp.iinfo(jnp.int32).min, tk), axis=0, keepdims=True)
        i1 = (S - 1) - (k1[0, 0] & (S - 1))
        i2 = (S - 1) - (k2[0, 0] & (S - 1))
        g1, g2 = i1 >> 5, i2 >> 5
        b1 = pl.multiple_of(i1 & 24, 8)
        b2 = pl.multiple_of(i2 & 24, 8)

        def two_blocks(ref):
            return jnp.concatenate([ref[g1, pl.ds(b1, 8), :].astype(F32),
                                    ref[g2, pl.ds(b2, 8), :].astype(F32)], axis=0)

        h2b = two_blocks(hbuf).astype(BF16)
        row = lax.broadcasted_iota(jnp.int32, (16, 1), 0)
        grow = jnp.where(row < 8, g1 * SEG + b1 + row, g2 * SEG + b2 + row - 8)
        ks = jnp.where(grow == i1, k1, k2)
        rsel = pltpu.bitcast((ks ^ ((ks >> 31) & 0x7FFF0000)) & -65536, F32)
        acts = []
        for j in range(FF // 128):
            gt = _rb(_dot(h2b, wg_s[j]))
            gt = _rb(gt * _rb(jax.nn.sigmoid(gt)))
            ut = _rb(_dot(h2b, wu_s[j]))
            acts.append((gt * ut).astype(BF16))
        act = jnp.concatenate(acts, axis=1)
        y = _rb(jnp.concatenate([_dot(act, wd_s[j]) for j in range(NT)], axis=1))
        y = _rb(y * _rb(jax.nn.sigmoid(rsel)))
        sel = jnp.logical_or(grow == i1, grow == i2)
        upd = jnp.concatenate([modv(5)] * 2, axis=0) * y
        fixed = (two_blocks(outs) + jnp.where(sel, upd, 0.0)).astype(BF16)

        with jax.named_scope("e_outwait"):
            out_copy(0, NSEG, 0, SEG).wait()
        outs[g1, pl.ds(b1, 8), :] = fixed[0:8]
        outs[g2, pl.ds(b2, 8), :] = fixed[8:16]
        out_copy(g1, 1, b1, 8, 0).start()

        @pl.when((i1 >> 3) != (i2 >> 3))
        def _():
            out_copy(g2, 1, b2, 8, 1).start()
            out_copy(g2, 1, b2, 8, 1).wait()

        out_copy(g1, 1, b1, 8, 0).wait()

    pl.run_scoped(
        main,
        pltpu.VMEM((FF // 128, D, 128), BF16),
        pltpu.VMEM((FF // 128, D, 128), BF16),
        pltpu.VMEM((NT, FF, 128), BF16),
        pltpu.VMEM((NSEG, SEG, D), BF16),
        pltpu.VMEM((NSEG, SEG, D), BF16),
        pltpu.VMEM((NSEG, SEG, D), BF16),
        pltpu.SemaphoreType.DMA((3,)),
    )


@functools.partial(jax.jit, static_argnames=("A_seg_len",))
def pallas_adaLN_cond__memory_aug_recurrent_mem_tr__moe_arch_mod__prompt_kernel(
    A_x: jax.Array,
    A_mem0: jax.Array,
    A_Wq: jax.Array,
    A_Wk: jax.Array,
    A_Wv: jax.Array,
    A_Wo: jax.Array,
    A_seg_len,
    B_x: jax.Array,
    B_w_r: jax.Array,
    B_w_gate: jax.Array,
    B_w_up: jax.Array,
    B_w_down: jax.Array,
    c: jax.Array,
    w_mod: jax.Array,
):
    assert A_seg_len == SEG and A_x.shape == (1, S, D)
    del B_x
    hbm = pl.BlockSpec(memory_space=pl.ANY)
    out = pl.pallas_call(
        _kernel,
        out_shape=jax.ShapeDtypeStruct((NSEG, SEG, D), BF16),
        in_specs=[hbm] * 12,
        out_specs=hbm,
        scratch_shapes=[
            pltpu.VMEM((NCHUNK, H, KQ // 2, DH), U32),
            pltpu.VMEM((NSEG + 1, NT, XR // 2, 128), U32),
            pltpu.VMEM((NT, (H * DH + H * DH // NT) // 2, 128), U32),
            pltpu.VMEM((3 * NP, NSEG, 2 * M, DH), F32),
            pltpu.VMEM((3 * H, SEG, DH), BF16),
            pltpu.VMEM((H, SEG // 2, DH), U32),
            pltpu.VMEM((H, NSEG // UNROLL, UNROLL * M // 2, DH), U32),
            pltpu.VMEM((NSEG, SEG, D), BF16),
            pltpu.VMEM((UNROLL, NT, SEG // 2, 128), U32),
            pltpu.VMEM((4, 4 * NT * UNROLL // NSEG, D, 128), BF16),
            pltpu.VMEM((7 * NT, M, 128), F32),
            pltpu.VMEM((PR, PR), F32),
            pltpu.VMEM((16, 1), jnp.int32),
            pltpu.VMEM((M, D), BF16),
            pltpu.VMEM((8 + PADS[2], 128), U32),
            pltpu.SemaphoreType.DMA((4,)),
            pltpu.SemaphoreType.DMA((2,)),
        ],
        compiler_params=pltpu.CompilerParams(vmem_limit_bytes=120 * 1024 * 1024,
                                             disable_bounds_checks=True),
    )(A_x.reshape(NSEG, SEG, D), A_mem0.reshape(M, D), A_Wq, A_Wk, A_Wv, A_Wo.reshape(H * DH, D),
      B_w_r, B_w_gate, B_w_up, B_w_down, c, w_mod)
    return out.reshape(1, S, D)
```

```python
import functools

import jax
import jax.numpy as jnp
from jax import lax
import jax.experimental.pallas as pl
import jax.experimental.pallas.tpu as pltpu

F32 = jnp.float32
BF16 = jnp.bfloat16
U32 = jnp.uint32

D = 1024
S = 2048
H = 32
DH = 128
M = 8
SEG = 32
NSEG = S // SEG
FF = 3584
NT = D // 128
XR = SEG - M
R0 = M * NSEG
CH = 8
KQ = D // 4
NCHUNK = 3 * D // KQ
NSLOT = 4
PR = 2 * SEG + 2 * M
NP = H // 2
EC = 128
NEC = R0 // EC
LOG2E = 1.4426950408889634
EPS = 1e-5
SCALE = DH ** -0.5
NEG_MASK = -1000000000.0

PHASES = ("pro", "step", "epi")
UNROLL = 4
FB = 32
BLK = 32
R_AT = ((0, 6, 16), (14, 22, 30), (30, 38, 46), (44, 52, 60))
F_AT = (5, 13)
L_AT = 5
OPAQUE = True
LATE_APPLY = False
LEAN = False
RB = 16
RB2 = 64
JOB_SPAN = 40
LNU = 16
EKH = 4
E_SPAN = 6
ZIN = "all"
PIN_OUT = False
EBLK = (128,)
PADS = (0, 0, 0)
MODS = ((-1, 4), (1, 4))
TOK_S = 9
TOK_P = None
TOK_STAG = 2
NORM_PRE = True
R1_END = 11
R2_0 = (3, 14)
LN_RANGE = (0, 29)
WO_RANGE = (12, 31)


def _schedule(mods):
    groups = [list(range(4 * g, 4 * g + 4)) for g in range(4)]
    ops = []

    def mod_at(pos):
        ops.extend(("M", u) for (u, q) in mods if q == pos)

    for t in range(4):
        for i, p in enumerate(groups[t]):
            ops.append(("Q", p, p == 0))
            if i == 0 and t >= 1:
                ops.extend(("S", q) for q in groups[t - 1])
                mod_at(10 + t)
            if i == 3 and t >= 1:
                ops.extend(("P", q) for q in groups[t - 1])
                mod_at(t)
    first = groups[0] + groups[1]
    for j in range(NT):
        ops.append(("O", j, first))
        if j == 1:
            ops.extend(("S", q) for q in groups[3])
            mod_at(14)
    ops.extend(("P", q) for q in groups[3])
    mod_at(4)
    ops.extend(("O", j, groups[2]) for j in range(NT))
    for j in range(NT):
        ops.append(("O", j, groups[3]))
        ops.append(("F", j))
    mod_at(5)
    return ops


def _rb(x):
    return x.astype(BF16).astype(F32)


def _recip(x):
    r = pl.reciprocal(x, approx=True)
    return r * (2.0 - x * r)


def _ln(x, zero=None, lean=False):
    xm = x if zero is None else jnp.concatenate([x[..., :128] + zero, x[..., 128:]], axis=-1)
    mu = jnp.mean(xm, axis=-1, keepdims=True)
    xc = x - mu
    v = _rb(_rb(jnp.mean(xc * xc, axis=-1, keepdims=True)) + EPS)
    inv = _recip(_rb(v * lax.rsqrt(v)))
    if lean:
        return x * inv - mu * inv
    return xc * inv


def _ln_mod(x, s1p, shift, zero=None, lean=False):
    return _ln(x, zero, lean) * s1p + shift


def _dot(a, b):
    return jnp.dot(a, b, preferred_element_type=F32)


def _as_bf16(u):
    return pltpu.bitcast(u, BF16)


def _as_u32(b):
    return pltpu.bitcast(b, U32)


def _cumsum(xs):
    out, r = [], 0
    for x in xs:
        out.append(r)
        r += x
    return out


def _spread(jobs, fns, lo, hi):
    for n, fn in enumerate(fns):
        jobs.setdefault(lo + n * (hi - lo) // len(fns), []).append(fn)


def _kernel(x_hbm, mem0_hbm, wq_hbm, wk_hbm, wv_hbm, wo_hbm, wr_hbm, wg_hbm, wu_hbm, wd_hbm,
            c_hbm, wmod_hbm, out_hbm,
            wqkv, hs, wo_s, pre, cur_s, olhs, odef, xbuf, lhs, wm_s, mod, mk,
            top, sc_s, zero_s, sem_m, sem_out):
    mt = 4 * NT * UNROLL // NSEG

    def modv(j):
        return jnp.concatenate([mod[j * NT + k] for k in range(NT)], axis=1)

    def mod_tile(wm, t):
        v = _rb(_dot(sc_s[...], wm))
        mod[t] = jnp.where(jnp.logical_or(t // NT == 1, t // NT == 4), _rb(1.0 + v), v)

    def wm_copy(it, u):
        col = pl.multiple_of((2 * NT + it * mt + u) * 128, 128)
        return pltpu.make_async_copy(wmod_hbm.at[:, pl.ds(col, 128)], wm_s.at[it & 3, u],
                                     sem_m.at[it & 3])

    def ln1(x, zero=None):
        x3 = x.astype(F32).reshape(x.shape[0] // 8, 8, D)
        zf = None if zero is None else pltpu.bitcast(zero, F32)
        if LATE_APPLY:
            return _ln(x3, zf, LEAN).reshape(x.shape[0], D).astype(BF16)
        return _ln_mod(x3, modv(1), modv(0), zf, LEAN).reshape(x.shape[0], D).astype(BF16)

    def zero_after(y):
        return (y if y.dtype == U32 else pltpu.bitcast(y, U32)) & zero_s[0:8, :]

    def or_tile(u, z):
        if z is None:
            return u
        return (u.reshape(u.shape[0] // 8, 8, 128) | z).reshape(u.shape)

    def prologue(stage, wo_raw, wmod_s, nrm, ha, hb, tmp, mem0_ref, wr_ref, c_ref, sem):
        w_hbms = (wq_hbm, wk_hbm, wv_hbm)
        wob = H * DH // NT
        S_X, S_C0, S_ST, S_WO, S_MOD, S_SM = 0, 2, 6, 6 + NSLOT, 6 + NSLOT + NT, 6 + NSLOT + 2 * NT

        def x_copy(i):
            lo, n = ((XR, M), (0, XR))[i]
            return pltpu.make_async_copy(x_hbm.at[:, pl.ds(lo, n), :], xbuf.at[:, pl.ds(lo, n), :],
                                         sem.at[S_X + i])

        def mod_copies(k):
            return [pltpu.make_async_copy(wmod_hbm.at[:, pl.ds(v * D + k * 128, 128)],
                                          wmod_s.at[k, v], sem.at[S_MOD + k]) for v in range(2)]

        def chunk_copy(mat, d0, g, slot, k):
            return pltpu.make_async_copy(w_hbms[mat].at[pl.ds(d0, KQ), pl.ds(g * CH, CH), :],
                                         stage.at[slot, g], sem.at[k])

        def wo_copy(j):
            return pltpu.make_async_copy(wo_hbm.at[pl.ds(pl.multiple_of(j * wob, wob), wob)],
                                         wo_raw.at[j], sem.at[S_WO + j])

        def relayout1(src, t0, z=None):
            v = src.reshape(RB * CH, 128)
            tmp[t0:t0 + RB * CH // 2, :] = or_tile(_as_u32(v), z)

        def relayout2(c, h0_, t0, d0, z=None):
            w = or_tile(tmp[pl.ds(t0, RB2, stride=CH // 2), :], z)
            rows = pl.ds(d0 // 2, RB2 // 2)
            wqkv[c, h0_, rows, :] = _as_u32(w.astype(jnp.uint16))
            wqkv[c, h0_ + 1, rows, :] = _as_u32((w >> 16).astype(jnp.uint16))

        def mod_pair(k):
            for v in range(2):
                mod_tile(wmod_s[k, v], v * NT + k)

        def fill(dst, q, t, r, z=None):
            k = 2 * q + t
            sh = mod[k] if z is None else mod[k] + pltpu.bitcast(z, F32)
            v = nrm[k, r:r + FB, :].reshape(FB // 8, 8, 128) * mod[NT + k] + sh
            dst[t, r // 2:(r + FB) // 2, :] = _as_u32(v.reshape(FB, 128).astype(BF16))

        small = [pltpu.make_async_copy(src, dst, sem.at[S_SM])
                 for src, dst in ((c_hbm, c_ref), (mem0_hbm, mem0_ref), (wr_hbm, wr_ref))]
        for cp in small:
            cp.start()
        x_copy(0).start()
        for cp in mod_copies(0) + mod_copies(1):
            cp.start()
        for g in range(4):
            chunk_copy(0, 0, g, 0, S_C0 + g).start()
        for c in range(1, NSLOT):
            for g in range(4):
                chunk_copy(c % 3, (c // 3) * KQ, g, c, S_ST + c).start()
            for cp in mod_copies(2 * c) + mod_copies(2 * c + 1):
                cp.start()

        def decode(i):
            lo = i < 2 * SEG
            head = jnp.where(lo, i // SEG, (i - 2 * SEG) // M)
            is_mem = jnp.logical_and(lo, i % SEG >= XR)
            pos = jnp.where(lo, i % SEG, XR + i % M)
            return head, is_mem, pos

        qh, qm, qp = decode(lax.broadcasted_iota(jnp.int32, (PR, PR), 0))
        kh, km, kp = decode(lax.broadcasted_iota(jnp.int32, (PR, PR), 1))
        vis = qm | km | (qp >= kp)
        mk[...] = jnp.where(qh == kh, jnp.where(vis, 0.0, NEG_MASK * LOG2E), -jnp.inf).astype(F32)
        mod[0:2 * NT] = jnp.zeros((2 * NT, M, 128), F32)
        zero_s[...] = jnp.zeros(zero_s.shape, U32)
        top[...] = jnp.full(top.shape, jnp.iinfo(jnp.int32).min, jnp.int32)
        for cp in small:
            cp.wait()
        wr = jnp.broadcast_to(wr_ref[...].astype(F32).reshape(1, D), (M, D))
        for k in range(NT):
            mod[6 * NT + k] = wr[:, k * 128:(k + 1) * 128]
        cv = c_ref[...].astype(F32)
        sc_s[...] = jnp.broadcast_to(cv * _rb(jax.nn.sigmoid(cv)), (M, D)).astype(BF16)
        mb = mem0_ref[...]
        for k in range(NT):
            lhs[0, k, XR // 2:, :] = _as_u32(mb[:, k * 128:(k + 1) * 128])

        def zero_body(i, c):
            wo_raw[NT, pl.ds(pl.multiple_of(i * 32, 32), 32), :] = jnp.zeros((32, D), BF16)
            return c

        lax.fori_loop(0, wob // 32, zero_body, 0)
        x_copy(0).wait()

        def ln_body(i, c):
            for u in range(LNU):
                q = i * LNU + u
                v = _ln(xbuf[q, XR:, :].astype(F32))
                for k in range(NT):
                    nrm[k, pl.ds(pl.multiple_of(q * 8, 8), 8), :] = v[:, k * 128:(k + 1) * 128]
            return c

        with jax.named_scope("p_ln"):
            lax.fori_loop(0, NSEG // LNU, ln_body, 0)

        def mod_body(k, c):
            pltpu.make_async_copy(wmod_s.at[k], wmod_s.at[k], sem.at[S_MOD + k]).wait()
            mod_pair(k)
            for r in range(0, R0, FB):
                fill(ha, 0, k, r)
            return c

        with jax.named_scope("p_mod"):
            lax.fori_loop(0, 2, mod_body, 0)

        def c0_body(g):
            chunk_copy(0, 0, 0, 0, S_C0 + g).wait()
            for d0 in range(0, KQ, RB):
                relayout1(stage[0, g, d0:d0 + RB], d0 * CH // 2)
            for j in range(CH // 2):
                for d0 in range(0, KQ, RB2):
                    relayout2(0, g * CH + 2 * j, d0 * CH // 2 + j, d0)

        def bulk(units, jobs, inserts):
            due = {}
            t0 = 0
            for n, (hq, c, h0_, pi, first, r0, nrow) in enumerate(units):
                nb = nrow // BLK
                parts = []
                for u in range(nb):
                    part = hq[0, (r0 + u * BLK) // 2:(r0 + (u + 1) * BLK) // 2, :]
                    for z in due.pop(t0 + u, ()):
                        part = jnp.concatenate([part[0:8] | z, part[8:]], axis=0)
                    parts.append(part)
                hv = jnp.concatenate([_as_bf16(jnp.concatenate(parts, axis=0)),
                                      _as_bf16(hq[1, r0 // 2:(r0 + nrow) // 2, :])], axis=1)
                w = jnp.concatenate([_as_bf16(wqkv[c, h0_]), _as_bf16(wqkv[c, h0_ + 1])], axis=1)
                y = _dot(hv, w)
                segs = slice(r0 // M, (r0 + nrow) // M)
                for a in range(2):
                    old = jnp.where(first, 0.0, pre[pi, segs, a * M:(a + 1) * M, :])
                    pre[pi, segs, a * M:(a + 1) * M, :] = (
                        y[:, a * DH:(a + 1) * DH].reshape(nrow // M, M, DH) + old)
                for fn in inserts.get(n, ()):
                    fn()
                for u in range(nb):
                    for job in jobs.get(t0 + u, ()):
                        res = job(zero_after(y[u * BLK:u * BLK + 8, 0:128]))
                        if res is not None:
                            due.setdefault(max(t0 + u + JOB_SPAN, t0 + nb), []).append(
                                zero_after(res))
                t0 += nb
            assert not due

        GP = CH // 2
        WO0 = NCHUNK - 1 - NT
        LN0 = 3 if LATE_APPLY else NT - 2
        SPI = -(-NSEG // (NCHUNK - 1 - LN0))

        def rot_body(i, c):
            slot = (i + 1) & (NSLOT - 1)
            pltpu.make_async_copy(stage.at[slot], stage.at[slot], sem.at[S_ST + slot]).wait()
            km = jnp.minimum(i + 1, NT - 1)

            @pl.when(jnp.logical_and(i >= 1, i + 1 < NT))
            def _():
                pltpu.make_async_copy(wmod_s.at[km], wmod_s.at[km], sem.at[S_MOD + km]).wait()

            @pl.when(i == LN0)
            def _():
                x_copy(1).wait()

            @pl.when(i >= WO0)
            def _():
                wo_copy(i - WO0).wait()

            nxt = i + NSLOT
            qn = (nxt * 43) >> 7
            for mat in range(3):
                @pl.when(jnp.logical_and(nxt < NCHUNK, nxt - 3 * qn == mat))
                def _():
                    for g in range(4):
                        chunk_copy(mat, qn * KQ, g, nxt & (NSLOT - 1),
                                   S_ST + (nxt & (NSLOT - 1))).start()

            @pl.when(i < NT)
            def _():
                wo_copy(i).start()

            @pl.when(i == 0)
            def _():
                x_copy(1).start()

            q0 = (i * 43) >> 7
            q1 = ((i + 1) * 43) >> 7
            pa = (i - 3 * q0) * NP + NP - GP
            units = ([(ha, i, H - CH, pa, q0 == 0, r, R0 // 2) for r in (0, R0 // 2)]
                     + [(ha, i, H - CH + 2 * n, pa + n, q0 == 0, 0, R0) for n in range(1, GP)]
                     + [(hb, i + 1, 2 * n, (i + 1 - 3 * q1) * NP + n, q1 == 0, 0, R0)
                        for n in range(NP - GP)])
            jw = jnp.where(i >= WO0, i - WO0, NT)

            def wo_job(b, z):
                v = wo_raw[jw, b * 16:(b + 1) * 16, :]
                rows = pl.ds(pl.multiple_of(jw * (wob // 2) + b * 8, 8), 8)
                for j in range(NT):
                    wo_s[j, rows, :] = _as_u32(v[:, j * 128:(j + 1) * 128]) | z

            def ln_job(b, z):
                r = (b % 3) * 8
                seg = (i - LN0) * SPI + b // 3
                live = jnp.logical_and(i >= LN0, seg < NSEG)
                src = jnp.where(live, seg, 0)
                hv = ln1(xbuf[src, pl.ds(pl.multiple_of(jnp.where(live, r, XR), 8), 8), :], z)
                u = [_as_u32(hv[:, k * 128:(k + 1) * 128]) for k in range(NT)]
                dst = jnp.where(live, seg, NSEG)
                for k in range(NT):
                    hs[dst, k, r // 2:r // 2 + 4, :] = u[k]
                res = jnp.concatenate(u[0:2], axis=0)
                for k in range(2, NT, 2):
                    res = res | jnp.concatenate(u[k:k + 2], axis=0)
                return res

            def r1_job(g, d0, z):
                relayout1(stage[slot, g, d0:d0 + RB], (g * KQ + d0) * CH // 2, z)

            def copy_job(t, r, z):
                ha[t, r:r + 32, :] = or_tile(hb[t, r:r + 32, :], z)

            P = functools.partial
            upb = R0 // BLK
            nr = NP * upb
            jobs = {}
            for g in range(4):
                lo, mid, hi = (x * upb // 4 for x in R_AT[g])
                _spread(jobs, [P(r1_job, g, d0) for d0 in range(0, KQ, RB)], lo, mid)
                _spread(jobs, [P(relayout2, i + 1, g * CH + 2 * j, (g * KQ + d0) * CH // 2 + j, d0)
                               for j in range(CH // 2) for d0 in range(0, KQ, RB2)], mid, hi)
            oz = (i >> 10) if OPAQUE else 0
            _spread(jobs, [P(fill, hb, q1, t + oz, r) for r in range(0, R0, FB) for t in range(2)],
                    F_AT[0] * upb // 4, F_AT[1] * upb // 4)
            _spread(jobs, [P(copy_job, t, r) for t in range(2) for r in range(0, R0 // 2, 32)],
                    2 * GP * upb, nr - upb)
            _spread(jobs, [P(ln_job, b) for b in range(3 * SPI)],
                    L_AT * upb // 4, nr - max(upb, JOB_SPAN))
            _spread(jobs, [P(wo_job, b) for b in range(wob // 16)], GP * upb, nr - upb)
            bulk(units, jobs, {0: [lambda: mod_tile(wmod_s[km, 0], km)],
                               1: [lambda: mod_tile(wmod_s[km, 1], NT + km)]})
            return c

        def outer(k, c):
            last = k == 4

            @pl.when(k < 4)
            def _():
                c0_body(k)

            @pl.when(k != 3)
            def _():
                g = jnp.minimum(k, 3)
                bulk([(ha, jnp.where(last, NCHUNK - 1, 0), g * CH + 2 * n,
                       jnp.where(last, 2 * NP, 0) + g * GP + n, k < 4, 0, R0)
                      for n in range(GP)], {}, {})

            @pl.when(k == 3)
            def _():
                with jax.named_scope("p_rot"):
                    lax.fori_loop(0, NCHUNK - 1, rot_body, 0)
                for it in range(2):
                    for u in range(mt):
                        wm_copy(it, u).start()

            return c

        with jax.named_scope("p_bulk"):
            lax.fori_loop(0, 5, outer, 0)

    if "pro" in PHASES: pl.run_scoped(
        prologue,
        pltpu.VMEM((NSLOT, H // CH, KQ, CH, 128), BF16),
        pltpu.VMEM((NT + 1, H * DH // NT, D), BF16),
        pltpu.VMEM((NT, 2, D, 128), BF16),
        pltpu.VMEM((NT, R0, 128), F32),
        pltpu.VMEM((2, R0 // 2 + PADS[0], 128), U32),
        pltpu.VMEM((2, R0 // 2 + PADS[0], 128), U32),
        pltpu.VMEM((D * CH // 2 + PADS[1], 128), U32),
        pltpu.VMEM((M, D), BF16),
        pltpu.VMEM((D,), BF16),
        pltpu.VMEM((1, D), BF16),
        pltpu.SemaphoreType.DMA((7 + NSLOT + 2 * NT,)),
    )

    def main(wg_s, wu_s, wd_s, ybuf, hbuf, outs, sem_f):
        def load_x_rows(slot, seg):
            for k in range(NT):
                if LATE_APPLY:
                    v = _as_bf16(hs[seg, k]).astype(F32).reshape(XR // 8, 8, 128)
                    v = (v * mod[NT + k] + mod[k]).reshape(XR, 128)
                    lhs[slot, k, 0:XR // 2, :] = _as_u32(v.astype(BF16))
                else:
                    lhs[slot, k, 0:XR // 2, :] = hs[seg, k]

        def post(seg, r, z=None):
            if z is not None and ZIN == "scalar":
                seg = seg + pltpu.bitcast(z, jnp.int32)[0, 0]
            rows = pl.ds(r, 8)
            t = modv(2) * ybuf[seg, rows, :].astype(F32)
            if z is not None and ZIN == "all":
                t = t + jnp.concatenate([pltpu.bitcast(z, F32)] * NT, axis=1)
            x1 = xbuf[seg, rows, :].astype(F32) + t
            h2 = _ln_mod(x1, modv(4), modv(3),
                         pltpu.bitcast(z, F32) if z is not None and ZIN == "mean" else None)
            hbuf[seg, rows, :] = h2.astype(BF16)
            o = x1 + modv(5) * h2
            outs[seg, rows, :] = o.astype(BF16)
            v = _rb(jnp.sum(h2 * modv(6), axis=-1, keepdims=True))
            b = pltpu.bitcast(jnp.where(v != v, -jnp.inf, v + 0.0), jnp.int32)
            low = (S - 1 - seg * SEG - r) - lax.broadcasted_iota(jnp.int32, (8, 1), 0)
            key = (b ^ ((b >> 31) & 0x7FFF0000)) | low
            m1, m2 = top[0:8, :], top[8:16, :]
            top[8:16, :] = jnp.maximum(m2, jnp.minimum(m1, key))
            top[0:8, :] = jnp.maximum(m1, key)
            if z is not None:
                res = pltpu.bitcast(jnp.broadcast_to(v, (8, 128)), U32)
                if PIN_OUT:
                    for k in range(NT):
                        res = res | pltpu.bitcast(o[:, k * 128:(k + 1) * 128], U32)
                return res

        def out_copy(g0, ng, r, n, k=0):
            return pltpu.make_async_copy(outs.at[pl.ds(g0, ng), pl.ds(r, n), :],
                                         out_hbm.at[pl.ds(g0, ng), pl.ds(r, n), :], sem_out.at[k])

        late = ((wg_hbm, wg_s, FF // 128), (wu_hbm, wu_s, FF // 128), (wd_hbm, wd_s, NT))

        def col_copy(k, j):
            return pltpu.make_async_copy(
                late[k][0].at[:, pl.ds(pl.multiple_of(j * 128, 128), 128)], late[k][1].at[j],
                sem_f.at[k])

        load_x_rows(0, 0)

        def step(it, cur, state):
            s = it * UNROLL + cur
            nxt = (cur + 1) % UNROLL

            def pay(t, cost):
                now = state.get("now", 0)
                due = state.setdefault("due", [])
                for z in [z for (d, z) in due if d <= now]:
                    t = jnp.concatenate([t[0:8] | z, t[8:]], axis=0)
                state["due"] = [(d, z) for (d, z) in due if d > now]
                state["now"] = now + cost
                return t

            def owe(lag, p, tiles):
                z = tiles[0]
                for t in tiles[1:]:
                    z = z | t
                state.setdefault("due", []).append(
                    (state.get("now", 0) + lag + (p % 4) * TOK_STAG, zero_after(z)))

            def lv(k0, k1):
                ts = [lhs[cur, k] for k in range(k0, k1)]
                ts[0] = pay(ts[0], (k1 - k0) / NT)
                return jnp.concatenate([_as_bf16(t) for t in ts], axis=1)

            def wmat(mat, h, q0, q1):
                return _as_bf16(jnp.concatenate([wqkv[3 * q + mat, h] for q in range(q0, q1)],
                                                axis=0))

            def qkv(p, split=False):
                part = {}
                if split:
                    for mat in range(3):
                        for a in range(2):
                            part[mat, a] = _dot(lv(0, NT // 2), wmat(mat, 2 * p + a, 0, 2))
                for mat in range(3):
                    for a in range(2):
                        hm = mat * H + 2 * p + a
                        if split:
                            y = _dot(lv(NT // 2, NT), wmat(mat, 2 * p + a, 2, 4)) + part[mat, a]
                        else:
                            y = _dot(lv(0, NT), wmat(mat, 2 * p + a, 0, 4))
                        cur_s[hm] = y.astype(BF16)

            def gather(mat, p):
                hm = mat * H + 2 * p
                return jnp.concatenate(
                    [cur_s[hm], cur_s[hm + 1], pre[mat * NP + p, s].astype(BF16)], axis=0)

            probs = {}

            def scores(p):
                sc = lax.dot_general(gather(0, p), gather(1, p), (((1,), (1,)), ((), ())),
                                     preferred_element_type=F32)
                mv = mk[...]
                sc = jnp.where(mv == 0.0, sc * (SCALE * LOG2E), mv)
                e = jnp.exp2(sc - jnp.max(sc, axis=-1, keepdims=True))
                inv = _recip(jnp.sum(e, axis=-1, keepdims=True))
                if NORM_PRE:
                    e = e * inv
                    if TOK_S is not None:
                        eu = pltpu.bitcast(e, U32)
                        z = eu[0:8]
                        for k in range(1, PR // 8):
                            z = z | eu[k * 8:(k + 1) * 8]
                        owe(TOK_S, p, [jnp.concatenate([z, jnp.zeros((8, 128 - PR), U32)], axis=1)])
                    probs[p] = (e.astype(BF16), None)
                else:
                    if TOK_S is not None:
                        iu = pltpu.bitcast(jnp.broadcast_to(inv, (PR, 128)), U32)
                        owe(TOK_S, p, [iu[k * 8:(k + 1) * 8] for k in range(PR // 8)])
                    probs[p] = (e.astype(BF16), inv)

            def pv(p):
                e, inv = probs.pop(p)
                o = _dot(e, gather(2, p))
                if inv is not None:
                    o = o * inv
                o = o.astype(BF16)
                if TOK_P is not None:
                    ou = _as_u32(o)
                    owe(TOK_P, p, [ou[k * 8:(k + 1) * 8] for k in range(PR // 16)])
                for a in range(2):
                    h = 2 * p + a
                    olhs[h] = _as_u32(o[a * SEG:(a + 1) * SEG])
                    odef[h, it, cur * 4:(cur + 1) * 4, :] = _as_u32(
                        o[2 * SEG + a * M:2 * SEG + (a + 1) * M])

            acc = [None] * NT

            def oproj(j, pairs):
                ts = [olhs[2 * p + a] for p in pairs for a in range(2)]
                ts[0] = pay(ts[0], len(pairs) / 4)
                ov = jnp.concatenate([_as_bf16(t) for t in ts], axis=1)
                w = wo_s[j, pairs[0] * DH:(pairs[-1] + 1) * DH, :]
                y = _dot(ov, _as_bf16(w))
                acc[j] = y if acc[j] is None else y + acc[j]

            def fin(j):
                yb = acc[j].astype(BF16)
                ybuf[s, 0:XR, j * 128:(j + 1) * 128] = yb[0:XR]
                lhs[nxt, j, XR // 2:, :] = _as_u32(yb[XR:])

            def late_mod(u):
                mod_tile(wm_s[it & 3, u], 2 * NT + it * mt + u)

            load_x_rows(nxt, jnp.minimum(s + 1, NSEG - 1))
            ops = dict(Q=qkv, S=scores, P=pv, O=oproj, F=fin, M=late_mod)
            for op in _schedule([(u, q) for u, (c_, q) in enumerate(MODS[:mt]) if c_ % UNROLL == cur]):
                ops[op[0]](*op[1:])

        def steps(it, carry):
            if "pro" in PHASES:
                pltpu.make_async_copy(wm_s.at[it & 3], wm_s.at[it & 3], sem_m.at[it & 3]).wait()

                @pl.when(it + 2 < NSEG // UNROLL)
                def _():
                    for u in range(mt):
                        wm_copy(it + 2, u).start()

            for u in range(UNROLL // 2):
                t = it * (UNROLL // 2) + u
                for k in range(3):
                    @pl.when(t < late[k][2])
                    def _():
                        col_copy(k, t).start()

            state = {}
            for u in range(UNROLL):
                step(it, u, state)
            return carry

        with jax.named_scope("m_steps"):
            if "step" in PHASES: lax.fori_loop(0, NSEG // UNROLL, steps, 0)
        for k in range(3):
            for j in range(late[k][2]):
                col_copy(k, j).wait()
        if "epi" not in PHASES:
            return

        ntail = EBLK[-1] // M
        ppi = (S // 8 - ntail) // NEC
        gpi = ppi // (XR // 8)
        gb_ = UNROLL * M

        def ep_body(i, c):
            @pl.when(i > 0)
            def _():
                out_copy((i - 1) * gpi, gpi, 0, XR).start()

            subs = []
            r0 = 0
            for nr in EBLK:
                kh = EKH * EC // nr if EC % nr == 0 else EKH
                for j in range(NT):
                    for h0_ in range(0, H, kh):
                        subs.append((r0, nr, j, h0_, kh))
                r0 += nr
            tot = sum(nr * kh for (_, nr, _, _, kh) in subs)
            span = E_SPAN * EC * EKH
            rel = [u * (tot - span) // ppi for u in range(ppi)]
            ready = {}
            due = []
            now = 0
            u = 0
            y = None
            for (r0, nr, j, h0_, kh) in subs:
                blk = pl.ds(i * (EC // gb_) + r0 // gb_, nr // gb_)
                ts = [odef[h, blk].reshape(nr // 2, DH) for h in range(h0_, h0_ + kh)]
                for z in [z for (d, z) in due if d <= now]:
                    ts[0] = jnp.concatenate([ts[0][0:8] | z, ts[0][8:]], axis=0)
                due = [(d, z) for (d, z) in due if d > now]
                w = wo_s[j, h0_ * DH // 2:(h0_ + kh) * DH // 2, :]
                yp = _dot(jnp.concatenate([_as_bf16(t) for t in ts], axis=1), _as_bf16(w))
                y = yp if h0_ == 0 else yp + y
                if h0_ + kh == H:
                    ybuf[pl.ds(i * (EC // M) + r0 // M, nr // M), XR:, j * 128:(j + 1) * 128] = (
                        y.reshape(nr // M, M, 128).astype(BF16))
                    if j == NT - 1:
                        ready[r0] = True
                start = now
                now += nr * kh
                while u < ppi and rel[u] < now:
                    d = (NEC - 1) * ppi + u - NSEG * (XR // 8) - (NEC - 1) * (EC // M)
                    if d >= 0 and sum(n for r, n in zip(_cumsum(EBLK), EBLK) if r in ready) <= d * M:
                        break
                    t = i * ppi + u
                    early = t < NSEG * (XR // 8)
                    seg = jnp.where(early, t // (XR // 8), t - NSEG * (XR // 8))
                    row = pl.multiple_of(jnp.where(early, (t % (XR // 8)) * 8, XR), 8)
                    res = post(seg, row, zero_after(y[0:8]))
                    due.append((start + span, zero_after(res)))
                    u += 1
            assert u == ppi
            return c

        with jax.named_scope("e_loop"):
            lax.fori_loop(0, NEC, ep_body, 0)
        done = (NEC - 1) * gpi
        tail = NSEG - ntail
        out_copy(done, NSEG - done, 0, XR).start()
        out_copy(0, tail, XR, M).start()
        for g in range(tail, NSEG):
            post(g, XR)
        out_copy(tail, NSEG - tail, XR, M).start()

        tk = top[...]
        k1 = jnp.max(tk[0:8], axis=0, keepdims=True)
        k2 = jnp.max(jnp.where(tk == k1, jnp.iinfo(jnp.int32).min, tk), axis=0, keepdims=True)
        i1 = (S - 1) - (k1[0, 0] & (S - 1))
        i2 = (S - 1) - (k2[0, 0] & (S - 1))
        g1, g2 = i1 >> 5, i2 >> 5
        b1 = pl.multiple_of(i1 & 24, 8)
        b2 = pl.multiple_of(i2 & 24, 8)

        def two_blocks(ref):
            return jnp.concatenate([ref[g1, pl.ds(b1, 8), :].astype(F32),
                                    ref[g2, pl.ds(b2, 8), :].astype(F32)], axis=0)

        h2b = two_blocks(hbuf).astype(BF16)
        row = lax.broadcasted_iota(jnp.int32, (16, 1), 0)
        grow = jnp.where(row < 8, g1 * SEG + b1 + row, g2 * SEG + b2 + row - 8)
        ks = jnp.where(grow == i1, k1, k2)
        rsel = pltpu.bitcast((ks ^ ((ks >> 31) & 0x7FFF0000)) & -65536, F32)
        acts = []
        for j in range(FF // 128):
            gt = _rb(_dot(h2b, wg_s[j]))
            gt = _rb(gt * _rb(jax.nn.sigmoid(gt)))
            ut = _rb(_dot(h2b, wu_s[j]))
            acts.append((gt * ut).astype(BF16))
        act = jnp.concatenate(acts, axis=1)
        y = _rb(jnp.concatenate([_dot(act, wd_s[j]) for j in range(NT)], axis=1))
        y = _rb(y * _rb(jax.nn.sigmoid(rsel)))
        sel = jnp.logical_or(grow == i1, grow == i2)
        upd = jnp.concatenate([modv(5)] * 2, axis=0) * y
        fixed = (two_blocks(outs) + jnp.where(sel, upd, 0.0)).astype(BF16)

        with jax.named_scope("e_outwait"):
            out_copy(0, NSEG, 0, SEG).wait()
        outs[g1, pl.ds(b1, 8), :] = fixed[0:8]
        outs[g2, pl.ds(b2, 8), :] = fixed[8:16]
        out_copy(g1, 1, b1, 8, 0).start()

        @pl.when((i1 >> 3) != (i2 >> 3))
        def _():
            out_copy(g2, 1, b2, 8, 1).start()
            out_copy(g2, 1, b2, 8, 1).wait()

        out_copy(g1, 1, b1, 8, 0).wait()

    pl.run_scoped(
        main,
        pltpu.VMEM((FF // 128, D, 128), BF16),
        pltpu.VMEM((FF // 128, D, 128), BF16),
        pltpu.VMEM((NT, FF, 128), BF16),
        pltpu.VMEM((NSEG, SEG, D), BF16),
        pltpu.VMEM((NSEG, SEG, D), BF16),
        pltpu.VMEM((NSEG, SEG, D), BF16),
        pltpu.SemaphoreType.DMA((3,)),
    )


@functools.partial(jax.jit, static_argnames=("A_seg_len",))
def pallas_adaLN_cond__memory_aug_recurrent_mem_tr__moe_arch_mod__prompt_kernel(
    A_x: jax.Array,
    A_mem0: jax.Array,
    A_Wq: jax.Array,
    A_Wk: jax.Array,
    A_Wv: jax.Array,
    A_Wo: jax.Array,
    A_seg_len,
    B_x: jax.Array,
    B_w_r: jax.Array,
    B_w_gate: jax.Array,
    B_w_up: jax.Array,
    B_w_down: jax.Array,
    c: jax.Array,
    w_mod: jax.Array,
):
    assert A_seg_len == SEG and A_x.shape == (1, S, D)
    del B_x
    hbm = pl.BlockSpec(memory_space=pl.ANY)
    out = pl.pallas_call(
        _kernel,
        out_shape=jax.ShapeDtypeStruct((NSEG, SEG, D), BF16),
        in_specs=[hbm] * 12,
        out_specs=hbm,
        scratch_shapes=[
            pltpu.VMEM((NCHUNK, H, KQ // 2, DH), U32),
            pltpu.VMEM((NSEG + 1, NT, XR // 2, 128), U32),
            pltpu.VMEM((NT, (H * DH + H * DH // NT) // 2, 128), U32),
            pltpu.VMEM((3 * NP, NSEG, 2 * M, DH), F32),
            pltpu.VMEM((3 * H, SEG, DH), BF16),
            pltpu.VMEM((H, SEG // 2, DH), U32),
            pltpu.VMEM((H, NSEG // UNROLL, UNROLL * M // 2, DH), U32),
            pltpu.VMEM((NSEG, SEG, D), BF16),
            pltpu.VMEM((UNROLL, NT, SEG // 2, 128), U32),
            pltpu.VMEM((4, 4 * NT * UNROLL // NSEG, D, 128), BF16),
            pltpu.VMEM((7 * NT, M, 128), F32),
            pltpu.VMEM((PR, PR), F32),
            pltpu.VMEM((16, 1), jnp.int32),
            pltpu.VMEM((M, D), BF16),
            pltpu.VMEM((8 + PADS[2], 128), U32),
            pltpu.SemaphoreType.DMA((4,)),
            pltpu.SemaphoreType.DMA((2,)),
        ],
        compiler_params=pltpu.CompilerParams(vmem_limit_bytes=120 * 1024 * 1024,
                                             disable_bounds_checks=True),
    )(A_x.reshape(NSEG, SEG, D), A_mem0.reshape(M, D), A_Wq, A_Wk, A_Wv, A_Wo.reshape(H * DH, D),
      B_w_r, B_w_gate, B_w_up, B_w_down, c, w_mod)
    return out.reshape(1, S, D)
```

```python
import functools

import jax
import jax.numpy as jnp
from jax import lax
import jax.experimental.pallas as pl
import jax.experimental.pallas.tpu as pltpu

F32 = jnp.float32
BF16 = jnp.bfloat16
U32 = jnp.uint32

D = 1024
S = 2048
H = 32
DH = 128
M = 8
SEG = 32
NSEG = S // SEG
FF = 3584
NT = D // 128
XR = SEG - M
R0 = M * NSEG
CH = 8
KQ = D // 4
NCHUNK = 3 * D // KQ
NSLOT = 4
PR = 2 * SEG + 2 * M
NP = H // 2
EC = 128
NEC = R0 // EC
LOG2E = 1.4426950408889634
EPS = 1e-5
SCALE = DH ** -0.5
NEG_MASK = -1000000000.0

PHASES = ("pro", "step", "epi")
UNROLL = 4
FB = 32
BLK = 32
R_AT = ((0, 6, 16), (14, 22, 30), (30, 38, 46), (44, 52, 60))
F_AT = (0, 13)
L_AT = 8
VPU_MOD = True
G_AT = (0, 1, 2, 3)
GR = 32
GV_AT = (16, 56)
GVR = 32
GV_FREE = 64
G_LAG = 2
OPAQUE = True
LATE_APPLY = False
LEAN = False
RB = 16
RB2 = 64
JOB_SPAN = 40
LNU = 16
EKH = 4
E_SPAN = 6
ZIN = "all"
PIN_OUT = False
EBLK = (128,)
PADS = (0, 0, 0)
MODS = ((-1, 4), (1, 4))
TOK_S = 9
TOK_P = None
TOK_STAG = 2
NORM_PRE = True
R1_END = 11
R2_0 = (3, 14)
LN_RANGE = (0, 29)
WO_RANGE = (12, 31)


def _schedule(mods):
    groups = [list(range(4 * g, 4 * g + 4)) for g in range(4)]
    ops = []

    def mod_at(pos):
        ops.extend(("M", u) for (u, q) in mods if q == pos)

    for t in range(4):
        for i, p in enumerate(groups[t]):
            ops.append(("Q", p, p == 0))
            if p in G_AT:
                ops.append(("G",))
            if i == 0 and t >= 1:
                ops.extend(("S", q) for q in groups[t - 1])
                mod_at(10 + t)
            if i == 3 and t >= 1:
                ops.extend(("P", q) for q in groups[t - 1])
                mod_at(t)
    first = groups[0] + groups[1]
    for j in range(NT):
        ops.append(("O", j, first))
        if j == 1:
            ops.extend(("S", q) for q in groups[3])
            mod_at(14)
    ops.extend(("P", q) for q in groups[3])
    mod_at(4)
    ops.extend(("O", j, groups[2]) for j in range(NT))
    for j in range(NT):
        ops.append(("O", j, groups[3]))
        ops.append(("F", j))
    mod_at(5)
    return ops


def _rb(x):
    return x.astype(BF16).astype(F32)


def _recip(x):
    r = pl.reciprocal(x, approx=True)
    return r * (2.0 - x * r)


def _ln(x, zero=None, lean=False):
    xm = x if zero is None else jnp.concatenate([x[..., :128] + zero, x[..., 128:]], axis=-1)
    mu = jnp.mean(xm, axis=-1, keepdims=True)
    xc = x - mu
    v = _rb(_rb(jnp.mean(xc * xc, axis=-1, keepdims=True)) + EPS)
    inv = _recip(_rb(v * lax.rsqrt(v)))
    if lean:
        return x * inv - mu * inv
    return xc * inv


def _ln_mod(x, s1p, shift, zero=None, lean=False):
    return _ln(x, zero, lean) * s1p + shift


def _dot(a, b):
    return jnp.dot(a, b, preferred_element_type=F32)


def _as_bf16(u):
    return pltpu.bitcast(u, BF16)


def _as_u32(b):
    return pltpu.bitcast(b, U32)


def _cumsum(xs):
    out, r = [], 0
    for x in xs:
        out.append(r)
        r += x
    return out


def _spread(jobs, fns, lo, hi):
    for n, fn in enumerate(fns):
        jobs.setdefault(lo + n * (hi - lo) // len(fns), []).append(fn)


def _kernel(x_hbm, mem0_hbm, wq_hbm, wk_hbm, wv_hbm, wo_hbm, wr_hbm, wg_hbm, wu_hbm, wd_hbm,
            c_hbm, wmod_hbm, out_hbm,
            wqkv, hs, wo_s, pre, cur_s, olhs, odef, xbuf, lhs, wm_s, mod, mk,
            top, sc_s, cb_s, zero_s, sem_m, sem_out):
    mt = 4 * NT * UNROLL // NSEG

    def modv(j):
        return jnp.concatenate([mod[j * NT + k] for k in range(NT)], axis=1)

    def mod_store(v, t):
        v = _rb(v)
        mod[t] = jnp.where(jnp.logical_or((t >> 3) == 1, (t >> 3) == 4), _rb(1.0 + v), v)

    def mod_tile(wm, t):
        mod_store(_dot(sc_s[...], wm), t)

    def gemv_part(w, d0, acc):
        n = w.shape[1]
        p = w.astype(F32) * cb_s[d0:d0 + n, :]
        p = jnp.sum(p.reshape(w.shape[0], n // 8, 8, 128), axis=1)
        return p if acc is None else p + acc

    def gemv_finish(acc, ts):
        for u, t in enumerate(ts):
            mod_store(jnp.broadcast_to(jnp.sum(acc[u], axis=0, keepdims=True), (M, 128)), t)

    def wm_copy(it, u):
        col = pl.multiple_of((2 * NT + it * mt + u) * 128, 128)
        return pltpu.make_async_copy(wmod_hbm.at[:, pl.ds(col, 128)], wm_s.at[it & 3, u],
                                     sem_m.at[it & 3])

    def ln1(x, zero=None):
        x3 = x.astype(F32).reshape(x.shape[0] // 8, 8, D)
        zf = None if zero is None else pltpu.bitcast(zero, F32)
        if LATE_APPLY:
            return _ln(x3, zf, LEAN).reshape(x.shape[0], D).astype(BF16)
        return _ln_mod(x3, modv(1), modv(0), zf, LEAN).reshape(x.shape[0], D).astype(BF16)

    def zero_after(y):
        return (y if y.dtype == U32 else pltpu.bitcast(y, U32)) & zero_s[0:8, :]

    def or_tile(u, z):
        if z is None:
            return u
        return (u.reshape(u.shape[0] // 8, 8, 128) | z).reshape(u.shape)

    def prologue(stage, wo_raw, wmod_s, nrm, ha, hb, tmp, mem0_ref, wr_ref, c_ref, sem):
        w_hbms = (wq_hbm, wk_hbm, wv_hbm)
        wob = H * DH // NT
        S_X, S_C0, S_ST, S_WO, S_MOD, S_SM = 0, 2, 6, 6 + NSLOT, 6 + NSLOT + NT, 6 + NSLOT + 2 * NT

        def x_copy(i):
            lo, n = ((XR, M), (0, XR))[i]
            return pltpu.make_async_copy(x_hbm.at[:, pl.ds(lo, n), :], xbuf.at[:, pl.ds(lo, n), :],
                                         sem.at[S_X + i])

        def mod_copies(k):
            return [pltpu.make_async_copy(wmod_hbm.at[:, pl.ds(v * D + k * 128, 128)],
                                          wmod_s.at[k, v], sem.at[S_MOD + (k if k < 2 else k & 6)])
                    for v in range(2)]

        def chunk_copy(mat, d0, g, slot, k):
            return pltpu.make_async_copy(w_hbms[mat].at[pl.ds(d0, KQ), pl.ds(g * CH, CH), :],
                                         stage.at[slot, g], sem.at[k])

        def wo_copy(j):
            return pltpu.make_async_copy(wo_hbm.at[pl.ds(pl.multiple_of(j * wob, wob), wob)],
                                         wo_raw.at[j], sem.at[S_WO + j])

        def relayout1(src, t0, z=None):
            v = src.reshape(RB * CH, 128)
            tmp[t0:t0 + RB * CH // 2, :] = or_tile(_as_u32(v), z)

        def relayout2(c, h0_, t0, d0, z=None):
            w = or_tile(tmp[pl.ds(t0, RB2, stride=CH // 2), :], z)
            rows = pl.ds(d0 // 2, RB2 // 2)
            wqkv[c, h0_, rows, :] = _as_u32(w.astype(jnp.uint16))
            wqkv[c, h0_ + 1, rows, :] = _as_u32((w >> 16).astype(jnp.uint16))

        def mod_pair(k):
            for v in range(2):
                mod_tile(wmod_s[k, v], v * NT + k)

        def fill(dst, q, t, r, z=None):
            k = 2 * q + t
            sh = mod[k] if z is None else mod[k] + pltpu.bitcast(z, F32)
            v = nrm[k, r:r + FB, :].reshape(FB // 8, 8, 128) * mod[NT + k] + sh
            dst[t, r // 2:(r + FB) // 2, :] = _as_u32(v.reshape(FB, 128).astype(BF16))

        small = [pltpu.make_async_copy(src, dst, sem.at[S_SM])
                 for src, dst in ((c_hbm, c_ref), (mem0_hbm, mem0_ref), (wr_hbm, wr_ref))]
        for cp in small:
            cp.start()
        x_copy(0).start()
        for cp in mod_copies(0) + mod_copies(1):
            cp.start()
        for g in range(4):
            chunk_copy(0, 0, g, 0, S_C0 + g).start()
        for c in range(1, NSLOT):
            for g in range(4):
                chunk_copy(c % 3, (c // 3) * KQ, g, c, S_ST + c).start()
            for cp in mod_copies(2 * c) + mod_copies(2 * c + 1):
                cp.start()

        def decode(i):
            lo = i < 2 * SEG
            head = jnp.where(lo, i // SEG, (i - 2 * SEG) // M)
            is_mem = jnp.logical_and(lo, i % SEG >= XR)
            pos = jnp.where(lo, i % SEG, XR + i % M)
            return head, is_mem, pos

        qh, qm, qp = decode(lax.broadcasted_iota(jnp.int32, (PR, PR), 0))
        kh, km, kp = decode(lax.broadcasted_iota(jnp.int32, (PR, PR), 1))
        vis = qm | km | (qp >= kp)
        mk[...] = jnp.where(qh == kh, jnp.where(vis, 0.0, NEG_MASK * LOG2E), -jnp.inf).astype(F32)
        mod[0:2 * NT] = jnp.zeros((2 * NT, M, 128), F32)
        zero_s[...] = jnp.zeros(zero_s.shape, U32)
        top[...] = jnp.full(top.shape, jnp.iinfo(jnp.int32).min, jnp.int32)
        for cp in small:
            cp.wait()
        wr = jnp.broadcast_to(wr_ref[...].astype(F32).reshape(1, D), (M, D))
        for k in range(NT):
            mod[6 * NT + k] = wr[:, k * 128:(k + 1) * 128]
        cv = c_ref[...].astype(F32)
        sc = _rb(cv * _rb(jax.nn.sigmoid(cv)))
        sc_s[...] = jnp.broadcast_to(sc, (M, D)).astype(BF16)
        for k in range(NT):
            cb_s[k * 128:(k + 1) * 128, :] = jnp.broadcast_to(
                sc[:, k * 128:(k + 1) * 128], (128, 128)).T
        mb = mem0_ref[...]
        for k in range(NT):
            lhs[0, k, XR // 2:, :] = _as_u32(mb[:, k * 128:(k + 1) * 128])

        def zero_body(i, c):
            wo_raw[NT, pl.ds(pl.multiple_of(i * 32, 32), 32), :] = jnp.zeros((32, D), BF16)
            return c

        lax.fori_loop(0, wob // 32, zero_body, 0)
        x_copy(0).wait()

        def ln_body(i, c):
            for u in range(LNU):
                q = i * LNU + u
                v = _ln(xbuf[q, XR:, :].astype(F32))
                for k in range(NT):
                    nrm[k, pl.ds(pl.multiple_of(q * 8, 8), 8), :] = v[:, k * 128:(k + 1) * 128]
            return c

        with jax.named_scope("p_ln"):
            lax.fori_loop(0, NSEG // LNU, ln_body, 0)

        def mod_body(k, c):
            pltpu.make_async_copy(wmod_s.at[k], wmod_s.at[k], sem.at[S_MOD + k]).wait()
            mod_pair(k)
            for r in range(0, R0, FB):
                fill(ha, 0, k, r)
            return c

        with jax.named_scope("p_mod"):
            lax.fori_loop(0, 2, mod_body, 0)

        def c0_body(g):
            chunk_copy(0, 0, 0, 0, S_C0 + g).wait()
            for d0 in range(0, KQ, RB):
                relayout1(stage[0, g, d0:d0 + RB], d0 * CH // 2)
            for j in range(CH // 2):
                for d0 in range(0, KQ, RB2):
                    relayout2(0, g * CH + 2 * j, d0 * CH // 2 + j, d0)

        def bulk(units, jobs, inserts):
            due = {}
            t0 = 0
            for n, (hq, c, h0_, pi, first, r0, nrow) in enumerate(units):
                nb = nrow // BLK
                parts = []
                for u in range(nb):
                    part = hq[0, (r0 + u * BLK) // 2:(r0 + (u + 1) * BLK) // 2, :]
                    for z in due.pop(t0 + u, ()):
                        part = jnp.concatenate([part[0:8] | z, part[8:]], axis=0)
                    parts.append(part)
                hv = jnp.concatenate([_as_bf16(jnp.concatenate(parts, axis=0)),
                                      _as_bf16(hq[1, r0 // 2:(r0 + nrow) // 2, :])], axis=1)
                w = jnp.concatenate([_as_bf16(wqkv[c, h0_]), _as_bf16(wqkv[c, h0_ + 1])], axis=1)
                y = _dot(hv, w)
                segs = slice(r0 // M, (r0 + nrow) // M)
                for a in range(2):
                    old = jnp.where(first, 0.0, pre[pi, segs, a * M:(a + 1) * M, :])
                    pre[pi, segs, a * M:(a + 1) * M, :] = (
                        y[:, a * DH:(a + 1) * DH].reshape(nrow // M, M, DH) + old)
                for fn in inserts.get(n, ()):
                    fn()
                for u in range(nb):
                    for job in jobs.get(t0 + u, ()):
                        res = job(zero_after(y[u * BLK:u * BLK + 8, 0:128]))
                        if res is not None:
                            due.setdefault(max(t0 + u + JOB_SPAN, t0 + nb), []).append(
                                zero_after(res))
                t0 += nb
            assert not due

        GP = CH // 2
        WO0 = NCHUNK - 1 - NT
        LN0 = 4
        SPI = -(-NSEG // (NCHUNK - 1 - LN0))

        def rot_body(i, c):
            slot = (i + 1) & (NSLOT - 1)
            pltpu.make_async_copy(stage.at[slot], stage.at[slot], sem.at[S_ST + slot]).wait()
            km = 2 * jnp.minimum(i, 3)

            @pl.when(jnp.logical_and(i >= 1, i <= 3))
            def _():
                wq = wmod_s.at[pl.ds(km, 2)]
                pltpu.make_async_copy(wq, wq, sem.at[S_MOD + km]).wait()

            @pl.when(i == LN0)
            def _():
                x_copy(1).wait()

            @pl.when(i >= WO0)
            def _():
                wo_copy(i - WO0).wait()

            nxt = i + NSLOT
            qn = (nxt * 43) >> 7
            for mat in range(3):
                @pl.when(jnp.logical_and(nxt < NCHUNK, nxt - 3 * qn == mat))
                def _():
                    for g in range(4):
                        chunk_copy(mat, qn * KQ, g, nxt & (NSLOT - 1),
                                   S_ST + (nxt & (NSLOT - 1))).start()

            @pl.when(i < NT)
            def _():
                wo_copy(i).start()

            @pl.when(i == 0)
            def _():
                x_copy(1).start()

            q0 = (i * 43) >> 7
            q1 = ((i + 1) * 43) >> 7
            pa = (i - 3 * q0) * NP + NP - GP
            units = ([(ha, i, H - CH + 2 * n, pa + n, q0 == 0, 0, R0) for n in range(GP)]
                     + [(hb, i + 1, 2 * n, (i + 1 - 3 * q1) * NP + n, q1 == 0, 0, R0)
                        for n in range(NP - GP)])
            jw = jnp.where(i >= WO0, i - WO0, NT)

            def wo_job(b, z):
                v = wo_raw[jw, b * 16:(b + 1) * 16, :]
                rows = pl.ds(pl.multiple_of(jw * (wob // 2) + b * 8, 8), 8)
                for j in range(NT):
                    wo_s[j, rows, :] = _as_u32(v[:, j * 128:(j + 1) * 128]) | z

            def ln_job(b, z):
                r = (b % 3) * 8
                seg = (i - LN0) * SPI + b // 3
                live = jnp.logical_and(i >= LN0, seg < NSEG)
                src = jnp.where(live, seg, 0)
                hv = ln1(xbuf[src, pl.ds(pl.multiple_of(jnp.where(live, r, XR), 8), 8), :], z)
                u = [_as_u32(hv[:, k * 128:(k + 1) * 128]) for k in range(NT)]
                dst = jnp.where(live, seg, NSEG)
                for k in range(NT):
                    hs[dst, k, r // 2:r // 2 + 4, :] = u[k]
                res = jnp.concatenate(u[0:2], axis=0)
                for k in range(2, NT, 2):
                    res = res | jnp.concatenate(u[k:k + 2], axis=0)
                return res

            def r1_job(g, d0, z):
                relayout1(stage[slot, g, d0:d0 + RB], (g * KQ + d0) * CH // 2, z)

            def copy_job(t, r, z):
                ha[t, r:r + 32, :] = or_tile(hb[t, r:r + 32, :], z)

            P = functools.partial
            upb = R0 // BLK
            nr = NP * upb
            jobs = {}
            for g in range(4):
                lo, mid, hi = (x * upb // 4 for x in R_AT[g])
                _spread(jobs, [P(r1_job, g, d0) for d0 in range(0, KQ, RB)], lo, mid)
                _spread(jobs, [P(relayout2, i + 1, g * CH + 2 * j, (g * KQ + d0) * CH // 2 + j, d0)
                               for j in range(CH // 2) for d0 in range(0, KQ, RB2)], mid, hi)
            oz = (i >> 10) if OPAQUE else 0
            _spread(jobs, [P(fill, hb, q1, t + oz, r) for r in range(0, R0, FB) for t in range(2)],
                    F_AT[0] * upb // 4, F_AT[1] * upb // 4)
            _spread(jobs, [P(copy_job, t, r) for t in range(2) for r in range(0, R0 // 2, 32)],
                    2 * GP * upb, nr - upb)
            _spread(jobs, [P(ln_job, b) for b in range(3 * SPI)],
                    L_AT * upb // 4, nr - max(upb, JOB_SPAN))
            _spread(jobs, [P(wo_job, b) for b in range(wob // 16)], GP * upb, nr - upb)
            gv = {}

            def gv_job(d0, n, z):
                w = wmod_s[pl.ds(km, 2), :, d0:d0 + n, :].reshape(4, n, 128)
                acc = gv.get("acc")
                if z is not None:
                    zf = pltpu.bitcast(z, F32)[None]
                    acc = jnp.broadcast_to(zf, (4, 8, 128)) if acc is None else acc + zf
                gv["acc"] = gemv_part(w, d0, acc)
                if z is not None:
                    au = pltpu.bitcast(gv["acc"], U32)
                    return au[0] | au[1] | au[2] | au[3]

            _spread(jobs, [P(gv_job, d0, GVR) for d0 in range(0, D - GV_FREE, GVR)],
                    GV_AT[0] * upb // 4, min(GV_AT[1] * upb // 4, nr - JOB_SPAN))
            bulk(units, jobs, {})
            if GV_FREE:
                gv_job(D - GV_FREE, GV_FREE, None)
            gemv_finish(gv["acc"], [km, NT + km, km + 1, NT + km + 1])
            return c

        def outer(k, c):
            last = k == 4

            @pl.when(k < 4)
            def _():
                c0_body(k)

            @pl.when(k != 3)
            def _():
                g = jnp.minimum(k, 3)
                bulk([(ha, jnp.where(last, NCHUNK - 1, 0), g * CH + 2 * n,
                       jnp.where(last, 2 * NP, 0) + g * GP + n, k < 4, 0, R0)
                      for n in range(GP)], {}, {})

            @pl.when(k == 3)
            def _():
                with jax.named_scope("p_rot"):
                    lax.fori_loop(0, NCHUNK - 1, rot_body, 0)
                for it in range(2):
                    for u in range(mt):
                        wm_copy(it, u).start()

            return c

        with jax.named_scope("p_bulk"):
            lax.fori_loop(0, 5, outer, 0)

    if "pro" in PHASES: pl.run_scoped(
        prologue,
        pltpu.VMEM((NSLOT, H // CH, KQ, CH, 128), BF16),
        pltpu.VMEM((NT + 1, H * DH // NT, D), BF16),
        pltpu.VMEM((NT, 2, D, 128), BF16),
        pltpu.VMEM((NT, R0, 128), F32),
        pltpu.VMEM((2, R0 // 2 + PADS[0], 128), U32),
        pltpu.VMEM((2, R0 // 2 + PADS[0], 128), U32),
        pltpu.VMEM((D * CH // 2 + PADS[1], 128), U32),
        pltpu.VMEM((M, D), BF16),
        pltpu.VMEM((D,), BF16),
        pltpu.VMEM((1, D), BF16),
        pltpu.SemaphoreType.DMA((7 + NSLOT + 2 * NT,)),
    )

    def main(wg_s, wu_s, wd_s, ybuf, hbuf, outs, sem_f):
        def load_x_rows(slot, seg):
            for k in range(NT):
                if LATE_APPLY:
                    v = _as_bf16(hs[seg, k]).astype(F32).reshape(XR // 8, 8, 128)
                    v = (v * mod[NT + k] + mod[k]).reshape(XR, 128)
                    lhs[slot, k, 0:XR // 2, :] = _as_u32(v.astype(BF16))
                else:
                    lhs[slot, k, 0:XR // 2, :] = hs[seg, k]

        def post(seg, r, z=None):
            if z is not None and ZIN == "scalar":
                seg = seg + pltpu.bitcast(z, jnp.int32)[0, 0]
            rows = pl.ds(r, 8)
            t = modv(2) * ybuf[seg, rows, :].astype(F32)
            if z is not None and ZIN == "all":
                t = t + jnp.concatenate([pltpu.bitcast(z, F32)] * NT, axis=1)
            x1 = xbuf[seg, rows, :].astype(F32) + t
            h2 = _ln_mod(x1, modv(4), modv(3),
                         pltpu.bitcast(z, F32) if z is not None and ZIN == "mean" else None)
            hbuf[seg, rows, :] = h2.astype(BF16)
            o = x1 + modv(5) * h2
            outs[seg, rows, :] = o.astype(BF16)
            v = _rb(jnp.sum(h2 * modv(6), axis=-1, keepdims=True))
            b = pltpu.bitcast(jnp.where(v != v, -jnp.inf, v + 0.0), jnp.int32)
            low = (S - 1 - seg * SEG - r) - lax.broadcasted_iota(jnp.int32, (8, 1), 0)
            key = (b ^ ((b >> 31) & 0x7FFF0000)) | low
            m1, m2 = top[0:8, :], top[8:16, :]
            top[8:16, :] = jnp.maximum(m2, jnp.minimum(m1, key))
            top[0:8, :] = jnp.maximum(m1, key)
            if z is not None:
                res = pltpu.bitcast(jnp.broadcast_to(v, (8, 128)), U32)
                if PIN_OUT:
                    for k in range(NT):
                        res = res | pltpu.bitcast(o[:, k * 128:(k + 1) * 128], U32)
                return res

        def out_copy(g0, ng, r, n, k=0):
            return pltpu.make_async_copy(outs.at[pl.ds(g0, ng), pl.ds(r, n), :],
                                         out_hbm.at[pl.ds(g0, ng), pl.ds(r, n), :], sem_out.at[k])

        late = ((wg_hbm, wg_s, FF // 128), (wu_hbm, wu_s, FF // 128), (wd_hbm, wd_s, NT))

        def col_copy(k, j):
            return pltpu.make_async_copy(
                late[k][0].at[:, pl.ds(pl.multiple_of(j * 128, 128), 128)], late[k][1].at[j],
                sem_f.at[k])

        load_x_rows(0, 0)

        def step(it, cur, state):
            s = it * UNROLL + cur
            nxt = (cur + 1) % UNROLL

            def pay(t, cost):
                now = state.get("now", 0)
                due = state.setdefault("due", [])
                for z in [z for (d, z) in due if d <= now]:
                    t = jnp.concatenate([t[0:8] | z, t[8:]], axis=0)
                state["due"] = [(d, z) for (d, z) in due if d > now]
                state["now"] = now + cost
                return t

            def owe(lag, p, tiles):
                z = tiles[0]
                for t in tiles[1:]:
                    z = z | t
                state.setdefault("due", []).append(
                    (state.get("now", 0) + lag + (p % 4) * TOK_STAG, zero_after(z)))

            def lv(k0, k1):
                ts = [lhs[cur, k] for k in range(k0, k1)]
                ts[0] = pay(ts[0], (k1 - k0) / NT)
                return jnp.concatenate([_as_bf16(t) for t in ts], axis=1)

            def wmat(mat, h, q0, q1):
                return _as_bf16(jnp.concatenate([wqkv[3 * q + mat, h] for q in range(q0, q1)],
                                                axis=0))

            def qkv(p, split=False):
                part = {}
                if split:
                    for mat in range(3):
                        for a in range(2):
                            part[mat, a] = _dot(lv(0, NT // 2), wmat(mat, 2 * p + a, 0, 2))
                for mat in range(3):
                    for a in range(2):
                        hm = mat * H + 2 * p + a
                        if split:
                            y = _dot(lv(NT // 2, NT), wmat(mat, 2 * p + a, 2, 4)) + part[mat, a]
                        else:
                            y = _dot(lv(0, NT), wmat(mat, 2 * p + a, 0, 4))
                        cur_s[hm] = y.astype(BF16)

            def gather(mat, p):
                hm = mat * H + 2 * p
                return jnp.concatenate(
                    [cur_s[hm], cur_s[hm + 1], pre[mat * NP + p, s].astype(BF16)], axis=0)

            probs = {}

            def scores(p):
                sc = lax.dot_general(gather(0, p), gather(1, p), (((1,), (1,)), ((), ())),
                                     preferred_element_type=F32)
                mv = mk[...]
                sc = jnp.where(mv == 0.0, sc * (SCALE * LOG2E), mv)
                e = jnp.exp2(sc - jnp.max(sc, axis=-1, keepdims=True))
                inv = _recip(jnp.sum(e, axis=-1, keepdims=True))
                if NORM_PRE:
                    e = e * inv
                    if TOK_S is not None:
                        eu = pltpu.bitcast(e, U32)
                        z = eu[0:8]
                        for k in range(1, PR // 8):
                            z = z | eu[k * 8:(k + 1) * 8]
                        owe(TOK_S, p, [jnp.concatenate([z, jnp.zeros((8, 128 - PR), U32)], axis=1)])
                    probs[p] = (e.astype(BF16), None)
                else:
                    if TOK_S is not None:
                        iu = pltpu.bitcast(jnp.broadcast_to(inv, (PR, 128)), U32)
                        owe(TOK_S, p, [iu[k * 8:(k + 1) * 8] for k in range(PR // 8)])
                    probs[p] = (e.astype(BF16), inv)

            def pv(p):
                e, inv = probs.pop(p)
                o = _dot(e, gather(2, p))
                if inv is not None:
                    o = o * inv
                o = o.astype(BF16)
                if TOK_P is not None:
                    ou = _as_u32(o)
                    owe(TOK_P, p, [ou[k * 8:(k + 1) * 8] for k in range(PR // 16)])
                for a in range(2):
                    h = 2 * p + a
                    olhs[h] = _as_u32(o[a * SEG:(a + 1) * SEG])
                    odef[h, it, cur * 4:(cur + 1) * 4, :] = _as_u32(
                        o[2 * SEG + a * M:2 * SEG + (a + 1) * M])

            acc = [None] * NT

            def oproj(j, pairs):
                ts = [olhs[2 * p + a] for p in pairs for a in range(2)]
                ts[0] = pay(ts[0], len(pairs) / 4)
                ov = jnp.concatenate([_as_bf16(t) for t in ts], axis=1)
                w = wo_s[j, pairs[0] * DH:(pairs[-1] + 1) * DH, :]
                y = _dot(ov, _as_bf16(w))
                acc[j] = y if acc[j] is None else y + acc[j]

            def fin(j):
                yb = acc[j].astype(BF16)
                ybuf[s, 0:XR, j * 128:(j + 1) * 128] = yb[0:XR]
                lhs[nxt, j, XR // 2:, :] = _as_u32(yb[XR:])

            def gemv():
                d0 = state.get("d0", 0)
                state["acc"] = gemv_part(wm_s[it & 3, :, d0:d0 + GR, :], d0, state.get("acc"))
                state["d0"] = d0 + GR
                au = pltpu.bitcast(state["acc"], U32)
                owe(G_LAG, 0, [au[u] for u in range(mt)])

            def late_mod(u):
                mod_tile(wm_s[it & 3, u], 2 * NT + it * mt + u)

            load_x_rows(nxt, jnp.minimum(s + 1, NSEG - 1))
            ops = dict(Q=qkv, S=scores, P=pv, O=oproj, F=fin, M=late_mod, G=gemv)
            for op in _schedule([(u, q) for u, (c_, q) in enumerate(MODS[:mt])
                                 if c_ % UNROLL == cur and not VPU_MOD]):
                ops[op[0]](*op[1:])

        def steps(it, carry):
            if "pro" in PHASES:
                pltpu.make_async_copy(wm_s.at[it & 3], wm_s.at[it & 3], sem_m.at[it & 3]).wait()

                @pl.when(it + 2 < NSEG // UNROLL)
                def _():
                    for u in range(mt):
                        wm_copy(it + 2, u).start()

            for u in range(UNROLL // 2):
                t = it * (UNROLL // 2) + u
                for k in range(3):
                    @pl.when(t < late[k][2])
                    def _():
                        col_copy(k, t).start()

            state = {}
            for u in range(UNROLL):
                step(it, u, state)
            if VPU_MOD:
                acc = state.get("acc")
                for d0 in range(state.get("d0", 0), D, 64):
                    acc = gemv_part(wm_s[it & 3, :, d0:d0 + 64, :], d0, acc)
                gemv_finish(acc, [2 * NT + it * mt + u for u in range(mt)])
            return carry

        with jax.named_scope("m_steps"):
            if "step" in PHASES: lax.fori_loop(0, NSEG // UNROLL, steps, 0)
        for k in range(3):
            for j in range(late[k][2]):
                col_copy(k, j).wait()
        if "epi" not in PHASES:
            return

        ntail = EBLK[-1] // M
        ppi = (S // 8 - ntail) // NEC
        gpi = ppi // (XR // 8)
        gb_ = UNROLL * M

        def ep_body(i, c):
            @pl.when(i > 0)
            def _():
                out_copy((i - 1) * gpi, gpi, 0, XR).start()

            subs = []
            r0 = 0
            for nr in EBLK:
                kh = EKH * EC // nr if EC % nr == 0 else EKH
                for j in range(NT):
                    for h0_ in range(0, H, kh):
                        subs.append((r0, nr, j, h0_, kh))
                r0 += nr
            tot = sum(nr * kh for (_, nr, _, _, kh) in subs)
            span = E_SPAN * EC * EKH
            rel = [u * (tot - span) // ppi for u in range(ppi)]
            ready = {}
            due = []
            now = 0
            u = 0
            y = None
            for (r0, nr, j, h0_, kh) in subs:
                blk = pl.ds(i * (EC // gb_) + r0 // gb_, nr // gb_)
                ts = [odef[h, blk].reshape(nr // 2, DH) for h in range(h0_, h0_ + kh)]
                for z in [z for (d, z) in due if d <= now]:
                    ts[0] = jnp.concatenate([ts[0][0:8] | z, ts[0][8:]], axis=0)
                due = [(d, z) for (d, z) in due if d > now]
                w = wo_s[j, h0_ * DH // 2:(h0_ + kh) * DH // 2, :]
                yp = _dot(jnp.concatenate([_as_bf16(t) for t in ts], axis=1), _as_bf16(w))
                y = yp if h0_ == 0 else yp + y
                if h0_ + kh == H:
                    ybuf[pl.ds(i * (EC // M) + r0 // M, nr // M), XR:, j * 128:(j + 1) * 128] = (
                        y.reshape(nr // M, M, 128).astype(BF16))
                    if j == NT - 1:
                        ready[r0] = True
                start = now
                now += nr * kh
                while u < ppi and rel[u] < now:
                    d = (NEC - 1) * ppi + u - NSEG * (XR // 8) - (NEC - 1) * (EC // M)
                    if d >= 0 and sum(n for r, n in zip(_cumsum(EBLK), EBLK) if r in ready) <= d * M:
                        break
                    t = i * ppi + u
                    early = t < NSEG * (XR // 8)
                    seg = jnp.where(early, t // (XR // 8), t - NSEG * (XR // 8))
                    row = pl.multiple_of(jnp.where(early, (t % (XR // 8)) * 8, XR), 8)
                    res = post(seg, row, zero_after(y[0:8]))
                    due.append((start + span, zero_after(res)))
                    u += 1
            assert u == ppi
            return c

        with jax.named_scope("e_loop"):
            lax.fori_loop(0, NEC, ep_body, 0)
        done = (NEC - 1) * gpi
        tail = NSEG - ntail
        out_copy(done, NSEG - done, 0, XR).start()
        out_copy(0, tail, XR, M).start()
        for g in range(tail, NSEG):
            post(g, XR)
        out_copy(tail, NSEG - tail, XR, M).start()

        tk = top[...]
        k1 = jnp.max(tk[0:8], axis=0, keepdims=True)
        k2 = jnp.max(jnp.where(tk == k1, jnp.iinfo(jnp.int32).min, tk), axis=0, keepdims=True)
        i1 = (S - 1) - (k1[0, 0] & (S - 1))
        i2 = (S - 1) - (k2[0, 0] & (S - 1))
        g1, g2 = i1 >> 5, i2 >> 5
        b1 = pl.multiple_of(i1 & 24, 8)
        b2 = pl.multiple_of(i2 & 24, 8)

        def two_blocks(ref):
            return jnp.concatenate([ref[g1, pl.ds(b1, 8), :].astype(F32),
                                    ref[g2, pl.ds(b2, 8), :].astype(F32)], axis=0)

        h2b = two_blocks(hbuf).astype(BF16)
        row = lax.broadcasted_iota(jnp.int32, (16, 1), 0)
        grow = jnp.where(row < 8, g1 * SEG + b1 + row, g2 * SEG + b2 + row - 8)
        ks = jnp.where(grow == i1, k1, k2)
        rsel = pltpu.bitcast((ks ^ ((ks >> 31) & 0x7FFF0000)) & -65536, F32)
        acts = []
        for j in range(FF // 128):
            gt = _rb(_dot(h2b, wg_s[j]))
            gt = _rb(gt * _rb(jax.nn.sigmoid(gt)))
            ut = _rb(_dot(h2b, wu_s[j]))
            acts.append((gt * ut).astype(BF16))
        act = jnp.concatenate(acts, axis=1)
        y = _rb(jnp.concatenate([_dot(act, wd_s[j]) for j in range(NT)], axis=1))
        y = _rb(y * _rb(jax.nn.sigmoid(rsel)))
        sel = jnp.logical_or(grow == i1, grow == i2)
        upd = jnp.concatenate([modv(5)] * 2, axis=0) * y
        fixed = (two_blocks(outs) + jnp.where(sel, upd, 0.0)).astype(BF16)

        with jax.named_scope("e_outwait"):
            out_copy(0, NSEG, 0, SEG).wait()
        outs[g1, pl.ds(b1, 8), :] = fixed[0:8]
        outs[g2, pl.ds(b2, 8), :] = fixed[8:16]
        out_copy(g1, 1, b1, 8, 0).start()

        @pl.when((i1 >> 3) != (i2 >> 3))
        def _():
            out_copy(g2, 1, b2, 8, 1).start()
            out_copy(g2, 1, b2, 8, 1).wait()

        out_copy(g1, 1, b1, 8, 0).wait()

    pl.run_scoped(
        main,
        pltpu.VMEM((FF // 128, D, 128), BF16),
        pltpu.VMEM((FF // 128, D, 128), BF16),
        pltpu.VMEM((NT, FF, 128), BF16),
        pltpu.VMEM((NSEG, SEG, D), BF16),
        pltpu.VMEM((NSEG, SEG, D), BF16),
        pltpu.VMEM((NSEG, SEG, D), BF16),
        pltpu.SemaphoreType.DMA((3,)),
    )


@functools.partial(jax.jit, static_argnames=("A_seg_len",))
def pallas_adaLN_cond__memory_aug_recurrent_mem_tr__moe_arch_mod__prompt_kernel(
    A_x: jax.Array,
    A_mem0: jax.Array,
    A_Wq: jax.Array,
    A_Wk: jax.Array,
    A_Wv: jax.Array,
    A_Wo: jax.Array,
    A_seg_len,
    B_x: jax.Array,
    B_w_r: jax.Array,
    B_w_gate: jax.Array,
    B_w_up: jax.Array,
    B_w_down: jax.Array,
    c: jax.Array,
    w_mod: jax.Array,
):
    assert A_seg_len == SEG and A_x.shape == (1, S, D)
    del B_x
    hbm = pl.BlockSpec(memory_space=pl.ANY)
    out = pl.pallas_call(
        _kernel,
        out_shape=jax.ShapeDtypeStruct((NSEG, SEG, D), BF16),
        in_specs=[hbm] * 12,
        out_specs=hbm,
        scratch_shapes=[
            pltpu.VMEM((NCHUNK, H, KQ // 2, DH), U32),
            pltpu.VMEM((NSEG + 1, NT, XR // 2, 128), U32),
            pltpu.VMEM((NT, (H * DH + H * DH // NT) // 2, 128), U32),
            pltpu.VMEM((3 * NP, NSEG, 2 * M, DH), F32),
            pltpu.VMEM((3 * H, SEG, DH), BF16),
            pltpu.VMEM((H, SEG // 2, DH), U32),
            pltpu.VMEM((H, NSEG // UNROLL, UNROLL * M // 2, DH), U32),
            pltpu.VMEM((NSEG, SEG, D), BF16),
            pltpu.VMEM((UNROLL, NT, SEG // 2, 128), U32),
            pltpu.VMEM((4, 4 * NT * UNROLL // NSEG, D, 128), BF16),
            pltpu.VMEM((7 * NT, M, 128), F32),
            pltpu.VMEM((PR, PR), F32),
            pltpu.VMEM((16, 1), jnp.int32),
            pltpu.VMEM((M, D), BF16),
            pltpu.VMEM((D, 128), F32),
            pltpu.VMEM((8 + PADS[2], 128), U32),
            pltpu.SemaphoreType.DMA((4,)),
            pltpu.SemaphoreType.DMA((2,)),
        ],
        compiler_params=pltpu.CompilerParams(vmem_limit_bytes=120 * 1024 * 1024,
                                             disable_bounds_checks=True),
    )(A_x.reshape(NSEG, SEG, D), A_mem0.reshape(M, D), A_Wq, A_Wk, A_Wv, A_Wo.reshape(H * DH, D),
      B_w_r, B_w_gate, B_w_up, B_w_down, c, w_mod)
    return out.reshape(1, S, D)
```

```python
import functools

import jax
import jax.numpy as jnp
from jax import lax
import jax.experimental.pallas as pl
import jax.experimental.pallas.tpu as pltpu

F32 = jnp.float32
BF16 = jnp.bfloat16
U32 = jnp.uint32

D = 1024
S = 2048
H = 32
DH = 128
M = 8
SEG = 32
NSEG = S // SEG
FF = 3584
NT = D // 128
XR = SEG - M
R0 = M * NSEG
CH = 8
KQ = D // 4
NCHUNK = 3 * D // KQ
NSLOT = 4
PR = 2 * SEG + 2 * M
NP = H // 2
EC = 128
NEC = R0 // EC
LOG2E = 1.4426950408889634
EPS = 1e-5
SCALE = DH ** -0.5
NEG_MASK = -1000000000.0

PHASES = ("pro", "step", "epi")
UNROLL = 4
FB = 32
BLK = 32
R_AT = ((0, 6, 16), (14, 22, 30), (30, 38, 46), (44, 52, 60))
F_AT = (0, 13)
L_AT = 8
VPU_MOD = True
G_AT = (0, 1, 2, 3)
GR = 32
GV_AT = (16, 56)
GVR = 32
GV_FREE = 64
G_LAG = 2
OPAQUE = True
LATE_APPLY = False
LEAN = False
RB = 16
RB2 = 64
JOB_SPAN = 40
LNU = 16
EKH = 4
E_SPAN = 5
EBLK = (128,)
PADS = (0, 0, 0)
MODS = ((-1, 4), (1, 4))
TOK_S = 9
TOK_P = None
TOK_STAG = 2
NORM_PRE = True
R1_END = 11
R2_0 = (3, 14)
LN_RANGE = (0, 29)
WO_RANGE = (12, 31)


def _schedule(mods):
    groups = [list(range(4 * g, 4 * g + 4)) for g in range(4)]
    ops = []

    def mod_at(pos):
        ops.extend(("M", u) for (u, q) in mods if q == pos)

    for t in range(4):
        for i, p in enumerate(groups[t]):
            ops.append(("Q", p, p == 0))
            if p in G_AT:
                ops.append(("G",))
            if i == 0 and t >= 1:
                ops.extend(("S", q) for q in groups[t - 1])
                mod_at(10 + t)
            if i == 3 and t >= 1:
                ops.extend(("P", q) for q in groups[t - 1])
                mod_at(t)
    first = groups[0] + groups[1]
    for j in range(NT):
        ops.append(("O", j, first))
        if j == 1:
            ops.extend(("S", q) for q in groups[3])
            mod_at(14)
    ops.extend(("P", q) for q in groups[3])
    mod_at(4)
    ops.extend(("O", j, groups[2]) for j in range(NT))
    for j in range(NT):
        ops.append(("O", j, groups[3]))
        ops.append(("F", j))
    mod_at(5)
    return ops


def _rb(x):
    return x.astype(BF16).astype(F32)


def _recip(x):
    r = pl.reciprocal(x, approx=True)
    return r * (2.0 - x * r)


def _inv_std(xc):
    v = _rb(_rb(jnp.mean(xc * xc, axis=-1, keepdims=True)) + EPS)
    return _recip(_rb(v * lax.rsqrt(v)))


def _ln(x, zero=None, lean=False):
    xm = x if zero is None else jnp.concatenate([x[..., :128] + zero, x[..., 128:]], axis=-1)
    mu = jnp.mean(xm, axis=-1, keepdims=True)
    xc = x - mu
    v = _rb(_rb(jnp.mean(xc * xc, axis=-1, keepdims=True)) + EPS)
    inv = _recip(_rb(v * lax.rsqrt(v)))
    if lean:
        return x * inv - mu * inv
    return xc * inv


def _ln_mod(x, s1p, shift, zero=None, lean=False):
    return _ln(x, zero, lean) * s1p + shift


def _dot(a, b):
    return jnp.dot(a, b, preferred_element_type=F32)


def _as_bf16(u):
    return pltpu.bitcast(u, BF16)


def _as_u32(b):
    return pltpu.bitcast(b, U32)


def _cumsum(xs):
    out, r = [], 0
    for x in xs:
        out.append(r)
        r += x
    return out


def _spread(jobs, fns, lo, hi):
    for n, fn in enumerate(fns):
        jobs.setdefault(lo + n * (hi - lo) // len(fns), []).append(fn)


def _kernel(x_hbm, mem0_hbm, wq_hbm, wk_hbm, wv_hbm, wo_hbm, wr_hbm, wg_hbm, wu_hbm, wd_hbm,
            c_hbm, wmod_hbm, out_hbm,
            wqkv, hs, wo_s, pre, cur_s, olhs, odef, xbuf, lhs, wm_s, mod, mk,
            top, sc_s, cb_s, zero_s, sem_m, sem_out):
    mt = 4 * NT * UNROLL // NSEG

    def modv(j):
        return jnp.concatenate([mod[j * NT + k] for k in range(NT)], axis=1)

    def mod_store(v, t):
        v = _rb(v)
        mod[t] = jnp.where(jnp.logical_or((t >> 3) == 1, (t >> 3) == 4), _rb(1.0 + v), v)

    def mod_tile(wm, t):
        mod_store(_dot(sc_s[...], wm), t)

    def gemv_part(w, d0, acc):
        n = w.shape[1]
        p = w.astype(F32) * cb_s[d0:d0 + n, :]
        p = jnp.sum(p.reshape(w.shape[0], n // 8, 8, 128), axis=1)
        return p if acc is None else p + acc

    def gemv_finish(acc, ts):
        for u, t in enumerate(ts):
            mod_store(jnp.broadcast_to(jnp.sum(acc[u], axis=0, keepdims=True), (M, 128)), t)

    def wm_copy(it, u):
        col = pl.multiple_of((2 * NT + it * mt + u) * 128, 128)
        return pltpu.make_async_copy(wmod_hbm.at[:, pl.ds(col, 128)], wm_s.at[it & 3, u],
                                     sem_m.at[it & 3])

    def ln1(x, zero=None):
        x3 = x.astype(F32).reshape(x.shape[0] // 8, 8, D)
        zf = None if zero is None else pltpu.bitcast(zero, F32)
        if LATE_APPLY:
            return _ln(x3, zf, LEAN).reshape(x.shape[0], D).astype(BF16)
        return _ln_mod(x3, modv(1), modv(0), zf, LEAN).reshape(x.shape[0], D).astype(BF16)

    def zero_after(y):
        return (y if y.dtype == U32 else pltpu.bitcast(y, U32)) & zero_s[0:8, :]

    def or_tile(u, z):
        if z is None:
            return u
        return (u.reshape(u.shape[0] // 8, 8, 128) | z).reshape(u.shape)

    def prologue(stage, wo_raw, wmod_s, nrm, ha, hb, tmp, mem0_ref, wr_ref, c_ref, sem):
        w_hbms = (wq_hbm, wk_hbm, wv_hbm)
        wob = H * DH // NT
        S_X, S_C0, S_ST, S_WO, S_MOD, S_SM = 0, 2, 6, 6 + NSLOT, 6 + NSLOT + NT, 6 + NSLOT + 2 * NT

        def x_copy(i):
            lo, n = ((XR, M), (0, XR))[i]
            return pltpu.make_async_copy(x_hbm.at[:, pl.ds(lo, n), :], xbuf.at[:, pl.ds(lo, n), :],
                                         sem.at[S_X + i])

        def mod_copies(k):
            return [pltpu.make_async_copy(wmod_hbm.at[:, pl.ds(v * D + k * 128, 128)],
                                          wmod_s.at[k, v], sem.at[S_MOD + (k if k < 2 else k & 6)])
                    for v in range(2)]

        def chunk_copy(mat, d0, g, slot, k):
            return pltpu.make_async_copy(w_hbms[mat].at[pl.ds(d0, KQ), pl.ds(g * CH, CH), :],
                                         stage.at[slot, g], sem.at[k])

        def wo_copy(j):
            return pltpu.make_async_copy(wo_hbm.at[pl.ds(pl.multiple_of(j * wob, wob), wob)],
                                         wo_raw.at[j], sem.at[S_WO + j])

        def relayout1(src, t0, z=None):
            v = src.reshape(RB * CH, 128)
            tmp[t0:t0 + RB * CH // 2, :] = or_tile(_as_u32(v), z)

        def relayout2(c, h0_, t0, d0, z=None):
            w = or_tile(tmp[pl.ds(t0, RB2, stride=CH // 2), :], z)
            rows = pl.ds(d0 // 2, RB2 // 2)
            wqkv[c, h0_, rows, :] = _as_u32(w.astype(jnp.uint16))
            wqkv[c, h0_ + 1, rows, :] = _as_u32((w >> 16).astype(jnp.uint16))

        def mod_pair(k):
            for v in range(2):
                mod_tile(wmod_s[k, v], v * NT + k)

        def fill(dst, q, t, r, z=None):
            k = 2 * q + t
            sh = mod[k] if z is None else mod[k] + pltpu.bitcast(z, F32)
            v = nrm[k, r:r + FB, :].reshape(FB // 8, 8, 128) * mod[NT + k] + sh
            dst[t, r // 2:(r + FB) // 2, :] = _as_u32(v.reshape(FB, 128).astype(BF16))

        small = [pltpu.make_async_copy(src, dst, sem.at[S_SM])
                 for src, dst in ((c_hbm, c_ref), (mem0_hbm, mem0_ref), (wr_hbm, wr_ref))]
        for cp in small:
            cp.start()
        x_copy(0).start()
        for cp in mod_copies(0) + mod_copies(1):
            cp.start()
        for g in range(4):
            chunk_copy(0, 0, g, 0, S_C0 + g).start()
        for c in range(1, NSLOT):
            for g in range(4):
                chunk_copy(c % 3, (c // 3) * KQ, g, c, S_ST + c).start()
            for cp in mod_copies(2 * c) + mod_copies(2 * c + 1):
                cp.start()

        def decode(i):
            lo = i < 2 * SEG
            head = jnp.where(lo, i // SEG, (i - 2 * SEG) // M)
            is_mem = jnp.logical_and(lo, i % SEG >= XR)
            pos = jnp.where(lo, i % SEG, XR + i % M)
            return head, is_mem, pos

        qh, qm, qp = decode(lax.broadcasted_iota(jnp.int32, (PR, PR), 0))
        kh, km, kp = decode(lax.broadcasted_iota(jnp.int32, (PR, PR), 1))
        vis = qm | km | (qp >= kp)
        mk[0:PR, :] = jnp.where(qh == kh, jnp.where(vis, 0.0, NEG_MASK * LOG2E), -jnp.inf).astype(F32)
        mod[0:2 * NT] = jnp.zeros((2 * NT, M, 128), F32)
        zero_s[...] = jnp.zeros(zero_s.shape, U32)
        top[...] = jnp.full(top.shape, jnp.iinfo(jnp.int32).min, jnp.int32)
        for cp in small:
            cp.wait()
        wr = jnp.broadcast_to(wr_ref[...].astype(F32).reshape(1, D), (M, D))
        for k in range(NT):
            mod[6 * NT + k] = wr[:, k * 128:(k + 1) * 128]
        cv = c_ref[...].astype(F32)
        sc = _rb(cv * _rb(jax.nn.sigmoid(cv)))
        sc_s[...] = jnp.broadcast_to(sc, (M, D)).astype(BF16)
        for k in range(NT):
            cb_s[k * 128:(k + 1) * 128, :] = jnp.broadcast_to(
                sc[:, k * 128:(k + 1) * 128], (128, 128)).T
        mb = mem0_ref[...]
        for k in range(NT):
            lhs[0, k, XR // 2:, :] = _as_u32(mb[:, k * 128:(k + 1) * 128])

        def zero_body(i, c):
            wo_raw[NT, pl.ds(pl.multiple_of(i * 32, 32), 32), :] = jnp.zeros((32, D), BF16)
            return c

        lax.fori_loop(0, wob // 32, zero_body, 0)
        x_copy(0).wait()

        def ln_body(i, c):
            for u in range(LNU):
                q = i * LNU + u
                v = _ln(xbuf[q, XR:, :].astype(F32))
                for k in range(NT):
                    nrm[k, pl.ds(pl.multiple_of(q * 8, 8), 8), :] = v[:, k * 128:(k + 1) * 128]
            return c

        with jax.named_scope("p_ln"):
            lax.fori_loop(0, NSEG // LNU, ln_body, 0)

        def mod_body(k, c):
            pltpu.make_async_copy(wmod_s.at[k], wmod_s.at[k], sem.at[S_MOD + k]).wait()
            mod_pair(k)
            for r in range(0, R0, FB):
                fill(ha, 0, k, r)
            return c

        with jax.named_scope("p_mod"):
            lax.fori_loop(0, 2, mod_body, 0)

        def c0_body(g):
            chunk_copy(0, 0, 0, 0, S_C0 + g).wait()
            for d0 in range(0, KQ, RB):
                relayout1(stage[0, g, d0:d0 + RB], d0 * CH // 2)
            for j in range(CH // 2):
                for d0 in range(0, KQ, RB2):
                    relayout2(0, g * CH + 2 * j, d0 * CH // 2 + j, d0)

        def bulk(units, jobs, inserts):
            due = {}
            t0 = 0
            for n, (hq, c, h0_, pi, first, r0, nrow) in enumerate(units):
                nb = nrow // BLK
                parts = []
                for u in range(nb):
                    part = hq[0, (r0 + u * BLK) // 2:(r0 + (u + 1) * BLK) // 2, :]
                    for z in due.pop(t0 + u, ()):
                        part = jnp.concatenate([part[0:8] | z, part[8:]], axis=0)
                    parts.append(part)
                hv = jnp.concatenate([_as_bf16(jnp.concatenate(parts, axis=0)),
                                      _as_bf16(hq[1, r0 // 2:(r0 + nrow) // 2, :])], axis=1)
                w = jnp.concatenate([_as_bf16(wqkv[c, h0_]), _as_bf16(wqkv[c, h0_ + 1])], axis=1)
                y = _dot(hv, w)
                segs = slice(r0 // M, (r0 + nrow) // M)
                for a in range(2):
                    old = jnp.where(first, 0.0, pre[pi, segs, a * M:(a + 1) * M, :])
                    pre[pi, segs, a * M:(a + 1) * M, :] = (
                        y[:, a * DH:(a + 1) * DH].reshape(nrow // M, M, DH) + old)
                for fn in inserts.get(n, ()):
                    fn()
                for u in range(nb):
                    for job in jobs.get(t0 + u, ()):
                        res = job(zero_after(y[u * BLK:u * BLK + 8, 0:128]))
                        if res is not None:
                            due.setdefault(max(t0 + u + JOB_SPAN, t0 + nb), []).append(
                                zero_after(res))
                t0 += nb
            assert not due

        GP = CH // 2
        WO0 = NCHUNK - 1 - NT
        LN0 = 4
        SPI = -(-NSEG // (NCHUNK - 1 - LN0))

        def rot_body(i, c):
            slot = (i + 1) & (NSLOT - 1)
            pltpu.make_async_copy(stage.at[slot], stage.at[slot], sem.at[S_ST + slot]).wait()
            km = 2 * jnp.minimum(i, 3)

            @pl.when(jnp.logical_and(i >= 1, i <= 3))
            def _():
                wq = wmod_s.at[pl.ds(km, 2)]
                pltpu.make_async_copy(wq, wq, sem.at[S_MOD + km]).wait()

            @pl.when(i == LN0)
            def _():
                x_copy(1).wait()

            @pl.when(i >= WO0)
            def _():
                wo_copy(i - WO0).wait()

            nxt = i + NSLOT
            qn = (nxt * 43) >> 7
            for mat in range(3):
                @pl.when(jnp.logical_and(nxt < NCHUNK, nxt - 3 * qn == mat))
                def _():
                    for g in range(4):
                        chunk_copy(mat, qn * KQ, g, nxt & (NSLOT - 1),
                                   S_ST + (nxt & (NSLOT - 1))).start()

            @pl.when(i < NT)
            def _():
                wo_copy(i).start()

            @pl.when(i == 0)
            def _():
                x_copy(1).start()

            q0 = (i * 43) >> 7
            q1 = ((i + 1) * 43) >> 7
            pa = (i - 3 * q0) * NP + NP - GP
            units = ([(ha, i, H - CH + 2 * n, pa + n, q0 == 0, 0, R0) for n in range(GP)]
                     + [(hb, i + 1, 2 * n, (i + 1 - 3 * q1) * NP + n, q1 == 0, 0, R0)
                        for n in range(NP - GP)])
            jw = jnp.where(i >= WO0, i - WO0, NT)

            def wo_job(b, z):
                v = wo_raw[jw, b * 16:(b + 1) * 16, :]
                rows = pl.ds(pl.multiple_of(jw * (wob // 2) + b * 8, 8), 8)
                for j in range(NT):
                    wo_s[j, rows, :] = _as_u32(v[:, j * 128:(j + 1) * 128]) | z

            def ln_job(b, z):
                r = (b % 3) * 8
                seg = (i - LN0) * SPI + b // 3
                live = jnp.logical_and(i >= LN0, seg < NSEG)
                src = jnp.where(live, seg, 0)
                hv = ln1(xbuf[src, pl.ds(pl.multiple_of(jnp.where(live, r, XR), 8), 8), :], z)
                u = [_as_u32(hv[:, k * 128:(k + 1) * 128]) for k in range(NT)]
                dst = jnp.where(live, seg, NSEG)
                for k in range(NT):
                    hs[dst, k, r // 2:r // 2 + 4, :] = u[k]
                res = jnp.concatenate(u[0:2], axis=0)
                for k in range(2, NT, 2):
                    res = res | jnp.concatenate(u[k:k + 2], axis=0)
                return res

            def r1_job(g, d0, z):
                relayout1(stage[slot, g, d0:d0 + RB], (g * KQ + d0) * CH // 2, z)

            def copy_job(t, r, z):
                ha[t, r:r + 32, :] = or_tile(hb[t, r:r + 32, :], z)

            P = functools.partial
            upb = R0 // BLK
            nr = NP * upb
            jobs = {}
            for g in range(4):
                lo, mid, hi = (x * upb // 4 for x in R_AT[g])
                _spread(jobs, [P(r1_job, g, d0) for d0 in range(0, KQ, RB)], lo, mid)
                _spread(jobs, [P(relayout2, i + 1, g * CH + 2 * j, (g * KQ + d0) * CH // 2 + j, d0)
                               for j in range(CH // 2) for d0 in range(0, KQ, RB2)], mid, hi)
            oz = (i >> 10) if OPAQUE else 0
            _spread(jobs, [P(fill, hb, q1, t + oz, r) for r in range(0, R0, FB) for t in range(2)],
                    F_AT[0] * upb // 4, F_AT[1] * upb // 4)
            _spread(jobs, [P(copy_job, t, r) for t in range(2) for r in range(0, R0 // 2, 32)],
                    2 * GP * upb, nr - upb)
            _spread(jobs, [P(ln_job, b) for b in range(3 * SPI)],
                    L_AT * upb // 4, nr - max(upb, JOB_SPAN))
            _spread(jobs, [P(wo_job, b) for b in range(wob // 16)], GP * upb, nr - upb)
            gv = {}

            def gv_job(d0, n, z):
                w = wmod_s[pl.ds(km, 2), :, d0:d0 + n, :].reshape(4, n, 128)
                acc = gv.get("acc")
                if z is not None:
                    zf = pltpu.bitcast(z, F32)[None]
                    acc = jnp.broadcast_to(zf, (4, 8, 128)) if acc is None else acc + zf
                gv["acc"] = gemv_part(w, d0, acc)
                if z is not None:
                    au = pltpu.bitcast(gv["acc"], U32)
                    return au[0] | au[1] | au[2] | au[3]

            _spread(jobs, [P(gv_job, d0, GVR) for d0 in range(0, D - GV_FREE, GVR)],
                    GV_AT[0] * upb // 4, min(GV_AT[1] * upb // 4, nr - JOB_SPAN))
            bulk(units, jobs, {})
            if GV_FREE:
                gv_job(D - GV_FREE, GV_FREE, None)
            gemv_finish(gv["acc"], [km, NT + km, km + 1, NT + km + 1])
            return c

        def outer(k, c):
            last = k == 4

            @pl.when(k < 4)
            def _():
                c0_body(k)

            @pl.when(k != 3)
            def _():
                g = jnp.minimum(k, 3)
                bulk([(ha, jnp.where(last, NCHUNK - 1, 0), g * CH + 2 * n,
                       jnp.where(last, 2 * NP, 0) + g * GP + n, k < 4, 0, R0)
                      for n in range(GP)], {}, {})

            @pl.when(k == 3)
            def _():
                with jax.named_scope("p_rot"):
                    lax.fori_loop(0, NCHUNK - 1, rot_body, 0)
                for it in range(2):
                    for u in range(mt):
                        wm_copy(it, u).start()

            return c

        with jax.named_scope("p_bulk"):
            lax.fori_loop(0, 5, outer, 0)

    if "pro" in PHASES: pl.run_scoped(
        prologue,
        pltpu.VMEM((NSLOT, H // CH, KQ, CH, 128), BF16),
        pltpu.VMEM((NT + 1, H * DH // NT, D), BF16),
        pltpu.VMEM((NT, 2, D, 128), BF16),
        pltpu.VMEM((NT, R0, 128), F32),
        pltpu.VMEM((2, R0 // 2 + PADS[0], 128), U32),
        pltpu.VMEM((2, R0 // 2 + PADS[0], 128), U32),
        pltpu.VMEM((D * CH // 2 + PADS[1], 128), U32),
        pltpu.VMEM((M, D), BF16),
        pltpu.VMEM((D,), BF16),
        pltpu.VMEM((1, D), BF16),
        pltpu.SemaphoreType.DMA((7 + NSLOT + 2 * NT,)),
    )

    def main(wg_s, wu_s, wd_s, ybuf, stat, outs, sem_f):
        def load_x_rows(slot, seg):
            for k in range(NT):
                if LATE_APPLY:
                    v = _as_bf16(hs[seg, k]).astype(F32).reshape(XR // 8, 8, 128)
                    v = (v * mod[NT + k] + mod[k]).reshape(XR, 128)
                    lhs[slot, k, 0:XR // 2, :] = _as_u32(v.astype(BF16))
                else:
                    lhs[slot, k, 0:XR // 2, :] = hs[seg, k]

        def resid(seg, r, z=None):
            rows = pl.ds(r, 8)
            t = modv(2) * ybuf[seg, rows, :].astype(F32)
            if z is not None:
                t = t + jnp.concatenate([pltpu.bitcast(z, F32)] * NT, axis=1)
            return xbuf[seg, rows, :].astype(F32) + t

        def wide(v):
            return jnp.concatenate([v] * NT, axis=1)

        def make_key(v, row0):
            b = pltpu.bitcast(jnp.where(v != v, -jnp.inf, v + 0.0), jnp.int32)
            low = (S - 1 - row0) - lax.broadcasted_iota(jnp.int32, (8, 128), 0)
            return (b ^ ((b >> 31) & 0x7FFF0000)) | low

        def post(seg, r, z):
            x1 = resid(seg, r, z)
            mu = jnp.mean(x1, axis=-1, keepdims=True)
            xc = x1 - mu
            inv = _inv_std(xc)
            stat[0, seg, pl.ds(r, 8), :] = jnp.broadcast_to(mu, (8, 128))
            stat[1, seg, pl.ds(r, 8), :] = jnp.broadcast_to(inv, (8, 128))
            v = _rb(inv * jnp.sum(xc * modv(7), axis=-1, keepdims=True) + mod[8 * NT])
            key = make_key(v, seg * SEG + r)
            m1, m2 = top[0:8, :], top[8:16, :]
            top[8:16, :] = jnp.maximum(m2, jnp.minimum(m1, key))
            top[0:8, :] = jnp.maximum(m1, key)
            o = x1 + modv(5) * (xc * inv * modv(4) + modv(3))
            outs[seg, pl.ds(r, 8), :] = o.astype(BF16)
            res = pltpu.bitcast(v, U32)
            for k in range(NT):
                res = res | pltpu.bitcast(o[:, k * 128:(k + 1) * 128], U32)
            return res

        def redo(seg, r, z=None):
            x1 = resid(seg, r, z)
            n = (x1 - wide(stat[0, seg, pl.ds(r, 8), :])) * wide(stat[1, seg, pl.ds(r, 8), :])
            return x1, n * modv(4) + modv(3)

        def out_copy(g0, ng, r, n, k=0):
            return pltpu.make_async_copy(outs.at[pl.ds(g0, ng), pl.ds(r, n), :],
                                         out_hbm.at[pl.ds(g0, ng), pl.ds(r, n), :], sem_out.at[k])

        late = ((wg_hbm, wg_s, FF // 128), (wu_hbm, wu_s, FF // 128), (wd_hbm, wd_s, NT))

        def col_copy(k, j):
            return pltpu.make_async_copy(
                late[k][0].at[:, pl.ds(pl.multiple_of(j * 128, 128), 128)], late[k][1].at[j],
                sem_f.at[k])

        load_x_rows(0, 0)

        def step(it, cur, state):
            s = it * UNROLL + cur
            nxt = (cur + 1) % UNROLL

            def pay(t, cost):
                now = state.get("now", 0)
                due = state.setdefault("due", [])
                for z in [z for (d, z) in due if d <= now]:
                    t = jnp.concatenate([t[0:8] | z, t[8:]], axis=0)
                state["due"] = [(d, z) for (d, z) in due if d > now]
                state["now"] = now + cost
                return t

            def owe(lag, p, tiles):
                z = tiles[0]
                for t in tiles[1:]:
                    z = z | t
                state.setdefault("due", []).append(
                    (state.get("now", 0) + lag + (p % 4) * TOK_STAG, zero_after(z)))

            def lv(k0, k1):
                ts = [lhs[cur, k] for k in range(k0, k1)]
                ts[0] = pay(ts[0], (k1 - k0) / NT)
                return jnp.concatenate([_as_bf16(t) for t in ts], axis=1)

            def wmat(mat, h, q0, q1):
                return _as_bf16(jnp.concatenate([wqkv[3 * q + mat, h] for q in range(q0, q1)],
                                                axis=0))

            def qkv(p, split=False):
                part = {}
                if split:
                    for mat in range(3):
                        for a in range(2):
                            part[mat, a] = _dot(lv(0, NT // 2), wmat(mat, 2 * p + a, 0, 2))
                for mat in range(3):
                    for a in range(2):
                        hm = mat * H + 2 * p + a
                        if split:
                            y = _dot(lv(NT // 2, NT), wmat(mat, 2 * p + a, 2, 4)) + part[mat, a]
                        else:
                            y = _dot(lv(0, NT), wmat(mat, 2 * p + a, 0, 4))
                        cur_s[hm] = y.astype(BF16)

            def gather(mat, p):
                hm = mat * H + 2 * p
                return jnp.concatenate(
                    [cur_s[hm], cur_s[hm + 1], pre[mat * NP + p, s].astype(BF16)], axis=0)

            probs = {}

            def scores(p):
                sc = lax.dot_general(gather(0, p), gather(1, p), (((1,), (1,)), ((), ())),
                                     preferred_element_type=F32)
                mv = mk[0:PR, :]
                sc = jnp.where(mv == 0.0, sc * (SCALE * LOG2E), mv)
                e = jnp.exp2(sc - jnp.max(sc, axis=-1, keepdims=True))
                inv = _recip(jnp.sum(e, axis=-1, keepdims=True))
                if NORM_PRE:
                    e = e * inv
                    if TOK_S is not None:
                        eu = pltpu.bitcast(e, U32)
                        z = eu[0:8]
                        for k in range(1, PR // 8):
                            z = z | eu[k * 8:(k + 1) * 8]
                        owe(TOK_S, p, [jnp.concatenate([z, jnp.zeros((8, 128 - PR), U32)], axis=1)])
                    probs[p] = (e.astype(BF16), None)
                else:
                    if TOK_S is not None:
                        iu = pltpu.bitcast(jnp.broadcast_to(inv, (PR, 128)), U32)
                        owe(TOK_S, p, [iu[k * 8:(k + 1) * 8] for k in range(PR // 8)])
                    probs[p] = (e.astype(BF16), inv)

            def pv(p):
                e, inv = probs.pop(p)
                o = _dot(e, gather(2, p))
                if inv is not None:
                    o = o * inv
                o = o.astype(BF16)
                if TOK_P is not None:
                    ou = _as_u32(o)
                    owe(TOK_P, p, [ou[k * 8:(k + 1) * 8] for k in range(PR // 16)])
                for a in range(2):
                    h = 2 * p + a
                    olhs[h] = _as_u32(o[a * SEG:(a + 1) * SEG])
                    odef[h, it, cur * 4:(cur + 1) * 4, :] = _as_u32(
                        o[2 * SEG + a * M:2 * SEG + (a + 1) * M])

            acc = [None] * NT

            def oproj(j, pairs):
                ts = [olhs[2 * p + a] for p in pairs for a in range(2)]
                ts[0] = pay(ts[0], len(pairs) / 4)
                ov = jnp.concatenate([_as_bf16(t) for t in ts], axis=1)
                w = wo_s[j, pairs[0] * DH:(pairs[-1] + 1) * DH, :]
                y = _dot(ov, _as_bf16(w))
                acc[j] = y if acc[j] is None else y + acc[j]

            def fin(j):
                yb = acc[j].astype(BF16)
                ybuf[s, 0:XR, j * 128:(j + 1) * 128] = yb[0:XR]
                lhs[nxt, j, XR // 2:, :] = _as_u32(yb[XR:])

            def gemv():
                d0 = state.get("d0", 0)
                state["acc"] = gemv_part(wm_s[it & 3, :, d0:d0 + GR, :], d0, state.get("acc"))
                state["d0"] = d0 + GR
                au = pltpu.bitcast(state["acc"], U32)
                owe(G_LAG, 0, [au[u] for u in range(mt)])

            def late_mod(u):
                mod_tile(wm_s[it & 3, u], 2 * NT + it * mt + u)

            load_x_rows(nxt, jnp.minimum(s + 1, NSEG - 1))
            ops = dict(Q=qkv, S=scores, P=pv, O=oproj, F=fin, M=late_mod, G=gemv)
            for op in _schedule([(u, q) for u, (c_, q) in enumerate(MODS[:mt])
                                 if c_ % UNROLL == cur and not VPU_MOD]):
                ops[op[0]](*op[1:])

        def steps(it, carry):
            if "pro" in PHASES:
                pltpu.make_async_copy(wm_s.at[it & 3], wm_s.at[it & 3], sem_m.at[it & 3]).wait()

                @pl.when(it + 2 < NSEG // UNROLL)
                def _():
                    for u in range(mt):
                        wm_copy(it + 2, u).start()

            for u in range(UNROLL // 2):
                t = it * (UNROLL // 2) + u
                for k in range(3):
                    @pl.when(t < late[k][2])
                    def _():
                        col_copy(k, t).start()

            state = {}
            for u in range(UNROLL):
                step(it, u, state)
            if VPU_MOD:
                acc = state.get("acc")
                for d0 in range(state.get("d0", 0), D, 64):
                    acc = gemv_part(wm_s[it & 3, :, d0:d0 + 64, :], d0, acc)
                gemv_finish(acc, [2 * NT + it * mt + u for u in range(mt)])
            return carry

        with jax.named_scope("m_steps"):
            if "step" in PHASES: lax.fori_loop(0, NSEG // UNROLL, steps, 0)
        for k in range(3):
            for j in range(late[k][2]):
                col_copy(k, j).wait()
        if "epi" not in PHASES:
            return

        ntail = EBLK[-1] // M
        ppi = (S // 8 - ntail) // NEC
        gpi = ppi // (XR // 8)
        gb_ = UNROLL * M

        def ep_body(i, c):
            @pl.when(i > 0)
            def _():
                out_copy((i - 1) * gpi, gpi, 0, XR).start()

            for k in range(NT):
                mod[7 * NT + k] = mod[4 * NT + k] * mod[6 * NT + k]
            mod[8 * NT] = jnp.broadcast_to(
                jnp.sum(modv(3) * modv(6), axis=-1, keepdims=True), (M, 128))

            subs = []
            r0 = 0
            for nr in EBLK:
                kh = EKH * EC // nr if EC % nr == 0 else EKH
                for j in range(NT):
                    for h0_ in range(0, H, kh):
                        subs.append((r0, nr, j, h0_, kh))
                r0 += nr
            tot = sum(nr * kh for (_, nr, _, _, kh) in subs)
            span = E_SPAN * EC * EKH
            rel = [u * (tot - span) // ppi for u in range(ppi)]
            ready = {}
            due = []
            now = 0
            u = 0
            y = None
            for (r0, nr, j, h0_, kh) in subs:
                blk = pl.ds(i * (EC // gb_) + r0 // gb_, nr // gb_)
                ts = [odef[h, blk].reshape(nr // 2, DH) for h in range(h0_, h0_ + kh)]
                for z in [z for (d, z) in due if d <= now]:
                    ts[0] = jnp.concatenate([ts[0][0:8] | z, ts[0][8:]], axis=0)
                due = [(d, z) for (d, z) in due if d > now]
                w = wo_s[j, h0_ * DH // 2:(h0_ + kh) * DH // 2, :]
                yp = _dot(jnp.concatenate([_as_bf16(t) for t in ts], axis=1), _as_bf16(w))
                y = yp if h0_ == 0 else yp + y
                if h0_ + kh == H:
                    ybuf[pl.ds(i * (EC // M) + r0 // M, nr // M), XR:, j * 128:(j + 1) * 128] = (
                        y.reshape(nr // M, M, 128).astype(BF16))
                    if j == NT - 1:
                        ready[r0] = True
                start = now
                now += nr * kh
                while u < ppi and rel[u] < now:
                    d = (NEC - 1) * ppi + u - NSEG * (XR // 8) - (NEC - 1) * (EC // M)
                    if d >= 0 and sum(n for r, n in zip(_cumsum(EBLK), EBLK) if r in ready) <= d * M:
                        break
                    t = i * ppi + u
                    early = t < NSEG * (XR // 8)
                    seg = jnp.where(early, t // (XR // 8), t - NSEG * (XR // 8))
                    row = pl.multiple_of(jnp.where(early, (t % (XR // 8)) * 8, XR), 8)
                    res = post(seg, row, zero_after(y[0:8]))
                    due.append((start + span, zero_after(res)))
                    u += 1
            assert u == ppi
            return c

        with jax.named_scope("e_loop"):
            lax.fori_loop(0, NEC, ep_body, 0)
        done = (NEC - 1) * gpi
        tail = NSEG - ntail
        out_copy(done, NSEG - done, 0, XR).start()
        out_copy(0, tail, XR, M).start()
        x1s = [resid(g, XR) for g in range(tail, NSEG)]
        mus = [jnp.mean(x1, axis=-1, keepdims=True) for x1 in x1s]
        pairs = [(top[0:8, :], top[8:16, :])]
        lowest = jnp.full((8, 128), jnp.iinfo(jnp.int32).min, jnp.int32)
        for g in range(tail, NSEG):
            xc = x1s[g - tail] - mus[g - tail]
            inv = _inv_std(xc)
            stat[0, g, XR:, :] = jnp.broadcast_to(mus[g - tail], (8, 128))
            stat[1, g, XR:, :] = jnp.broadcast_to(inv, (8, 128))
            v = _rb(inv * jnp.sum(xc * modv(7), axis=-1, keepdims=True) + mod[8 * NT])
            pairs.append((make_key(v, g * SEG + XR), lowest))
        while len(pairs) > 1:
            (a1, a2), (c1, c2) = pairs.pop(0), pairs.pop(0)
            pairs.append((jnp.maximum(a1, c1),
                          jnp.maximum(jnp.minimum(a1, c1), jnp.maximum(a2, c2))))

        tk = jnp.concatenate(pairs[0], axis=0)[:, 0:1]
        k1 = jnp.max(tk[0:8], axis=0, keepdims=True)
        k2 = jnp.max(jnp.where(tk == k1, jnp.iinfo(jnp.int32).min, tk), axis=0, keepdims=True)
        i1 = (S - 1) - (k1[0, 0] & (S - 1))
        i2 = (S - 1) - (k2[0, 0] & (S - 1))
        g1, g2 = i1 >> 5, i2 >> 5
        b1 = pl.multiple_of(i1 & 24, 8)
        b2 = pl.multiple_of(i2 & 24, 8)

        xa, ha_ = redo(g1, b1)
        xb_, hb_ = redo(g2, b2)
        x1 = jnp.concatenate([xa, xb_], axis=0)
        h2 = jnp.concatenate([ha_, hb_], axis=0)
        h2b = h2.astype(BF16)
        row = lax.broadcasted_iota(jnp.int32, (16, 1), 0)
        grow = jnp.where(row < 8, g1 * SEG + b1 + row, g2 * SEG + b2 + row - 8)
        ks = jnp.where(grow == i1, k1, k2)
        rsel = pltpu.bitcast((ks ^ ((ks >> 31) & 0x7FFF0000)) & -65536, F32)
        acts = []
        for j in range(FF // 128):
            gt = _rb(_dot(h2b, wg_s[j]))
            gt = _rb(gt * _rb(jax.nn.sigmoid(gt)))
            ut = _rb(_dot(h2b, wu_s[j]))
            acts.append((gt * ut).astype(BF16))
            if j < ntail:
                xo_, ho_ = redo(tail + j, XR, zero_after(ut[0:8]))
                outs[tail + j, XR:, :] = (xo_ + modv(5) * ho_).astype(BF16)
            if j == ntail - 1:
                out_copy(tail, NSEG - tail, XR, M).start()
        act = jnp.concatenate(acts, axis=1)
        y = _rb(jnp.concatenate([_dot(act, wd_s[j]) for j in range(NT)], axis=1))
        y = _rb(y * _rb(jax.nn.sigmoid(rsel)))
        sel = jnp.logical_or(grow == i1, grow == i2)
        gb2 = jnp.concatenate([modv(5)] * 2, axis=0)
        fixed = (x1 + gb2 * (h2 + jnp.where(sel, y, 0.0))).astype(BF16)

        with jax.named_scope("e_outwait"):
            out_copy(0, NSEG, 0, SEG).wait()
        outs[g1, pl.ds(b1, 8), :] = fixed[0:8]
        outs[g2, pl.ds(b2, 8), :] = fixed[8:16]
        out_copy(g1, 1, b1, 8, 0).start()

        @pl.when((i1 >> 3) != (i2 >> 3))
        def _():
            out_copy(g2, 1, b2, 8, 1).start()
            out_copy(g2, 1, b2, 8, 1).wait()

        out_copy(g1, 1, b1, 8, 0).wait()

    pl.run_scoped(
        main,
        pltpu.VMEM((FF // 128, D, 128), BF16),
        pltpu.VMEM((FF // 128, D, 128), BF16),
        pltpu.VMEM((NT, FF, 128), BF16),
        pltpu.VMEM((NSEG, SEG, D), BF16),
        pltpu.VMEM((2, NSEG, SEG, 128), F32),
        pltpu.VMEM((NSEG, SEG, D), BF16),
        pltpu.SemaphoreType.DMA((3,)),
    )


@functools.partial(jax.jit, static_argnames=("A_seg_len",))
def pallas_adaLN_cond__memory_aug_recurrent_mem_tr__moe_arch_mod__prompt_kernel(
    A_x: jax.Array,
    A_mem0: jax.Array,
    A_Wq: jax.Array,
    A_Wk: jax.Array,
    A_Wv: jax.Array,
    A_Wo: jax.Array,
    A_seg_len,
    B_x: jax.Array,
    B_w_r: jax.Array,
    B_w_gate: jax.Array,
    B_w_up: jax.Array,
    B_w_down: jax.Array,
    c: jax.Array,
    w_mod: jax.Array,
):
    assert A_seg_len == SEG and A_x.shape == (1, S, D)
    del B_x
    hbm = pl.BlockSpec(memory_space=pl.ANY)
    out = pl.pallas_call(
        _kernel,
        out_shape=jax.ShapeDtypeStruct((NSEG, SEG, D), BF16),
        in_specs=[hbm] * 12,
        out_specs=hbm,
        scratch_shapes=[
            pltpu.VMEM((NCHUNK, H, KQ // 2, DH), U32),
            pltpu.VMEM((NSEG + 1, NT, XR // 2, 128), U32),
            pltpu.VMEM((NT, (H * DH + H * DH // NT) // 2, 128), U32),
            pltpu.VMEM((3 * NP, NSEG, 2 * M, DH), F32),
            pltpu.VMEM((3 * H, SEG, DH), BF16),
            pltpu.VMEM((H, SEG // 2, DH), U32),
            pltpu.VMEM((H, NSEG // UNROLL, UNROLL * M // 2, DH), U32),
            pltpu.VMEM((NSEG, SEG, D), BF16),
            pltpu.VMEM((UNROLL, NT, SEG // 2, 128), U32),
            pltpu.VMEM((4, 4 * NT * UNROLL // NSEG, D, 128), BF16),
            pltpu.VMEM((8 * NT + 4, M, 128), F32),
            pltpu.VMEM((96, PR), F32),
            pltpu.VMEM((32, 128), jnp.int32),
            pltpu.VMEM((M, D), BF16),
            pltpu.VMEM((D, 128), F32),
            pltpu.VMEM((8 + PADS[2], 128), U32),
            pltpu.SemaphoreType.DMA((4,)),
            pltpu.SemaphoreType.DMA((2,)),
        ],
        compiler_params=pltpu.CompilerParams(vmem_limit_bytes=120 * 1024 * 1024,
                                             disable_bounds_checks=True),
    )(A_x.reshape(NSEG, SEG, D), A_mem0.reshape(M, D), A_Wq, A_Wk, A_Wv, A_Wo.reshape(H * DH, D),
      B_w_r, B_w_gate, B_w_up, B_w_down, c, w_mod)
    return out.reshape(1, S, D)
```

```python
import functools

import jax
import jax.numpy as jnp
from jax import lax
import jax.experimental.pallas as pl
import jax.experimental.pallas.tpu as pltpu

F32 = jnp.float32
BF16 = jnp.bfloat16
U32 = jnp.uint32

D = 1024
S = 2048
H = 32
DH = 128
M = 8
SEG = 32
NSEG = S // SEG
FF = 3584
NT = D // 128
XR = SEG - M
R0 = M * NSEG
CH = 8
KQ = D // 4
NCHUNK = 3 * D // KQ
NSLOT = 4
PR = 2 * SEG + 2 * M
NP = H // 2
EC = 128
NEC = R0 // EC
LOG2E = 1.4426950408889634
EPS = 1e-5
SCALE = DH ** -0.5
NEG_MASK = -1000000000.0

PHASES = ("pro", "step", "epi")
UNROLL = 4
FB = 32
BLK = 32
R_AT = ((0, 6, 16), (14, 22, 30), (30, 38, 46), (44, 52, 60))
F_AT = (0, 13)
L_AT = 8
VPU_MOD = True
REL_S = 2
REL_STAG = 2
PG = 4
LAG_S = 1
LAG_P = 4
O_PARTS = (0, 8, 12)
O_TH = (256, 256, 256, 1216)
TR_MODE = "bf16"
G_AT = (0, 1, 2, 3)
GR = 32
GV_AT = (16, 56)
GVR = 32
GV_FREE = 64
G_LAG = 2
OPAQUE = True
LATE_APPLY = False
LEAN = False
RB = 16
RB2 = 64
JOB_SPAN = 40
LNU = 16
EKH = 4
E_SPAN = 5
EBLK = (128,)
PADS = (0, 0, 24)
MODS = ((-1, 4), (1, 4))
TOK_S = None
TOK_P = None
TOK_STAG = 2
NORM_PRE = True
R1_END = 11
R2_0 = (3, 14)
LN_RANGE = (0, 29)
WO_RANGE = (12, 31)


def _schedule(mods):
    groups = [list(range(g, g + PG)) for g in range(0, NP, PG)]
    at = {}
    for g, grp in enumerate(groups):
        at.setdefault(grp[-1] + LAG_P, []).extend(("P", q) for q in grp)
    for g, grp in enumerate(groups):
        at.setdefault(grp[-1] + LAG_S, []).extend(("S", q) for q in grp)
    ops = []
    for p in range(NP):
        ops.append(("Q", p, p == 0))
        if p in G_AT:
            ops.append(("G",))
        ops.extend(at.pop(p, []))
    bounds = list(O_PARTS) + [NP]
    t = NP
    done = 0
    for n in range(len(O_PARTS)):
        part = list(range(bounds[n], bounds[n + 1]))
        assert all(("P", q) in ops for q in part), (n, ops)
        for j in range(NT):
            ops.append(("O", j, part))
            if n == len(O_PARTS) - 1:
                ops.append(("F", j))
            done += len(part) * 16
            while t - NP < len(O_TH) and done >= O_TH[t - NP]:
                ops.extend(at.pop(t, []))
                t += 1
    assert not at
    return ops


def _rb(x):
    return x.astype(BF16).astype(F32)


def _recip(x):
    r = pl.reciprocal(x, approx=True)
    return r * (2.0 - x * r)


def _inv_std(xc):
    v = _rb(_rb(jnp.mean(xc * xc, axis=-1, keepdims=True)) + EPS)
    return _recip(_rb(v * lax.rsqrt(v)))


def _ln(x, zero=None, lean=False):
    xm = x if zero is None else jnp.concatenate([x[..., :128] + zero, x[..., 128:]], axis=-1)
    mu = jnp.mean(xm, axis=-1, keepdims=True)
    xc = x - mu
    v = _rb(_rb(jnp.mean(xc * xc, axis=-1, keepdims=True)) + EPS)
    inv = _recip(_rb(v * lax.rsqrt(v)))
    if lean:
        return x * inv - mu * inv
    return xc * inv


def _ln_mod(x, s1p, shift, zero=None, lean=False):
    return _ln(x, zero, lean) * s1p + shift


def _dot(a, b):
    return jnp.dot(a, b, preferred_element_type=F32)


def _as_bf16(u):
    return pltpu.bitcast(u, BF16)


def _as_u32(b):
    return pltpu.bitcast(b, U32)


def _cumsum(xs):
    out, r = [], 0
    for x in xs:
        out.append(r)
        r += x
    return out


def _spread(jobs, fns, lo, hi):
    for n, fn in enumerate(fns):
        jobs.setdefault(lo + n * (hi - lo) // len(fns), []).append(fn)


def _kernel(x_hbm, mem0_hbm, wq_hbm, wk_hbm, wv_hbm, wo_hbm, wr_hbm, wg_hbm, wu_hbm, wd_hbm,
            c_hbm, wmod_hbm, out_hbm,
            wqkv, hs, wo_s, pre, cur_s, olhs, odef, xbuf, lhs, wm_s, mod, mk,
            top, sc_s, cb_s, ts_s, zero_s, sem_m, sem_out):
    mt = 4 * NT * UNROLL // NSEG

    def modv(j):
        return jnp.concatenate([mod[j * NT + k] for k in range(NT)], axis=1)

    def mod_store(v, t):
        v = _rb(v)
        mod[t] = jnp.where(jnp.logical_or((t >> 3) == 1, (t >> 3) == 4), _rb(1.0 + v), v)

    def mod_tile(wm, t):
        mod_store(_dot(sc_s[...], wm), t)

    def gemv_part(w, d0, acc):
        n = w.shape[1]
        p = w.astype(F32) * cb_s[d0:d0 + n, :]
        p = jnp.sum(p.reshape(w.shape[0], n // 8, 8, 128), axis=1)
        return p if acc is None else p + acc

    def gemv_finish(acc, ts):
        for u, t in enumerate(ts):
            mod_store(jnp.broadcast_to(jnp.sum(acc[u], axis=0, keepdims=True), (M, 128)), t)

    def wm_copy(it, u):
        col = pl.multiple_of((2 * NT + it * mt + u) * 128, 128)
        return pltpu.make_async_copy(wmod_hbm.at[:, pl.ds(col, 128)], wm_s.at[it & 3, u],
                                     sem_m.at[it & 3])

    def ln1(x, zero=None):
        x3 = x.astype(F32).reshape(x.shape[0] // 8, 8, D)
        zf = None if zero is None else pltpu.bitcast(zero, F32)
        if LATE_APPLY:
            return _ln(x3, zf, LEAN).reshape(x.shape[0], D).astype(BF16)
        return _ln_mod(x3, modv(1), modv(0), zf, LEAN).reshape(x.shape[0], D).astype(BF16)

    def zero_after(y):
        return (y if y.dtype == U32 else pltpu.bitcast(y, U32)) & zero_s[0:8, :]

    def or_tile(u, z):
        if z is None:
            return u
        return (u.reshape(u.shape[0] // 8, 8, 128) | z).reshape(u.shape)

    def prologue(stage, wo_raw, wmod_s, nrm, ha, hb, tmp, mem0_ref, wr_ref, c_ref, sem):
        w_hbms = (wq_hbm, wk_hbm, wv_hbm)
        wob = H * DH // NT
        S_X, S_C0, S_ST, S_WO, S_MOD, S_SM = 0, 2, 6, 6 + NSLOT, 6 + NSLOT + NT, 6 + NSLOT + 2 * NT

        def x_copy(i):
            lo, n = ((XR, M), (0, XR))[i]
            return pltpu.make_async_copy(x_hbm.at[:, pl.ds(lo, n), :], xbuf.at[:, pl.ds(lo, n), :],
                                         sem.at[S_X + i])

        def mod_copies(k):
            return [pltpu.make_async_copy(wmod_hbm.at[:, pl.ds(v * D + k * 128, 128)],
                                          wmod_s.at[k, v], sem.at[S_MOD + (k if k < 2 else k & 6)])
                    for v in range(2)]

        def chunk_copy(mat, d0, g, slot, k):
            return pltpu.make_async_copy(w_hbms[mat].at[pl.ds(d0, KQ), pl.ds(g * CH, CH), :],
                                         stage.at[slot, g], sem.at[k])

        def wo_copy(j):
            return pltpu.make_async_copy(wo_hbm.at[pl.ds(pl.multiple_of(j * wob, wob), wob)],
                                         wo_raw.at[j], sem.at[S_WO + j])

        def relayout1(src, t0, z=None):
            v = src.reshape(RB * CH, 128)
            tmp[t0:t0 + RB * CH // 2, :] = or_tile(_as_u32(v), z)

        def relayout2(c, h0_, t0, d0, z=None):
            w = or_tile(tmp[pl.ds(t0, RB2, stride=CH // 2), :], z)
            rows = pl.ds(d0 // 2, RB2 // 2)
            wqkv[c, h0_, rows, :] = _as_u32(w.astype(jnp.uint16))
            wqkv[c, h0_ + 1, rows, :] = _as_u32((w >> 16).astype(jnp.uint16))

        def mod_pair(k):
            for v in range(2):
                mod_tile(wmod_s[k, v], v * NT + k)

        def fill(dst, q, t, r, z=None):
            k = 2 * q + t
            sh = mod[k] if z is None else mod[k] + pltpu.bitcast(z, F32)
            v = nrm[k, r:r + FB, :].reshape(FB // 8, 8, 128) * mod[NT + k] + sh
            dst[t, r // 2:(r + FB) // 2, :] = _as_u32(v.reshape(FB, 128).astype(BF16))

        small = [pltpu.make_async_copy(src, dst, sem.at[S_SM])
                 for src, dst in ((c_hbm, c_ref), (mem0_hbm, mem0_ref), (wr_hbm, wr_ref))]
        for cp in small:
            cp.start()
        x_copy(0).start()
        for cp in mod_copies(0) + mod_copies(1):
            cp.start()
        for g in range(4):
            chunk_copy(0, 0, g, 0, S_C0 + g).start()
        for c in range(1, NSLOT):
            for g in range(4):
                chunk_copy(c % 3, (c // 3) * KQ, g, c, S_ST + c).start()
            for cp in mod_copies(2 * c) + mod_copies(2 * c + 1):
                cp.start()

        def decode(i):
            lo = i < 2 * SEG
            head = jnp.where(lo, i // SEG, (i - 2 * SEG) // M)
            is_mem = jnp.logical_and(lo, i % SEG >= XR)
            pos = jnp.where(lo, i % SEG, XR + i % M)
            return head, is_mem, pos

        qh, qm, qp = decode(lax.broadcasted_iota(jnp.int32, (PR, PR), 0))
        kh, km, kp = decode(lax.broadcasted_iota(jnp.int32, (PR, PR), 1))
        vis = qm | km | (qp >= kp)
        if TR_MODE:
            kk = lax.broadcasted_iota(jnp.int32, (SEG + M, PR), 0)
            _, qm2, qp2 = decode(lax.broadcasted_iota(jnp.int32, (SEG + M, PR), 1))
            km2 = jnp.logical_and(kk >= XR, kk < SEG)
            kp2 = jnp.where(kk < SEG, kk, kk - M)
            mk[0:SEG + M, :] = jnp.where(qm2 | km2 | (qp2 >= kp2), 0.0, 1.0).astype(F32)
        if not TR_MODE: mk[0:PR, :] = jnp.where(qh == kh, jnp.where(vis, 0.0, NEG_MASK * LOG2E), -jnp.inf).astype(F32)
        mod[0:2 * NT] = jnp.zeros((2 * NT, M, 128), F32)
        zero_s[...] = jnp.zeros(zero_s.shape, U32)
        top[...] = jnp.full(top.shape, jnp.iinfo(jnp.int32).min, jnp.int32)
        for cp in small:
            cp.wait()
        wr = jnp.broadcast_to(wr_ref[...].astype(F32).reshape(1, D), (M, D))
        for k in range(NT):
            mod[6 * NT + k] = wr[:, k * 128:(k + 1) * 128]
        cv = c_ref[...].astype(F32)
        sc = _rb(cv * _rb(jax.nn.sigmoid(cv)))
        sc_s[...] = jnp.broadcast_to(sc, (M, D)).astype(BF16)
        for k in range(NT):
            cb_s[k * 128:(k + 1) * 128, :] = jnp.broadcast_to(
                sc[:, k * 128:(k + 1) * 128], (128, 128)).T
        mb = mem0_ref[...]
        for k in range(NT):
            lhs[0, k, XR // 2:, :] = _as_u32(mb[:, k * 128:(k + 1) * 128])

        def zero_body(i, c):
            wo_raw[NT, pl.ds(pl.multiple_of(i * 32, 32), 32), :] = jnp.zeros((32, D), BF16)
            return c

        lax.fori_loop(0, wob // 32, zero_body, 0)
        x_copy(0).wait()

        def ln_body(i, c):
            for u in range(LNU):
                q = i * LNU + u
                v = _ln(xbuf[q, XR:, :].astype(F32))
                for k in range(NT):
                    nrm[k, pl.ds(pl.multiple_of(q * 8, 8), 8), :] = v[:, k * 128:(k + 1) * 128]
            return c

        with jax.named_scope("p_ln"):
            lax.fori_loop(0, NSEG // LNU, ln_body, 0)

        def mod_body(k, c):
            pltpu.make_async_copy(wmod_s.at[k], wmod_s.at[k], sem.at[S_MOD + k]).wait()
            mod_pair(k)
            for r in range(0, R0, FB):
                fill(ha, 0, k, r)
            return c

        with jax.named_scope("p_mod"):
            lax.fori_loop(0, 2, mod_body, 0)

        def c0_body(g):
            chunk_copy(0, 0, 0, 0, S_C0 + g).wait()
            for d0 in range(0, KQ, RB):
                relayout1(stage[0, g, d0:d0 + RB], d0 * CH // 2)
            for j in range(CH // 2):
                for d0 in range(0, KQ, RB2):
                    relayout2(0, g * CH + 2 * j, d0 * CH // 2 + j, d0)

        def bulk(units, jobs, inserts):
            due = {}
            t0 = 0
            for n, (hq, c, h0_, pi, first, r0, nrow) in enumerate(units):
                nb = nrow // BLK
                parts = []
                for u in range(nb):
                    part = hq[0, (r0 + u * BLK) // 2:(r0 + (u + 1) * BLK) // 2, :]
                    for z in due.pop(t0 + u, ()):
                        part = jnp.concatenate([part[0:8] | z, part[8:]], axis=0)
                    parts.append(part)
                hv = jnp.concatenate([_as_bf16(jnp.concatenate(parts, axis=0)),
                                      _as_bf16(hq[1, r0 // 2:(r0 + nrow) // 2, :])], axis=1)
                w = jnp.concatenate([_as_bf16(wqkv[c, h0_]), _as_bf16(wqkv[c, h0_ + 1])], axis=1)
                y = _dot(hv, w)
                segs = slice(r0 // M, (r0 + nrow) // M)
                for a in range(2):
                    old = jnp.where(first, 0.0, pre[pi, segs, a * M:(a + 1) * M, :])
                    pre[pi, segs, a * M:(a + 1) * M, :] = (
                        y[:, a * DH:(a + 1) * DH].reshape(nrow // M, M, DH) + old)
                for fn in inserts.get(n, ()):
                    fn()
                for u in range(nb):
                    for job in jobs.get(t0 + u, ()):
                        res = job(zero_after(y[u * BLK:u * BLK + 8, 0:128]))
                        if res is not None:
                            due.setdefault(max(t0 + u + JOB_SPAN, t0 + nb), []).append(
                                zero_after(res))
                t0 += nb
            assert not due

        GP = CH // 2
        WO0 = NCHUNK - 1 - NT
        LN0 = 4
        SPI = -(-NSEG // (NCHUNK - 1 - LN0))

        def rot_body(i, c):
            slot = (i + 1) & (NSLOT - 1)
            pltpu.make_async_copy(stage.at[slot], stage.at[slot], sem.at[S_ST + slot]).wait()
            km = 2 * jnp.minimum(i, 3)

            @pl.when(jnp.logical_and(i >= 1, i <= 3))
            def _():
                wq = wmod_s.at[pl.ds(km, 2)]
                pltpu.make_async_copy(wq, wq, sem.at[S_MOD + km]).wait()

            @pl.when(i == LN0)
            def _():
                x_copy(1).wait()

            @pl.when(i >= WO0)
            def _():
                wo_copy(i - WO0).wait()

            nxt = i + NSLOT
            qn = (nxt * 43) >> 7
            for mat in range(3):
                @pl.when(jnp.logical_and(nxt < NCHUNK, nxt - 3 * qn == mat))
                def _():
                    for g in range(4):
                        chunk_copy(mat, qn * KQ, g, nxt & (NSLOT - 1),
                                   S_ST + (nxt & (NSLOT - 1))).start()

            @pl.when(i < NT)
            def _():
                wo_copy(i).start()

            @pl.when(i == 0)
            def _():
                x_copy(1).start()

            q0 = (i * 43) >> 7
            q1 = ((i + 1) * 43) >> 7
            pa = (i - 3 * q0) * NP + NP - GP
            units = ([(ha, i, H - CH + 2 * n, pa + n, q0 == 0, 0, R0) for n in range(GP)]
                     + [(hb, i + 1, 2 * n, (i + 1 - 3 * q1) * NP + n, q1 == 0, 0, R0)
                        for n in range(NP - GP)])
            jw = jnp.where(i >= WO0, i - WO0, NT)

            def wo_job(b, z):
                v = wo_raw[jw, b * 16:(b + 1) * 16, :]
                rows = pl.ds(pl.multiple_of(jw * (wob // 2) + b * 8, 8), 8)
                for j in range(NT):
                    wo_s[j, rows, :] = _as_u32(v[:, j * 128:(j + 1) * 128]) | z

            def ln_job(b, z):
                r = (b % 3) * 8
                seg = (i - LN0) * SPI + b // 3
                live = jnp.logical_and(i >= LN0, seg < NSEG)
                src = jnp.where(live, seg, 0)
                hv = ln1(xbuf[src, pl.ds(pl.multiple_of(jnp.where(live, r, XR), 8), 8), :], z)
                u = [_as_u32(hv[:, k * 128:(k + 1) * 128]) for k in range(NT)]
                dst = jnp.where(live, seg, NSEG)
                for k in range(NT):
                    hs[dst, k, r // 2:r // 2 + 4, :] = u[k]
                res = jnp.concatenate(u[0:2], axis=0)
                for k in range(2, NT, 2):
                    res = res | jnp.concatenate(u[k:k + 2], axis=0)
                return res

            def r1_job(g, d0, z):
                relayout1(stage[slot, g, d0:d0 + RB], (g * KQ + d0) * CH // 2, z)

            def copy_job(t, r, z):
                ha[t, r:r + 32, :] = or_tile(hb[t, r:r + 32, :], z)

            P = functools.partial
            upb = R0 // BLK
            nr = NP * upb
            jobs = {}
            for g in range(4):
                lo, mid, hi = (x * upb // 4 for x in R_AT[g])
                _spread(jobs, [P(r1_job, g, d0) for d0 in range(0, KQ, RB)], lo, mid)
                _spread(jobs, [P(relayout2, i + 1, g * CH + 2 * j, (g * KQ + d0) * CH // 2 + j, d0)
                               for j in range(CH // 2) for d0 in range(0, KQ, RB2)], mid, hi)
            oz = (i >> 10) if OPAQUE else 0
            _spread(jobs, [P(fill, hb, q1, t + oz, r) for r in range(0, R0, FB) for t in range(2)],
                    F_AT[0] * upb // 4, F_AT[1] * upb // 4)
            _spread(jobs, [P(copy_job, t, r) for t in range(2) for r in range(0, R0 // 2, 32)],
                    2 * GP * upb, nr - upb)
            _spread(jobs, [P(ln_job, b) for b in range(3 * SPI)],
                    L_AT * upb // 4, nr - max(upb, JOB_SPAN))
            _spread(jobs, [P(wo_job, b) for b in range(wob // 16)], GP * upb, nr - upb)
            gv = {}

            def gv_job(d0, n, z):
                w = wmod_s[pl.ds(km, 2), :, d0:d0 + n, :].reshape(4, n, 128)
                acc = gv.get("acc")
                if z is not None:
                    zf = pltpu.bitcast(z, F32)[None]
                    acc = jnp.broadcast_to(zf, (4, 8, 128)) if acc is None else acc + zf
                gv["acc"] = gemv_part(w, d0, acc)
                if z is not None:
                    au = pltpu.bitcast(gv["acc"], U32)
                    return au[0] | au[1] | au[2] | au[3]

            _spread(jobs, [P(gv_job, d0, GVR) for d0 in range(0, D - GV_FREE, GVR)],
                    GV_AT[0] * upb // 4, min(GV_AT[1] * upb // 4, nr - JOB_SPAN))
            bulk(units, jobs, {})
            if GV_FREE:
                gv_job(D - GV_FREE, GV_FREE, None)
            gemv_finish(gv["acc"], [km, NT + km, km + 1, NT + km + 1])
            return c

        def outer(k, c):
            last = k == 4

            @pl.when(k < 4)
            def _():
                c0_body(k)

            @pl.when(k != 3)
            def _():
                g = jnp.minimum(k, 3)
                bulk([(ha, jnp.where(last, NCHUNK - 1, 0), g * CH + 2 * n,
                       jnp.where(last, 2 * NP, 0) + g * GP + n, k < 4, 0, R0)
                      for n in range(GP)], {}, {})

            @pl.when(k == 3)
            def _():
                with jax.named_scope("p_rot"):
                    lax.fori_loop(0, NCHUNK - 1, rot_body, 0)
                for it in range(2):
                    for u in range(mt):
                        wm_copy(it, u).start()

            return c

        with jax.named_scope("p_bulk"):
            lax.fori_loop(0, 5, outer, 0)

    if "pro" in PHASES: pl.run_scoped(
        prologue,
        pltpu.VMEM((NSLOT, H // CH, KQ, CH, 128), BF16),
        pltpu.VMEM((NT + 1, H * DH // NT, D), BF16),
        pltpu.VMEM((NT, 2, D, 128), BF16),
        pltpu.VMEM((NT, R0, 128), F32),
        pltpu.VMEM((2, R0 // 2 + PADS[0], 128), U32),
        pltpu.VMEM((2, R0 // 2 + PADS[0], 128), U32),
        pltpu.VMEM((D * CH // 2 + PADS[1], 128), U32),
        pltpu.VMEM((M, D), BF16),
        pltpu.VMEM((D,), BF16),
        pltpu.VMEM((1, D), BF16),
        pltpu.SemaphoreType.DMA((7 + NSLOT + 2 * NT,)),
    )

    def main(wg_s, wu_s, wd_s, ybuf, stat, outs, sem_f):
        def load_x_rows(slot, seg):
            for k in range(NT):
                if LATE_APPLY:
                    v = _as_bf16(hs[seg, k]).astype(F32).reshape(XR // 8, 8, 128)
                    v = (v * mod[NT + k] + mod[k]).reshape(XR, 128)
                    lhs[slot, k, 0:XR // 2, :] = _as_u32(v.astype(BF16))
                else:
                    lhs[slot, k, 0:XR // 2, :] = hs[seg, k]

        def resid(seg, r, z=None):
            rows = pl.ds(r, 8)
            t = modv(2) * ybuf[seg, rows, :].astype(F32)
            if z is not None:
                t = t + jnp.concatenate([pltpu.bitcast(z, F32)] * NT, axis=1)
            return xbuf[seg, rows, :].astype(F32) + t

        def wide(v):
            return jnp.concatenate([v] * NT, axis=1)

        def make_key(v, row0):
            b = pltpu.bitcast(jnp.where(v != v, -jnp.inf, v + 0.0), jnp.int32)
            low = (S - 1 - row0) - lax.broadcasted_iota(jnp.int32, (8, 128), 0)
            return (b ^ ((b >> 31) & 0x7FFF0000)) | low

        def post(seg, r, z):
            x1 = resid(seg, r, z)
            mu = jnp.mean(x1, axis=-1, keepdims=True)
            xc = x1 - mu
            inv = _inv_std(xc)
            stat[0, seg, pl.ds(r, 8), :] = jnp.broadcast_to(mu, (8, 128))
            stat[1, seg, pl.ds(r, 8), :] = jnp.broadcast_to(inv, (8, 128))
            v = _rb(inv * jnp.sum(xc * modv(7), axis=-1, keepdims=True) + mod[8 * NT])
            key = make_key(v, seg * SEG + r)
            m1, m2 = top[0:8, :], top[8:16, :]
            top[8:16, :] = jnp.maximum(m2, jnp.minimum(m1, key))
            top[0:8, :] = jnp.maximum(m1, key)
            o = x1 + modv(5) * (xc * inv * modv(4) + modv(3))
            outs[seg, pl.ds(r, 8), :] = o.astype(BF16)
            res = pltpu.bitcast(v, U32)
            for k in range(NT):
                res = res | pltpu.bitcast(o[:, k * 128:(k + 1) * 128], U32)
            return res

        def redo(seg, r, z=None):
            x1 = resid(seg, r, z)
            n = (x1 - wide(stat[0, seg, pl.ds(r, 8), :])) * wide(stat[1, seg, pl.ds(r, 8), :])
            return x1, n * modv(4) + modv(3)

        def out_copy(g0, ng, r, n, k=0):
            return pltpu.make_async_copy(outs.at[pl.ds(g0, ng), pl.ds(r, n), :],
                                         out_hbm.at[pl.ds(g0, ng), pl.ds(r, n), :], sem_out.at[k])

        late = ((wg_hbm, wg_s, FF // 128), (wu_hbm, wu_s, FF // 128), (wd_hbm, wd_s, NT))

        def col_copy(k, j):
            return pltpu.make_async_copy(
                late[k][0].at[:, pl.ds(pl.multiple_of(j * 128, 128), 128)], late[k][1].at[j],
                sem_f.at[k])

        load_x_rows(0, 0)

        def step(it, cur, state):
            s = it * UNROLL + cur
            nxt = (cur + 1) % UNROLL

            def pay(t, cost):
                now = state.get("now", 0)
                due = state.setdefault("due", [])
                for z in [z for (d, z) in due if d <= now]:
                    t = jnp.concatenate([t[0:8] | z, t[8:]], axis=0)
                state["due"] = [(d, z) for (d, z) in due if d > now]
                state["now"] = now + cost
                return t

            def owe(lag, p, tiles):
                z = tiles[0]
                for t in tiles[1:]:
                    z = z | t
                state.setdefault("due", []).append(
                    (state.get("now", 0) + lag + (p % PG) * TOK_STAG, zero_after(z)))

            def lv(k0, k1):
                ts = [lhs[cur, k] for k in range(k0, k1)]
                ts[0] = pay(ts[0], (k1 - k0) / NT)
                return jnp.concatenate([_as_bf16(t) for t in ts], axis=1)

            def wmat(mat, h, q0, q1):
                return _as_bf16(jnp.concatenate([wqkv[3 * q + mat, h] for q in range(q0, q1)],
                                                axis=0))

            def qkv(p, split=False):
                part = {}
                if split:
                    for mat in range(3):
                        for a in range(2):
                            part[mat, a] = _dot(lv(0, NT // 2), wmat(mat, 2 * p + a, 0, 2))
                for mat in range(3):
                    for a in range(2):
                        hm = mat * H + 2 * p + a
                        if split:
                            y = _dot(lv(NT // 2, NT), wmat(mat, 2 * p + a, 2, 4)) + part[mat, a]
                        else:
                            y = _dot(lv(0, NT), wmat(mat, 2 * p + a, 0, 4))
                        cur_s[hm] = y.astype(BF16)
                        release(y)

            def gather(mat, p):
                hm = mat * H + 2 * p
                return jnp.concatenate(
                    [cur_s[hm], cur_s[hm + 1], pre[mat * NP + p, s].astype(BF16)], axis=0)

            probs = {}

            def scores_t(p):
                st = lax.dot_general(gather(1, p), gather(0, p), (((1,), (1,)), ((), ())),
                                     preferred_element_type=F32)
                lane = lax.broadcasted_iota(jnp.int32, (1, PR), 1)
                is_a = jnp.logical_or(lane < SEG,
                                      jnp.logical_and(lane >= 2 * SEG, lane < 2 * SEG + M))
                ka = jnp.concatenate([st[0:SEG], st[2 * SEG:2 * SEG + M]], axis=0)
                kb = jnp.concatenate([st[SEG:2 * SEG], st[2 * SEG + M:]], axis=0)
                t = jnp.where(is_a, ka, kb) * (SCALE * LOG2E)
                t = jnp.where(mk[0:SEG + M, :] == 0.0, t, NEG_MASK * LOG2E)
                if REL_S is None:
                    return softmax_t(p, is_a, t)
                ts_s[p + (it >> 10)] = t

                def later(z):
                    zf = pltpu.bitcast(z, F32)[:, 0:PR]
                    t2 = (ts_s[p].reshape(-1, 8, PR) + zf).reshape(SEG + M, PR)
                    softmax_t(p, is_a, t2)

                state.setdefault("pend", []).append(
                    (state.get("now", 0) + REL_S + (p % PG) * REL_STAG, later))

            def release(y):
                now = state.get("now", 0)
                pend = state.get("pend", [])
                state["pend"] = [(d, f) for (d, f) in pend if d > now]
                for (d, f) in pend:
                    if d <= now:
                        f(zero_after(y[0:8]))

            def softmax_t(p, is_a, t):
                e = jnp.exp2(t - jnp.max(t, axis=0, keepdims=True))
                e = e * _recip(jnp.sum(e, axis=0, keepdims=True))
                pa = jnp.where(is_a, e, 0.0)
                pb = jnp.where(is_a, 0.0, e)
                pt = jnp.concatenate([pa[0:SEG], pb[0:SEG], pa[SEG:], pb[SEG:]], axis=0)
                if TOK_S is not None:
                    eu = pltpu.bitcast(e, U32)
                    z = eu[0:8]
                    for k in range(1, (SEG + M) // 8):
                        z = z | eu[k * 8:(k + 1) * 8]
                    owe(TOK_S, p, [jnp.concatenate([z, jnp.zeros((8, 128 - PR), U32)], axis=1)])
                probs[p] = (pt.astype(BF16), "t")

            def scores(p):
                sc = lax.dot_general(gather(0, p), gather(1, p), (((1,), (1,)), ((), ())),
                                     preferred_element_type=F32)
                mv = mk[0:PR, :]
                sc = jnp.where(mv == 0.0, sc * (SCALE * LOG2E), mv)
                e = jnp.exp2(sc - jnp.max(sc, axis=-1, keepdims=True))
                inv = _recip(jnp.sum(e, axis=-1, keepdims=True))
                if NORM_PRE:
                    e = e * inv
                    if TOK_S is not None:
                        eu = pltpu.bitcast(e, U32)
                        z = eu[0:8]
                        for k in range(1, PR // 8):
                            z = z | eu[k * 8:(k + 1) * 8]
                        owe(TOK_S, p, [jnp.concatenate([z, jnp.zeros((8, 128 - PR), U32)], axis=1)])
                    probs[p] = (e.astype(BF16), None)
                else:
                    if TOK_S is not None:
                        iu = pltpu.bitcast(jnp.broadcast_to(inv, (PR, 128)), U32)
                        owe(TOK_S, p, [iu[k * 8:(k + 1) * 8] for k in range(PR // 8)])
                    probs[p] = (e.astype(BF16), inv)

            def pv(p):
                e, inv = probs.pop(p)
                if isinstance(inv, str):
                    o = lax.dot_general(e, gather(2, p), (((0,), (0,)), ((), ())),
                                        preferred_element_type=F32)
                else:
                    o = _dot(e, gather(2, p))
                    if inv is not None:
                        o = o * inv
                o = o.astype(BF16)
                if TOK_P is not None:
                    ou = _as_u32(o)
                    owe(TOK_P, p, [ou[k * 8:(k + 1) * 8] for k in range(PR // 16)])
                for a in range(2):
                    h = 2 * p + a
                    olhs[h] = _as_u32(o[a * SEG:(a + 1) * SEG])
                    odef[h, it, cur * 4:(cur + 1) * 4, :] = _as_u32(
                        o[2 * SEG + a * M:2 * SEG + (a + 1) * M])

            acc = [None] * NT

            def oproj(j, pairs):
                ts = [olhs[2 * p + a] for p in pairs for a in range(2)]
                ts[0] = pay(ts[0], len(pairs) / 4)
                ov = jnp.concatenate([_as_bf16(t) for t in ts], axis=1)
                w = wo_s[j, pairs[0] * DH:(pairs[-1] + 1) * DH, :]
                y = _dot(ov, _as_bf16(w))
                acc[j] = y if acc[j] is None else y + acc[j]
                release(acc[j])

            def fin(j):
                yb = acc[j].astype(BF16)
                ybuf[s, 0:XR, j * 128:(j + 1) * 128] = yb[0:XR]
                lhs[nxt, j, XR // 2:, :] = _as_u32(yb[XR:])

            def gemv():
                d0 = state.get("d0", 0)
                state["acc"] = gemv_part(wm_s[it & 3, :, d0:d0 + GR, :], d0, state.get("acc"))
                state["d0"] = d0 + GR
                au = pltpu.bitcast(state["acc"], U32)
                owe(G_LAG, 0, [au[u] for u in range(mt)])

            def late_mod(u):
                mod_tile(wm_s[it & 3, u], 2 * NT + it * mt + u)

            load_x_rows(nxt, jnp.minimum(s + 1, NSEG - 1))
            ops = dict(Q=qkv, S=scores_t if TR_MODE else scores, P=pv, O=oproj, F=fin, M=late_mod, G=gemv)
            for op in _schedule([(u, q) for u, (c_, q) in enumerate(MODS[:mt])
                                 if c_ % UNROLL == cur and not VPU_MOD]):
                ops[op[0]](*op[1:])

        def steps(it, carry):
            if "pro" in PHASES:
                pltpu.make_async_copy(wm_s.at[it & 3], wm_s.at[it & 3], sem_m.at[it & 3]).wait()

                @pl.when(it + 2 < NSEG // UNROLL)
                def _():
                    for u in range(mt):
                        wm_copy(it + 2, u).start()

            for u in range(UNROLL // 2):
                t = it * (UNROLL // 2) + u
                for k in range(3):
                    @pl.when(t < late[k][2])
                    def _():
                        col_copy(k, t).start()

            state = {}
            for u in range(UNROLL):
                step(it, u, state)
            if VPU_MOD:
                acc = state.get("acc")
                for d0 in range(state.get("d0", 0), D, 64):
                    acc = gemv_part(wm_s[it & 3, :, d0:d0 + 64, :], d0, acc)
                gemv_finish(acc, [2 * NT + it * mt + u for u in range(mt)])
            return carry

        with jax.named_scope("m_steps"):
            if "step" in PHASES: lax.fori_loop(0, NSEG // UNROLL, steps, 0)
        for k in range(3):
            for j in range(late[k][2]):
                col_copy(k, j).wait()
        if "epi" not in PHASES:
            return

        ntail = EBLK[-1] // M
        ppi = (S // 8 - ntail) // NEC
        gpi = ppi // (XR // 8)
        gb_ = UNROLL * M

        def ep_body(i, c):
            @pl.when(i > 0)
            def _():
                out_copy((i - 1) * gpi, gpi, 0, XR).start()

            for k in range(NT):
                mod[7 * NT + k] = mod[4 * NT + k] * mod[6 * NT + k]
            mod[8 * NT] = jnp.broadcast_to(
                jnp.sum(modv(3) * modv(6), axis=-1, keepdims=True), (M, 128))

            subs = []
            r0 = 0
            for nr in EBLK:
                kh = EKH * EC // nr if EC % nr == 0 else EKH
                for j in range(NT):
                    for h0_ in range(0, H, kh):
                        subs.append((r0, nr, j, h0_, kh))
                r0 += nr
            tot = sum(nr * kh for (_, nr, _, _, kh) in subs)
            span = E_SPAN * EC * EKH
            rel = [u * (tot - span) // ppi for u in range(ppi)]
            ready = {}
            due = []
            now = 0
            u = 0
            y = None
            for (r0, nr, j, h0_, kh) in subs:
                blk = pl.ds(i * (EC // gb_) + r0 // gb_, nr // gb_)
                ts = [odef[h, blk].reshape(nr // 2, DH) for h in range(h0_, h0_ + kh)]
                for z in [z for (d, z) in due if d <= now]:
                    ts[0] = jnp.concatenate([ts[0][0:8] | z, ts[0][8:]], axis=0)
                due = [(d, z) for (d, z) in due if d > now]
                w = wo_s[j, h0_ * DH // 2:(h0_ + kh) * DH // 2, :]
                yp = _dot(jnp.concatenate([_as_bf16(t) for t in ts], axis=1), _as_bf16(w))
                y = yp if h0_ == 0 else yp + y
                if h0_ + kh == H:
                    ybuf[pl.ds(i * (EC // M) + r0 // M, nr // M), XR:, j * 128:(j + 1) * 128] = (
                        y.reshape(nr // M, M, 128).astype(BF16))
                    if j == NT - 1:
                        ready[r0] = True
                start = now
                now += nr * kh
                while u < ppi and rel[u] < now:
                    d = (NEC - 1) * ppi + u - NSEG * (XR // 8) - (NEC - 1) * (EC // M)
                    if d >= 0 and sum(n for r, n in zip(_cumsum(EBLK), EBLK) if r in ready) <= d * M:
                        break
                    t = i * ppi + u
                    early = t < NSEG * (XR // 8)
                    seg = jnp.where(early, t // (XR // 8), t - NSEG * (XR // 8))
                    row = pl.multiple_of(jnp.where(early, (t % (XR // 8)) * 8, XR), 8)
                    res = post(seg, row, zero_after(y[0:8]))
                    due.append((start + span, zero_after(res)))
                    u += 1
            assert u == ppi
            return c

        with jax.named_scope("e_loop"):
            lax.fori_loop(0, NEC, ep_body, 0)
        done = (NEC - 1) * gpi
        tail = NSEG - ntail
        out_copy(done, NSEG - done, 0, XR).start()
        out_copy(0, tail, XR, M).start()
        x1s = [resid(g, XR) for g in range(tail, NSEG)]
        mus = [jnp.mean(x1, axis=-1, keepdims=True) for x1 in x1s]
        pairs = [(top[0:8, :], top[8:16, :])]
        lowest = jnp.full((8, 128), jnp.iinfo(jnp.int32).min, jnp.int32)
        for g in range(tail, NSEG):
            xc = x1s[g - tail] - mus[g - tail]
            inv = _inv_std(xc)
            stat[0, g, XR:, :] = jnp.broadcast_to(mus[g - tail], (8, 128))
            stat[1, g, XR:, :] = jnp.broadcast_to(inv, (8, 128))
            v = _rb(inv * jnp.sum(xc * modv(7), axis=-1, keepdims=True) + mod[8 * NT])
            pairs.append((make_key(v, g * SEG + XR), lowest))
        while len(pairs) > 1:
            (a1, a2), (c1, c2) = pairs.pop(0), pairs.pop(0)
            pairs.append((jnp.maximum(a1, c1),
                          jnp.maximum(jnp.minimum(a1, c1), jnp.maximum(a2, c2))))

        tk = jnp.concatenate(pairs[0], axis=0)[:, 0:1]
        k1 = jnp.max(tk[0:8], axis=0, keepdims=True)
        k2 = jnp.max(jnp.where(tk == k1, jnp.iinfo(jnp.int32).min, tk), axis=0, keepdims=True)
        i1 = (S - 1) - (k1[0, 0] & (S - 1))
        i2 = (S - 1) - (k2[0, 0] & (S - 1))
        g1, g2 = i1 >> 5, i2 >> 5
        b1 = pl.multiple_of(i1 & 24, 8)
        b2 = pl.multiple_of(i2 & 24, 8)

        xa, ha_ = redo(g1, b1)
        xb_, hb_ = redo(g2, b2)
        x1 = jnp.concatenate([xa, xb_], axis=0)
        h2 = jnp.concatenate([ha_, hb_], axis=0)
        h2b = h2.astype(BF16)
        row = lax.broadcasted_iota(jnp.int32, (16, 1), 0)
        grow = jnp.where(row < 8, g1 * SEG + b1 + row, g2 * SEG + b2 + row - 8)
        ks = jnp.where(grow == i1, k1, k2)
        rsel = pltpu.bitcast((ks ^ ((ks >> 31) & 0x7FFF0000)) & -65536, F32)
        acts = []
        for j in range(FF // 128):
            gt = _rb(_dot(h2b, wg_s[j]))
            gt = _rb(gt * _rb(jax.nn.sigmoid(gt)))
            ut = _rb(_dot(h2b, wu_s[j]))
            acts.append((gt * ut).astype(BF16))
            if j < ntail:
                xo_, ho_ = redo(tail + j, XR, zero_after(ut[0:8]))
                outs[tail + j, XR:, :] = (xo_ + modv(5) * ho_).astype(BF16)
            if j == ntail - 1:
                out_copy(tail, NSEG - tail, XR, M).start()
        act = jnp.concatenate(acts, axis=1)
        y = _rb(jnp.concatenate([_dot(act, wd_s[j]) for j in range(NT)], axis=1))
        y = _rb(y * _rb(jax.nn.sigmoid(rsel)))
        sel = jnp.logical_or(grow == i1, grow == i2)
        gb2 = jnp.concatenate([modv(5)] * 2, axis=0)
        fixed = (x1 + gb2 * (h2 + jnp.where(sel, y, 0.0))).astype(BF16)

        with jax.named_scope("e_outwait"):
            out_copy(0, NSEG, 0, SEG).wait()
        outs[g1, pl.ds(b1, 8), :] = fixed[0:8]
        outs[g2, pl.ds(b2, 8), :] = fixed[8:16]
        out_copy(g1, 1, b1, 8, 0).start()

        @pl.when((i1 >> 3) != (i2 >> 3))
        def _():
            out_copy(g2, 1, b2, 8, 1).start()
            out_copy(g2, 1, b2, 8, 1).wait()

        out_copy(g1, 1, b1, 8, 0).wait()

    pl.run_scoped(
        main,
        pltpu.VMEM((FF // 128, D, 128), BF16),
        pltpu.VMEM((FF // 128, D, 128), BF16),
        pltpu.VMEM((NT, FF, 128), BF16),
        pltpu.VMEM((NSEG, SEG, D), BF16),
        pltpu.VMEM((2, NSEG, SEG, 128), F32),
        pltpu.VMEM((NSEG, SEG, D), BF16),
        pltpu.SemaphoreType.DMA((3,)),
    )


def _entry(*refs):
    pl.run_scoped(
        functools.partial(_kernel, *refs),
        pltpu.VMEM((NCHUNK, H, KQ // 2, DH), U32),
        pltpu.VMEM((NSEG + 1, NT, XR // 2, 128), U32),
        pltpu.VMEM((NT, (H * DH + H * DH // NT) // 2, 128), U32),
        pltpu.VMEM((3 * NP, NSEG, 2 * M, DH), F32),
        pltpu.VMEM((3 * H, SEG, DH), BF16),
        pltpu.VMEM((H, SEG // 2, DH), U32),
        pltpu.VMEM((H, NSEG // UNROLL, UNROLL * M // 2, DH), U32),
        pltpu.VMEM((NSEG, SEG, D), BF16),
        pltpu.VMEM((UNROLL, NT, SEG // 2, 128), U32),
        pltpu.VMEM((4, 4 * NT * UNROLL // NSEG, D, 128), BF16),
        pltpu.VMEM((8 * NT + 4, M, 128), F32),
        pltpu.VMEM((96, PR), F32),
        pltpu.VMEM((32, 128), jnp.int32),
        pltpu.VMEM((M, D), BF16),
        pltpu.VMEM((D, 128), F32),
        pltpu.VMEM((NP, SEG + M, PR), F32),
        pltpu.VMEM((8 + PADS[2], 128), U32),
        pltpu.SemaphoreType.DMA((4,)),
        pltpu.SemaphoreType.DMA((2,)),
    )


@functools.partial(jax.jit, static_argnames=("A_seg_len",))
def pallas_adaLN_cond__memory_aug_recurrent_mem_tr__moe_arch_mod__prompt_kernel(
    A_x: jax.Array,
    A_mem0: jax.Array,
    A_Wq: jax.Array,
    A_Wk: jax.Array,
    A_Wv: jax.Array,
    A_Wo: jax.Array,
    A_seg_len,
    B_x: jax.Array,
    B_w_r: jax.Array,
    B_w_gate: jax.Array,
    B_w_up: jax.Array,
    B_w_down: jax.Array,
    c: jax.Array,
    w_mod: jax.Array,
):
    assert A_seg_len == SEG and A_x.shape == (1, S, D)
    del B_x
    hbm = pl.BlockSpec(memory_space=pl.ANY)
    out = pl.pallas_call(
        _entry,
        out_shape=jax.ShapeDtypeStruct((NSEG, SEG, D), BF16),
        in_specs=[hbm] * 12,
        out_specs=hbm,
        compiler_params=pltpu.CompilerParams(vmem_limit_bytes=120 * 1024 * 1024,
                                             disable_bounds_checks=True),
    )(A_x.reshape(NSEG, SEG, D), A_mem0.reshape(M, D), A_Wq, A_Wk, A_Wv, A_Wo.reshape(H * DH, D),
      B_w_r, B_w_gate, B_w_up, B_w_down, c, w_mod)
    return out.reshape(1, S, D)
```

```python
import functools

import jax
import jax.numpy as jnp
from jax import lax
import jax.experimental.pallas as pl
import jax.experimental.pallas.tpu as pltpu

F32 = jnp.float32
BF16 = jnp.bfloat16
U32 = jnp.uint32

D = 1024
S = 2048
H = 32
DH = 128
M = 8
SEG = 32
NSEG = S // SEG
FF = 3584
NT = D // 128
XR = SEG - M
R0 = M * NSEG
CH = 8
KQ = D // 4
NCHUNK = 3 * D // KQ
NSLOT = 4
PR = 2 * SEG + 2 * M
NP = H // 2
EC = 128
NEC = R0 // EC
LOG2E = 1.4426950408889634
EPS = 1e-5
SCALE = DH ** -0.5
NEG_MASK = -1000000000.0

PHASES = ("pro", "step", "epi")
UNROLL = 4
FB = 32
BLK = 32
R_AT = ((0, 6, 16), (14, 22, 30), (30, 38, 46), (44, 52, 60))
F_AT = (0, 13)
L_AT = 8
VPU_MOD = True
REL_S = 2
REL_STAG = 2
PG = 4
LAG_S = 1
LAG_P = 4
O_PARTS = (0, 8, 12)
O_TH = (256, 256, 256, 1216)
TR_MODE = "bf16"
G_AT = (0, 1, 2, 3)
GR = 32
GV_AT = (16, 56)
GVR = 32
GV_FREE = 64
G_LAG = 2
OPAQUE = True
LATE_APPLY = False
LEAN = False
RB = 16
RB2 = 64
JOB_SPAN = 40
LNU = 16
EKH = 4
E_SPAN = 5
EBLK = (128,)
PADS = (0, 0, 24)
MODS = ((-1, 4), (1, 4))
TOK_S = None
TOK_P = None
TOK_STAG = 2
NORM_PRE = True
R1_END = 11
R2_0 = (3, 14)
LN_RANGE = (0, 29)
WO_RANGE = (12, 31)


def _schedule(mods):
    groups = [list(range(g, g + PG)) for g in range(0, NP, PG)]
    at = {}
    for g, grp in enumerate(groups):
        at.setdefault(grp[-1] + LAG_P, []).extend(("P", q) for q in grp)
    for g, grp in enumerate(groups):
        at.setdefault(grp[-1] + LAG_S, []).extend(("S", q) for q in grp)
    ops = []
    for p in range(NP):
        ops.append(("Q", p, p == 0))
        if p in G_AT:
            ops.append(("G",))
        ops.extend(at.pop(p, []))
    bounds = list(O_PARTS) + [NP]
    t = NP
    done = 0
    for n in range(len(O_PARTS)):
        part = list(range(bounds[n], bounds[n + 1]))
        assert all(("P", q) in ops for q in part), (n, ops)
        for j in range(NT):
            ops.append(("O", j, part))
            if n == len(O_PARTS) - 1:
                ops.append(("F", j))
            done += len(part) * 16
            while t - NP < len(O_TH) and done >= O_TH[t - NP]:
                ops.extend(at.pop(t, []))
                t += 1
    assert not at
    return ops


def _rb(x):
    return x.astype(BF16).astype(F32)


def _recip(x):
    r = pl.reciprocal(x, approx=True)
    return r * (2.0 - x * r)


def _inv_std(xc):
    v = _rb(_rb(jnp.mean(xc * xc, axis=-1, keepdims=True)) + EPS)
    return _recip(_rb(v * lax.rsqrt(v)))


def _ln(x, zero=None, lean=False):
    xm = x if zero is None else jnp.concatenate([x[..., :128] + zero, x[..., 128:]], axis=-1)
    mu = jnp.mean(xm, axis=-1, keepdims=True)
    xc = x - mu
    v = _rb(_rb(jnp.mean(xc * xc, axis=-1, keepdims=True)) + EPS)
    inv = _recip(_rb(v * lax.rsqrt(v)))
    if lean:
        return x * inv - mu * inv
    return xc * inv


def _ln_mod(x, s1p, shift, zero=None, lean=False):
    return _ln(x, zero, lean) * s1p + shift


def _dot(a, b):
    return jnp.dot(a, b, preferred_element_type=F32)


def _as_bf16(u):
    return pltpu.bitcast(u, BF16)


def _as_u32(b):
    return pltpu.bitcast(b, U32)


def _cumsum(xs):
    out, r = [], 0
    for x in xs:
        out.append(r)
        r += x
    return out


def _spread(jobs, fns, lo, hi):
    for n, fn in enumerate(fns):
        jobs.setdefault(lo + n * (hi - lo) // len(fns), []).append(fn)


def _kernel(x_hbm, mem0_hbm, wq_hbm, wk_hbm, wv_hbm, wo_hbm, wr_hbm, wg_hbm, wu_hbm, wd_hbm,
            c_hbm, wmod_hbm, out_hbm,
            wqkv, hs, wo_s, pre, cur_s, olhs, odef, xbuf, lhs, wm_s, mod, mk,
            top, sc_s, cb_s, ts_s, zero_s, sem_m, sem_out):
    mt = 4 * NT * UNROLL // NSEG

    def modv(j):
        return jnp.concatenate([mod[j * NT + k] for k in range(NT)], axis=1)

    def mod_store(v, t):
        v = _rb(v)
        mod[t] = jnp.where(jnp.logical_or((t >> 3) == 1, (t >> 3) == 4), _rb(1.0 + v), v)

    def mod_tile(wm, t):
        mod_store(_dot(sc_s[...], wm), t)

    def gemv_part(w, d0, acc):
        n = w.shape[1]
        p = w.astype(F32) * cb_s[d0:d0 + n, :]
        p = jnp.sum(p.reshape(w.shape[0], n // 8, 8, 128), axis=1)
        return p if acc is None else p + acc

    def gemv_finish(acc, ts):
        for u, t in enumerate(ts):
            mod_store(jnp.broadcast_to(jnp.sum(acc[u], axis=0, keepdims=True), (M, 128)), t)

    def wm_copy(it, u):
        col = pl.multiple_of((2 * NT + it * mt + u) * 128, 128)
        return pltpu.make_async_copy(wmod_hbm.at[:, pl.ds(col, 128)], wm_s.at[it & 3, u],
                                     sem_m.at[it & 3])

    def ln1(x, zero=None):
        x3 = x.astype(F32).reshape(x.shape[0] // 8, 8, D)
        zf = None if zero is None else pltpu.bitcast(zero, F32)
        if LATE_APPLY:
            return _ln(x3, zf, LEAN).reshape(x.shape[0], D).astype(BF16)
        return _ln_mod(x3, modv(1), modv(0), zf, LEAN).reshape(x.shape[0], D).astype(BF16)

    def zero_after(y):
        return (y if y.dtype == U32 else pltpu.bitcast(y, U32)) & zero_s[0:8, :]

    def or_tile(u, z):
        if z is None:
            return u
        return (u.reshape(u.shape[0] // 8, 8, 128) | z).reshape(u.shape)

    def prologue(stage, wo_raw, wmod_s, nrm, ha, hb, tmp, mem0_ref, wr_ref, c_ref, sem):
        w_hbms = (wq_hbm, wk_hbm, wv_hbm)
        wob = H * DH // NT
        S_X, S_C0, S_ST, S_WO, S_MOD, S_SM = 0, 2, 6, 6 + NSLOT, 6 + NSLOT + NT, 6 + NSLOT + 2 * NT

        def x_copy(i):
            lo, n = ((XR, M), (0, XR))[i]
            return pltpu.make_async_copy(x_hbm.at[:, pl.ds(lo, n), :], xbuf.at[:, pl.ds(lo, n), :],
                                         sem.at[S_X + i])

        def mod_copies(k):
            return [pltpu.make_async_copy(wmod_hbm.at[:, pl.ds(v * D + k * 128, 128)],
                                          wmod_s.at[k, v], sem.at[S_MOD + (k if k < 2 else k & 6)])
                    for v in range(2)]

        def chunk_copy(mat, d0, g, slot, k):
            return pltpu.make_async_copy(w_hbms[mat].at[pl.ds(d0, KQ), pl.ds(g * CH, CH), :],
                                         stage.at[slot, g], sem.at[k])

        def wo_copy(j):
            return pltpu.make_async_copy(wo_hbm.at[pl.ds(pl.multiple_of(j * wob, wob), wob)],
                                         wo_raw.at[j], sem.at[S_WO + j])

        def relayout1(src, t0, z=None):
            v = src.reshape(RB * CH, 128)
            tmp[t0:t0 + RB * CH // 2, :] = or_tile(_as_u32(v), z)

        def relayout2(c, h0_, t0, d0, z=None, src=tmp):
            w = or_tile(src[pl.ds(t0, RB2, stride=CH // 2), :], z)
            rows = pl.ds(d0 // 2, RB2 // 2)
            wqkv[c, h0_, rows, :] = _as_u32(w.astype(jnp.uint16))
            wqkv[c, h0_ + 1, rows, :] = _as_u32((w >> 16).astype(jnp.uint16))

        def mod_pair(k):
            for v in range(2):
                mod_tile(wmod_s[k, v], v * NT + k)

        def fill(dst, q, t, r, z=None):
            k = 2 * q + t
            sh = mod[k] if z is None else mod[k] + pltpu.bitcast(z, F32)
            v = nrm[k, r:r + FB, :].reshape(FB // 8, 8, 128) * mod[NT + k] + sh
            dst[t, r // 2:(r + FB) // 2, :] = _as_u32(v.reshape(FB, 128).astype(BF16))

        small = [pltpu.make_async_copy(src, dst, sem.at[S_SM])
                 for src, dst in ((c_hbm, c_ref), (mem0_hbm, mem0_ref), (wr_hbm, wr_ref))]
        for cp in small:
            cp.start()
        x_copy(0).start()
        for cp in mod_copies(0) + mod_copies(1):
            cp.start()
        for g in range(4):
            chunk_copy(0, 0, g, 0, S_C0 + g).start()
        for c in range(1, NSLOT):
            for g in range(4):
                chunk_copy(c % 3, (c // 3) * KQ, g, c, S_ST + c).start()
            for cp in mod_copies(2 * c) + mod_copies(2 * c + 1):
                cp.start()

        def decode(i):
            lo = i < 2 * SEG
            head = jnp.where(lo, i // SEG, (i - 2 * SEG) // M)
            is_mem = jnp.logical_and(lo, i % SEG >= XR)
            pos = jnp.where(lo, i % SEG, XR + i % M)
            return head, is_mem, pos

        qh, qm, qp = decode(lax.broadcasted_iota(jnp.int32, (PR, PR), 0))
        kh, km, kp = decode(lax.broadcasted_iota(jnp.int32, (PR, PR), 1))
        vis = qm | km | (qp >= kp)
        if TR_MODE:
            kk = lax.broadcasted_iota(jnp.int32, (SEG + M, PR), 0)
            _, qm2, qp2 = decode(lax.broadcasted_iota(jnp.int32, (SEG + M, PR), 1))
            km2 = jnp.logical_and(kk >= XR, kk < SEG)
            kp2 = jnp.where(kk < SEG, kk, kk - M)
            mk[0:SEG + M, :] = jnp.where(qm2 | km2 | (qp2 >= kp2), 0.0, 1.0).astype(F32)
        if not TR_MODE: mk[0:PR, :] = jnp.where(qh == kh, jnp.where(vis, 0.0, NEG_MASK * LOG2E), -jnp.inf).astype(F32)
        mod[0:2 * NT] = jnp.zeros((2 * NT, M, 128), F32)
        zero_s[...] = jnp.zeros(zero_s.shape, U32)
        top[...] = jnp.full(top.shape, jnp.iinfo(jnp.int32).min, jnp.int32)
        for cp in small:
            cp.wait()
        wr = jnp.broadcast_to(wr_ref[...].astype(F32).reshape(1, D), (M, D))
        for k in range(NT):
            mod[6 * NT + k] = wr[:, k * 128:(k + 1) * 128]
        cv = c_ref[...].astype(F32)
        sc = _rb(cv * _rb(jax.nn.sigmoid(cv)))
        sc_s[...] = jnp.broadcast_to(sc, (M, D)).astype(BF16)
        for k in range(NT):
            cb_s[k * 128:(k + 1) * 128, :] = jnp.broadcast_to(
                sc[:, k * 128:(k + 1) * 128], (128, 128)).T
        mb = mem0_ref[...]
        for k in range(NT):
            lhs[0, k, XR // 2:, :] = _as_u32(mb[:, k * 128:(k + 1) * 128])

        def zero_body(i, c):
            wo_raw[NT, pl.ds(pl.multiple_of(i * 32, 32), 32), :] = jnp.zeros((32, D), BF16)
            return c

        lax.fori_loop(0, wob // 32, zero_body, 0)
        x_copy(0).wait()

        def ln_body(i, c):
            for u in range(LNU):
                q = i * LNU + u
                v = _ln(xbuf[q, XR:, :].astype(F32))
                for k in range(NT):
                    nrm[k, pl.ds(pl.multiple_of(q * 8, 8), 8), :] = v[:, k * 128:(k + 1) * 128]
            return c

        with jax.named_scope("p_ln"):
            lax.fori_loop(0, NSEG // LNU, ln_body, 0)

        def mod_body(k, c):
            pltpu.make_async_copy(wmod_s.at[k], wmod_s.at[k], sem.at[S_MOD + k]).wait()
            mod_pair(k)
            for r in range(0, R0, FB):
                fill(ha, 0, k, r)
            return c

        with jax.named_scope("p_mod"):
            lax.fori_loop(0, 2, mod_body, 0)

        def hop1(g):
            chunk_copy(0, 0, 0, 0, S_C0 + g).wait()

            def body(i, c):
                d0 = pl.multiple_of(i * 128, 128)
                v = stage[0, g, pl.ds(d0, 128)].reshape(128 * CH, 128)
                t0 = pl.multiple_of((g * KQ + d0) * (CH // 2), 512)
                tmp[pl.ds(t0, 128 * CH // 2), :] = _as_u32(v)
                return c

            lax.fori_loop(0, KQ // 128, body, 0)

        def hop2(c, g, j):
            src = tmp.at[pl.ds(pl.multiple_of(g * (KQ * CH // 2), 512), KQ * CH // 2)]
            for d0 in range(0, KQ, RB2):
                relayout2(c, g * CH + 2 * j, d0 * CH // 2 + j, d0, src=src)

        def bulk(units, jobs, inserts):
            due = {}
            t0 = 0
            for n, (hq, c, h0_, pi, first, r0, nrow) in enumerate(units):
                nb = nrow // BLK
                parts = []
                for u in range(nb):
                    part = hq[0, (r0 + u * BLK) // 2:(r0 + (u + 1) * BLK) // 2, :]
                    for z in due.pop(t0 + u, ()):
                        part = jnp.concatenate([part[0:8] | z, part[8:]], axis=0)
                    parts.append(part)
                hv = jnp.concatenate([_as_bf16(jnp.concatenate(parts, axis=0)),
                                      _as_bf16(hq[1, r0 // 2:(r0 + nrow) // 2, :])], axis=1)
                w = jnp.concatenate([_as_bf16(wqkv[c, h0_]), _as_bf16(wqkv[c, h0_ + 1])], axis=1)
                y = _dot(hv, w)
                segs = slice(r0 // M, (r0 + nrow) // M)
                for a in range(2):
                    old = jnp.where(first, 0.0, pre[pi, segs, a * M:(a + 1) * M, :])
                    pre[pi, segs, a * M:(a + 1) * M, :] = (
                        y[:, a * DH:(a + 1) * DH].reshape(nrow // M, M, DH) + old)
                for fn in inserts.get(n, ()):
                    fn()
                for u in range(nb):
                    for job in jobs.get(t0 + u, ()):
                        res = job(zero_after(y[u * BLK:u * BLK + 8, 0:128]))
                        if res is not None:
                            due.setdefault(max(t0 + u + JOB_SPAN, t0 + nb), []).append(
                                zero_after(res))
                t0 += nb
            assert not due

        GP = CH // 2
        WO0 = NCHUNK - 1 - NT
        LN0 = 4
        SPI = -(-NSEG // (NCHUNK - 1 - LN0))

        def rot_body(i, c):
            slot = (i + 1) & (NSLOT - 1)
            pltpu.make_async_copy(stage.at[slot], stage.at[slot], sem.at[S_ST + slot]).wait()
            km = 2 * jnp.minimum(i, 3)

            @pl.when(jnp.logical_and(i >= 1, i <= 3))
            def _():
                wq = wmod_s.at[pl.ds(km, 2)]
                pltpu.make_async_copy(wq, wq, sem.at[S_MOD + km]).wait()

            @pl.when(i == LN0)
            def _():
                x_copy(1).wait()

            @pl.when(i >= WO0)
            def _():
                wo_copy(i - WO0).wait()

            nxt = i + NSLOT
            qn = (nxt * 43) >> 7
            for mat in range(3):
                @pl.when(jnp.logical_and(nxt < NCHUNK, nxt - 3 * qn == mat))
                def _():
                    for g in range(4):
                        chunk_copy(mat, qn * KQ, g, nxt & (NSLOT - 1),
                                   S_ST + (nxt & (NSLOT - 1))).start()

            @pl.when(i < NT)
            def _():
                wo_copy(i).start()

            @pl.when(i == 0)
            def _():
                x_copy(1).start()

            q0 = (i * 43) >> 7
            q1 = ((i + 1) * 43) >> 7
            pa = (i - 3 * q0) * NP + NP - GP
            units = ([(ha, i, H - CH + 2 * n, pa + n, q0 == 0, 0, R0) for n in range(GP)]
                     + [(hb, i + 1, 2 * n, (i + 1 - 3 * q1) * NP + n, q1 == 0, 0, R0)
                        for n in range(NP - GP)])
            jw = jnp.where(i >= WO0, i - WO0, NT)

            def wo_job(b, z):
                v = wo_raw[jw, b * 16:(b + 1) * 16, :]
                rows = pl.ds(pl.multiple_of(jw * (wob // 2) + b * 8, 8), 8)
                for j in range(NT):
                    wo_s[j, rows, :] = _as_u32(v[:, j * 128:(j + 1) * 128]) | z

            def ln_job(b, z):
                r = (b % 3) * 8
                seg = (i - LN0) * SPI + b // 3
                live = jnp.logical_and(i >= LN0, seg < NSEG)
                src = jnp.where(live, seg, 0)
                hv = ln1(xbuf[src, pl.ds(pl.multiple_of(jnp.where(live, r, XR), 8), 8), :], z)
                u = [_as_u32(hv[:, k * 128:(k + 1) * 128]) for k in range(NT)]
                dst = jnp.where(live, seg, NSEG)
                for k in range(NT):
                    hs[dst, k, r // 2:r // 2 + 4, :] = u[k]
                res = jnp.concatenate(u[0:2], axis=0)
                for k in range(2, NT, 2):
                    res = res | jnp.concatenate(u[k:k + 2], axis=0)
                return res

            def r1_job(g, d0, z):
                relayout1(stage[slot, g, d0:d0 + RB], (g * KQ + d0) * CH // 2, z)

            def copy_job(t, r, z):
                ha[t, r:r + 32, :] = or_tile(hb[t, r:r + 32, :], z)

            P = functools.partial
            upb = R0 // BLK
            nr = NP * upb
            jobs = {}
            for g in range(4):
                lo, mid, hi = (x * upb // 4 for x in R_AT[g])
                _spread(jobs, [P(r1_job, g, d0) for d0 in range(0, KQ, RB)], lo, mid)
                _spread(jobs, [P(relayout2, i + 1, g * CH + 2 * j, (g * KQ + d0) * CH // 2 + j, d0)
                               for j in range(CH // 2) for d0 in range(0, KQ, RB2)], mid, hi)
            oz = (i >> 10) if OPAQUE else 0
            _spread(jobs, [P(fill, hb, q1, t + oz, r) for r in range(0, R0, FB) for t in range(2)],
                    F_AT[0] * upb // 4, F_AT[1] * upb // 4)
            _spread(jobs, [P(copy_job, t, r) for t in range(2) for r in range(0, R0 // 2, 32)],
                    2 * GP * upb, nr - upb)
            _spread(jobs, [P(ln_job, b) for b in range(3 * SPI)],
                    L_AT * upb // 4, nr - max(upb, JOB_SPAN))
            _spread(jobs, [P(wo_job, b) for b in range(wob // 16)], GP * upb, nr - upb)
            gv = {}

            def gv_job(d0, n, z):
                w = wmod_s[pl.ds(km, 2), :, d0:d0 + n, :].reshape(4, n, 128)
                acc = gv.get("acc")
                if z is not None:
                    zf = pltpu.bitcast(z, F32)[None]
                    acc = jnp.broadcast_to(zf, (4, 8, 128)) if acc is None else acc + zf
                gv["acc"] = gemv_part(w, d0, acc)
                if z is not None:
                    au = pltpu.bitcast(gv["acc"], U32)
                    return au[0] | au[1] | au[2] | au[3]

            _spread(jobs, [P(gv_job, d0, GVR) for d0 in range(0, D - GV_FREE, GVR)],
                    GV_AT[0] * upb // 4, min(GV_AT[1] * upb // 4, nr - JOB_SPAN))
            bulk(units, jobs, {})
            if GV_FREE:
                gv_job(D - GV_FREE, GV_FREE, None)
            gemv_finish(gv["acc"], [km, NT + km, km + 1, NT + km + 1])
            return c

        def outer(k, c):
            last = k == 4

            @pl.when(k < 4)
            def _():
                hop1(k)

            @pl.when(k != 3)
            def _():
                g = jnp.minimum(k, 3)
                cc = jnp.where(last, NCHUNK - 1, 0)
                for j in range(GP):
                    hop2(cc, g, j)
                bulk([(ha, cc, g * CH + 2 * n, jnp.where(last, 2 * NP, 0) + g * GP + n, k < 4,
                       0, R0) for n in range(GP)], {}, {})

            @pl.when(k == 3)
            def _():
                for j in range(GP):
                    hop2(0, 3, j)
                with jax.named_scope("p_rot"):
                    lax.fori_loop(0, NCHUNK - 1, rot_body, 0)
                for it in range(2):
                    for u in range(mt):
                        wm_copy(it, u).start()

            return c

        with jax.named_scope("p_bulk"):
            lax.fori_loop(0, 5, outer, 0)

    if "pro" in PHASES: pl.run_scoped(
        prologue,
        pltpu.VMEM((NSLOT, H // CH, KQ, CH, 128), BF16),
        pltpu.VMEM((NT + 1, H * DH // NT, D), BF16),
        pltpu.VMEM((NT, 2, D, 128), BF16),
        pltpu.VMEM((NT, R0, 128), F32),
        pltpu.VMEM((2, R0 // 2 + PADS[0], 128), U32),
        pltpu.VMEM((2, R0 // 2 + PADS[0], 128), U32),
        pltpu.VMEM((D * CH // 2 + PADS[1], 128), U32),
        pltpu.VMEM((M, D), BF16),
        pltpu.VMEM((D,), BF16),
        pltpu.VMEM((1, D), BF16),
        pltpu.SemaphoreType.DMA((7 + NSLOT + 2 * NT,)),
    )

    def main(wg_s, wu_s, wd_s, ybuf, stat, outs, sem_f):
        def load_x_rows(slot, seg):
            for k in range(NT):
                if LATE_APPLY:
                    v = _as_bf16(hs[seg, k]).astype(F32).reshape(XR // 8, 8, 128)
                    v = (v * mod[NT + k] + mod[k]).reshape(XR, 128)
                    lhs[slot, k, 0:XR // 2, :] = _as_u32(v.astype(BF16))
                else:
                    lhs[slot, k, 0:XR // 2, :] = hs[seg, k]

        def resid(seg, r, z=None):
            rows = pl.ds(r, 8)
            t = modv(2) * ybuf[seg, rows, :].astype(F32)
            if z is not None:
                t = t + jnp.concatenate([pltpu.bitcast(z, F32)] * NT, axis=1)
            return xbuf[seg, rows, :].astype(F32) + t

        def wide(v):
            return jnp.concatenate([v] * NT, axis=1)

        def make_key(v, row0):
            b = pltpu.bitcast(jnp.where(v != v, -jnp.inf, v + 0.0), jnp.int32)
            low = (S - 1 - row0) - lax.broadcasted_iota(jnp.int32, (8, 128), 0)
            return (b ^ ((b >> 31) & 0x7FFF0000)) | low

        def post(seg, r, z):
            x1 = resid(seg, r, z)
            mu = jnp.mean(x1, axis=-1, keepdims=True)
            xc = x1 - mu
            inv = _inv_std(xc)
            stat[0, seg, pl.ds(r, 8), :] = jnp.broadcast_to(mu, (8, 128))
            stat[1, seg, pl.ds(r, 8), :] = jnp.broadcast_to(inv, (8, 128))
            v = _rb(inv * jnp.sum(xc * modv(7), axis=-1, keepdims=True) + mod[8 * NT])
            key = make_key(v, seg * SEG + r)
            m1, m2 = top[0:8, :], top[8:16, :]
            top[8:16, :] = jnp.maximum(m2, jnp.minimum(m1, key))
            top[0:8, :] = jnp.maximum(m1, key)
            o = x1 + modv(5) * (xc * inv * modv(4) + modv(3))
            outs[seg, pl.ds(r, 8), :] = o.astype(BF16)
            res = pltpu.bitcast(v, U32)
            for k in range(NT):
                res = res | pltpu.bitcast(o[:, k * 128:(k + 1) * 128], U32)
            return res

        def redo(seg, r, z=None):
            x1 = resid(seg, r, z)
            n = (x1 - wide(stat[0, seg, pl.ds(r, 8), :])) * wide(stat[1, seg, pl.ds(r, 8), :])
            return x1, n * modv(4) + modv(3)

        def out_copy(g0, ng, r, n, k=0):
            return pltpu.make_async_copy(outs.at[pl.ds(g0, ng), pl.ds(r, n), :],
                                         out_hbm.at[pl.ds(g0, ng), pl.ds(r, n), :], sem_out.at[k])

        late = ((wg_hbm, wg_s, FF // 128), (wu_hbm, wu_s, FF // 128), (wd_hbm, wd_s, NT))

        def col_copy(k, j):
            return pltpu.make_async_copy(
                late[k][0].at[:, pl.ds(pl.multiple_of(j * 128, 128), 128)], late[k][1].at[j],
                sem_f.at[k])

        load_x_rows(0, 0)

        def step(it, cur, state):
            s = it * UNROLL + cur
            nxt = (cur + 1) % UNROLL

            def pay(t, cost):
                now = state.get("now", 0)
                due = state.setdefault("due", [])
                for z in [z for (d, z) in due if d <= now]:
                    t = jnp.concatenate([t[0:8] | z, t[8:]], axis=0)
                state["due"] = [(d, z) for (d, z) in due if d > now]
                state["now"] = now + cost
                return t

            def owe(lag, p, tiles):
                z = tiles[0]
                for t in tiles[1:]:
                    z = z | t
                state.setdefault("due", []).append(
                    (state.get("now", 0) + lag + (p % PG) * TOK_STAG, zero_after(z)))

            def lv(k0, k1):
                ts = [lhs[cur, k] for k in range(k0, k1)]
                ts[0] = pay(ts[0], (k1 - k0) / NT)
                return jnp.concatenate([_as_bf16(t) for t in ts], axis=1)

            def wmat(mat, h, q0, q1):
                return _as_bf16(jnp.concatenate([wqkv[3 * q + mat, h] for q in range(q0, q1)],
                                                axis=0))

            def qkv(p, split=False):
                part = {}
                if split:
                    for mat in range(3):
                        for a in range(2):
                            part[mat, a] = _dot(lv(0, NT // 2), wmat(mat, 2 * p + a, 0, 2))
                for mat in range(3):
                    for a in range(2):
                        hm = mat * H + 2 * p + a
                        if split:
                            y = _dot(lv(NT // 2, NT), wmat(mat, 2 * p + a, 2, 4)) + part[mat, a]
                        else:
                            y = _dot(lv(0, NT), wmat(mat, 2 * p + a, 0, 4))
                        cur_s[hm] = y.astype(BF16)
                        release(y)

            def gather(mat, p):
                hm = mat * H + 2 * p
                return jnp.concatenate(
                    [cur_s[hm], cur_s[hm + 1], pre[mat * NP + p, s].astype(BF16)], axis=0)

            probs = {}

            def scores_t(p):
                st = lax.dot_general(gather(1, p), gather(0, p), (((1,), (1,)), ((), ())),
                                     preferred_element_type=F32)
                lane = lax.broadcasted_iota(jnp.int32, (1, PR), 1)
                is_a = jnp.logical_or(lane < SEG,
                                      jnp.logical_and(lane >= 2 * SEG, lane < 2 * SEG + M))
                ka = jnp.concatenate([st[0:SEG], st[2 * SEG:2 * SEG + M]], axis=0)
                kb = jnp.concatenate([st[SEG:2 * SEG], st[2 * SEG + M:]], axis=0)
                t = jnp.where(is_a, ka, kb) * (SCALE * LOG2E)
                t = jnp.where(mk[0:SEG + M, :] == 0.0, t, NEG_MASK * LOG2E)
                if REL_S is None:
                    return softmax_t(p, is_a, t)
                ts_s[p + (it >> 10)] = t

                def later(z):
                    zf = pltpu.bitcast(z, F32)[:, 0:PR]
                    t2 = (ts_s[p].reshape(-1, 8, PR) + zf).reshape(SEG + M, PR)
                    softmax_t(p, is_a, t2)

                state.setdefault("pend", []).append(
                    (state.get("now", 0) + REL_S + (p % PG) * REL_STAG, later))

            def release(y):
                now = state.get("now", 0)
                pend = state.get("pend", [])
                state["pend"] = [(d, f) for (d, f) in pend if d > now]
                for (d, f) in pend:
                    if d <= now:
                        f(zero_after(y[0:8]))

            def softmax_t(p, is_a, t):
                e = jnp.exp2(t - jnp.max(t, axis=0, keepdims=True))
                e = e * _recip(jnp.sum(e, axis=0, keepdims=True))
                pa = jnp.where(is_a, e, 0.0)
                pb = jnp.where(is_a, 0.0, e)
                pt = jnp.concatenate([pa[0:SEG], pb[0:SEG], pa[SEG:], pb[SEG:]], axis=0)
                if TOK_S is not None:
                    eu = pltpu.bitcast(e, U32)
                    z = eu[0:8]
                    for k in range(1, (SEG + M) // 8):
                        z = z | eu[k * 8:(k + 1) * 8]
                    owe(TOK_S, p, [jnp.concatenate([z, jnp.zeros((8, 128 - PR), U32)], axis=1)])
                probs[p] = (pt.astype(BF16), "t")

            def scores(p):
                sc = lax.dot_general(gather(0, p), gather(1, p), (((1,), (1,)), ((), ())),
                                     preferred_element_type=F32)
                mv = mk[0:PR, :]
                sc = jnp.where(mv == 0.0, sc * (SCALE * LOG2E), mv)
                e = jnp.exp2(sc - jnp.max(sc, axis=-1, keepdims=True))
                inv = _recip(jnp.sum(e, axis=-1, keepdims=True))
                if NORM_PRE:
                    e = e * inv
                    if TOK_S is not None:
                        eu = pltpu.bitcast(e, U32)
                        z = eu[0:8]
                        for k in range(1, PR // 8):
                            z = z | eu[k * 8:(k + 1) * 8]
                        owe(TOK_S, p, [jnp.concatenate([z, jnp.zeros((8, 128 - PR), U32)], axis=1)])
                    probs[p] = (e.astype(BF16), None)
                else:
                    if TOK_S is not None:
                        iu = pltpu.bitcast(jnp.broadcast_to(inv, (PR, 128)), U32)
                        owe(TOK_S, p, [iu[k * 8:(k + 1) * 8] for k in range(PR // 8)])
                    probs[p] = (e.astype(BF16), inv)

            def pv(p):
                e, inv = probs.pop(p)
                if isinstance(inv, str):
                    o = lax.dot_general(e, gather(2, p), (((0,), (0,)), ((), ())),
                                        preferred_element_type=F32)
                else:
                    o = _dot(e, gather(2, p))
                    if inv is not None:
                        o = o * inv
                o = o.astype(BF16)
                if TOK_P is not None:
                    ou = _as_u32(o)
                    owe(TOK_P, p, [ou[k * 8:(k + 1) * 8] for k in range(PR // 16)])
                for a in range(2):
                    h = 2 * p + a
                    olhs[h] = _as_u32(o[a * SEG:(a + 1) * SEG])
                    odef[h, it, cur * 4:(cur + 1) * 4, :] = _as_u32(
                        o[2 * SEG + a * M:2 * SEG + (a + 1) * M])

            acc = [None] * NT

            def oproj(j, pairs):
                ts = [olhs[2 * p + a] for p in pairs for a in range(2)]
                ts[0] = pay(ts[0], len(pairs) / 4)
                ov = jnp.concatenate([_as_bf16(t) for t in ts], axis=1)
                w = wo_s[j, pairs[0] * DH:(pairs[-1] + 1) * DH, :]
                y = _dot(ov, _as_bf16(w))
                acc[j] = y if acc[j] is None else y + acc[j]
                release(acc[j])

            def fin(j):
                yb = acc[j].astype(BF16)
                ybuf[s, 0:XR, j * 128:(j + 1) * 128] = yb[0:XR]
                lhs[nxt, j, XR // 2:, :] = _as_u32(yb[XR:])

            def gemv():
                d0 = state.get("d0", 0)
                state["acc"] = gemv_part(wm_s[it & 3, :, d0:d0 + GR, :], d0, state.get("acc"))
                state["d0"] = d0 + GR
                au = pltpu.bitcast(state["acc"], U32)
                owe(G_LAG, 0, [au[u] for u in range(mt)])

            def late_mod(u):
                mod_tile(wm_s[it & 3, u], 2 * NT + it * mt + u)

            load_x_rows(nxt, jnp.minimum(s + 1, NSEG - 1))
            ops = dict(Q=qkv, S=scores_t if TR_MODE else scores, P=pv, O=oproj, F=fin, M=late_mod, G=gemv)
            for op in _schedule([(u, q) for u, (c_, q) in enumerate(MODS[:mt])
                                 if c_ % UNROLL == cur and not VPU_MOD]):
                ops[op[0]](*op[1:])

        def steps(it, carry):
            if "pro" in PHASES:
                pltpu.make_async_copy(wm_s.at[it & 3], wm_s.at[it & 3], sem_m.at[it & 3]).wait()

                @pl.when(it + 2 < NSEG // UNROLL)
                def _():
                    for u in range(mt):
                        wm_copy(it + 2, u).start()

            for u in range(UNROLL // 2):
                t = it * (UNROLL // 2) + u
                for k in range(3):
                    @pl.when(t < late[k][2])
                    def _():
                        col_copy(k, t).start()

            state = {}
            for u in range(UNROLL):
                step(it, u, state)
            if VPU_MOD:
                acc = state.get("acc")
                for d0 in range(state.get("d0", 0), D, 64):
                    acc = gemv_part(wm_s[it & 3, :, d0:d0 + 64, :], d0, acc)
                gemv_finish(acc, [2 * NT + it * mt + u for u in range(mt)])
            return carry

        with jax.named_scope("m_steps"):
            if "step" in PHASES: lax.fori_loop(0, NSEG // UNROLL, steps, 0)
        for k in range(3):
            for j in range(late[k][2]):
                col_copy(k, j).wait()
        if "epi" not in PHASES:
            cp = pltpu.make_async_copy(ybuf, out_hbm, sem_out.at[0])
            cp.start()
            cp.wait()
            return

        ntail = EBLK[-1] // M
        ppi = (S // 8 - ntail) // NEC
        gpi = ppi // (XR // 8)
        gb_ = UNROLL * M

        def ep_body(i, c):
            @pl.when(i > 0)
            def _():
                out_copy((i - 1) * gpi, gpi, 0, XR).start()

            for k in range(NT):
                mod[7 * NT + k] = mod[4 * NT + k] * mod[6 * NT + k]
            mod[8 * NT] = jnp.broadcast_to(
                jnp.sum(modv(3) * modv(6), axis=-1, keepdims=True), (M, 128))

            subs = []
            r0 = 0
            for nr in EBLK:
                kh = EKH * EC // nr if EC % nr == 0 else EKH
                for j in range(NT):
                    for h0_ in range(0, H, kh):
                        subs.append((r0, nr, j, h0_, kh))
                r0 += nr
            tot = sum(nr * kh for (_, nr, _, _, kh) in subs)
            span = E_SPAN * EC * EKH
            rel = [u * (tot - span) // ppi for u in range(ppi)]
            ready = {}
            due = []
            now = 0
            u = 0
            y = None
            for (r0, nr, j, h0_, kh) in subs:
                blk = pl.ds(i * (EC // gb_) + r0 // gb_, nr // gb_)
                ts = [odef[h, blk].reshape(nr // 2, DH) for h in range(h0_, h0_ + kh)]
                for z in [z for (d, z) in due if d <= now]:
                    ts[0] = jnp.concatenate([ts[0][0:8] | z, ts[0][8:]], axis=0)
                due = [(d, z) for (d, z) in due if d > now]
                w = wo_s[j, h0_ * DH // 2:(h0_ + kh) * DH // 2, :]
                yp = _dot(jnp.concatenate([_as_bf16(t) for t in ts], axis=1), _as_bf16(w))
                y = yp if h0_ == 0 else yp + y
                if h0_ + kh == H:
                    ybuf[pl.ds(i * (EC // M) + r0 // M, nr // M), XR:, j * 128:(j + 1) * 128] = (
                        y.reshape(nr // M, M, 128).astype(BF16))
                    if j == NT - 1:
                        ready[r0] = True
                start = now
                now += nr * kh
                while u < ppi and rel[u] < now:
                    d = (NEC - 1) * ppi + u - NSEG * (XR // 8) - (NEC - 1) * (EC // M)
                    if d >= 0 and sum(n for r, n in zip(_cumsum(EBLK), EBLK) if r in ready) <= d * M:
                        break
                    t = i * ppi + u
                    early = t < NSEG * (XR // 8)
                    seg = jnp.where(early, t // (XR // 8), t - NSEG * (XR // 8))
                    row = pl.multiple_of(jnp.where(early, (t % (XR // 8)) * 8, XR), 8)
                    res = post(seg, row, zero_after(y[0:8]))
                    due.append((start + span, zero_after(res)))
                    u += 1
            assert u == ppi
            return c

        with jax.named_scope("e_loop"):
            lax.fori_loop(0, NEC, ep_body, 0)
        done = (NEC - 1) * gpi
        tail = NSEG - ntail
        out_copy(done, NSEG - done, 0, XR).start()
        out_copy(0, tail, XR, M).start()
        x1s = [resid(g, XR) for g in range(tail, NSEG)]
        mus = [jnp.mean(x1, axis=-1, keepdims=True) for x1 in x1s]
        pairs = [(top[0:8, :], top[8:16, :])]
        lowest = jnp.full((8, 128), jnp.iinfo(jnp.int32).min, jnp.int32)
        for g in range(tail, NSEG):
            xc = x1s[g - tail] - mus[g - tail]
            inv = _inv_std(xc)
            stat[0, g, XR:, :] = jnp.broadcast_to(mus[g - tail], (8, 128))
            stat[1, g, XR:, :] = jnp.broadcast_to(inv, (8, 128))
            v = _rb(inv * jnp.sum(xc * modv(7), axis=-1, keepdims=True) + mod[8 * NT])
            pairs.append((make_key(v, g * SEG + XR), lowest))
        while len(pairs) > 1:
            (a1, a2), (c1, c2) = pairs.pop(0), pairs.pop(0)
            pairs.append((jnp.maximum(a1, c1),
                          jnp.maximum(jnp.minimum(a1, c1), jnp.maximum(a2, c2))))

        tk = jnp.concatenate(pairs[0], axis=0)[:, 0:1]
        k1 = jnp.max(tk[0:8], axis=0, keepdims=True)
        k2 = jnp.max(jnp.where(tk == k1, jnp.iinfo(jnp.int32).min, tk), axis=0, keepdims=True)
        i1 = (S - 1) - (k1[0, 0] & (S - 1))
        i2 = (S - 1) - (k2[0, 0] & (S - 1))
        g1, g2 = i1 >> 5, i2 >> 5
        b1 = pl.multiple_of(i1 & 24, 8)
        b2 = pl.multiple_of(i2 & 24, 8)

        xa, ha_ = redo(g1, b1)
        xb_, hb_ = redo(g2, b2)
        x1 = jnp.concatenate([xa, xb_], axis=0)
        h2 = jnp.concatenate([ha_, hb_], axis=0)
        h2b = h2.astype(BF16)
        row = lax.broadcasted_iota(jnp.int32, (16, 1), 0)
        grow = jnp.where(row < 8, g1 * SEG + b1 + row, g2 * SEG + b2 + row - 8)
        ks = jnp.where(grow == i1, k1, k2)
        rsel = pltpu.bitcast((ks ^ ((ks >> 31) & 0x7FFF0000)) & -65536, F32)
        acts = []
        for j in range(FF // 128):
            gt = _rb(_dot(h2b, wg_s[j]))
            gt = _rb(gt * _rb(jax.nn.sigmoid(gt)))
            ut = _rb(_dot(h2b, wu_s[j]))
            acts.append((gt * ut).astype(BF16))
            if j < ntail:
                xo_, ho_ = redo(tail + j, XR, zero_after(ut[0:8]))
                outs[tail + j, XR:, :] = (xo_ + modv(5) * ho_).astype(BF16)
            if j == ntail - 1:
                out_copy(tail, NSEG - tail, XR, M).start()
        act = jnp.concatenate(acts, axis=1)
        y = _rb(jnp.concatenate([_dot(act, wd_s[j]) for j in range(NT)], axis=1))
        y = _rb(y * _rb(jax.nn.sigmoid(rsel)))
        sel = jnp.logical_or(grow == i1, grow == i2)
        gb2 = jnp.concatenate([modv(5)] * 2, axis=0)
        fixed = (x1 + gb2 * (h2 + jnp.where(sel, y, 0.0))).astype(BF16)

        with jax.named_scope("e_outwait"):
            out_copy(0, NSEG, 0, SEG).wait()
        outs[g1, pl.ds(b1, 8), :] = fixed[0:8]
        outs[g2, pl.ds(b2, 8), :] = fixed[8:16]
        out_copy(g1, 1, b1, 8, 0).start()

        @pl.when((i1 >> 3) != (i2 >> 3))
        def _():
            out_copy(g2, 1, b2, 8, 1).start()
            out_copy(g2, 1, b2, 8, 1).wait()

        out_copy(g1, 1, b1, 8, 0).wait()

    pl.run_scoped(
        main,
        pltpu.VMEM((FF // 128, D, 128), BF16),
        pltpu.VMEM((FF // 128, D, 128), BF16),
        pltpu.VMEM((NT, FF, 128), BF16),
        pltpu.VMEM((NSEG, SEG, D), BF16),
        pltpu.VMEM((2, NSEG, SEG, 128), F32),
        pltpu.VMEM((NSEG, SEG, D), BF16),
        pltpu.SemaphoreType.DMA((3,)),
    )


def _entry(*refs):
    pl.run_scoped(
        functools.partial(_kernel, *refs),
        pltpu.VMEM((NCHUNK, H, KQ // 2, DH), U32),
        pltpu.VMEM((NSEG + 1, NT, XR // 2, 128), U32),
        pltpu.VMEM((NT, (H * DH + H * DH // NT) // 2, 128), U32),
        pltpu.VMEM((3 * NP, NSEG, 2 * M, DH), F32),
        pltpu.VMEM((3 * H, SEG, DH), BF16),
        pltpu.VMEM((H, SEG // 2, DH), U32),
        pltpu.VMEM((H, NSEG // UNROLL, UNROLL * M // 2, DH), U32),
        pltpu.VMEM((NSEG, SEG, D), BF16),
        pltpu.VMEM((UNROLL, NT, SEG // 2, 128), U32),
        pltpu.VMEM((4, 4 * NT * UNROLL // NSEG, D, 128), BF16),
        pltpu.VMEM((8 * NT + 4, M, 128), F32),
        pltpu.VMEM((96, PR), F32),
        pltpu.VMEM((32, 128), jnp.int32),
        pltpu.VMEM((M, D), BF16),
        pltpu.VMEM((D, 128), F32),
        pltpu.VMEM((NP, SEG + M, PR), F32),
        pltpu.VMEM((8 + PADS[2], 128), U32),
        pltpu.SemaphoreType.DMA((4,)),
        pltpu.SemaphoreType.DMA((2,)),
    )


@functools.partial(jax.jit, static_argnames=("A_seg_len",))
def pallas_adaLN_cond__memory_aug_recurrent_mem_tr__moe_arch_mod__prompt_kernel(
    A_x: jax.Array,
    A_mem0: jax.Array,
    A_Wq: jax.Array,
    A_Wk: jax.Array,
    A_Wv: jax.Array,
    A_Wo: jax.Array,
    A_seg_len,
    B_x: jax.Array,
    B_w_r: jax.Array,
    B_w_gate: jax.Array,
    B_w_up: jax.Array,
    B_w_down: jax.Array,
    c: jax.Array,
    w_mod: jax.Array,
):
    assert A_seg_len == SEG and A_x.shape == (1, S, D)
    del B_x
    hbm = pl.BlockSpec(memory_space=pl.ANY)
    out = pl.pallas_call(
        _entry,
        out_shape=jax.ShapeDtypeStruct((NSEG, SEG, D), BF16),
        in_specs=[hbm] * 12,
        out_specs=hbm,
        compiler_params=pltpu.CompilerParams(vmem_limit_bytes=120 * 1024 * 1024,
                                             disable_bounds_checks=True),
    )(A_x.reshape(NSEG, SEG, D), A_mem0.reshape(M, D), A_Wq, A_Wk, A_Wv, A_Wo.reshape(H * DH, D),
      B_w_r, B_w_gate, B_w_up, B_w_down, c, w_mod)
    return out.reshape(1, S, D)
```

```python
import functools

import jax
import jax.numpy as jnp
from jax import lax
import jax.experimental.pallas as pl
import jax.experimental.pallas.tpu as pltpu

F32 = jnp.float32
BF16 = jnp.bfloat16
U32 = jnp.uint32

D = 1024
S = 2048
H = 32
DH = 128
M = 8
SEG = 32
NSEG = S // SEG
FF = 3584
NT = D // 128
XR = SEG - M
R0 = M * NSEG
CH = 8
KQ = D // 4
NCHUNK = 3 * D // KQ
NSLOT = 4
PR = 2 * SEG + 2 * M
NP = H // 2
EC = 128
NEC = R0 // EC
LOG2E = 1.4426950408889634
EPS = 1e-5
SCALE = DH ** -0.5
NEG_MASK = -1000000000.0

PHASES = ("pro", "step", "epi")

UNROLL = 4
PG = 4
LAG_S = 1
LAG_P = 4
O_PARTS = (0, 8, 12)
O_TH = (256, 256, 256, 1216)
REL_S = 2
REL_STAG = 2
G_AT = (0, 1, 2, 3)
GR = 32
G_LAG = 2
BLK = 32
JOB_SPAN = 40
RB = 16
RB2 = 64
FB = 32
GVR = 32
GV_FREE = 64
R_AT = ((0, 6, 16), (14, 22, 30), (30, 38, 46), (44, 52, 60))
F_AT = (0, 13)
L_AT = 8
GV_AT = (16, 56)
LNU = 16
EKH = 4
E_SPAN = 5
PAD = 24


def _schedule():
    groups = [list(range(g, g + PG)) for g in range(0, NP, PG)]
    at = {}
    for g, grp in enumerate(groups):
        at.setdefault(grp[-1] + LAG_P, []).extend(("P", q) for q in grp)
    for g, grp in enumerate(groups):
        at.setdefault(grp[-1] + LAG_S, []).extend(("S", q) for q in grp)
    ops = []
    for p in range(NP):
        ops.append(("Q", p, p == 0))
        if p in G_AT:
            ops.append(("G",))
        ops.extend(at.pop(p, []))
    bounds = list(O_PARTS) + [NP]
    t = NP
    done = 0
    for n in range(len(O_PARTS)):
        part = list(range(bounds[n], bounds[n + 1]))
        assert all(("P", q) in ops for q in part), (n, ops)
        for j in range(NT):
            ops.append(("O", j, part))
            if n == len(O_PARTS) - 1:
                ops.append(("F", j))
            done += len(part) * 16
            while t - NP < len(O_TH) and done >= O_TH[t - NP]:
                ops.extend(at.pop(t, []))
                t += 1
    assert not at
    return ops


def _rb(x):
    return x.astype(BF16).astype(F32)


def _recip(x):
    r = pl.reciprocal(x, approx=True)
    return r * (2.0 - x * r)


def _inv_std(xc):
    v = _rb(_rb(jnp.mean(xc * xc, axis=-1, keepdims=True)) + EPS)
    return _recip(_rb(v * lax.rsqrt(v)))


def _ln(x, zero=None):
    xm = x if zero is None else jnp.concatenate([x[..., :128] + zero, x[..., 128:]], axis=-1)
    xc = x - jnp.mean(xm, axis=-1, keepdims=True)
    return xc * _inv_std(xc)


def _dot(a, b):
    return jnp.dot(a, b, preferred_element_type=F32)


def _as_bf16(u):
    return pltpu.bitcast(u, BF16)


def _as_u32(b):
    return pltpu.bitcast(b, U32)


def _spread(jobs, fns, lo, hi):
    for n, fn in enumerate(fns):
        jobs.setdefault(lo + n * (hi - lo) // len(fns), []).append(fn)


def _kernel(x_hbm, mem0_hbm, wq_hbm, wk_hbm, wv_hbm, wo_hbm, wr_hbm, wg_hbm, wu_hbm, wd_hbm,
            c_hbm, wmod_hbm, out_hbm,
            wqkv, hs, wo_s, pre, cur_s, olhs, odef, xbuf, lhs, wm_s, mod, mk,
            top, sc_s, cb_s, ts_s, zero_s, sem_m, sem_out):
    mt = 4 * NT * UNROLL // NSEG

    def modv(j):
        return jnp.concatenate([mod[j * NT + k] for k in range(NT)], axis=1)

    def mod_store(v, t):
        v = _rb(v)
        mod[t] = jnp.where(jnp.logical_or((t >> 3) == 1, (t >> 3) == 4), _rb(1.0 + v), v)

    def mod_tile(wm, t):
        mod_store(_dot(sc_s[...], wm), t)

    def gemv_part(w, d0, acc):
        n = w.shape[1]
        p = w.astype(F32) * cb_s[d0:d0 + n, :]
        p = jnp.sum(p.reshape(w.shape[0], n // 8, 8, 128), axis=1)
        return p if acc is None else p + acc

    def gemv_finish(acc, ts):
        for u, t in enumerate(ts):
            mod_store(jnp.broadcast_to(jnp.sum(acc[u], axis=0, keepdims=True), (M, 128)), t)

    def wm_copy(it, u):
        col = pl.multiple_of((2 * NT + it * mt + u) * 128, 128)
        return pltpu.make_async_copy(wmod_hbm.at[:, pl.ds(col, 128)], wm_s.at[it & 3, u],
                                     sem_m.at[it & 3])

    def zero_after(y):
        return (y if y.dtype == U32 else pltpu.bitcast(y, U32)) & zero_s[0:8, :]

    def or_tile(u, z):
        if z is None:
            return u
        return (u.reshape(u.shape[0] // 8, 8, 128) | z).reshape(u.shape)

    def prologue(stage, wo_raw, wmod_s, nrm, ha, hb, tmp, mem0_ref, wr_ref, c_ref, sem):
        w_hbms = (wq_hbm, wk_hbm, wv_hbm)
        wob = H * DH // NT
        S_X, S_C0, S_ST, S_WO, S_MOD, S_SM = 0, 2, 6, 6 + NSLOT, 6 + NSLOT + NT, 6 + NSLOT + 2 * NT

        def x_copy(i):
            lo, n = ((XR, M), (0, XR))[i]
            return pltpu.make_async_copy(x_hbm.at[:, pl.ds(lo, n), :], xbuf.at[:, pl.ds(lo, n), :],
                                         sem.at[S_X + i])

        def mod_copies(k):
            return [pltpu.make_async_copy(wmod_hbm.at[:, pl.ds(v * D + k * 128, 128)],
                                          wmod_s.at[k, v], sem.at[S_MOD + (k if k < 2 else k & 6)])
                    for v in range(2)]

        def chunk_copy(mat, d0, g, slot, k):
            heads = pl.ds(pl.multiple_of(g * CH, CH), CH)
            return pltpu.make_async_copy(w_hbms[mat].at[pl.ds(d0, KQ), heads, :],
                                         stage.at[slot, g], sem.at[k])

        def wo_copy(j):
            return pltpu.make_async_copy(wo_hbm.at[pl.ds(pl.multiple_of(j * wob, wob), wob)],
                                         wo_raw.at[j], sem.at[S_WO + j])

        def relayout1(src, t0, z=None):
            v = src.reshape(RB * CH, 128)
            tmp[t0:t0 + RB * CH // 2, :] = or_tile(_as_u32(v), z)

        def relayout2(c, h0_, t0, d0, z=None, src=tmp):
            w = or_tile(src[pl.ds(t0, RB2, stride=CH // 2), :], z)
            rows = pl.ds(d0 // 2, RB2 // 2)
            wqkv[c, h0_, rows, :] = _as_u32(w.astype(jnp.uint16))
            wqkv[c, h0_ + 1, rows, :] = _as_u32((w >> 16).astype(jnp.uint16))

        def mod_pair(k):
            for v in range(2):
                mod_tile(wmod_s[k, v], v * NT + k)

        def fill(dst, q, t, r, z=None):
            k = 2 * q + t
            sh = mod[k] if z is None else mod[k] + pltpu.bitcast(z, F32)
            v = nrm[k, r:r + FB, :].reshape(FB // 8, 8, 128) * mod[NT + k] + sh
            dst[t, r // 2:(r + FB) // 2, :] = _as_u32(v.reshape(FB, 128).astype(BF16))

        small = [pltpu.make_async_copy(src, dst, sem.at[S_SM])
                 for src, dst in ((c_hbm, c_ref), (mem0_hbm, mem0_ref), (wr_hbm, wr_ref))]
        for cp in small:
            cp.start()
        x_copy(0).start()
        for cp in mod_copies(0) + mod_copies(1):
            cp.start()
        for g in range(4):
            chunk_copy(0, 0, g, 0, S_C0 + g).start()
        for c in range(1, NSLOT):
            for g in range(4):
                chunk_copy(c % 3, (c // 3) * KQ, g, c, S_ST + c).start()
            for cp in mod_copies(2 * c) + mod_copies(2 * c + 1):
                cp.start()

        kk = lax.broadcasted_iota(jnp.int32, (SEG + M, PR), 0)
        qq = lax.broadcasted_iota(jnp.int32, (SEG + M, PR), 1)
        k_mem = jnp.logical_and(kk >= XR, kk < SEG)
        k_pos = jnp.where(kk < SEG, kk, kk - M)
        q_mem = jnp.logical_and(qq < 2 * SEG, qq % SEG >= XR)
        q_pos = jnp.where(qq < 2 * SEG, qq % SEG, XR + qq % M)
        mk[0:SEG + M, :] = jnp.where(q_mem | k_mem | (q_pos >= k_pos), 0.0, 1.0).astype(F32)
        mod[0:2 * NT] = jnp.zeros((2 * NT, M, 128), F32)
        zero_s[...] = jnp.zeros(zero_s.shape, U32)
        top[...] = jnp.full(top.shape, jnp.iinfo(jnp.int32).min, jnp.int32)
        for cp in small:
            cp.wait()
        wr = jnp.broadcast_to(wr_ref[...].astype(F32).reshape(1, D), (M, D))
        for k in range(NT):
            mod[6 * NT + k] = wr[:, k * 128:(k + 1) * 128]
        cv = c_ref[...].astype(F32)
        sc = _rb(cv * _rb(jax.nn.sigmoid(cv)))
        sc_s[...] = jnp.broadcast_to(sc, (M, D)).astype(BF16)
        for k in range(NT):
            cb_s[k * 128:(k + 1) * 128, :] = jnp.broadcast_to(
                sc[:, k * 128:(k + 1) * 128], (128, 128)).T
        mb = mem0_ref[...]
        for k in range(NT):
            lhs[0, k, XR // 2:, :] = _as_u32(mb[:, k * 128:(k + 1) * 128])

        def zero_body(i, c):
            wo_raw[NT, pl.ds(pl.multiple_of(i * 32, 32), 32), :] = jnp.zeros((32, D), BF16)
            return c

        lax.fori_loop(0, wob // 32, zero_body, 0)
        x_copy(0).wait()

        def ln_body(i, c):
            for u in range(LNU):
                q = i * LNU + u
                v = _ln(xbuf[q, XR:, :].astype(F32))
                for k in range(NT):
                    nrm[k, pl.ds(pl.multiple_of(q * 8, 8), 8), :] = v[:, k * 128:(k + 1) * 128]
            return c

        with jax.named_scope("p_ln"):
            lax.fori_loop(0, NSEG // LNU, ln_body, 0)

        def mod_body(k, c):
            pltpu.make_async_copy(wmod_s.at[k], wmod_s.at[k], sem.at[S_MOD + k]).wait()
            mod_pair(k)
            for r in range(0, R0, FB):
                fill(ha, 0, k, r)
            return c

        with jax.named_scope("p_mod"):
            lax.fori_loop(0, 2, mod_body, 0)

        def hop1(g):
            chunk_copy(0, 0, g, 0, S_C0 + g).wait()

            def body(i, c):
                d0 = pl.multiple_of(i * 128, 128)
                v = stage[0, g, pl.ds(d0, 128)].reshape(128 * CH, 128)
                t0 = pl.multiple_of((g * KQ + d0) * (CH // 2), 512)
                tmp[pl.ds(t0, 128 * CH // 2), :] = _as_u32(v)
                return c

            lax.fori_loop(0, KQ // 128, body, 0)

        def hop2(c, g, j):
            src = tmp.at[pl.ds(pl.multiple_of(g * (KQ * CH // 2), 512), KQ * CH // 2 + 8)]
            for d0 in range(0, KQ, RB2):
                relayout2(c, g * CH + 2 * j, d0 * CH // 2 + j, d0, src=src)

        def bulk(units, jobs):
            due = {}
            t0 = 0
            for n, (hq, c, h0_, pi, first, r0, nrow) in enumerate(units):
                nb = nrow // BLK
                parts = []
                for u in range(nb):
                    part = hq[0, (r0 + u * BLK) // 2:(r0 + (u + 1) * BLK) // 2, :]
                    for z in due.pop(t0 + u, ()):
                        part = jnp.concatenate([part[0:8] | z, part[8:]], axis=0)
                    parts.append(part)
                hv = jnp.concatenate([_as_bf16(jnp.concatenate(parts, axis=0)),
                                      _as_bf16(hq[1, r0 // 2:(r0 + nrow) // 2, :])], axis=1)
                w = jnp.concatenate([_as_bf16(wqkv[c, h0_]), _as_bf16(wqkv[c, h0_ + 1])], axis=1)
                y = _dot(hv, w)
                segs = slice(r0 // M, (r0 + nrow) // M)
                for a in range(2):
                    old = jnp.where(first, 0.0, pre[pi, segs, a * M:(a + 1) * M, :])
                    pre[pi, segs, a * M:(a + 1) * M, :] = (
                        y[:, a * DH:(a + 1) * DH].reshape(nrow // M, M, DH) + old)
                for u in range(nb):
                    for job in jobs.get(t0 + u, ()):
                        res = job(zero_after(y[u * BLK:u * BLK + 8, 0:128]))
                        if res is not None:
                            due.setdefault(max(t0 + u + JOB_SPAN, t0 + nb), []).append(
                                zero_after(res))
                t0 += nb
            assert not due

        GP = CH // 2
        WO0 = NCHUNK - 1 - NT
        LN0 = 4
        SPI = -(-NSEG // (NCHUNK - 1 - LN0))

        def rot_body(i, c):
            slot = (i + 1) & (NSLOT - 1)
            pltpu.make_async_copy(stage.at[slot], stage.at[slot], sem.at[S_ST + slot]).wait()
            km = 2 * jnp.minimum(i, 3)

            @pl.when(jnp.logical_and(i >= 1, i <= 3))
            def _():
                wq = wmod_s.at[pl.ds(km, 2)]
                pltpu.make_async_copy(wq, wq, sem.at[S_MOD + km]).wait()

            @pl.when(i == LN0)
            def _():
                x_copy(1).wait()

            @pl.when(i >= WO0)
            def _():
                wo_copy(i - WO0).wait()

            nxt = i + NSLOT
            qn = (nxt * 43) >> 7
            for mat in range(3):
                @pl.when(jnp.logical_and(nxt < NCHUNK, nxt - 3 * qn == mat))
                def _():
                    for g in range(4):
                        chunk_copy(mat, qn * KQ, g, nxt & (NSLOT - 1),
                                   S_ST + (nxt & (NSLOT - 1))).start()

            @pl.when(i < NT)
            def _():
                wo_copy(i).start()

            @pl.when(i == 0)
            def _():
                x_copy(1).start()

            q0 = (i * 43) >> 7
            q1 = ((i + 1) * 43) >> 7
            pa = (i - 3 * q0) * NP + NP - GP
            units = ([(ha, i, H - CH + 2 * n, pa + n, q0 == 0, 0, R0) for n in range(GP)]
                     + [(hb, i + 1, 2 * n, (i + 1 - 3 * q1) * NP + n, q1 == 0, 0, R0)
                        for n in range(NP - GP)])
            jw = jnp.where(i >= WO0, i - WO0, NT)

            def wo_job(b, z):
                v = wo_raw[jw, b * 16:(b + 1) * 16, :]
                rows = pl.ds(pl.multiple_of(jw * (wob // 2) + b * 8, 8), 8)
                for j in range(NT):
                    wo_s[j, rows, :] = _as_u32(v[:, j * 128:(j + 1) * 128]) | z

            def ln_job(b, z):
                r = (b % 3) * 8
                seg = (i - LN0) * SPI + b // 3
                live = jnp.logical_and(i >= LN0, seg < NSEG)
                src = jnp.where(live, seg, 0)
                x = xbuf[src, pl.ds(pl.multiple_of(jnp.where(live, r, XR), 8), 8), :].astype(F32)
                hv = (_ln(x, pltpu.bitcast(z, F32)) * modv(1) + modv(0)).astype(BF16)
                u = [_as_u32(hv[:, k * 128:(k + 1) * 128]) for k in range(NT)]
                dst = jnp.where(live, seg, NSEG)
                for k in range(NT):
                    hs[dst, k, r // 2:r // 2 + 4, :] = u[k]
                res = jnp.concatenate(u[0:2], axis=0)
                for k in range(2, NT, 2):
                    res = res | jnp.concatenate(u[k:k + 2], axis=0)
                return res

            def r1_job(g, d0, z):
                relayout1(stage[slot, g, d0:d0 + RB], (g * KQ + d0) * CH // 2, z)

            def copy_job(t, r, z):
                ha[t, r:r + 32, :] = or_tile(hb[t, r:r + 32, :], z)

            P = functools.partial
            upb = R0 // BLK
            nr = NP * upb
            jobs = {}
            for g in range(4):
                lo, mid, hi = (x * upb // 4 for x in R_AT[g])
                _spread(jobs, [P(r1_job, g, d0) for d0 in range(0, KQ, RB)], lo, mid)
                _spread(jobs, [P(relayout2, i + 1, g * CH + 2 * j, (g * KQ + d0) * CH // 2 + j, d0)
                               for j in range(CH // 2) for d0 in range(0, KQ, RB2)], mid, hi)
            oz = i >> 10
            _spread(jobs, [P(fill, hb, q1, t + oz, r) for r in range(0, R0, FB) for t in range(2)],
                    F_AT[0] * upb // 4, F_AT[1] * upb // 4)
            _spread(jobs, [P(copy_job, t, r) for t in range(2) for r in range(0, R0 // 2, 32)],
                    2 * GP * upb, nr - upb)
            _spread(jobs, [P(ln_job, b) for b in range(3 * SPI)],
                    L_AT * upb // 4, nr - max(upb, JOB_SPAN))
            _spread(jobs, [P(wo_job, b) for b in range(wob // 16)], GP * upb, nr - upb)
            gv = {}

            def gv_job(d0, n, z):
                w = wmod_s[pl.ds(km, 2), :, d0:d0 + n, :].reshape(4, n, 128)
                acc = gv.get("acc")
                if z is not None:
                    zf = pltpu.bitcast(z, F32)[None]
                    acc = jnp.broadcast_to(zf, (4, 8, 128)) if acc is None else acc + zf
                gv["acc"] = gemv_part(w, d0, acc)
                if z is not None:
                    au = pltpu.bitcast(gv["acc"], U32)
                    return au[0] | au[1] | au[2] | au[3]

            _spread(jobs, [P(gv_job, d0, GVR) for d0 in range(0, D - GV_FREE, GVR)],
                    GV_AT[0] * upb // 4, min(GV_AT[1] * upb // 4, nr - JOB_SPAN))
            bulk(units, jobs)
            if GV_FREE:
                gv_job(D - GV_FREE, GV_FREE, None)
            gemv_finish(gv["acc"], [km, NT + km, km + 1, NT + km + 1])
            return c

        def outer(k, c):
            last = k == 4

            @pl.when(k < 4)
            def _():
                hop1(k)

            @pl.when(k != 3)
            def _():
                g = jnp.minimum(k, 3)
                cc = jnp.where(last, NCHUNK - 1, 0)
                for j in range(GP):
                    hop2(cc, g, j)
                bulk([(ha, cc, g * CH + 2 * n, jnp.where(last, 2 * NP, 0) + g * GP + n, k < 4,
                       0, R0) for n in range(GP)], {})

            @pl.when(k == 3)
            def _():
                for j in range(GP):
                    hop2(0, 3, j)
                with jax.named_scope("p_rot"):
                    lax.fori_loop(0, NCHUNK - 1, rot_body, 0)
                for it in range(2):
                    for u in range(mt):
                        wm_copy(it, u).start()

            return c

        with jax.named_scope("p_bulk"):
            lax.fori_loop(0, 5, outer, 0)

    if "pro" in PHASES: pl.run_scoped(
        prologue,
        pltpu.VMEM((NSLOT, H // CH, KQ, CH, 128), BF16),
        pltpu.VMEM((NT + 1, H * DH // NT, D), BF16),
        pltpu.VMEM((NT, 2, D, 128), BF16),
        pltpu.VMEM((NT, R0, 128), F32),
        pltpu.VMEM((2, R0 // 2, 128), U32),
        pltpu.VMEM((2, R0 // 2, 128), U32),
        pltpu.VMEM((D * CH // 2 + 32, 128), U32),
        pltpu.VMEM((M, D), BF16),
        pltpu.VMEM((D,), BF16),
        pltpu.VMEM((1, D), BF16),
        pltpu.SemaphoreType.DMA((7 + NSLOT + 2 * NT,)),
    )

    def main(wg_s, wu_s, wd_s, ybuf, stat, outs, sem_f):
        def load_x_rows(slot, seg):
            for k in range(NT):
                lhs[slot, k, 0:XR // 2, :] = hs[seg, k]

        def resid(seg, r, z=None):
            rows = pl.ds(r, 8)
            t = modv(2) * ybuf[seg, rows, :].astype(F32)
            if z is not None:
                t = t + jnp.concatenate([pltpu.bitcast(z, F32)] * NT, axis=1)
            return xbuf[seg, rows, :].astype(F32) + t

        def wide(v):
            return jnp.concatenate([v] * NT, axis=1)

        def make_key(v, row0):
            b = pltpu.bitcast(jnp.where(v != v, -jnp.inf, v + 0.0), jnp.int32)
            low = (S - 1 - row0) - lax.broadcasted_iota(jnp.int32, (8, 128), 0)
            return (b ^ ((b >> 31) & 0x7FFF0000)) | low

        def post(seg, r, z):
            x1 = resid(seg, r, z)
            mu = jnp.mean(x1, axis=-1, keepdims=True)
            xc = x1 - mu
            inv = _inv_std(xc)
            stat[0, seg, pl.ds(r, 8), :] = jnp.broadcast_to(mu, (8, 128))
            stat[1, seg, pl.ds(r, 8), :] = jnp.broadcast_to(inv, (8, 128))
            v = _rb(inv * jnp.sum(xc * modv(7), axis=-1, keepdims=True) + mod[8 * NT])
            key = make_key(v, seg * SEG + r)
            m1, m2 = top[0:8, :], top[8:16, :]
            top[8:16, :] = jnp.maximum(m2, jnp.minimum(m1, key))
            top[0:8, :] = jnp.maximum(m1, key)
            o = x1 + modv(5) * (xc * inv * modv(4) + modv(3))
            outs[seg, pl.ds(r, 8), :] = o.astype(BF16)
            res = pltpu.bitcast(v, U32)
            for k in range(NT):
                res = res | pltpu.bitcast(o[:, k * 128:(k + 1) * 128], U32)
            return res

        def redo(seg, r, z=None):
            x1 = resid(seg, r, z)
            n = (x1 - wide(stat[0, seg, pl.ds(r, 8), :])) * wide(stat[1, seg, pl.ds(r, 8), :])
            return x1, n * modv(4) + modv(3)

        def out_copy(g0, ng, r, n, k=0):
            return pltpu.make_async_copy(outs.at[pl.ds(g0, ng), pl.ds(r, n), :],
                                         out_hbm.at[pl.ds(g0, ng), pl.ds(r, n), :], sem_out.at[k])

        late = ((wg_hbm, wg_s, FF // 128), (wu_hbm, wu_s, FF // 128), (wd_hbm, wd_s, NT))

        def col_copy(k, j):
            return pltpu.make_async_copy(
                late[k][0].at[:, pl.ds(pl.multiple_of(j * 128, 128), 128)], late[k][1].at[j],
                sem_f.at[k])

        load_x_rows(0, 0)

        def step(it, cur, state):
            s = it * UNROLL + cur
            nxt = (cur + 1) % UNROLL

            def pay(t, cost):
                now, due = state["now"], state["due"]
                for z in [z for (d, z) in due if d <= now]:
                    t = jnp.concatenate([t[0:8] | z, t[8:]], axis=0)
                state["due"] = [(d, z) for (d, z) in due if d > now]
                state["now"] = now + cost
                return t

            def release(y):
                now = state["now"]
                pend, state["pend"] = state["pend"], [e for e in state["pend"] if e[0] > now]
                for (d, f) in pend:
                    if d <= now:
                        f(zero_after(y[0:8]))

            def lv(k0, k1):
                ts = [lhs[cur, k] for k in range(k0, k1)]
                ts[0] = pay(ts[0], (k1 - k0) / NT)
                return jnp.concatenate([_as_bf16(t) for t in ts], axis=1)

            def wmat(mat, h, q0, q1):
                return _as_bf16(jnp.concatenate([wqkv[3 * q + mat, h] for q in range(q0, q1)],
                                                axis=0))

            def qkv(p, split=False):
                part = {}
                if split:
                    for mat in range(3):
                        for a in range(2):
                            part[mat, a] = _dot(lv(0, NT // 2), wmat(mat, 2 * p + a, 0, 2))
                for mat in range(3):
                    for a in range(2):
                        hm = mat * H + 2 * p + a
                        if split:
                            y = _dot(lv(NT // 2, NT), wmat(mat, 2 * p + a, 2, 4)) + part[mat, a]
                        else:
                            y = _dot(lv(0, NT), wmat(mat, 2 * p + a, 0, 4))
                        cur_s[hm] = y.astype(BF16)
                        release(y)

            def gather(mat, p):
                hm = mat * H + 2 * p
                return jnp.concatenate(
                    [cur_s[hm], cur_s[hm + 1], pre[mat * NP + p, s].astype(BF16)], axis=0)

            probs = {}

            def scores(p):
                st = lax.dot_general(gather(1, p), gather(0, p), (((1,), (1,)), ((), ())),
                                     preferred_element_type=F32)
                lane = lax.broadcasted_iota(jnp.int32, (1, PR), 1)
                is_a = jnp.logical_or(lane < SEG,
                                      jnp.logical_and(lane >= 2 * SEG, lane < 2 * SEG + M))
                ka = jnp.concatenate([st[0:SEG], st[2 * SEG:2 * SEG + M]], axis=0)
                kb = jnp.concatenate([st[SEG:2 * SEG], st[2 * SEG + M:]], axis=0)
                t = jnp.where(is_a, ka, kb) * (SCALE * LOG2E)
                ts_s[p + (it >> 10)] = jnp.where(mk[0:SEG + M, :] == 0.0, t, NEG_MASK * LOG2E)

                def softmax(z):
                    zf = pltpu.bitcast(z, F32)[:, 0:PR]
                    t = (ts_s[p].reshape(-1, 8, PR) + zf).reshape(SEG + M, PR)
                    e = jnp.exp2(t - jnp.max(t, axis=0, keepdims=True))
                    e = e * _recip(jnp.sum(e, axis=0, keepdims=True))
                    pa = jnp.where(is_a, e, 0.0)
                    pb = jnp.where(is_a, 0.0, e)
                    probs[p] = jnp.concatenate(
                        [pa[0:SEG], pb[0:SEG], pa[SEG:], pb[SEG:]], axis=0).astype(BF16)

                state["pend"].append((state["now"] + REL_S + (p % PG) * REL_STAG, softmax))

            def pv(p):
                o = lax.dot_general(probs.pop(p), gather(2, p), (((0,), (0,)), ((), ())),
                                    preferred_element_type=F32).astype(BF16)
                for a in range(2):
                    h = 2 * p + a
                    olhs[h] = _as_u32(o[a * SEG:(a + 1) * SEG])
                    odef[h, it, cur * 4:(cur + 1) * 4, :] = _as_u32(
                        o[2 * SEG + a * M:2 * SEG + (a + 1) * M])

            acc = [None] * NT

            def oproj(j, pairs):
                ts = [olhs[2 * p + a] for p in pairs for a in range(2)]
                ts[0] = pay(ts[0], len(pairs) / 4)
                ov = jnp.concatenate([_as_bf16(t) for t in ts], axis=1)
                w = wo_s[j, pairs[0] * DH:(pairs[-1] + 1) * DH, :]
                y = _dot(ov, _as_bf16(w))
                acc[j] = y if acc[j] is None else y + acc[j]
                release(acc[j])

            def fin(j):
                yb = acc[j].astype(BF16)
                ybuf[s, 0:XR, j * 128:(j + 1) * 128] = yb[0:XR]
                lhs[nxt, j, XR // 2:, :] = _as_u32(yb[XR:])

            def gemv():
                d0 = state["d0"]
                state["acc"] = gemv_part(wm_s[it & 3, :, d0:d0 + GR, :], d0, state["acc"])
                state["d0"] = d0 + GR
                au = pltpu.bitcast(state["acc"], U32)
                z = functools.reduce(lambda a, b: a | b, [au[u] for u in range(mt)])
                state["due"].append((state["now"] + G_LAG, zero_after(z)))

            load_x_rows(nxt, jnp.minimum(s + 1, NSEG - 1))
            ops = dict(Q=qkv, S=scores, P=pv, O=oproj, F=fin, G=gemv)
            for op in _schedule():
                ops[op[0]](*op[1:])

        def steps(it, carry):
            if "pro" in PHASES:
                pltpu.make_async_copy(wm_s.at[it & 3], wm_s.at[it & 3], sem_m.at[it & 3]).wait()

                @pl.when(it + 2 < NSEG // UNROLL)
                def _():
                    for u in range(mt):
                        wm_copy(it + 2, u).start()

            for u in range(UNROLL // 2):
                t = it * (UNROLL // 2) + u
                for k in range(3):
                    @pl.when(t < late[k][2])
                    def _():
                        col_copy(k, t).start()

            state = dict(now=0, due=[], pend=[], d0=0, acc=None)
            for u in range(UNROLL):
                step(it, u, state)
            acc = state["acc"]
            for d0 in range(state["d0"], D, 64):
                acc = gemv_part(wm_s[it & 3, :, d0:min(d0 + 64, D), :], d0, acc)
            gemv_finish(acc, [2 * NT + it * mt + u for u in range(mt)])
            return carry

        with jax.named_scope("m_steps"):
            if "step" in PHASES: lax.fori_loop(0, NSEG // UNROLL, steps, 0)
        for k in range(3):
            for j in range(late[k][2]):
                col_copy(k, j).wait()
        if "epi" not in PHASES:
            cp = pltpu.make_async_copy(ybuf, out_hbm, sem_out.at[0])
            cp.start()
            cp.wait()
            return

        ntail = EC // M
        ppi = (S // 8 - ntail) // NEC
        gpi = ppi // (XR // 8)
        nblk = EC // (UNROLL * M)

        def ep_body(i, c):
            @pl.when(i > 0)
            def _():
                out_copy((i - 1) * gpi, gpi, 0, XR).start()

            for k in range(NT):
                mod[7 * NT + k] = mod[4 * NT + k] * mod[6 * NT + k]
            mod[8 * NT] = jnp.broadcast_to(
                jnp.sum(modv(3) * modv(6), axis=-1, keepdims=True), (M, 128))

            jobs = {}
            _spread(jobs, list(range(ppi)), 0, NT * H // EKH - E_SPAN)
            due = {}
            n = 0
            for j in range(NT):
                for h0_ in range(0, H, EKH):
                    ts = [odef[h, pl.ds(i * nblk, nblk)].reshape(EC // 2, DH)
                          for h in range(h0_, h0_ + EKH)]
                    for z in due.pop(n, ()):
                        ts[0] = jnp.concatenate([ts[0][0:8] | z, ts[0][8:]], axis=0)
                    w = wo_s[j, h0_ * DH // 2:(h0_ + EKH) * DH // 2, :]
                    yp = _dot(jnp.concatenate([_as_bf16(t) for t in ts], axis=1), _as_bf16(w))
                    y = yp if h0_ == 0 else yp + y
                    if h0_ + EKH == H:
                        ybuf[pl.ds(i * ntail, ntail), XR:, j * 128:(j + 1) * 128] = (
                            y.reshape(ntail, M, 128).astype(BF16))
                    for u in jobs.get(n, ()):
                        t = i * ppi + u
                        early = t < NSEG * (XR // 8)
                        seg = jnp.where(early, t // (XR // 8), t - NSEG * (XR // 8))
                        row = pl.multiple_of(jnp.where(early, (t % (XR // 8)) * 8, XR), 8)
                        res = post(seg, row, zero_after(y[0:8]))
                        due.setdefault(n + E_SPAN, []).append(zero_after(res))
                    n += 1
            return c

        with jax.named_scope("e_loop"):
            lax.fori_loop(0, NEC, ep_body, 0)
        done = (NEC - 1) * gpi
        tail = NSEG - ntail
        out_copy(done, NSEG - done, 0, XR).start()
        out_copy(0, tail, XR, M).start()
        x1s = [resid(g, XR) for g in range(tail, NSEG)]
        mus = [jnp.mean(x1, axis=-1, keepdims=True) for x1 in x1s]
        pairs = [(top[0:8, :], top[8:16, :])]
        lowest = jnp.full((8, 128), jnp.iinfo(jnp.int32).min, jnp.int32)
        for g in range(tail, NSEG):
            xc = x1s[g - tail] - mus[g - tail]
            inv = _inv_std(xc)
            stat[0, g, XR:, :] = jnp.broadcast_to(mus[g - tail], (8, 128))
            stat[1, g, XR:, :] = jnp.broadcast_to(inv, (8, 128))
            v = _rb(inv * jnp.sum(xc * modv(7), axis=-1, keepdims=True) + mod[8 * NT])
            pairs.append((make_key(v, g * SEG + XR), lowest))
        while len(pairs) > 1:
            (a1, a2), (c1, c2) = pairs.pop(0), pairs.pop(0)
            pairs.append((jnp.maximum(a1, c1),
                          jnp.maximum(jnp.minimum(a1, c1), jnp.maximum(a2, c2))))

        tk = jnp.concatenate(pairs[0], axis=0)[:, 0:1]
        k1 = jnp.max(tk[0:8], axis=0, keepdims=True)
        k2 = jnp.max(jnp.where(tk == k1, jnp.iinfo(jnp.int32).min, tk), axis=0, keepdims=True)
        i1 = (S - 1) - (k1[0, 0] & (S - 1))
        i2 = (S - 1) - (k2[0, 0] & (S - 1))
        g1, g2 = i1 >> 5, i2 >> 5
        b1 = pl.multiple_of(i1 & 24, 8)
        b2 = pl.multiple_of(i2 & 24, 8)

        xa, ha_ = redo(g1, b1)
        xb_, hb_ = redo(g2, b2)
        x1 = jnp.concatenate([xa, xb_], axis=0)
        h2 = jnp.concatenate([ha_, hb_], axis=0)
        h2b = h2.astype(BF16)
        row = lax.broadcasted_iota(jnp.int32, (16, 1), 0)
        grow = jnp.where(row < 8, g1 * SEG + b1 + row, g2 * SEG + b2 + row - 8)
        ks = jnp.where(grow == i1, k1, k2)
        rsel = pltpu.bitcast((ks ^ ((ks >> 31) & 0x7FFF0000)) & -65536, F32)
        acts = []
        for j in range(FF // 128):
            gt = _rb(_dot(h2b, wg_s[j]))
            gt = _rb(gt * _rb(jax.nn.sigmoid(gt)))
            ut = _rb(_dot(h2b, wu_s[j]))
            acts.append((gt * ut).astype(BF16))
            if j < ntail:
                xo_, ho_ = redo(tail + j, XR, zero_after(ut[0:8]))
                outs[tail + j, XR:, :] = (xo_ + modv(5) * ho_).astype(BF16)
            if j == ntail - 1:
                out_copy(tail, NSEG - tail, XR, M).start()
        act = jnp.concatenate(acts, axis=1)
        y = _rb(jnp.concatenate([_dot(act, wd_s[j]) for j in range(NT)], axis=1))
        y = _rb(y * _rb(jax.nn.sigmoid(rsel)))
        sel = jnp.logical_or(grow == i1, grow == i2)
        gb2 = jnp.concatenate([modv(5)] * 2, axis=0)
        fixed = (x1 + gb2 * (h2 + jnp.where(sel, y, 0.0))).astype(BF16)

        with jax.named_scope("e_outwait"):
            out_copy(0, NSEG, 0, SEG).wait()
        outs[g1, pl.ds(b1, 8), :] = fixed[0:8]
        outs[g2, pl.ds(b2, 8), :] = fixed[8:16]
        out_copy(g1, 1, b1, 8, 0).start()

        @pl.when((i1 >> 3) != (i2 >> 3))
        def _():
            out_copy(g2, 1, b2, 8, 1).start()
            out_copy(g2, 1, b2, 8, 1).wait()

        out_copy(g1, 1, b1, 8, 0).wait()

    pl.run_scoped(
        main,
        pltpu.VMEM((FF // 128, D, 128), BF16),
        pltpu.VMEM((FF // 128, D, 128), BF16),
        pltpu.VMEM((NT, FF, 128), BF16),
        pltpu.VMEM((NSEG, SEG, D), BF16),
        pltpu.VMEM((2, NSEG, SEG, 128), F32),
        pltpu.VMEM((NSEG, SEG, D), BF16),
        pltpu.SemaphoreType.DMA((3,)),
    )


def _entry(*refs):
    pl.run_scoped(
        functools.partial(_kernel, *refs),
        pltpu.VMEM((NCHUNK, H, KQ // 2, DH), U32),
        pltpu.VMEM((NSEG + 1, NT, XR // 2, 128), U32),
        pltpu.VMEM((NT, (H * DH + H * DH // NT) // 2, 128), U32),
        pltpu.VMEM((3 * NP, NSEG, 2 * M, DH), F32),
        pltpu.VMEM((3 * H, SEG, DH), BF16),
        pltpu.VMEM((H, SEG // 2, DH), U32),
        pltpu.VMEM((H, NSEG // UNROLL, UNROLL * M // 2, DH), U32),
        pltpu.VMEM((NSEG, SEG, D), BF16),
        pltpu.VMEM((UNROLL, NT, SEG // 2, 128), U32),
        pltpu.VMEM((4, 4 * NT * UNROLL // NSEG, D, 128), BF16),
        pltpu.VMEM((8 * NT + 4, M, 128), F32),
        pltpu.VMEM((64, PR), F32),
        pltpu.VMEM((32, 128), jnp.int32),
        pltpu.VMEM((M, D), BF16),
        pltpu.VMEM((D, 128), F32),
        pltpu.VMEM((NP, SEG + M, PR), F32),
        pltpu.VMEM((8 + PAD, 128), U32),
        pltpu.SemaphoreType.DMA((4,)),
        pltpu.SemaphoreType.DMA((2,)),
    )


@functools.partial(jax.jit, static_argnames=("A_seg_len",))
def pallas_adaLN_cond__memory_aug_recurrent_mem_tr__moe_arch_mod__prompt_kernel(
    A_x: jax.Array,
    A_mem0: jax.Array,
    A_Wq: jax.Array,
    A_Wk: jax.Array,
    A_Wv: jax.Array,
    A_Wo: jax.Array,
    A_seg_len,
    B_x: jax.Array,
    B_w_r: jax.Array,
    B_w_gate: jax.Array,
    B_w_up: jax.Array,
    B_w_down: jax.Array,
    c: jax.Array,
    w_mod: jax.Array,
):
    assert A_seg_len == SEG and A_x.shape == (1, S, D)
    del B_x
    hbm = pl.BlockSpec(memory_space=pl.ANY)
    out = pl.pallas_call(
        _entry,
        out_shape=jax.ShapeDtypeStruct((NSEG, SEG, D), BF16),
        in_specs=[hbm] * 12,
        out_specs=hbm,
        compiler_params=pltpu.CompilerParams(vmem_limit_bytes=120 * 1024 * 1024,
                                             disable_bounds_checks=True),
    )(A_x.reshape(NSEG, SEG, D), A_mem0.reshape(M, D), A_Wq, A_Wk, A_Wv, A_Wo.reshape(H * DH, D),
      B_w_r, B_w_gate, B_w_up, B_w_down, c, w_mod)
    return out.reshape(1, S, D)
```

```python
import functools

import jax
import jax.numpy as jnp
from jax import lax
import jax.experimental.pallas as pl
import jax.experimental.pallas.tpu as pltpu

F32 = jnp.float32
BF16 = jnp.bfloat16
U32 = jnp.uint32

D = 1024
S = 2048
H = 32
DH = 128
M = 8
SEG = 32
NSEG = S // SEG
FF = 3584
NT = D // 128
XR = SEG - M
R0 = M * NSEG
CH = 8
KQ = D // 4
NCHUNK = 3 * D // KQ
NSLOT = 4
PR = 2 * SEG + 2 * M
NP = H // 2
EC = 128
NEC = R0 // EC
LOG2E = 1.4426950408889634
EPS = 1e-5
SCALE = DH ** -0.5
NEG_MASK = -1000000000.0

PHASES = ("pro", "step", "epi")

UNROLL = 4
PG = 4
LAG_S = 1
LAG_P = 4
O_PARTS = (0, 8, 12)
O_TH = (256, 256, 256, 1280)
REL_S = 3
REL_STAG = 2
G_AT = (0, 1, 2, 3, 7, 11)
GR = 32
G_LAG = 3
BLK = 32
JOB_SPAN = 40
RB = 16
RB2 = 64
FB = 32
GVR = 32
GV_FREE = 64
R_AT = ((0, 6, 16), (14, 22, 30), (30, 38, 46), (44, 52, 60))
F_AT = (0, 13)
L_AT = 8
GV_AT = (16, 56)
LNU = 16
LN_PH = (0, 8, 18)
EKH = 4
E_SPAN = 5
PAD = 24


def _schedule():
    groups = [list(range(g, g + PG)) for g in range(0, NP, PG)]
    at = {}
    for g, grp in enumerate(groups):
        at.setdefault(grp[-1] + LAG_P, []).extend(("P", q) for q in grp)
    for g, grp in enumerate(groups):
        at.setdefault(grp[-1] + LAG_S, []).extend(("S", q) for q in grp)
    ops = []
    for p in range(NP):
        ops.append(("Q", p, p == 0))
        if p in G_AT:
            ops.append(("G",))
        ops.extend(at.pop(p, []))
    bounds = list(O_PARTS) + [NP]
    t = NP
    done = 0
    for n in range(len(O_PARTS)):
        part = list(range(bounds[n], bounds[n + 1]))
        assert all(("P", q) in ops for q in part), (n, ops)
        for j in range(NT):
            ops.append(("O", j, part))
            if n == len(O_PARTS) - 1:
                ops.append(("F", j))
            done += len(part) * 16
            while t - NP < len(O_TH) and done >= O_TH[t - NP]:
                ops.extend(at.pop(t, []))
                t += 1
    assert not at
    return ops


def _rb(x):
    return x.astype(BF16).astype(F32)


def _recip(x):
    r = pl.reciprocal(x, approx=True)
    return r * (2.0 - x * r)


def _inv_std(xc):
    v = _rb(_rb(jnp.mean(xc * xc, axis=-1, keepdims=True)) + EPS)
    return _recip(_rb(v * lax.rsqrt(v)))


def _ln(x, zero=None):
    xm = x if zero is None else jnp.concatenate([x[..., :128] + zero, x[..., 128:]], axis=-1)
    xc = x - jnp.mean(xm, axis=-1, keepdims=True)
    return xc * _inv_std(xc)


def _dot(a, b):
    return jnp.dot(a, b, preferred_element_type=F32)


def _as_bf16(u):
    return pltpu.bitcast(u, BF16)


def _as_u32(b):
    return pltpu.bitcast(b, U32)


def _spread(jobs, fns, lo, hi):
    for n, fn in enumerate(fns):
        jobs.setdefault(lo + n * (hi - lo) // len(fns), []).append(fn)


def _kernel(x_hbm, mem0_hbm, wq_hbm, wk_hbm, wv_hbm, wo_hbm, wr_hbm, wg_hbm, wu_hbm, wd_hbm,
            c_hbm, wmod_hbm, out_hbm,
            wqkv, hs, wo_s, pre, cur_s, olhs, odef, xbuf, lhs, wm_s, mod, mk,
            top, sc_s, cb_s, ts_s, zero_s, sem_m, sem_out):
    mt = 4 * NT * UNROLL // NSEG

    def modv(j):
        return jnp.concatenate([mod[j * NT + k] for k in range(NT)], axis=1)

    def mod_store(v, t):
        v = _rb(v)
        mod[t] = jnp.where(jnp.logical_or((t >> 3) == 1, (t >> 3) == 4), _rb(1.0 + v), v)

    def mod_tile(wm, t):
        mod_store(_dot(sc_s[...], wm), t)

    def gemv_part(w, d0, acc):
        n = w.shape[1]
        p = w.astype(F32) * cb_s[d0:d0 + n, :]
        p = jnp.sum(p.reshape(w.shape[0], n // 8, 8, 128), axis=1)
        return p if acc is None else p + acc

    def gemv_finish(acc, ts):
        for u, t in enumerate(ts):
            mod_store(jnp.broadcast_to(jnp.sum(acc[u], axis=0, keepdims=True), (M, 128)), t)

    def wm_copy(it, u):
        col = pl.multiple_of((2 * NT + it * mt + u) * 128, 128)
        return pltpu.make_async_copy(wmod_hbm.at[:, pl.ds(col, 128)], wm_s.at[it & 3, u],
                                     sem_m.at[it & 3])

    def zero_after(y):
        return (y if y.dtype == U32 else pltpu.bitcast(y, U32)) & zero_s[0:8, :]

    def or_tile(u, z):
        if z is None:
            return u
        return (u.reshape(u.shape[0] // 8, 8, 128) | z).reshape(u.shape)

    def prologue(stage, wo_raw, wmod_s, nrm, ha, hb, tmp, mem0_ref, wr_ref, c_ref, sem):
        w_hbms = (wq_hbm, wk_hbm, wv_hbm)
        wob = H * DH // NT
        S_X, S_C0, S_ST, S_WO, S_MOD, S_SM = 0, 2, 6, 6 + NSLOT, 6 + NSLOT + NT, 6 + NSLOT + 2 * NT

        def x_copy(i):
            lo, n = ((XR, M), (0, XR))[i]
            return pltpu.make_async_copy(x_hbm.at[:, pl.ds(lo, n), :], xbuf.at[:, pl.ds(lo, n), :],
                                         sem.at[S_X + i])

        def mod_copies(k):
            return [pltpu.make_async_copy(wmod_hbm.at[:, pl.ds(v * D + k * 128, 128)],
                                          wmod_s.at[k, v], sem.at[S_MOD + (k if k < 2 else k & 6)])
                    for v in range(2)]

        def chunk_copy(mat, d0, g, slot, k):
            heads = pl.ds(pl.multiple_of(g * CH, CH), CH)
            return pltpu.make_async_copy(w_hbms[mat].at[pl.ds(d0, KQ), heads, :],
                                         stage.at[slot, g], sem.at[k])

        def wo_copy(j):
            return pltpu.make_async_copy(wo_hbm.at[pl.ds(pl.multiple_of(j * wob, wob), wob)],
                                         wo_raw.at[j], sem.at[S_WO + j])

        def relayout1(src, t0, z=None):
            v = src.reshape(RB * CH, 128)
            tmp[t0:t0 + RB * CH // 2, :] = or_tile(_as_u32(v), z)

        def relayout2(c, h0_, t0, d0, z=None, src=tmp):
            w = or_tile(src[pl.ds(t0, RB2, stride=CH // 2), :], z)
            rows = pl.ds(d0 // 2, RB2 // 2)
            wqkv[c, h0_, rows, :] = _as_u32(w.astype(jnp.uint16))
            wqkv[c, h0_ + 1, rows, :] = _as_u32((w >> 16).astype(jnp.uint16))

        def mod_pair(k):
            for v in range(2):
                mod_tile(wmod_s[k, v], v * NT + k)

        def fill(dst, q, t, r, z=None):
            k = 2 * q + t
            sh = mod[k] if z is None else mod[k] + pltpu.bitcast(z, F32)
            v = nrm[k, r:r + FB, :].reshape(FB // 8, 8, 128) * mod[NT + k] + sh
            dst[t, r // 2:(r + FB) // 2, :] = _as_u32(v.reshape(FB, 128).astype(BF16))

        small = [pltpu.make_async_copy(src, dst, sem.at[S_SM])
                 for src, dst in ((c_hbm, c_ref), (mem0_hbm, mem0_ref), (wr_hbm, wr_ref))]
        for cp in small:
            cp.start()
        x_copy(0).start()
        for cp in mod_copies(0) + mod_copies(1):
            cp.start()
        for g in range(4):
            chunk_copy(0, 0, g, 0, S_C0 + g).start()
        for c in range(1, NSLOT):
            for g in range(4):
                chunk_copy(c % 3, (c // 3) * KQ, g, c, S_ST + c).start()
            for cp in mod_copies(2 * c) + mod_copies(2 * c + 1):
                cp.start()

        kk = lax.broadcasted_iota(jnp.int32, (SEG + M, PR), 0)
        qq = lax.broadcasted_iota(jnp.int32, (SEG + M, PR), 1)
        k_mem = jnp.logical_and(kk >= XR, kk < SEG)
        k_pos = jnp.where(kk < SEG, kk, kk - M)
        q_mem = jnp.logical_and(qq < 2 * SEG, qq % SEG >= XR)
        q_pos = jnp.where(qq < 2 * SEG, qq % SEG, XR + qq % M)
        mk[0:SEG + M, :] = jnp.where(q_mem | k_mem | (q_pos >= k_pos), 0.0, 1.0).astype(F32)
        mod[0:2 * NT] = jnp.zeros((2 * NT, M, 128), F32)
        zero_s[...] = jnp.zeros(zero_s.shape, U32)
        top[...] = jnp.full(top.shape, jnp.iinfo(jnp.int32).min, jnp.int32)
        for cp in small:
            cp.wait()
        wr = jnp.broadcast_to(wr_ref[...].astype(F32).reshape(1, D), (M, D))
        for k in range(NT):
            mod[6 * NT + k] = wr[:, k * 128:(k + 1) * 128]
        cv = c_ref[...].astype(F32)
        sc = _rb(cv * _rb(jax.nn.sigmoid(cv)))
        sc_s[...] = jnp.broadcast_to(sc, (M, D)).astype(BF16)
        for k in range(NT):
            cb_s[k * 128:(k + 1) * 128, :] = jnp.broadcast_to(
                sc[:, k * 128:(k + 1) * 128], (128, 128)).T
        mb = mem0_ref[...]
        for k in range(NT):
            lhs[0, k, XR // 2:, :] = _as_u32(mb[:, k * 128:(k + 1) * 128])

        def zero_body(i, c):
            wo_raw[NT, pl.ds(pl.multiple_of(i * 32, 32), 32), :] = jnp.zeros((32, D), BF16)
            return c

        lax.fori_loop(0, wob // 32, zero_body, 0)
        x_copy(0).wait()

        def ln_body(i, c):
            for u in range(LNU):
                q = i * LNU + u
                v = _ln(xbuf[q, XR:, :].astype(F32))
                for k in range(NT):
                    nrm[k, pl.ds(pl.multiple_of(q * 8, 8), 8), :] = v[:, k * 128:(k + 1) * 128]
            return c

        with jax.named_scope("p_ln"):
            lax.fori_loop(0, NSEG // LNU, ln_body, 0)

        def mod_body(k, c):
            pltpu.make_async_copy(wmod_s.at[k], wmod_s.at[k], sem.at[S_MOD + k]).wait()
            mod_pair(k)
            for r in range(0, R0, FB):
                fill(ha, 0, k, r)
            return c

        with jax.named_scope("p_mod"):
            lax.fori_loop(0, 2, mod_body, 0)

        def hop1(g):
            chunk_copy(0, 0, g, 0, S_C0 + g).wait()

            def body(i, c):
                d0 = pl.multiple_of(i * 128, 128)
                v = stage[0, g, pl.ds(d0, 128)].reshape(128 * CH, 128)
                t0 = pl.multiple_of((g * KQ + d0) * (CH // 2), 512)
                tmp[pl.ds(t0, 128 * CH // 2), :] = _as_u32(v)
                return c

            lax.fori_loop(0, KQ // 128, body, 0)

        def hop2(c, g, j):
            src = tmp.at[pl.ds(pl.multiple_of(g * (KQ * CH // 2), 512), KQ * CH // 2 + 8)]
            for d0 in range(0, KQ, RB2):
                relayout2(c, g * CH + 2 * j, d0 * CH // 2 + j, d0, src=src)

        def bulk(units, jobs):
            due = {}
            t0 = 0
            for n, (hq, c, h0_, pi, first, r0, nrow) in enumerate(units):
                nb = nrow // BLK
                parts = []
                for u in range(nb):
                    part = hq[0, (r0 + u * BLK) // 2:(r0 + (u + 1) * BLK) // 2, :]
                    for z in due.pop(t0 + u, ()):
                        part = jnp.concatenate([part[0:8] | z, part[8:]], axis=0)
                    parts.append(part)
                hv = jnp.concatenate([_as_bf16(jnp.concatenate(parts, axis=0)),
                                      _as_bf16(hq[1, r0 // 2:(r0 + nrow) // 2, :])], axis=1)
                w = jnp.concatenate([_as_bf16(wqkv[c, h0_]), _as_bf16(wqkv[c, h0_ + 1])], axis=1)
                y = _dot(hv, w)
                segs = slice(r0 // M, (r0 + nrow) // M)
                for a in range(2):
                    old = jnp.where(first, 0.0, pre[pi, segs, a * M:(a + 1) * M, :])
                    pre[pi, segs, a * M:(a + 1) * M, :] = (
                        y[:, a * DH:(a + 1) * DH].reshape(nrow // M, M, DH) + old)
                for u in range(nb):
                    for job in jobs.get(t0 + u, ()):
                        res = job(zero_after(y[u * BLK:u * BLK + 8, 0:128]))
                        if res is not None:
                            due.setdefault(max(t0 + u + JOB_SPAN, t0 + nb), []).append(
                                zero_after(res))
                t0 += nb
            assert not due

        GP = CH // 2
        WO0 = NCHUNK - 1 - NT
        LN0 = 4
        SPI = -(-NSEG // (NCHUNK - 1 - LN0))

        def rot_body(i, c):
            slot = (i + 1) & (NSLOT - 1)
            pltpu.make_async_copy(stage.at[slot], stage.at[slot], sem.at[S_ST + slot]).wait()
            km = 2 * jnp.minimum(i, 3)

            @pl.when(jnp.logical_and(i >= 1, i <= 3))
            def _():
                wq = wmod_s.at[pl.ds(km, 2)]
                pltpu.make_async_copy(wq, wq, sem.at[S_MOD + km]).wait()

            @pl.when(i == LN0)
            def _():
                x_copy(1).wait()

            @pl.when(i >= WO0)
            def _():
                wo_copy(i - WO0).wait()

            nxt = i + NSLOT
            qn = (nxt * 43) >> 7
            for mat in range(3):
                @pl.when(jnp.logical_and(nxt < NCHUNK, nxt - 3 * qn == mat))
                def _():
                    for g in range(4):
                        chunk_copy(mat, qn * KQ, g, nxt & (NSLOT - 1),
                                   S_ST + (nxt & (NSLOT - 1))).start()

            @pl.when(i < NT)
            def _():
                wo_copy(i).start()

            @pl.when(i == 0)
            def _():
                x_copy(1).start()

            q0 = (i * 43) >> 7
            q1 = ((i + 1) * 43) >> 7
            pa = (i - 3 * q0) * NP + NP - GP
            units = ([(ha, i, H - CH + 2 * n, pa + n, q0 == 0, 0, R0) for n in range(GP)]
                     + [(hb, i + 1, 2 * n, (i + 1 - 3 * q1) * NP + n, q1 == 0, 0, R0)
                        for n in range(NP - GP)])
            jw = jnp.where(i >= WO0, i - WO0, NT)

            def wo_job(b, z):
                v = wo_raw[jw, b * 16:(b + 1) * 16, :]
                rows = pl.ds(pl.multiple_of(jw * (wob // 2) + b * 8, 8), 8)
                for j in range(NT):
                    wo_s[j, rows, :] = _as_u32(v[:, j * 128:(j + 1) * 128]) | z

            lst = {}

            def ln_job(b, ph, z):
                r = (b % 3) * 8
                seg = (i - LN0) * SPI + b // 3
                live = jnp.logical_and(i >= LN0, seg < NSEG)
                src = jnp.where(live, seg, 0) + (i >> (10 + ph))
                x = xbuf[src, pl.ds(pl.multiple_of(jnp.where(live, r, XR), 8), 8), :].astype(F32)
                zf = pltpu.bitcast(z, F32)
                if ph == 0:
                    xm = jnp.concatenate([x[:, :128] + zf, x[:, 128:]], axis=1)
                    mu = jnp.mean(xm, axis=-1, keepdims=True)
                    lst[2 * b] = jnp.broadcast_to(mu, (8, 128))
                    return None
                xc = x - jnp.concatenate([lst[2 * b] + zf] * NT, axis=1)
                if ph == 1:
                    lst[2 * b + 1] = jnp.broadcast_to(_inv_std(xc), (8, 128))
                    return None
                inv = jnp.concatenate([lst[2 * b + 1]] * NT, axis=1)
                hv = (xc * inv * modv(1) + modv(0)).astype(BF16)
                u = [_as_u32(hv[:, k * 128:(k + 1) * 128]) for k in range(NT)]
                dst = jnp.where(live, seg, NSEG)
                for k in range(NT):
                    hs[dst, k, r // 2:r // 2 + 4, :] = u[k]
                res = jnp.concatenate(u[0:2], axis=0)
                for k in range(2, NT, 2):
                    res = res | jnp.concatenate(u[k:k + 2], axis=0)
                return res

            def r1_job(g, d0, z):
                relayout1(stage[slot, g, d0:d0 + RB], (g * KQ + d0) * CH // 2, z)

            def copy_job(t, r, z):
                ha[t, r:r + 32, :] = or_tile(hb[t, r:r + 32, :], z)

            P = functools.partial
            upb = R0 // BLK
            nr = NP * upb
            jobs = {}
            for g in range(4):
                lo, mid, hi = (x * upb // 4 for x in R_AT[g])
                _spread(jobs, [P(r1_job, g, d0) for d0 in range(0, KQ, RB)], lo, mid)
                _spread(jobs, [P(relayout2, i + 1, g * CH + 2 * j, (g * KQ + d0) * CH // 2 + j, d0)
                               for j in range(CH // 2) for d0 in range(0, KQ, RB2)], mid, hi)
            oz = i >> 10
            _spread(jobs, [P(fill, hb, q1, t + oz, r) for r in range(0, R0, FB) for t in range(2)],
                    F_AT[0] * upb // 4, F_AT[1] * upb // 4)
            _spread(jobs, [P(copy_job, t, r) for t in range(2) for r in range(0, R0 // 2, 32)],
                    2 * GP * upb, nr - upb)
            for ph in range(3):
                off = LN_PH[ph] - LN_PH[2]
                _spread(jobs, [P(ln_job, b, ph) for b in range(3 * SPI)],
                        L_AT * upb // 4 + LN_PH[ph], nr - max(upb, JOB_SPAN) + off)
            _spread(jobs, [P(wo_job, b) for b in range(wob // 16)], GP * upb, nr - upb)
            gv = {}

            def gv_job(d0, n, z):
                w = wmod_s[pl.ds(km, 2), :, d0:d0 + n, :].reshape(4, n, 128)
                acc = gv.get("acc")
                if z is not None:
                    zf = pltpu.bitcast(z, F32)[None]
                    acc = jnp.broadcast_to(zf, (4, 8, 128)) if acc is None else acc + zf
                gv["acc"] = gemv_part(w, d0, acc)
                if z is not None:
                    au = pltpu.bitcast(gv["acc"], U32)
                    return au[0] | au[1] | au[2] | au[3]

            _spread(jobs, [P(gv_job, d0, GVR) for d0 in range(0, D - GV_FREE, GVR)],
                    GV_AT[0] * upb // 4, min(GV_AT[1] * upb // 4, nr - JOB_SPAN))
            bulk(units, jobs)
            if GV_FREE:
                gv_job(D - GV_FREE, GV_FREE, None)
            gemv_finish(gv["acc"], [km, NT + km, km + 1, NT + km + 1])
            return c

        def outer(k, c):
            last = k == 4

            @pl.when(k < 4)
            def _():
                hop1(k)

            @pl.when(k != 3)
            def _():
                g = jnp.minimum(k, 3)
                cc = jnp.where(last, NCHUNK - 1, 0)
                for j in range(GP):
                    hop2(cc, g, j)
                bulk([(ha, cc, g * CH + 2 * n, jnp.where(last, 2 * NP, 0) + g * GP + n, k < 4,
                       0, R0) for n in range(GP)], {})

            @pl.when(k == 3)
            def _():
                for j in range(GP):
                    hop2(0, 3, j)
                with jax.named_scope("p_rot"):
                    lax.fori_loop(0, NCHUNK - 1, rot_body, 0)
                for it in range(2):
                    for u in range(mt):
                        wm_copy(it, u).start()

            return c

        with jax.named_scope("p_bulk"):
            lax.fori_loop(0, 5, outer, 0)

    if "pro" in PHASES: pl.run_scoped(
        prologue,
        pltpu.VMEM((NSLOT, H // CH, KQ, CH, 128), BF16),
        pltpu.VMEM((NT + 1, H * DH // NT, D), BF16),
        pltpu.VMEM((NT, 2, D, 128), BF16),
        pltpu.VMEM((NT, R0, 128), F32),
        pltpu.VMEM((2, R0 // 2, 128), U32),
        pltpu.VMEM((2, R0 // 2, 128), U32),
        pltpu.VMEM((D * CH // 2 + 32, 128), U32),
        pltpu.VMEM((M, D), BF16),
        pltpu.VMEM((D,), BF16),
        pltpu.VMEM((1, D), BF16),
        pltpu.SemaphoreType.DMA((7 + NSLOT + 2 * NT,)),
    )

    def main(wg_s, wu_s, wd_s, ybuf, stat, outs, sem_f):
        def load_x_rows(slot, seg):
            for k in range(NT):
                lhs[slot, k, 0:XR // 2, :] = hs[seg, k]

        def resid(seg, r, z=None):
            rows = pl.ds(r, 8)
            t = modv(2) * ybuf[seg, rows, :].astype(F32)
            if z is not None:
                t = t + jnp.concatenate([pltpu.bitcast(z, F32)] * NT, axis=1)
            return xbuf[seg, rows, :].astype(F32) + t

        def wide(v):
            return jnp.concatenate([v] * NT, axis=1)

        def make_key(v, row0):
            b = pltpu.bitcast(jnp.where(v != v, -jnp.inf, v + 0.0), jnp.int32)
            low = (S - 1 - row0) - lax.broadcasted_iota(jnp.int32, (8, 128), 0)
            return (b ^ ((b >> 31) & 0x7FFF0000)) | low

        def post(seg, r, z):
            x1 = resid(seg, r, z)
            mu = jnp.mean(x1, axis=-1, keepdims=True)
            xc = x1 - mu
            inv = _inv_std(xc)
            stat[0, seg, pl.ds(r, 8), :] = jnp.broadcast_to(mu, (8, 128))
            stat[1, seg, pl.ds(r, 8), :] = jnp.broadcast_to(inv, (8, 128))
            v = _rb(inv * jnp.sum(xc * modv(7), axis=-1, keepdims=True) + mod[8 * NT])
            key = make_key(v, seg * SEG + r)
            m1, m2 = top[0:8, :], top[8:16, :]
            top[8:16, :] = jnp.maximum(m2, jnp.minimum(m1, key))
            top[0:8, :] = jnp.maximum(m1, key)
            o = x1 + modv(5) * (xc * inv * modv(4) + modv(3))
            outs[seg, pl.ds(r, 8), :] = o.astype(BF16)
            res = pltpu.bitcast(v, U32)
            for k in range(NT):
                res = res | pltpu.bitcast(o[:, k * 128:(k + 1) * 128], U32)
            return res

        def redo(seg, r, z=None):
            x1 = resid(seg, r, z)
            n = (x1 - wide(stat[0, seg, pl.ds(r, 8), :])) * wide(stat[1, seg, pl.ds(r, 8), :])
            return x1, n * modv(4) + modv(3)

        def out_copy(g0, ng, r, n, k=0):
            return pltpu.make_async_copy(outs.at[pl.ds(g0, ng), pl.ds(r, n), :],
                                         out_hbm.at[pl.ds(g0, ng), pl.ds(r, n), :], sem_out.at[k])

        late = ((wg_hbm, wg_s, FF // 128), (wu_hbm, wu_s, FF // 128), (wd_hbm, wd_s, NT))

        def col_copy(k, j):
            return pltpu.make_async_copy(
                late[k][0].at[:, pl.ds(pl.multiple_of(j * 128, 128), 128)], late[k][1].at[j],
                sem_f.at[k])

        load_x_rows(0, 0)

        def step(it, cur, state):
            s = it * UNROLL + cur
            nxt = (cur + 1) % UNROLL

            def pay(t, cost):
                now, due = state["now"], state["due"]
                for z in [z for (d, z) in due if d <= now]:
                    t = jnp.concatenate([t[0:8] | z, t[8:]], axis=0)
                state["due"] = [(d, z) for (d, z) in due if d > now]
                state["now"] = now + cost
                return t

            def release(y):
                now = state["now"]
                pend, state["pend"] = state["pend"], [e for e in state["pend"] if e[0] > now]
                for (d, f) in pend:
                    if d <= now:
                        f(zero_after(y[0:8]))

            def lv(k0, k1):
                ts = [lhs[cur, k] for k in range(k0, k1)]
                ts[0] = pay(ts[0], (k1 - k0) / NT)
                return jnp.concatenate([_as_bf16(t) for t in ts], axis=1)

            def wmat(mat, h, q0, q1):
                return _as_bf16(jnp.concatenate([wqkv[3 * q + mat, h] for q in range(q0, q1)],
                                                axis=0))

            def qkv(p, split=False):
                part = {}
                if split:
                    for mat in range(3):
                        for a in range(2):
                            part[mat, a] = _dot(lv(0, NT // 2), wmat(mat, 2 * p + a, 0, 2))
                for mat in range(3):
                    for a in range(2):
                        hm = mat * H + 2 * p + a
                        if split:
                            y = _dot(lv(NT // 2, NT), wmat(mat, 2 * p + a, 2, 4)) + part[mat, a]
                        else:
                            y = _dot(lv(0, NT), wmat(mat, 2 * p + a, 0, 4))
                        cur_s[hm] = y.astype(BF16)
                        release(y)

            def gather(mat, p):
                hm = mat * H + 2 * p
                return jnp.concatenate(
                    [cur_s[hm], cur_s[hm + 1], pre[mat * NP + p, s].astype(BF16)], axis=0)

            probs = {}

            def scores(p):
                st = lax.dot_general(gather(1, p), gather(0, p), (((1,), (1,)), ((), ())),
                                     preferred_element_type=F32)
                lane = lax.broadcasted_iota(jnp.int32, (1, PR), 1)
                is_a = jnp.logical_or(lane < SEG,
                                      jnp.logical_and(lane >= 2 * SEG, lane < 2 * SEG + M))
                ka = jnp.concatenate([st[0:SEG], st[2 * SEG:2 * SEG + M]], axis=0)
                kb = jnp.concatenate([st[SEG:2 * SEG], st[2 * SEG + M:]], axis=0)
                t = jnp.where(is_a, ka, kb) * (SCALE * LOG2E)
                ts_s[p + (it >> 10)] = jnp.where(mk[0:SEG + M, :] == 0.0, t, NEG_MASK * LOG2E)

                def softmax(z):
                    zf = pltpu.bitcast(z, F32)[:, 0:PR]
                    t = (ts_s[p].reshape(-1, 8, PR) + zf).reshape(SEG + M, PR)
                    e = jnp.exp2(t - jnp.max(t, axis=0, keepdims=True))
                    e = e * _recip(jnp.sum(e, axis=0, keepdims=True))
                    pa = jnp.where(is_a, e, 0.0)
                    pb = jnp.where(is_a, 0.0, e)
                    probs[p] = jnp.concatenate(
                        [pa[0:SEG], pb[0:SEG], pa[SEG:], pb[SEG:]], axis=0).astype(BF16)

                state["pend"].append((state["now"] + REL_S + (p % PG) * REL_STAG, softmax))

            def pv(p):
                o = lax.dot_general(probs.pop(p), gather(2, p), (((0,), (0,)), ((), ())),
                                    preferred_element_type=F32).astype(BF16)
                for a in range(2):
                    h = 2 * p + a
                    olhs[h] = _as_u32(o[a * SEG:(a + 1) * SEG])
                    odef[h, it, cur * 4:(cur + 1) * 4, :] = _as_u32(
                        o[2 * SEG + a * M:2 * SEG + (a + 1) * M])

            acc = [None] * NT

            def oproj(j, pairs):
                ts = [olhs[2 * p + a] for p in pairs for a in range(2)]
                ts[0] = pay(ts[0], len(pairs) / 4)
                ov = jnp.concatenate([_as_bf16(t) for t in ts], axis=1)
                w = wo_s[j, pairs[0] * DH:(pairs[-1] + 1) * DH, :]
                y = _dot(ov, _as_bf16(w))
                acc[j] = y if acc[j] is None else y + acc[j]
                release(acc[j])

            def fin(j):
                yb = acc[j].astype(BF16)
                ybuf[s, 0:XR, j * 128:(j + 1) * 128] = yb[0:XR]
                lhs[nxt, j, XR // 2:, :] = _as_u32(yb[XR:])

            def gemv():
                d0 = state["d0"]
                state["acc"] = gemv_part(wm_s[it & 3, :, d0:d0 + GR, :], d0, state["acc"])
                state["d0"] = d0 + GR
                au = pltpu.bitcast(state["acc"], U32)
                z = functools.reduce(lambda a, b: a | b, [au[u] for u in range(mt)])
                state["due"].append((state["now"] + G_LAG, zero_after(z)))

            load_x_rows(nxt, jnp.minimum(s + 1, NSEG - 1))
            ops = dict(Q=qkv, S=scores, P=pv, O=oproj, F=fin, G=gemv)
            for op in _schedule():
                ops[op[0]](*op[1:])

        def steps(it, carry):
            if "pro" in PHASES:
                pltpu.make_async_copy(wm_s.at[it & 3], wm_s.at[it & 3], sem_m.at[it & 3]).wait()

                @pl.when(it + 2 < NSEG // UNROLL)
                def _():
                    for u in range(mt):
                        wm_copy(it + 2, u).start()

            for u in range(UNROLL // 2):
                t = it * (UNROLL // 2) + u
                for k in range(3):
                    @pl.when(t < late[k][2])
                    def _():
                        col_copy(k, t).start()

            state = dict(now=0, due=[], pend=[], d0=0, acc=None)
            for u in range(UNROLL):
                step(it, u, state)
            acc = state["acc"]
            for d0 in range(state["d0"], D, 64):
                acc = gemv_part(wm_s[it & 3, :, d0:min(d0 + 64, D), :], d0, acc)
            gemv_finish(acc, [2 * NT + it * mt + u for u in range(mt)])
            return carry

        with jax.named_scope("m_steps"):
            if "step" in PHASES: lax.fori_loop(0, NSEG // UNROLL, steps, 0)
        for k in range(3):
            for j in range(late[k][2]):
                col_copy(k, j).wait()
        if "epi" not in PHASES:
            cp = pltpu.make_async_copy(ybuf, out_hbm, sem_out.at[0])
            cp.start()
            cp.wait()
            return

        ntail = EC // M
        ppi = (S // 8 - ntail) // NEC
        gpi = ppi // (XR // 8)
        nblk = EC // (UNROLL * M)

        def ep_body(i, c):
            @pl.when(i > 0)
            def _():
                out_copy((i - 1) * gpi, gpi, 0, XR).start()

            for k in range(NT):
                mod[7 * NT + k] = mod[4 * NT + k] * mod[6 * NT + k]
            mod[8 * NT] = jnp.broadcast_to(
                jnp.sum(modv(3) * modv(6), axis=-1, keepdims=True), (M, 128))

            jobs = {}
            _spread(jobs, list(range(ppi)), 0, NT * H // EKH - E_SPAN)
            due = {}
            n = 0
            for j in range(NT):
                for h0_ in range(0, H, EKH):
                    ts = [odef[h, pl.ds(i * nblk, nblk)].reshape(EC // 2, DH)
                          for h in range(h0_, h0_ + EKH)]
                    for z in due.pop(n, ()):
                        ts[0] = jnp.concatenate([ts[0][0:8] | z, ts[0][8:]], axis=0)
                    w = wo_s[j, h0_ * DH // 2:(h0_ + EKH) * DH // 2, :]
                    yp = _dot(jnp.concatenate([_as_bf16(t) for t in ts], axis=1), _as_bf16(w))
                    y = yp if h0_ == 0 else yp + y
                    if h0_ + EKH == H:
                        ybuf[pl.ds(i * ntail, ntail), XR:, j * 128:(j + 1) * 128] = (
                            y.reshape(ntail, M, 128).astype(BF16))
                    for u in jobs.get(n, ()):
                        t = i * ppi + u
                        early = t < NSEG * (XR // 8)
                        seg = jnp.where(early, t // (XR // 8), t - NSEG * (XR // 8))
                        row = pl.multiple_of(jnp.where(early, (t % (XR // 8)) * 8, XR), 8)
                        res = post(seg, row, zero_after(y[0:8]))
                        due.setdefault(n + E_SPAN, []).append(zero_after(res))
                    n += 1
            return c

        with jax.named_scope("e_loop"):
            lax.fori_loop(0, NEC, ep_body, 0)
        done = (NEC - 1) * gpi
        tail = NSEG - ntail
        out_copy(done, NSEG - done, 0, XR).start()
        out_copy(0, tail, XR, M).start()
        x1s = [resid(g, XR) for g in range(tail, NSEG)]
        mus = [jnp.mean(x1, axis=-1, keepdims=True) for x1 in x1s]
        pairs = [(top[0:8, :], top[8:16, :])]
        lowest = jnp.full((8, 128), jnp.iinfo(jnp.int32).min, jnp.int32)
        for g in range(tail, NSEG):
            xc = x1s[g - tail] - mus[g - tail]
            inv = _inv_std(xc)
            stat[0, g, XR:, :] = jnp.broadcast_to(mus[g - tail], (8, 128))
            stat[1, g, XR:, :] = jnp.broadcast_to(inv, (8, 128))
            v = _rb(inv * jnp.sum(xc * modv(7), axis=-1, keepdims=True) + mod[8 * NT])
            pairs.append((make_key(v, g * SEG + XR), lowest))
        while len(pairs) > 1:
            (a1, a2), (c1, c2) = pairs.pop(0), pairs.pop(0)
            pairs.append((jnp.maximum(a1, c1),
                          jnp.maximum(jnp.minimum(a1, c1), jnp.maximum(a2, c2))))

        tk = jnp.concatenate(pairs[0], axis=0)[:, 0:1]
        k1 = jnp.max(tk[0:8], axis=0, keepdims=True)
        k2 = jnp.max(jnp.where(tk == k1, jnp.iinfo(jnp.int32).min, tk), axis=0, keepdims=True)
        i1 = (S - 1) - (k1[0, 0] & (S - 1))
        i2 = (S - 1) - (k2[0, 0] & (S - 1))
        g1, g2 = i1 >> 5, i2 >> 5
        b1 = pl.multiple_of(i1 & 24, 8)
        b2 = pl.multiple_of(i2 & 24, 8)

        xa, ha_ = redo(g1, b1)
        xb_, hb_ = redo(g2, b2)
        x1 = jnp.concatenate([xa, xb_], axis=0)
        h2 = jnp.concatenate([ha_, hb_], axis=0)
        h2b = h2.astype(BF16)
        row = lax.broadcasted_iota(jnp.int32, (16, 1), 0)
        grow = jnp.where(row < 8, g1 * SEG + b1 + row, g2 * SEG + b2 + row - 8)
        ks = jnp.where(grow == i1, k1, k2)
        rsel = pltpu.bitcast((ks ^ ((ks >> 31) & 0x7FFF0000)) & -65536, F32)
        acts = []
        for j in range(FF // 128):
            gt = _rb(_dot(h2b, wg_s[j]))
            gt = _rb(gt * _rb(jax.nn.sigmoid(gt)))
            ut = _rb(_dot(h2b, wu_s[j]))
            acts.append((gt * ut).astype(BF16))
            if j < ntail:
                xo_, ho_ = redo(tail + j, XR, zero_after(ut[0:8]))
                outs[tail + j, XR:, :] = (xo_ + modv(5) * ho_).astype(BF16)
            if j == ntail - 1:
                out_copy(tail, NSEG - tail, XR, M).start()
        act = jnp.concatenate(acts, axis=1)
        y = _rb(jnp.concatenate([_dot(act, wd_s[j]) for j in range(NT)], axis=1))
        y = _rb(y * _rb(jax.nn.sigmoid(rsel)))
        sel = jnp.logical_or(grow == i1, grow == i2)
        gb2 = jnp.concatenate([modv(5)] * 2, axis=0)
        fixed = (x1 + gb2 * (h2 + jnp.where(sel, y, 0.0))).astype(BF16)

        with jax.named_scope("e_outwait"):
            out_copy(0, NSEG, 0, SEG).wait()
        outs[g1, pl.ds(b1, 8), :] = fixed[0:8]
        outs[g2, pl.ds(b2, 8), :] = fixed[8:16]
        out_copy(g1, 1, b1, 8, 0).start()

        @pl.when((i1 >> 3) != (i2 >> 3))
        def _():
            out_copy(g2, 1, b2, 8, 1).start()
            out_copy(g2, 1, b2, 8, 1).wait()

        out_copy(g1, 1, b1, 8, 0).wait()

    pl.run_scoped(
        main,
        pltpu.VMEM((FF // 128, D, 128), BF16),
        pltpu.VMEM((FF // 128, D, 128), BF16),
        pltpu.VMEM((NT, FF, 128), BF16),
        pltpu.VMEM((NSEG, SEG, D), BF16),
        pltpu.VMEM((2, NSEG, SEG, 128), F32),
        pltpu.VMEM((NSEG, SEG, D), BF16),
        pltpu.SemaphoreType.DMA((3,)),
    )


def _entry(*refs):
    pl.run_scoped(
        functools.partial(_kernel, *refs),
        pltpu.VMEM((NCHUNK, H, KQ // 2, DH), U32),
        pltpu.VMEM((NSEG + 1, NT, XR // 2, 128), U32),
        pltpu.VMEM((NT, (H * DH + H * DH // NT) // 2, 128), U32),
        pltpu.VMEM((3 * NP, NSEG, 2 * M, DH), F32),
        pltpu.VMEM((3 * H, SEG, DH), BF16),
        pltpu.VMEM((H, SEG // 2, DH), U32),
        pltpu.VMEM((H, NSEG // UNROLL, UNROLL * M // 2, DH), U32),
        pltpu.VMEM((NSEG, SEG, D), BF16),
        pltpu.VMEM((UNROLL, NT, SEG // 2, 128), U32),
        pltpu.VMEM((4, 4 * NT * UNROLL // NSEG, D, 128), BF16),
        pltpu.VMEM((8 * NT + 4, M, 128), F32),
        pltpu.VMEM((64, PR), F32),
        pltpu.VMEM((32, 128), jnp.int32),
        pltpu.VMEM((M, D), BF16),
        pltpu.VMEM((D, 128), F32),
        pltpu.VMEM((NP, SEG + M, PR), F32),
        pltpu.VMEM((8 + PAD, 128), U32),
        pltpu.SemaphoreType.DMA((4,)),
        pltpu.SemaphoreType.DMA((2,)),
    )


@functools.partial(jax.jit, static_argnames=("A_seg_len",))
def pallas_adaLN_cond__memory_aug_recurrent_mem_tr__moe_arch_mod__prompt_kernel(
    A_x: jax.Array,
    A_mem0: jax.Array,
    A_Wq: jax.Array,
    A_Wk: jax.Array,
    A_Wv: jax.Array,
    A_Wo: jax.Array,
    A_seg_len,
    B_x: jax.Array,
    B_w_r: jax.Array,
    B_w_gate: jax.Array,
    B_w_up: jax.Array,
    B_w_down: jax.Array,
    c: jax.Array,
    w_mod: jax.Array,
):
    assert A_seg_len == SEG and A_x.shape == (1, S, D)
    del B_x
    hbm = pl.BlockSpec(memory_space=pl.ANY)
    out = pl.pallas_call(
        _entry,
        out_shape=jax.ShapeDtypeStruct((NSEG, SEG, D), BF16),
        in_specs=[hbm] * 12,
        out_specs=hbm,
        compiler_params=pltpu.CompilerParams(vmem_limit_bytes=120 * 1024 * 1024,
                                             disable_bounds_checks=True),
    )(A_x.reshape(NSEG, SEG, D), A_mem0.reshape(M, D), A_Wq, A_Wk, A_Wv, A_Wo.reshape(H * DH, D),
      B_w_r, B_w_gate, B_w_up, B_w_down, c, w_mod)
    return out.reshape(1, S, D)
```

```python
import functools

import jax
import jax.numpy as jnp
from jax import lax
import jax.experimental.pallas as pl
import jax.experimental.pallas.tpu as pltpu

F32 = jnp.float32
BF16 = jnp.bfloat16
U32 = jnp.uint32

D = 1024
S = 2048
H = 32
DH = 128
M = 8
SEG = 32
NSEG = S // SEG
FF = 3584
NT = D // 128
XR = SEG - M
R0 = M * NSEG
CH = 8
KQ = D // 4
NCHUNK = 3 * D // KQ
NSLOT = 4
PR = 2 * SEG + 2 * M
NP = H // 2
EC = 128
NEC = R0 // EC
LOG2E = 1.4426950408889634
EPS = 1e-5
SCALE = DH ** -0.5
NEG_MASK = -1000000000.0

PHASES = ("pro", "step", "epi")

UNROLL = 4
PG = 4
LAG_S = 1
LAG_P = 4
O_PARTS = (0, 8, 12)
O_TH = (256, 256, 256, 1280)
REL_S = 3
REL_STAG = 2
G_AT = (0, 1, 2, 3, 7, 11)
GR = 32
G_LAG = 3
BLK = 32
JOB_SPAN = 40
RB = 16
RB2 = 64
FB = 32
GVR = 32
GV_FREE = 64
R_AT = ((0, 6, 16), (14, 22, 30), (30, 38, 46), (44, 52, 60))
F_AT = (0, 13)
L_AT = 8
GV_AT = (16, 56)
LNU = 16
LN_PH = (0, 8, 18)
EKH = 4
E_SPAN = 5
TW = 4
T_END = 32
PAD = 24


def _schedule():
    groups = [list(range(g, g + PG)) for g in range(0, NP, PG)]
    at = {}
    for g, grp in enumerate(groups):
        at.setdefault(grp[-1] + LAG_P, []).extend(("P", q) for q in grp)
    for g, grp in enumerate(groups):
        at.setdefault(grp[-1] + LAG_S, []).extend(("S", q) for q in grp)
    ops = []
    for p in range(NP):
        ops.append(("Q", p, p == 0))
        if p in G_AT:
            ops.append(("G",))
        ops.extend(at.pop(p, []))
    bounds = list(O_PARTS) + [NP]
    t = NP
    done = 0
    for n in range(len(O_PARTS)):
        part = list(range(bounds[n], bounds[n + 1]))
        assert all(("P", q) in ops for q in part), (n, ops)
        for j in range(NT):
            ops.append(("O", j, part))
            if n == len(O_PARTS) - 1:
                ops.append(("F", j))
            done += len(part) * 16
            while t - NP < len(O_TH) and done >= O_TH[t - NP]:
                ops.extend(at.pop(t, []))
                t += 1
    assert not at
    return ops


def _rb(x):
    return x.astype(BF16).astype(F32)


def _recip(x):
    r = pl.reciprocal(x, approx=True)
    return r * (2.0 - x * r)


def _inv_std(xc):
    v = _rb(_rb(jnp.mean(xc * xc, axis=-1, keepdims=True)) + EPS)
    return _recip(_rb(v * lax.rsqrt(v)))


def _ln(x, zero=None):
    xm = x if zero is None else jnp.concatenate([x[..., :128] + zero, x[..., 128:]], axis=-1)
    xc = x - jnp.mean(xm, axis=-1, keepdims=True)
    return xc * _inv_std(xc)


def _dot(a, b):
    return jnp.dot(a, b, preferred_element_type=F32)


def _as_bf16(u):
    return pltpu.bitcast(u, BF16)


def _as_u32(b):
    return pltpu.bitcast(b, U32)


def _spread(jobs, fns, lo, hi):
    for n, fn in enumerate(fns):
        jobs.setdefault(lo + n * (hi - lo) // len(fns), []).append(fn)


def _kernel(x_hbm, mem0_hbm, wq_hbm, wk_hbm, wv_hbm, wo_hbm, wr_hbm, wg_hbm, wu_hbm, wd_hbm,
            c_hbm, wmod_hbm, out_hbm,
            wqkv, hs, wo_s, pre, cur_s, olhs, odef, xbuf, lhs, wm_s, mod, mk,
            top, sc_s, cb_s, ts_s, zero_s, sem_m, sem_out):
    mt = 4 * NT * UNROLL // NSEG

    def modv(j):
        return jnp.concatenate([mod[j * NT + k] for k in range(NT)], axis=1)

    def mod_store(v, t):
        v = _rb(v)
        mod[t] = jnp.where(jnp.logical_or((t >> 3) == 1, (t >> 3) == 4), _rb(1.0 + v), v)

    def mod_tile(wm, t):
        mod_store(_dot(sc_s[...], wm), t)

    def gemv_part(w, d0, acc):
        n = w.shape[1]
        p = w.astype(F32) * cb_s[d0:d0 + n, :]
        p = jnp.sum(p.reshape(w.shape[0], n // 8, 8, 128), axis=1)
        return p if acc is None else p + acc

    def gemv_finish(acc, ts):
        for u, t in enumerate(ts):
            mod_store(jnp.broadcast_to(jnp.sum(acc[u], axis=0, keepdims=True), (M, 128)), t)

    def wm_copy(it, u):
        col = pl.multiple_of((2 * NT + it * mt + u) * 128, 128)
        return pltpu.make_async_copy(wmod_hbm.at[:, pl.ds(col, 128)], wm_s.at[it & 3, u],
                                     sem_m.at[it & 3])

    def zero_after(y):
        return (y if y.dtype == U32 else pltpu.bitcast(y, U32)) & zero_s[0:8, :]

    def or_tile(u, z):
        if z is None:
            return u
        return (u.reshape(u.shape[0] // 8, 8, 128) | z).reshape(u.shape)

    def prologue(stage, wo_raw, wmod_s, nrm, ha, hb, tmp, mem0_ref, wr_ref, c_ref, sem):
        w_hbms = (wq_hbm, wk_hbm, wv_hbm)
        wob = H * DH // NT
        S_X, S_C0, S_ST, S_WO, S_MOD, S_SM = 0, 2, 6, 6 + NSLOT, 6 + NSLOT + NT, 6 + NSLOT + 2 * NT

        def x_copy(i):
            lo, n = ((XR, M), (0, XR))[i]
            return pltpu.make_async_copy(x_hbm.at[:, pl.ds(lo, n), :], xbuf.at[:, pl.ds(lo, n), :],
                                         sem.at[S_X + i])

        def mod_copies(k):
            return [pltpu.make_async_copy(wmod_hbm.at[:, pl.ds(v * D + k * 128, 128)],
                                          wmod_s.at[k, v], sem.at[S_MOD + (k if k < 2 else k & 6)])
                    for v in range(2)]

        def chunk_copy(mat, d0, g, slot, k):
            heads = pl.ds(pl.multiple_of(g * CH, CH), CH)
            return pltpu.make_async_copy(w_hbms[mat].at[pl.ds(d0, KQ), heads, :],
                                         stage.at[slot, g], sem.at[k])

        def wo_copy(j):
            return pltpu.make_async_copy(wo_hbm.at[pl.ds(pl.multiple_of(j * wob, wob), wob)],
                                         wo_raw.at[j], sem.at[S_WO + j])

        def relayout1(src, t0, z=None):
            v = src.reshape(RB * CH, 128)
            tmp[t0:t0 + RB * CH // 2, :] = or_tile(_as_u32(v), z)

        def relayout2(c, h0_, t0, d0, z=None, src=tmp):
            w = or_tile(src[pl.ds(t0, RB2, stride=CH // 2), :], z)
            rows = pl.ds(d0 // 2, RB2 // 2)
            wqkv[c, h0_, rows, :] = _as_u32(w.astype(jnp.uint16))
            wqkv[c, h0_ + 1, rows, :] = _as_u32((w >> 16).astype(jnp.uint16))

        def mod_pair(k):
            for v in range(2):
                mod_tile(wmod_s[k, v], v * NT + k)

        def fill(dst, q, t, r, z=None):
            k = 2 * q + t
            sh = mod[k] if z is None else mod[k] + pltpu.bitcast(z, F32)
            v = nrm[k, r:r + FB, :].reshape(FB // 8, 8, 128) * mod[NT + k] + sh
            dst[t, r // 2:(r + FB) // 2, :] = _as_u32(v.reshape(FB, 128).astype(BF16))

        small = [pltpu.make_async_copy(src, dst, sem.at[S_SM])
                 for src, dst in ((c_hbm, c_ref), (mem0_hbm, mem0_ref), (wr_hbm, wr_ref))]
        for cp in small:
            cp.start()
        x_copy(0).start()
        for cp in mod_copies(0) + mod_copies(1):
            cp.start()
        for g in range(4):
            chunk_copy(0, 0, g, 0, S_C0 + g).start()
        for c in range(1, NSLOT):
            for g in range(4):
                chunk_copy(c % 3, (c // 3) * KQ, g, c, S_ST + c).start()
            for cp in mod_copies(2 * c) + mod_copies(2 * c + 1):
                cp.start()

        kk = lax.broadcasted_iota(jnp.int32, (SEG + M, PR), 0)
        qq = lax.broadcasted_iota(jnp.int32, (SEG + M, PR), 1)
        k_mem = jnp.logical_and(kk >= XR, kk < SEG)
        k_pos = jnp.where(kk < SEG, kk, kk - M)
        q_mem = jnp.logical_and(qq < 2 * SEG, qq % SEG >= XR)
        q_pos = jnp.where(qq < 2 * SEG, qq % SEG, XR + qq % M)
        mk[0:SEG + M, :] = jnp.where(q_mem | k_mem | (q_pos >= k_pos), 0.0, 1.0).astype(F32)
        mod[0:2 * NT] = jnp.zeros((2 * NT, M, 128), F32)
        zero_s[...] = jnp.zeros(zero_s.shape, U32)
        top[...] = jnp.full(top.shape, jnp.iinfo(jnp.int32).min, jnp.int32)
        for cp in small:
            cp.wait()
        wr = jnp.broadcast_to(wr_ref[...].astype(F32).reshape(1, D), (M, D))
        for k in range(NT):
            mod[6 * NT + k] = wr[:, k * 128:(k + 1) * 128]
        cv = c_ref[...].astype(F32)
        sc = _rb(cv * _rb(jax.nn.sigmoid(cv)))
        sc_s[...] = jnp.broadcast_to(sc, (M, D)).astype(BF16)
        for k in range(NT):
            cb_s[k * 128:(k + 1) * 128, :] = jnp.broadcast_to(
                sc[:, k * 128:(k + 1) * 128], (128, 128)).T
        mb = mem0_ref[...]
        for k in range(NT):
            lhs[0, k, XR // 2:, :] = _as_u32(mb[:, k * 128:(k + 1) * 128])

        def zero_body(i, c):
            wo_raw[NT, pl.ds(pl.multiple_of(i * 32, 32), 32), :] = jnp.zeros((32, D), BF16)
            return c

        lax.fori_loop(0, wob // 32, zero_body, 0)
        x_copy(0).wait()

        def ln_body(i, c):
            for u in range(LNU):
                q = i * LNU + u
                v = _ln(xbuf[q, XR:, :].astype(F32))
                for k in range(NT):
                    nrm[k, pl.ds(pl.multiple_of(q * 8, 8), 8), :] = v[:, k * 128:(k + 1) * 128]
            return c

        with jax.named_scope("p_ln"):
            lax.fori_loop(0, NSEG // LNU, ln_body, 0)

        def mod_body(k, c):
            pltpu.make_async_copy(wmod_s.at[k], wmod_s.at[k], sem.at[S_MOD + k]).wait()
            mod_pair(k)
            for r in range(0, R0, FB):
                fill(ha, 0, k, r)
            return c

        with jax.named_scope("p_mod"):
            lax.fori_loop(0, 2, mod_body, 0)

        def hop1(g):
            chunk_copy(0, 0, g, 0, S_C0 + g).wait()

            def body(i, c):
                d0 = pl.multiple_of(i * 128, 128)
                v = stage[0, g, pl.ds(d0, 128)].reshape(128 * CH, 128)
                t0 = pl.multiple_of((g * KQ + d0) * (CH // 2), 512)
                tmp[pl.ds(t0, 128 * CH // 2), :] = _as_u32(v)
                return c

            lax.fori_loop(0, KQ // 128, body, 0)

        def hop2(c, g, j):
            src = tmp.at[pl.ds(pl.multiple_of(g * (KQ * CH // 2), 512), KQ * CH // 2 + 8)]
            for d0 in range(0, KQ, RB2):
                relayout2(c, g * CH + 2 * j, d0 * CH // 2 + j, d0, src=src)

        def bulk(units, jobs):
            due = {}
            t0 = 0
            for n, (hq, c, h0_, pi, first, r0, nrow) in enumerate(units):
                nb = nrow // BLK
                parts = []
                for u in range(nb):
                    part = hq[0, (r0 + u * BLK) // 2:(r0 + (u + 1) * BLK) // 2, :]
                    for z in due.pop(t0 + u, ()):
                        part = jnp.concatenate([part[0:8] | z, part[8:]], axis=0)
                    parts.append(part)
                hv = jnp.concatenate([_as_bf16(jnp.concatenate(parts, axis=0)),
                                      _as_bf16(hq[1, r0 // 2:(r0 + nrow) // 2, :])], axis=1)
                w = jnp.concatenate([_as_bf16(wqkv[c, h0_]), _as_bf16(wqkv[c, h0_ + 1])], axis=1)
                y = _dot(hv, w)
                segs = slice(r0 // M, (r0 + nrow) // M)
                for a in range(2):
                    old = jnp.where(first, 0.0, pre[pi, segs, a * M:(a + 1) * M, :])
                    pre[pi, segs, a * M:(a + 1) * M, :] = (
                        y[:, a * DH:(a + 1) * DH].reshape(nrow // M, M, DH) + old)
                for u in range(nb):
                    for job in jobs.get(t0 + u, ()):
                        res = job(zero_after(y[u * BLK:u * BLK + 8, 0:128]))
                        if res is not None:
                            due.setdefault(max(t0 + u + JOB_SPAN, t0 + nb), []).append(
                                zero_after(res))
                t0 += nb
            assert not due

        GP = CH // 2
        WO0 = NCHUNK - 1 - NT
        LN0 = 4
        SPI = -(-NSEG // (NCHUNK - 1 - LN0))

        def rot_body(i, c):
            slot = (i + 1) & (NSLOT - 1)
            pltpu.make_async_copy(stage.at[slot], stage.at[slot], sem.at[S_ST + slot]).wait()
            km = 2 * jnp.minimum(i, 3)

            @pl.when(jnp.logical_and(i >= 1, i <= 3))
            def _():
                wq = wmod_s.at[pl.ds(km, 2)]
                pltpu.make_async_copy(wq, wq, sem.at[S_MOD + km]).wait()

            @pl.when(i == LN0)
            def _():
                x_copy(1).wait()

            @pl.when(i >= WO0)
            def _():
                wo_copy(i - WO0).wait()

            nxt = i + NSLOT
            qn = (nxt * 43) >> 7
            for mat in range(3):
                @pl.when(jnp.logical_and(nxt < NCHUNK, nxt - 3 * qn == mat))
                def _():
                    for g in range(4):
                        chunk_copy(mat, qn * KQ, g, nxt & (NSLOT - 1),
                                   S_ST + (nxt & (NSLOT - 1))).start()

            @pl.when(i < NT)
            def _():
                wo_copy(i).start()

            @pl.when(i == 0)
            def _():
                x_copy(1).start()

            q0 = (i * 43) >> 7
            q1 = ((i + 1) * 43) >> 7
            pa = (i - 3 * q0) * NP + NP - GP
            units = ([(ha, i, H - CH + 2 * n, pa + n, q0 == 0, 0, R0) for n in range(GP)]
                     + [(hb, i + 1, 2 * n, (i + 1 - 3 * q1) * NP + n, q1 == 0, 0, R0)
                        for n in range(NP - GP)])
            jw = jnp.where(i >= WO0, i - WO0, NT)

            def wo_job(b, z):
                v = wo_raw[jw, b * 16:(b + 1) * 16, :]
                rows = pl.ds(pl.multiple_of(jw * (wob // 2) + b * 8, 8), 8)
                for j in range(NT):
                    wo_s[j, rows, :] = _as_u32(v[:, j * 128:(j + 1) * 128]) | z

            lst = {}

            def ln_job(b, ph, z):
                r = (b % 3) * 8
                seg = (i - LN0) * SPI + b // 3
                live = jnp.logical_and(i >= LN0, seg < NSEG)
                src = jnp.where(live, seg, 0) + (i >> (10 + ph))
                x = xbuf[src, pl.ds(pl.multiple_of(jnp.where(live, r, XR), 8), 8), :].astype(F32)
                zf = pltpu.bitcast(z, F32)
                if ph == 0:
                    xm = jnp.concatenate([x[:, :128] + zf, x[:, 128:]], axis=1)
                    mu = jnp.mean(xm, axis=-1, keepdims=True)
                    lst[2 * b] = jnp.broadcast_to(mu, (8, 128))
                    return None
                xc = x - jnp.concatenate([lst[2 * b] + zf] * NT, axis=1)
                if ph == 1:
                    lst[2 * b + 1] = jnp.broadcast_to(_inv_std(xc), (8, 128))
                    return None
                inv = jnp.concatenate([lst[2 * b + 1]] * NT, axis=1)
                hv = (xc * inv * modv(1) + modv(0)).astype(BF16)
                u = [_as_u32(hv[:, k * 128:(k + 1) * 128]) for k in range(NT)]
                dst = jnp.where(live, seg, NSEG)
                for k in range(NT):
                    hs[dst, k, r // 2:r // 2 + 4, :] = u[k]
                res = jnp.concatenate(u[0:2], axis=0)
                for k in range(2, NT, 2):
                    res = res | jnp.concatenate(u[k:k + 2], axis=0)
                return res

            def r1_job(g, d0, z):
                relayout1(stage[slot, g, d0:d0 + RB], (g * KQ + d0) * CH // 2, z)

            def copy_job(t, r, z):
                ha[t, r:r + 32, :] = or_tile(hb[t, r:r + 32, :], z)

            P = functools.partial
            upb = R0 // BLK
            nr = NP * upb
            jobs = {}
            for g in range(4):
                lo, mid, hi = (x * upb // 4 for x in R_AT[g])
                _spread(jobs, [P(r1_job, g, d0) for d0 in range(0, KQ, RB)], lo, mid)
                _spread(jobs, [P(relayout2, i + 1, g * CH + 2 * j, (g * KQ + d0) * CH // 2 + j, d0)
                               for j in range(CH // 2) for d0 in range(0, KQ, RB2)], mid, hi)
            oz = i >> 10
            _spread(jobs, [P(fill, hb, q1, t + oz, r) for r in range(0, R0, FB) for t in range(2)],
                    F_AT[0] * upb // 4, F_AT[1] * upb // 4)
            _spread(jobs, [P(copy_job, t, r) for t in range(2) for r in range(0, R0 // 2, 32)],
                    2 * GP * upb, nr - upb)
            for ph in range(3):
                off = LN_PH[ph] - LN_PH[2]
                _spread(jobs, [P(ln_job, b, ph) for b in range(3 * SPI)],
                        L_AT * upb // 4 + LN_PH[ph], nr - max(upb, JOB_SPAN) + off)
            _spread(jobs, [P(wo_job, b) for b in range(wob // 16)], GP * upb, nr - upb)
            gv = {}

            def gv_job(d0, n, z):
                w = wmod_s[pl.ds(km, 2), :, d0:d0 + n, :].reshape(4, n, 128)
                acc = gv.get("acc")
                if z is not None:
                    zf = pltpu.bitcast(z, F32)[None]
                    acc = jnp.broadcast_to(zf, (4, 8, 128)) if acc is None else acc + zf
                gv["acc"] = gemv_part(w, d0, acc)
                if z is not None:
                    au = pltpu.bitcast(gv["acc"], U32)
                    return au[0] | au[1] | au[2] | au[3]

            _spread(jobs, [P(gv_job, d0, GVR) for d0 in range(0, D - GV_FREE, GVR)],
                    GV_AT[0] * upb // 4, min(GV_AT[1] * upb // 4, nr - JOB_SPAN))
            bulk(units, jobs)
            if GV_FREE:
                gv_job(D - GV_FREE, GV_FREE, None)
            gemv_finish(gv["acc"], [km, NT + km, km + 1, NT + km + 1])
            return c

        def outer(k, c):
            last = k == 4

            @pl.when(k < 4)
            def _():
                hop1(k)

            @pl.when(k != 3)
            def _():
                g = jnp.minimum(k, 3)
                cc = jnp.where(last, NCHUNK - 1, 0)
                for j in range(GP):
                    hop2(cc, g, j)
                bulk([(ha, cc, g * CH + 2 * n, jnp.where(last, 2 * NP, 0) + g * GP + n, k < 4,
                       0, R0) for n in range(GP)], {})

            @pl.when(k == 3)
            def _():
                for j in range(GP):
                    hop2(0, 3, j)
                with jax.named_scope("p_rot"):
                    lax.fori_loop(0, NCHUNK - 1, rot_body, 0)
                for it in range(2):
                    for u in range(mt):
                        wm_copy(it, u).start()

            return c

        with jax.named_scope("p_bulk"):
            lax.fori_loop(0, 5, outer, 0)

    if "pro" in PHASES: pl.run_scoped(
        prologue,
        pltpu.VMEM((NSLOT, H // CH, KQ, CH, 128), BF16),
        pltpu.VMEM((NT + 1, H * DH // NT, D), BF16),
        pltpu.VMEM((NT, 2, D, 128), BF16),
        pltpu.VMEM((NT, R0, 128), F32),
        pltpu.VMEM((2, R0 // 2, 128), U32),
        pltpu.VMEM((2, R0 // 2, 128), U32),
        pltpu.VMEM((D * CH // 2 + 32, 128), U32),
        pltpu.VMEM((M, D), BF16),
        pltpu.VMEM((D,), BF16),
        pltpu.VMEM((1, D), BF16),
        pltpu.SemaphoreType.DMA((7 + NSLOT + 2 * NT,)),
    )

    def main(wg_s, wu_s, wd_s, ybuf, stat, outs, sem_f):
        def load_x_rows(slot, seg):
            for k in range(NT):
                lhs[slot, k, 0:XR // 2, :] = hs[seg, k]

        def resid(seg, r, z=None):
            rows = pl.ds(r, 8)
            t = modv(2) * ybuf[seg, rows, :].astype(F32)
            if z is not None:
                t = t + jnp.concatenate([pltpu.bitcast(z, F32)] * NT, axis=1)
            return xbuf[seg, rows, :].astype(F32) + t

        def wide(v):
            return jnp.concatenate([v] * NT, axis=1)

        def make_key(v, row0):
            b = pltpu.bitcast(jnp.where(v != v, -jnp.inf, v + 0.0), jnp.int32)
            low = (S - 1 - row0) - lax.broadcasted_iota(jnp.int32, (8, 128), 0)
            return (b ^ ((b >> 31) & 0x7FFF0000)) | low

        def post(seg, r, z):
            x1 = resid(seg, r, z)
            mu = jnp.mean(x1, axis=-1, keepdims=True)
            xc = x1 - mu
            inv = _inv_std(xc)
            stat[0, seg, pl.ds(r, 8), :] = jnp.broadcast_to(mu, (8, 128))
            stat[1, seg, pl.ds(r, 8), :] = jnp.broadcast_to(inv, (8, 128))
            v = _rb(inv * jnp.sum(xc * modv(7), axis=-1, keepdims=True) + mod[8 * NT])
            key = make_key(v, seg * SEG + r)
            m1, m2 = top[0:8, :], top[8:16, :]
            top[8:16, :] = jnp.maximum(m2, jnp.minimum(m1, key))
            top[0:8, :] = jnp.maximum(m1, key)
            o = x1 + modv(5) * (xc * inv * modv(4) + modv(3))
            outs[seg, pl.ds(r, 8), :] = o.astype(BF16)
            res = pltpu.bitcast(v, U32)
            for k in range(NT):
                res = res | pltpu.bitcast(o[:, k * 128:(k + 1) * 128], U32)
            return res

        def redo(seg, r, z=None):
            x1 = resid(seg, r, z)
            n = (x1 - wide(stat[0, seg, pl.ds(r, 8), :])) * wide(stat[1, seg, pl.ds(r, 8), :])
            return x1, n * modv(4) + modv(3)

        def out_copy(g0, ng, r, n, k=0):
            return pltpu.make_async_copy(outs.at[pl.ds(g0, ng), pl.ds(r, n), :],
                                         out_hbm.at[pl.ds(g0, ng), pl.ds(r, n), :], sem_out.at[k])

        late = ((wg_hbm, wg_s, FF // 128), (wu_hbm, wu_s, FF // 128), (wd_hbm, wd_s, NT))

        def col_copy(k, j):
            return pltpu.make_async_copy(
                late[k][0].at[:, pl.ds(pl.multiple_of(j * 128, 128), 128)], late[k][1].at[j],
                sem_f.at[k])

        load_x_rows(0, 0)

        def step(it, cur, state):
            s = it * UNROLL + cur
            nxt = (cur + 1) % UNROLL

            def pay(t, cost):
                now, due = state["now"], state["due"]
                for z in [z for (d, z) in due if d <= now]:
                    t = jnp.concatenate([t[0:8] | z, t[8:]], axis=0)
                state["due"] = [(d, z) for (d, z) in due if d > now]
                state["now"] = now + cost
                return t

            def release(y):
                now = state["now"]
                pend, state["pend"] = state["pend"], [e for e in state["pend"] if e[0] > now]
                for (d, f) in pend:
                    if d <= now:
                        f(zero_after(y[0:8]))

            def lv(k0, k1):
                ts = [lhs[cur, k] for k in range(k0, k1)]
                ts[0] = pay(ts[0], (k1 - k0) / NT)
                return jnp.concatenate([_as_bf16(t) for t in ts], axis=1)

            def wmat(mat, h, q0, q1):
                return _as_bf16(jnp.concatenate([wqkv[3 * q + mat, h] for q in range(q0, q1)],
                                                axis=0))

            def qkv(p, split=False):
                part = {}
                if split:
                    for mat in range(3):
                        for a in range(2):
                            part[mat, a] = _dot(lv(0, NT // 2), wmat(mat, 2 * p + a, 0, 2))
                for mat in range(3):
                    for a in range(2):
                        hm = mat * H + 2 * p + a
                        if split:
                            y = _dot(lv(NT // 2, NT), wmat(mat, 2 * p + a, 2, 4)) + part[mat, a]
                        else:
                            y = _dot(lv(0, NT), wmat(mat, 2 * p + a, 0, 4))
                        cur_s[hm] = y.astype(BF16)
                        release(y)

            def gather(mat, p):
                hm = mat * H + 2 * p
                return jnp.concatenate(
                    [cur_s[hm], cur_s[hm + 1], pre[mat * NP + p, s].astype(BF16)], axis=0)

            probs = {}

            def scores(p):
                st = lax.dot_general(gather(1, p), gather(0, p), (((1,), (1,)), ((), ())),
                                     preferred_element_type=F32)
                lane = lax.broadcasted_iota(jnp.int32, (1, PR), 1)
                is_a = jnp.logical_or(lane < SEG,
                                      jnp.logical_and(lane >= 2 * SEG, lane < 2 * SEG + M))
                ka = jnp.concatenate([st[0:SEG], st[2 * SEG:2 * SEG + M]], axis=0)
                kb = jnp.concatenate([st[SEG:2 * SEG], st[2 * SEG + M:]], axis=0)
                t = jnp.where(is_a, ka, kb) * (SCALE * LOG2E)
                ts_s[p + (it >> 10)] = jnp.where(mk[0:SEG + M, :] == 0.0, t, NEG_MASK * LOG2E)

                def softmax(z):
                    zf = pltpu.bitcast(z, F32)[:, 0:PR]
                    t = (ts_s[p].reshape(-1, 8, PR) + zf).reshape(SEG + M, PR)
                    e = jnp.exp2(t - jnp.max(t, axis=0, keepdims=True))
                    e = e * _recip(jnp.sum(e, axis=0, keepdims=True))
                    pa = jnp.where(is_a, e, 0.0)
                    pb = jnp.where(is_a, 0.0, e)
                    probs[p] = jnp.concatenate(
                        [pa[0:SEG], pb[0:SEG], pa[SEG:], pb[SEG:]], axis=0).astype(BF16)

                state["pend"].append((state["now"] + REL_S + (p % PG) * REL_STAG, softmax))

            def pv(p):
                o = lax.dot_general(probs.pop(p), gather(2, p), (((0,), (0,)), ((), ())),
                                    preferred_element_type=F32).astype(BF16)
                for a in range(2):
                    h = 2 * p + a
                    olhs[h] = _as_u32(o[a * SEG:(a + 1) * SEG])
                    odef[h, it, cur * 4:(cur + 1) * 4, :] = _as_u32(
                        o[2 * SEG + a * M:2 * SEG + (a + 1) * M])

            acc = [None] * NT

            def oproj(j, pairs):
                ts = [olhs[2 * p + a] for p in pairs for a in range(2)]
                ts[0] = pay(ts[0], len(pairs) / 4)
                ov = jnp.concatenate([_as_bf16(t) for t in ts], axis=1)
                w = wo_s[j, pairs[0] * DH:(pairs[-1] + 1) * DH, :]
                y = _dot(ov, _as_bf16(w))
                acc[j] = y if acc[j] is None else y + acc[j]
                release(acc[j])

            def fin(j):
                yb = acc[j].astype(BF16)
                ybuf[s, 0:XR, j * 128:(j + 1) * 128] = yb[0:XR]
                lhs[nxt, j, XR // 2:, :] = _as_u32(yb[XR:])

            def gemv():
                d0 = state["d0"]
                state["acc"] = gemv_part(wm_s[it & 3, :, d0:d0 + GR, :], d0, state["acc"])
                state["d0"] = d0 + GR
                au = pltpu.bitcast(state["acc"], U32)
                z = functools.reduce(lambda a, b: a | b, [au[u] for u in range(mt)])
                state["due"].append((state["now"] + G_LAG, zero_after(z)))

            load_x_rows(nxt, jnp.minimum(s + 1, NSEG - 1))
            ops = dict(Q=qkv, S=scores, P=pv, O=oproj, F=fin, G=gemv)
            for op in _schedule():
                ops[op[0]](*op[1:])

        def steps(it, carry):
            if "pro" in PHASES:
                pltpu.make_async_copy(wm_s.at[it & 3], wm_s.at[it & 3], sem_m.at[it & 3]).wait()

                @pl.when(it + 2 < NSEG // UNROLL)
                def _():
                    for u in range(mt):
                        wm_copy(it + 2, u).start()

            for u in range(UNROLL // 2):
                t = it * (UNROLL // 2) + u
                for k in range(3):
                    @pl.when(t < late[k][2])
                    def _():
                        col_copy(k, t).start()

            state = dict(now=0, due=[], pend=[], d0=0, acc=None)
            for u in range(UNROLL):
                step(it, u, state)
            acc = state["acc"]
            for d0 in range(state["d0"], D, 64):
                acc = gemv_part(wm_s[it & 3, :, d0:min(d0 + 64, D), :], d0, acc)
            gemv_finish(acc, [2 * NT + it * mt + u for u in range(mt)])
            return carry

        with jax.named_scope("m_steps"):
            if "step" in PHASES: lax.fori_loop(0, NSEG // UNROLL, steps, 0)
        for k in range(3):
            for j in range(late[k][2]):
                col_copy(k, j).wait()
        if "epi" not in PHASES:
            cp = pltpu.make_async_copy(ybuf, out_hbm, sem_out.at[0])
            cp.start()
            cp.wait()
            return

        ntail = EC // M
        ppi = (S // 8 - ntail) // NEC
        gpi = ppi // (XR // 8)
        nblk = EC // (UNROLL * M)

        def ep_body(i, c):
            @pl.when(i > 0)
            def _():
                out_copy((i - 1) * gpi, gpi, 0, XR).start()

            for k in range(NT):
                mod[7 * NT + k] = mod[4 * NT + k] * mod[6 * NT + k]
            mod[8 * NT] = jnp.broadcast_to(
                jnp.sum(modv(3) * modv(6), axis=-1, keepdims=True), (M, 128))

            jobs = {}
            _spread(jobs, list(range(ppi)), 0, NT * H // EKH - E_SPAN)
            due = {}
            n = 0
            for j in range(NT):
                for h0_ in range(0, H, EKH):
                    ts = [odef[h, pl.ds(i * nblk, nblk)].reshape(EC // 2, DH)
                          for h in range(h0_, h0_ + EKH)]
                    for z in due.pop(n, ()):
                        ts[0] = jnp.concatenate([ts[0][0:8] | z, ts[0][8:]], axis=0)
                    w = wo_s[j, h0_ * DH // 2:(h0_ + EKH) * DH // 2, :]
                    yp = _dot(jnp.concatenate([_as_bf16(t) for t in ts], axis=1), _as_bf16(w))
                    y = yp if h0_ == 0 else yp + y
                    if h0_ + EKH == H:
                        ybuf[pl.ds(i * ntail, ntail), XR:, j * 128:(j + 1) * 128] = (
                            y.reshape(ntail, M, 128).astype(BF16))
                    for u in jobs.get(n, ()):
                        t = i * ppi + u
                        early = t < NSEG * (XR // 8)
                        seg = jnp.where(early, t // (XR // 8), t - NSEG * (XR // 8))
                        row = pl.multiple_of(jnp.where(early, (t % (XR // 8)) * 8, XR), 8)
                        res = post(seg, row, zero_after(y[0:8]))
                        due.setdefault(n + E_SPAN, []).append(zero_after(res))
                    n += 1
            return c

        with jax.named_scope("e_loop"):
            lax.fori_loop(0, NEC, ep_body, 0)
        done = (NEC - 1) * gpi
        tail = NSEG - ntail
        out_copy(done, NSEG - done, 0, XR).start()
        out_copy(0, tail, XR, M).start()
        x1s = [resid(g, XR) for g in range(tail, NSEG)]
        mus = [jnp.mean(x1, axis=-1, keepdims=True) for x1 in x1s]
        pairs = [(top[0:8, :], top[8:16, :])]
        lowest = jnp.full((8, 128), jnp.iinfo(jnp.int32).min, jnp.int32)
        for g in range(tail, NSEG):
            xc = x1s[g - tail] - mus[g - tail]
            inv = _inv_std(xc)
            stat[0, g, XR:, :] = jnp.broadcast_to(mus[g - tail], (8, 128))
            stat[1, g, XR:, :] = jnp.broadcast_to(inv, (8, 128))
            v = _rb(inv * jnp.sum(xc * modv(7), axis=-1, keepdims=True) + mod[8 * NT])
            pairs.append((make_key(v, g * SEG + XR), lowest))
        while len(pairs) > 1:
            (a1, a2), (c1, c2) = pairs.pop(0), pairs.pop(0)
            pairs.append((jnp.maximum(a1, c1),
                          jnp.maximum(jnp.minimum(a1, c1), jnp.maximum(a2, c2))))

        tk = jnp.concatenate(pairs[0], axis=0)[:, 0:1]
        k1 = jnp.max(tk[0:8], axis=0, keepdims=True)
        k2 = jnp.max(jnp.where(tk == k1, jnp.iinfo(jnp.int32).min, tk), axis=0, keepdims=True)
        i1 = (S - 1) - (k1[0, 0] & (S - 1))
        i2 = (S - 1) - (k2[0, 0] & (S - 1))
        g1, g2 = i1 >> 5, i2 >> 5
        b1 = pl.multiple_of(i1 & 24, 8)
        b2 = pl.multiple_of(i2 & 24, 8)

        def tail_out(n, z):
            g, k0 = tail + n // (NT // TW), (n % (NT // TW)) * TW
            zf = pltpu.bitcast(z, F32)
            for k in range(k0, k0 + TW, 2):
                cols = slice(k * 128, (k + 2) * 128)
                m = lambda j: jnp.concatenate([mod[j * NT + k], mod[j * NT + k + 1]], axis=1)
                two = lambda v: jnp.concatenate([v, v], axis=1)
                x1_ = (xbuf[g, XR:, cols].astype(F32)
                       + (m(2) * ybuf[g, XR:, cols].astype(F32) + two(zf)))
                h_ = (x1_ - two(stat[0, g, XR:, :])) * two(stat[1, g, XR:, :]) * m(4) + m(3)
                outs[g, XR:, cols] = (x1_ + m(5) * h_).astype(BF16)

        xa, ha_ = redo(g1, b1)
        xb_, hb_ = redo(g2, b2)
        x1 = jnp.concatenate([xa, xb_], axis=0)
        h2 = jnp.concatenate([ha_, hb_], axis=0)
        h2b = h2.astype(BF16)
        row = lax.broadcasted_iota(jnp.int32, (16, 1), 0)
        grow = jnp.where(row < 8, g1 * SEG + b1 + row, g2 * SEG + b2 + row - 8)
        ks = jnp.where(grow == i1, k1, k2)
        rsel = pltpu.bitcast((ks ^ ((ks >> 31) & 0x7FFF0000)) & -65536, F32)
        acts = []
        jobs = {}
        _spread(jobs, list(range(ntail * NT // TW)), 0, T_END)
        for j in range(FF // 128):
            gt = _rb(_dot(h2b, wg_s[j]))
            for n in jobs.get(2 * j, ()):
                tail_out(n, zero_after(gt[0:8]))
            gt = _rb(gt * _rb(jax.nn.sigmoid(gt)))
            ut = _rb(_dot(h2b, wu_s[j]))
            for n in jobs.get(2 * j + 1, ()):
                tail_out(n, zero_after(ut[0:8]))
            acts.append((gt * ut).astype(BF16))
        out_copy(tail, NSEG - tail, XR, M).start()
        act = jnp.concatenate(acts, axis=1)
        y = _rb(jnp.concatenate([_dot(act, wd_s[j]) for j in range(NT)], axis=1))
        y = _rb(y * _rb(jax.nn.sigmoid(rsel)))
        sel = jnp.logical_or(grow == i1, grow == i2)
        gb2 = jnp.concatenate([modv(5)] * 2, axis=0)
        fixed = (x1 + gb2 * (h2 + jnp.where(sel, y, 0.0))).astype(BF16)

        with jax.named_scope("e_outwait"):
            out_copy(0, NSEG, 0, SEG).wait()
        outs[g1, pl.ds(b1, 8), :] = fixed[0:8]
        outs[g2, pl.ds(b2, 8), :] = fixed[8:16]
        out_copy(g1, 1, b1, 8, 0).start()

        @pl.when((i1 >> 3) != (i2 >> 3))
        def _():
            out_copy(g2, 1, b2, 8, 1).start()
            out_copy(g2, 1, b2, 8, 1).wait()

        out_copy(g1, 1, b1, 8, 0).wait()

    pl.run_scoped(
        main,
        pltpu.VMEM((FF // 128, D, 128), BF16),
        pltpu.VMEM((FF // 128, D, 128), BF16),
        pltpu.VMEM((NT, FF, 128), BF16),
        pltpu.VMEM((NSEG, SEG, D), BF16),
        pltpu.VMEM((2, NSEG, SEG, 128), F32),
        pltpu.VMEM((NSEG, SEG, D), BF16),
        pltpu.SemaphoreType.DMA((3,)),
    )


def _entry(*refs):
    pl.run_scoped(
        functools.partial(_kernel, *refs),
        pltpu.VMEM((NCHUNK, H, KQ // 2, DH), U32),
        pltpu.VMEM((NSEG + 1, NT, XR // 2, 128), U32),
        pltpu.VMEM((NT, (H * DH + H * DH // NT) // 2, 128), U32),
        pltpu.VMEM((3 * NP, NSEG, 2 * M, DH), F32),
        pltpu.VMEM((3 * H, SEG, DH), BF16),
        pltpu.VMEM((H, SEG // 2, DH), U32),
        pltpu.VMEM((H, NSEG // UNROLL, UNROLL * M // 2, DH), U32),
        pltpu.VMEM((NSEG, SEG, D), BF16),
        pltpu.VMEM((UNROLL, NT, SEG // 2, 128), U32),
        pltpu.VMEM((4, 4 * NT * UNROLL // NSEG, D, 128), BF16),
        pltpu.VMEM((8 * NT + 4, M, 128), F32),
        pltpu.VMEM((64, PR), F32),
        pltpu.VMEM((32, 128), jnp.int32),
        pltpu.VMEM((M, D), BF16),
        pltpu.VMEM((D, 128), F32),
        pltpu.VMEM((NP, SEG + M, PR), F32),
        pltpu.VMEM((8 + PAD, 128), U32),
        pltpu.SemaphoreType.DMA((4,)),
        pltpu.SemaphoreType.DMA((2,)),
    )


@functools.partial(jax.jit, static_argnames=("A_seg_len",))
def pallas_adaLN_cond__memory_aug_recurrent_mem_tr__moe_arch_mod__prompt_kernel(
    A_x: jax.Array,
    A_mem0: jax.Array,
    A_Wq: jax.Array,
    A_Wk: jax.Array,
    A_Wv: jax.Array,
    A_Wo: jax.Array,
    A_seg_len,
    B_x: jax.Array,
    B_w_r: jax.Array,
    B_w_gate: jax.Array,
    B_w_up: jax.Array,
    B_w_down: jax.Array,
    c: jax.Array,
    w_mod: jax.Array,
):
    assert A_seg_len == SEG and A_x.shape == (1, S, D)
    del B_x
    hbm = pl.BlockSpec(memory_space=pl.ANY)
    out = pl.pallas_call(
        _entry,
        out_shape=jax.ShapeDtypeStruct((NSEG, SEG, D), BF16),
        in_specs=[hbm] * 12,
        out_specs=hbm,
        compiler_params=pltpu.CompilerParams(vmem_limit_bytes=120 * 1024 * 1024,
                                             disable_bounds_checks=True),
    )(A_x.reshape(NSEG, SEG, D), A_mem0.reshape(M, D), A_Wq, A_Wk, A_Wv, A_Wo.reshape(H * DH, D),
      B_w_r, B_w_gate, B_w_up, B_w_down, c, w_mod)
    return out.reshape(1, S, D)
```

```python
import functools

import jax
import jax.numpy as jnp
from jax import lax
import jax.experimental.pallas as pl
import jax.experimental.pallas.tpu as pltpu

F32 = jnp.float32
BF16 = jnp.bfloat16
U32 = jnp.uint32

D = 1024
S = 2048
H = 32
DH = 128
M = 8
SEG = 32
NSEG = S // SEG
FF = 3584
NT = D // 128
XR = SEG - M
R0 = M * NSEG
CH = 8
KQ = D // 4
NCHUNK = 3 * D // KQ
NSLOT = 4
PR = 2 * SEG + 2 * M
NP = H // 2
EC = 128
NEC = R0 // EC
LOG2E = 1.4426950408889634
EPS = 1e-5
SCALE = DH ** -0.5
NEG_MASK = -1000000000.0

PHASES = ("pro", "step", "epi")

UNROLL = 4
PG = 4
LAG_S = 1
LAG_P = 4
O_PARTS = (0, 8, 12)
O_TH = (256, 256, 256, 1280)
REL_S = 3
REL_STAG = 2
G_AT = (0, 1, 2, 3, 7, 11)
GR = 32
G_LAG = 3
BLK = 32
JOB_SPAN = 40
RB = 16
RB2 = 32
FB = 32
GVR = 32
GV_FREE = 64
R_AT = ((0, 6, 16), (14, 22, 30), (30, 38, 46), (44, 52, 60))
F_AT = (0, 13)
L_AT = 6
GV_AT = (16, 56)
LNU = 16
LN_PH = (0, 10, 20)
EKH = 4
E_SPAN = 4
E_REL = 4
E_PH = (0, 10, 20)
TW = 4
T_END = 32
PAD = 24


def _schedule():
    groups = [list(range(g, g + PG)) for g in range(0, NP, PG)]
    at = {}
    for g, grp in enumerate(groups):
        at.setdefault(grp[-1] + LAG_P, []).extend(("P", q) for q in grp)
    for g, grp in enumerate(groups):
        at.setdefault(grp[-1] + LAG_S, []).extend(("S", q) for q in grp)
    ops = []
    for p in range(NP):
        ops.append(("Q", p, p == 0))
        if p in G_AT:
            ops.append(("G",))
        ops.extend(at.pop(p, []))
    bounds = list(O_PARTS) + [NP]
    t = NP
    done = 0
    for n in range(len(O_PARTS)):
        part = list(range(bounds[n], bounds[n + 1]))
        assert all(("P", q) in ops for q in part), (n, ops)
        for j in range(NT):
            ops.append(("O", j, part))
            if n == len(O_PARTS) - 1:
                ops.append(("F", j))
            done += len(part) * 16
            while t - NP < len(O_TH) and done >= O_TH[t - NP]:
                ops.extend(at.pop(t, []))
                t += 1
    assert not at
    return ops


def _rb(x):
    return x.astype(BF16).astype(F32)


def _recip(x):
    r = pl.reciprocal(x, approx=True)
    return r * (2.0 - x * r)


def _inv_std(var):
    v = _rb(_rb(var) + EPS)
    return _recip(_rb(v * lax.rsqrt(v)))


def _rstd(xc):
    return lax.rsqrt(jnp.mean(xc * xc, axis=-1, keepdims=True) + EPS)


def _dot(a, b):
    return jnp.dot(a, b, preferred_element_type=F32)


def _as_bf16(u):
    return pltpu.bitcast(u, BF16)


def _as_u32(b):
    return pltpu.bitcast(b, U32)


def _spread(jobs, fns, lo, hi):
    for n, fn in enumerate(fns):
        jobs.setdefault(lo + n * (hi - lo) // len(fns), []).append(fn)


def _kernel(x_hbm, mem0_hbm, wq_hbm, wk_hbm, wv_hbm, wo_hbm, wr_hbm, wg_hbm, wu_hbm, wd_hbm,
            c_hbm, wmod_hbm, out_hbm,
            wqkv, hs, wo_s, pre, cur_s, olhs, odef, xbuf, lhs, wm_s, mod, mk,
            top, sc_s, cb_s, ts_s, zero_s, sem_m, sem_out):
    mt = 4 * NT * UNROLL // NSEG

    def modv(j):
        return jnp.concatenate([mod[j * NT + k] for k in range(NT)], axis=1)

    def mod_store(v, t):
        v = _rb(v)
        mod[t] = jnp.where(jnp.logical_or((t >> 3) == 1, (t >> 3) == 4), _rb(1.0 + v), v)

    def mod_tile(wm, t):
        mod_store(_dot(sc_s[...], wm), t)

    def gemv_part(w, d0, acc):
        n = w.shape[1]
        p = w.astype(F32) * cb_s[d0:d0 + n, :]
        p = jnp.sum(p.reshape(w.shape[0], n // 8, 8, 128), axis=1)
        return p if acc is None else p + acc

    def gemv_finish(acc, ts):
        for u, t in enumerate(ts):
            mod_store(jnp.broadcast_to(jnp.sum(acc[u], axis=0, keepdims=True), (M, 128)), t)

    def wm_copy(it, u):
        col = pl.multiple_of((2 * NT + it * mt + u) * 128, 128)
        return pltpu.make_async_copy(wmod_hbm.at[:, pl.ds(col, 128)], wm_s.at[it & 3, u],
                                     sem_m.at[it & 3])

    def zero_after(y):
        return (y if y.dtype == U32 else pltpu.bitcast(y, U32)) & zero_s[0:8, :]

    def or_tile(u, z):
        if z is None:
            return u
        return (u.reshape(u.shape[0] // 8, 8, 128) | z).reshape(u.shape)

    def prologue(stage, wo_raw, wmod_s, nrm, ha, hb, tmp, mem0_ref, wr_ref, c_ref, sem):
        w_hbms = (wq_hbm, wk_hbm, wv_hbm)
        wob = H * DH // NT
        S_X, S_C0, S_ST, S_WO, S_MOD, S_SM = 0, 2, 6, 6 + NSLOT, 6 + NSLOT + NT, 6 + NSLOT + 2 * NT

        def x_copy(i):
            lo, n = ((XR, M), (0, XR))[i]
            return pltpu.make_async_copy(x_hbm.at[:, pl.ds(lo, n), :], xbuf.at[:, pl.ds(lo, n), :],
                                         sem.at[S_X + i])

        def mod_copies(k):
            return [pltpu.make_async_copy(wmod_hbm.at[:, pl.ds(v * D + k * 128, 128)],
                                          wmod_s.at[k, v], sem.at[S_MOD + (k if k < 2 else k & 6)])
                    for v in range(2)]

        def chunk_copy(mat, d0, g, slot, k):
            heads = pl.ds(pl.multiple_of(g * CH, CH), CH)
            return pltpu.make_async_copy(w_hbms[mat].at[pl.ds(d0, KQ), heads, :],
                                         stage.at[slot, g], sem.at[k])

        def wo_copy(j):
            return pltpu.make_async_copy(wo_hbm.at[pl.ds(pl.multiple_of(j * wob, wob), wob)],
                                         wo_raw.at[j], sem.at[S_WO + j])

        def relayout1(src, t0, z=None):
            v = src.reshape(RB * CH, 128)
            tmp[t0:t0 + RB * CH // 2, :] = or_tile(_as_u32(v), z)

        def relayout2(c, h0_, t0, d0, z=None, src=tmp):
            w = or_tile(src[pl.ds(t0, RB2, stride=CH // 2), :], z)
            rows = pl.ds(d0 // 2, RB2 // 2)
            wqkv[c, h0_, rows, :] = _as_u32(w.astype(jnp.uint16))
            wqkv[c, h0_ + 1, rows, :] = _as_u32((w >> 16).astype(jnp.uint16))

        def mod_pair(k):
            for v in range(2):
                mod_tile(wmod_s[k, v], v * NT + k)

        def fill(dst, q, t, r, z=None):
            k = 2 * q + t
            sh = mod[k] if z is None else mod[k] + pltpu.bitcast(z, F32)
            v = nrm[k, r:r + FB, :].reshape(FB // 8, 8, 128) * mod[NT + k] + sh
            dst[t, r // 2:(r + FB) // 2, :] = _as_u32(v.reshape(FB, 128).astype(BF16))

        small = [pltpu.make_async_copy(src, dst, sem.at[S_SM])
                 for src, dst in ((c_hbm, c_ref), (mem0_hbm, mem0_ref), (wr_hbm, wr_ref))]
        for cp in small:
            cp.start()
        x_copy(0).start()
        for cp in mod_copies(0) + mod_copies(1):
            cp.start()
        for g in range(4):
            chunk_copy(0, 0, g, 0, S_C0 + g).start()
        for c in range(1, NSLOT):
            for g in range(4):
                chunk_copy(c % 3, (c // 3) * KQ, g, c, S_ST + c).start()
            for cp in mod_copies(2 * c) + mod_copies(2 * c + 1):
                cp.start()

        kk = lax.broadcasted_iota(jnp.int32, (SEG + M, PR), 0)
        qq = lax.broadcasted_iota(jnp.int32, (SEG + M, PR), 1)
        k_mem = jnp.logical_and(kk >= XR, kk < SEG)
        k_pos = jnp.where(kk < SEG, kk, kk - M)
        q_mem = jnp.logical_and(qq < 2 * SEG, qq % SEG >= XR)
        q_pos = jnp.where(qq < 2 * SEG, qq % SEG, XR + qq % M)
        mk[0:SEG + M, :] = jnp.where(q_mem | k_mem | (q_pos >= k_pos), 0.0, 1.0).astype(F32)
        mod[0:2 * NT] = jnp.zeros((2 * NT, M, 128), F32)
        zero_s[...] = jnp.zeros(zero_s.shape, U32)
        top[...] = jnp.full(top.shape, jnp.iinfo(jnp.int32).min, jnp.int32)
        for cp in small:
            cp.wait()
        wr = jnp.broadcast_to(wr_ref[...].astype(F32).reshape(1, D), (M, D))
        for k in range(NT):
            mod[6 * NT + k] = wr[:, k * 128:(k + 1) * 128]
        cv = c_ref[...].astype(F32)
        sc = _rb(cv * _rb(jax.nn.sigmoid(cv)))
        sc_s[...] = jnp.broadcast_to(sc, (M, D)).astype(BF16)
        for k in range(NT):
            cb_s[k * 128:(k + 1) * 128, :] = jnp.broadcast_to(
                sc[:, k * 128:(k + 1) * 128], (128, 128)).T
        mb = mem0_ref[...]
        for k in range(NT):
            lhs[0, k, XR // 2:, :] = _as_u32(mb[:, k * 128:(k + 1) * 128])

        def zero_body(i, c):
            wo_raw[NT, pl.ds(pl.multiple_of(i * 32, 32), 32), :] = jnp.zeros((32, D), BF16)
            return c

        lax.fori_loop(0, wob // 32, zero_body, 0)
        x_copy(0).wait()

        def ln_body(i, c):
            for u in range(LNU):
                q = i * LNU + u
                x = xbuf[q, XR:, :].astype(F32)
                xc = x - jnp.mean(x, axis=-1, keepdims=True)
                v = xc * _rstd(xc)
                for k in range(NT):
                    nrm[k, pl.ds(pl.multiple_of(q * 8, 8), 8), :] = v[:, k * 128:(k + 1) * 128]
            return c

        with jax.named_scope("p_ln"):
            lax.fori_loop(0, NSEG // LNU, ln_body, 0)

        def mod_body(k, c):
            pltpu.make_async_copy(wmod_s.at[k], wmod_s.at[k], sem.at[S_MOD + k]).wait()
            mod_pair(k)
            for r in range(0, R0, FB):
                fill(ha, 0, k, r)
            return c

        with jax.named_scope("p_mod"):
            lax.fori_loop(0, 2, mod_body, 0)

        def hop1(g):
            chunk_copy(0, 0, g, 0, S_C0 + g).wait()

            def body(i, c):
                d0 = pl.multiple_of(i * 128, 128)
                v = stage[0, g, pl.ds(d0, 128)].reshape(128 * CH, 128)
                t0 = pl.multiple_of((g * KQ + d0) * (CH // 2), 512)
                tmp[pl.ds(t0, 128 * CH // 2), :] = _as_u32(v)
                return c

            lax.fori_loop(0, KQ // 128, body, 0)

        def hop2(c, g, j):
            src = tmp.at[pl.ds(pl.multiple_of(g * (KQ * CH // 2), 512), KQ * CH // 2 + 8)]
            for d0 in range(0, KQ, RB2):
                relayout2(c, g * CH + 2 * j, d0 * CH // 2 + j, d0, src=src)

        def bulk(units, jobs):
            due = {}
            t0 = 0
            for n, (hq, c, h0_, pi, first, r0, nrow) in enumerate(units):
                nb = nrow // BLK
                parts = []
                for u in range(nb):
                    part = hq[0, (r0 + u * BLK) // 2:(r0 + (u + 1) * BLK) // 2, :]
                    for z in due.pop(t0 + u, ()):
                        part = jnp.concatenate([part[0:8] | z, part[8:]], axis=0)
                    parts.append(part)
                hv = jnp.concatenate([_as_bf16(jnp.concatenate(parts, axis=0)),
                                      _as_bf16(hq[1, r0 // 2:(r0 + nrow) // 2, :])], axis=1)
                w = jnp.concatenate([_as_bf16(wqkv[c, h0_]), _as_bf16(wqkv[c, h0_ + 1])], axis=1)
                y = _dot(hv, w)
                segs = slice(r0 // M, (r0 + nrow) // M)
                for a in range(2):
                    old = jnp.where(first, 0.0, pre[pi, segs, a * M:(a + 1) * M, :])
                    pre[pi, segs, a * M:(a + 1) * M, :] = (
                        y[:, a * DH:(a + 1) * DH].reshape(nrow // M, M, DH) + old)
                for u in range(nb):
                    for job in jobs.get(t0 + u, ()):
                        res = job(zero_after(y[u * BLK:u * BLK + 8, 0:128]))
                        if res is not None:
                            due.setdefault(max(t0 + u + JOB_SPAN, t0 + nb), []).append(
                                zero_after(res))
                t0 += nb
            assert not due

        GP = CH // 2
        WO0 = NCHUNK - 1 - NT
        LN0 = 4
        SPI = -(-NSEG // (NCHUNK - 1 - LN0))

        def rot_body(i, c):
            slot = (i + 1) & (NSLOT - 1)
            pltpu.make_async_copy(stage.at[slot], stage.at[slot], sem.at[S_ST + slot]).wait()
            km = 2 * jnp.minimum(i, 3)

            @pl.when(jnp.logical_and(i >= 1, i <= 3))
            def _():
                wq = wmod_s.at[pl.ds(km, 2)]
                pltpu.make_async_copy(wq, wq, sem.at[S_MOD + km]).wait()

            @pl.when(i == LN0)
            def _():
                x_copy(1).wait()

            @pl.when(i >= WO0)
            def _():
                wo_copy(i - WO0).wait()

            nxt = i + NSLOT
            qn = (nxt * 43) >> 7
            for mat in range(3):
                @pl.when(jnp.logical_and(nxt < NCHUNK, nxt - 3 * qn == mat))
                def _():
                    for g in range(4):
                        chunk_copy(mat, qn * KQ, g, nxt & (NSLOT - 1),
                                   S_ST + (nxt & (NSLOT - 1))).start()

            @pl.when(i < NT)
            def _():
                wo_copy(i).start()

            @pl.when(i == 0)
            def _():
                x_copy(1).start()

            q0 = (i * 43) >> 7
            q1 = ((i + 1) * 43) >> 7
            pa = (i - 3 * q0) * NP + NP - GP
            units = ([(ha, i, H - CH + 2 * n, pa + n, q0 == 0, 0, R0) for n in range(GP)]
                     + [(hb, i + 1, 2 * n, (i + 1 - 3 * q1) * NP + n, q1 == 0, 0, R0)
                        for n in range(NP - GP)])
            jw = jnp.where(i >= WO0, i - WO0, NT)

            def wo_job(b, z):
                v = wo_raw[jw, b * 16:(b + 1) * 16, :]
                rows = pl.ds(pl.multiple_of(jw * (wob // 2) + b * 8, 8), 8)
                for j in range(NT):
                    wo_s[j, rows, :] = _as_u32(v[:, j * 128:(j + 1) * 128]) | z

            lst = {}

            def ln_job(b, ph, z):
                r = (b % 3) * 8
                seg = (i - LN0) * SPI + b // 3
                live = jnp.logical_and(i >= LN0, seg < NSEG)
                src = jnp.where(live, seg, 0) + (i >> (10 + ph))
                x = xbuf[src, pl.ds(pl.multiple_of(jnp.where(live, r, XR), 8), 8), :].astype(F32)
                zf = pltpu.bitcast(z, F32)
                if ph == 0:
                    xm = jnp.concatenate([x[:, :128] + zf, x[:, 128:]], axis=1)
                    mu = jnp.mean(xm, axis=-1, keepdims=True)
                    lst[2 * b] = jnp.broadcast_to(mu, (8, 128))
                    return None
                xc = x - jnp.concatenate([lst[2 * b] + zf] * NT, axis=1)
                if ph == 1:
                    lst[2 * b + 1] = jnp.broadcast_to(_rstd(xc), (8, 128))
                    return None
                inv = jnp.concatenate([lst[2 * b + 1]] * NT, axis=1)
                hv = (xc * inv * modv(1) + modv(0)).astype(BF16)
                u = [_as_u32(hv[:, k * 128:(k + 1) * 128]) for k in range(NT)]
                dst = jnp.where(live, seg, NSEG)
                for k in range(NT):
                    hs[dst, k, r // 2:r // 2 + 4, :] = u[k]
                res = jnp.concatenate(u[0:2], axis=0)
                for k in range(2, NT, 2):
                    res = res | jnp.concatenate(u[k:k + 2], axis=0)
                return res

            def r1_job(g, d0, z):
                relayout1(stage[slot, g, d0:d0 + RB], (g * KQ + d0) * CH // 2, z)

            def copy_job(t, r, z):
                ha[t, r:r + 32, :] = or_tile(hb[t, r:r + 32, :], z)

            P = functools.partial
            upb = R0 // BLK
            nr = NP * upb
            jobs = {}
            for g in range(4):
                lo, mid, hi = (x * upb // 4 for x in R_AT[g])
                _spread(jobs, [P(r1_job, g, d0) for d0 in range(0, KQ, RB)], lo, mid)
                _spread(jobs, [P(relayout2, i + 1, g * CH + 2 * j, (g * KQ + d0) * CH // 2 + j, d0)
                               for j in range(CH // 2) for d0 in range(0, KQ, RB2)], mid, hi)
            oz = i >> 10
            _spread(jobs, [P(fill, hb, q1, t + oz, r) for r in range(0, R0, FB) for t in range(2)],
                    F_AT[0] * upb // 4, F_AT[1] * upb // 4)
            _spread(jobs, [P(copy_job, t, r) for t in range(2) for r in range(0, R0 // 2, 32)],
                    2 * GP * upb, nr - upb)
            for ph in range(3):
                off = LN_PH[ph] - LN_PH[2]
                _spread(jobs, [P(ln_job, b, ph) for b in range(3 * SPI)],
                        L_AT * upb // 4 + LN_PH[ph], nr - max(upb, JOB_SPAN) + off)
            _spread(jobs, [P(wo_job, b) for b in range(wob // 16)], GP * upb, nr - upb)
            gv = {}

            def gv_job(d0, n, z):
                w = wmod_s[pl.ds(km, 2), :, d0:d0 + n, :].reshape(4, n, 128)
                acc = gv.get("acc")
                if z is not None:
                    zf = pltpu.bitcast(z, F32)[None]
                    acc = jnp.broadcast_to(zf, (4, 8, 128)) if acc is None else acc + zf
                gv["acc"] = gemv_part(w, d0, acc)
                if z is not None:
                    au = pltpu.bitcast(gv["acc"], U32)
                    return au[0] | au[1] | au[2] | au[3]

            _spread(jobs, [P(gv_job, d0, GVR) for d0 in range(0, D - GV_FREE, GVR)],
                    GV_AT[0] * upb // 4, min(GV_AT[1] * upb // 4, nr - JOB_SPAN))
            bulk(units, jobs)
            if GV_FREE:
                gv_job(D - GV_FREE, GV_FREE, None)
            gemv_finish(gv["acc"], [km, NT + km, km + 1, NT + km + 1])
            return c

        def outer(k, c):
            last = k == 4

            @pl.when(k < 4)
            def _():
                hop1(k)

            @pl.when(k != 3)
            def _():
                g = jnp.minimum(k, 3)
                cc = jnp.where(last, NCHUNK - 1, 0)
                for j in range(GP):
                    hop2(cc, g, j)
                bulk([(ha, cc, g * CH + 2 * n, jnp.where(last, 2 * NP, 0) + g * GP + n, k < 4,
                       0, R0) for n in range(GP)], {})

            @pl.when(k == 3)
            def _():
                for j in range(GP):
                    hop2(0, 3, j)
                with jax.named_scope("p_rot"):
                    lax.fori_loop(0, NCHUNK - 1, rot_body, 0)
                for it in range(2):
                    for u in range(mt):
                        wm_copy(it, u).start()

            return c

        with jax.named_scope("p_bulk"):
            lax.fori_loop(0, 5, outer, 0)

    if "pro" in PHASES: pl.run_scoped(
        prologue,
        pltpu.VMEM((NSLOT, H // CH, KQ, CH, 128), BF16),
        pltpu.VMEM((NT + 1, H * DH // NT, D), BF16),
        pltpu.VMEM((NT, 2, D, 128), BF16),
        pltpu.VMEM((NT, R0, 128), F32),
        pltpu.VMEM((2, R0 // 2, 128), U32),
        pltpu.VMEM((2, R0 // 2, 128), U32),
        pltpu.VMEM((D * CH // 2 + 32, 128), U32),
        pltpu.VMEM((M, D), BF16),
        pltpu.VMEM((D,), BF16),
        pltpu.VMEM((1, D), BF16),
        pltpu.SemaphoreType.DMA((7 + NSLOT + 2 * NT,)),
    )

    def main(wg_s, wu_s, wd_s, ybuf, stat, outs, sem_f):
        def load_x_rows(slot, seg):
            for k in range(NT):
                lhs[slot, k, 0:XR // 2, :] = hs[seg, k]

        def resid(seg, r, z=None):
            rows = pl.ds(r, 8)
            t = modv(2) * ybuf[seg, rows, :].astype(F32)
            if z is not None:
                t = t + jnp.concatenate([pltpu.bitcast(z, F32)] * NT, axis=1)
            return xbuf[seg, rows, :].astype(F32) + t

        def wide(v):
            return jnp.concatenate([v] * NT, axis=1)

        def make_key(v, row0):
            b = pltpu.bitcast(jnp.where(v != v, -jnp.inf, v + 0.0), jnp.int32)
            low = (S - 1 - row0) - lax.broadcasted_iota(jnp.int32, (8, 128), 0)
            return (b ^ ((b >> 31) & 0x7FFF0000)) | low

        def post(st, ph, seg, r, z):
            zf = pltpu.bitcast(z, F32)
            if ph == 0:
                st["x1"] = resid(seg, r, z)
                st["mu"] = jnp.broadcast_to(jnp.mean(st["x1"], axis=-1, keepdims=True), (8, 128))
                return None
            if ph == 1:
                mu = st["mu"] + zf
                stat[0, seg, pl.ds(r, 8), :] = mu
                xc = st["xc"] = st["x1"] - wide(mu)
                st["var"] = jnp.mean(xc * xc, axis=-1, keepdims=True)
                st["dot"] = jnp.sum(xc * modv(7), axis=-1, keepdims=True)
                return None
            inv = _inv_std(st["var"]) + zf
            stat[1, seg, pl.ds(r, 8), :] = inv
            v = _rb(inv * st["dot"] + mod[8 * NT])
            key = make_key(v, seg * SEG + r)
            m1, m2 = top[0:8, :], top[8:16, :]
            top[8:16, :] = jnp.maximum(m2, jnp.minimum(m1, key))
            top[0:8, :] = jnp.maximum(m1, key)
            o = st["x1"] + modv(5) * (st["xc"] * wide(inv) * modv(4) + modv(3))
            outs[seg, pl.ds(r, 8), :] = o.astype(BF16)
            res = pltpu.bitcast(v, U32)
            for k in range(NT):
                res = res | pltpu.bitcast(o[:, k * 128:(k + 1) * 128], U32)
            return res

        def redo(seg, r, z=None):
            x1 = resid(seg, r, z)
            n = (x1 - wide(stat[0, seg, pl.ds(r, 8), :])) * wide(stat[1, seg, pl.ds(r, 8), :])
            return x1, n * modv(4) + modv(3)

        def out_copy(g0, ng, r, n, k=0):
            return pltpu.make_async_copy(outs.at[pl.ds(g0, ng), pl.ds(r, n), :],
                                         out_hbm.at[pl.ds(g0, ng), pl.ds(r, n), :], sem_out.at[k])

        late = ((wg_hbm, wg_s, FF // 128), (wu_hbm, wu_s, FF // 128), (wd_hbm, wd_s, NT))

        def col_copy(k, j):
            return pltpu.make_async_copy(
                late[k][0].at[:, pl.ds(pl.multiple_of(j * 128, 128), 128)], late[k][1].at[j],
                sem_f.at[k])

        load_x_rows(0, 0)

        def step(it, cur, state):
            s = it * UNROLL + cur
            nxt = (cur + 1) % UNROLL

            def pay(t, cost):
                now, due = state["now"], state["due"]
                for z in [z for (d, z) in due if d <= now]:
                    t = jnp.concatenate([t[0:8] | z, t[8:]], axis=0)
                state["due"] = [(d, z) for (d, z) in due if d > now]
                state["now"] = now + cost
                return t

            def release(y):
                now = state["now"]
                pend, state["pend"] = state["pend"], [e for e in state["pend"] if e[0] > now]
                for (d, f) in pend:
                    if d <= now:
                        f(zero_after(y[0:8]))

            def lv(k0, k1):
                ts = [lhs[cur, k] for k in range(k0, k1)]
                ts[0] = pay(ts[0], (k1 - k0) / NT)
                return jnp.concatenate([_as_bf16(t) for t in ts], axis=1)

            def wmat(mat, h, q0, q1):
                return _as_bf16(jnp.concatenate([wqkv[3 * q + mat, h] for q in range(q0, q1)],
                                                axis=0))

            def qkv(p, split=False):
                part = {}
                if split:
                    for mat in range(3):
                        for a in range(2):
                            part[mat, a] = _dot(lv(0, NT // 2), wmat(mat, 2 * p + a, 0, 2))
                for mat in range(3):
                    for a in range(2):
                        hm = mat * H + 2 * p + a
                        if split:
                            y = _dot(lv(NT // 2, NT), wmat(mat, 2 * p + a, 2, 4)) + part[mat, a]
                        else:
                            y = _dot(lv(0, NT), wmat(mat, 2 * p + a, 0, 4))
                        cur_s[hm] = y.astype(BF16)
                        release(y)

            def gather(mat, p):
                hm = mat * H + 2 * p
                return jnp.concatenate(
                    [cur_s[hm], cur_s[hm + 1], pre[mat * NP + p, s].astype(BF16)], axis=0)

            probs = {}

            def scores(p):
                st = lax.dot_general(gather(1, p), gather(0, p), (((1,), (1,)), ((), ())),
                                     preferred_element_type=F32)
                lane = lax.broadcasted_iota(jnp.int32, (1, PR), 1)
                is_a = jnp.logical_or(lane < SEG,
                                      jnp.logical_and(lane >= 2 * SEG, lane < 2 * SEG + M))
                ka = jnp.concatenate([st[0:SEG], st[2 * SEG:2 * SEG + M]], axis=0)
                kb = jnp.concatenate([st[SEG:2 * SEG], st[2 * SEG + M:]], axis=0)
                t = jnp.where(is_a, ka, kb) * (SCALE * LOG2E)
                ts_s[p + (it >> 10)] = jnp.where(mk[0:SEG + M, :] == 0.0, t, NEG_MASK * LOG2E)

                def softmax(z):
                    zf = pltpu.bitcast(z, F32)[:, 0:PR]
                    t = (ts_s[p].reshape(-1, 8, PR) + zf).reshape(SEG + M, PR)
                    e = jnp.exp2(t - jnp.max(t, axis=0, keepdims=True))
                    e = e * _recip(jnp.sum(e, axis=0, keepdims=True))
                    pa = jnp.where(is_a, e, 0.0)
                    pb = jnp.where(is_a, 0.0, e)
                    probs[p] = jnp.concatenate(
                        [pa[0:SEG], pb[0:SEG], pa[SEG:], pb[SEG:]], axis=0).astype(BF16)

                state["pend"].append((state["now"] + REL_S + (p % PG) * REL_STAG, softmax))

            def pv(p):
                o = lax.dot_general(probs.pop(p), gather(2, p), (((0,), (0,)), ((), ())),
                                    preferred_element_type=F32).astype(BF16)
                for a in range(2):
                    h = 2 * p + a
                    olhs[h] = _as_u32(o[a * SEG:(a + 1) * SEG])
                    odef[h, it, cur * 4:(cur + 1) * 4, :] = _as_u32(
                        o[2 * SEG + a * M:2 * SEG + (a + 1) * M])

            acc = [None] * NT

            def oproj(j, pairs):
                ts = [olhs[2 * p + a] for p in pairs for a in range(2)]
                ts[0] = pay(ts[0], len(pairs) / 4)
                ov = jnp.concatenate([_as_bf16(t) for t in ts], axis=1)
                w = wo_s[j, pairs[0] * DH:(pairs[-1] + 1) * DH, :]
                y = _dot(ov, _as_bf16(w))
                acc[j] = y if acc[j] is None else y + acc[j]
                release(acc[j])

            def fin(j):
                yb = acc[j].astype(BF16)
                ybuf[s, 0:XR, j * 128:(j + 1) * 128] = yb[0:XR]
                lhs[nxt, j, XR // 2:, :] = _as_u32(yb[XR:])

            def gemv():
                d0 = state["d0"]
                state["acc"] = gemv_part(wm_s[it & 3, :, d0:d0 + GR, :], d0, state["acc"])
                state["d0"] = d0 + GR
                au = pltpu.bitcast(state["acc"], U32)
                z = functools.reduce(lambda a, b: a | b, [au[u] for u in range(mt)])
                state["due"].append((state["now"] + G_LAG, zero_after(z)))

            load_x_rows(nxt, jnp.minimum(s + 1, NSEG - 1))
            ops = dict(Q=qkv, S=scores, P=pv, O=oproj, F=fin, G=gemv)
            for op in _schedule():
                ops[op[0]](*op[1:])

        def steps(it, carry):
            if "pro" in PHASES:
                pltpu.make_async_copy(wm_s.at[it & 3], wm_s.at[it & 3], sem_m.at[it & 3]).wait()

                @pl.when(it + 2 < NSEG // UNROLL)
                def _():
                    for u in range(mt):
                        wm_copy(it + 2, u).start()

            for u in range(UNROLL // 2):
                t = it * (UNROLL // 2) + u
                for k in range(3):
                    @pl.when(t < late[k][2])
                    def _():
                        col_copy(k, t).start()

            state = dict(now=0, due=[], pend=[], d0=0, acc=None)
            for u in range(UNROLL):
                step(it, u, state)
            acc = state["acc"]
            for d0 in range(state["d0"], D, 64):
                acc = gemv_part(wm_s[it & 3, :, d0:min(d0 + 64, D), :], d0, acc)
            gemv_finish(acc, [2 * NT + it * mt + u for u in range(mt)])
            return carry

        with jax.named_scope("m_steps"):
            if "step" in PHASES: lax.fori_loop(0, NSEG // UNROLL, steps, 0)
        for k in range(3):
            for j in range(late[k][2]):
                col_copy(k, j).wait()
        if "epi" not in PHASES:
            cp = pltpu.make_async_copy(ybuf, out_hbm, sem_out.at[0])
            cp.start()
            cp.wait()
            return

        ntail = EC // M
        ppi = (S // 8 - ntail) // NEC
        gpi = ppi // (XR // 8)
        nblk = EC // (UNROLL * M)

        def ep_body(i, c):
            @pl.when(i > 0)
            def _():
                out_copy((i - 1) * gpi, gpi, 0, XR).start()

            for k in range(NT):
                mod[7 * NT + k] = mod[4 * NT + k] * mod[6 * NT + k]
            mod[8 * NT] = jnp.broadcast_to(
                jnp.sum(modv(3) * modv(6), axis=-1, keepdims=True), (M, 128))

            jobs = {}
            for ph in range(3):
                _spread(jobs, [(u, ph) for u in range(ppi)], E_PH[ph],
                        (NT * H // EKH - E_SPAN) * E_REL - E_PH[2] + E_PH[ph])
            sts = [{} for _ in range(ppi)]
            due = {}
            n = 0
            for j in range(NT):
                for h0_ in range(0, H, EKH):
                    ts = [odef[h, pl.ds(i * nblk, nblk)].reshape(EC // 2, DH)
                          for h in range(h0_, h0_ + EKH)]
                    for z in due.pop(n, ()):
                        ts[0] = jnp.concatenate([ts[0][0:8] | z, ts[0][8:]], axis=0)
                    w = wo_s[j, h0_ * DH // 2:(h0_ + EKH) * DH // 2, :]
                    yp = _dot(jnp.concatenate([_as_bf16(t) for t in ts], axis=1), _as_bf16(w))
                    y = yp if h0_ == 0 else yp + y
                    if h0_ + EKH == H:
                        ybuf[pl.ds(i * ntail, ntail), XR:, j * 128:(j + 1) * 128] = (
                            y.reshape(ntail, M, 128).astype(BF16))
                    for q in range(E_REL):
                        for (u, ph) in jobs.get(n * E_REL + q, ()):
                            t = i * ppi + u
                            early = t < NSEG * (XR // 8)
                            seg = jnp.where(early, t // (XR // 8), t - NSEG * (XR // 8))
                            row = pl.multiple_of(jnp.where(early, (t % (XR // 8)) * 8, XR), 8)
                            zr = q * (EC // E_REL)
                            res = post(sts[u], ph, seg, row, zero_after(y[zr:zr + 8]))
                            if res is not None:
                                due.setdefault(n + E_SPAN, []).append(zero_after(res))
                    n += 1
            return c

        with jax.named_scope("e_loop"):
            lax.fori_loop(0, NEC, ep_body, 0)
        done = (NEC - 1) * gpi
        tail = NSEG - ntail
        out_copy(done, NSEG - done, 0, XR).start()
        out_copy(0, tail, XR, M).start()
        x1s = [resid(g, XR) for g in range(tail, NSEG)]
        mus = [jnp.mean(x1, axis=-1, keepdims=True) for x1 in x1s]
        pairs = [(top[0:8, :], top[8:16, :])]
        lowest = jnp.full((8, 128), jnp.iinfo(jnp.int32).min, jnp.int32)
        for g in range(tail, NSEG):
            xc = x1s[g - tail] - mus[g - tail]
            inv = _inv_std(jnp.mean(xc * xc, axis=-1, keepdims=True))
            stat[0, g, XR:, :] = jnp.broadcast_to(mus[g - tail], (8, 128))
            stat[1, g, XR:, :] = jnp.broadcast_to(inv, (8, 128))
            v = _rb(inv * jnp.sum(xc * modv(7), axis=-1, keepdims=True) + mod[8 * NT])
            pairs.append((make_key(v, g * SEG + XR), lowest))
        while len(pairs) > 1:
            (a1, a2), (c1, c2) = pairs.pop(0), pairs.pop(0)
            pairs.append((jnp.maximum(a1, c1),
                          jnp.maximum(jnp.minimum(a1, c1), jnp.maximum(a2, c2))))

        tk = jnp.concatenate(pairs[0], axis=0)[:, 0:1]
        k1 = jnp.max(tk[0:8], axis=0, keepdims=True)
        k2 = jnp.max(jnp.where(tk == k1, jnp.iinfo(jnp.int32).min, tk), axis=0, keepdims=True)
        i1 = (S - 1) - (k1[0, 0] & (S - 1))
        i2 = (S - 1) - (k2[0, 0] & (S - 1))
        g1, g2 = i1 >> 5, i2 >> 5
        b1 = pl.multiple_of(i1 & 24, 8)
        b2 = pl.multiple_of(i2 & 24, 8)

        def tail_out(n, z):
            g, k0 = tail + n // (NT // TW), (n % (NT // TW)) * TW
            zf = pltpu.bitcast(z, F32)
            for k in range(k0, k0 + TW, 2):
                cols = slice(k * 128, (k + 2) * 128)
                m = lambda j: jnp.concatenate([mod[j * NT + k], mod[j * NT + k + 1]], axis=1)
                two = lambda v: jnp.concatenate([v, v], axis=1)
                x1_ = (xbuf[g, XR:, cols].astype(F32)
                       + (m(2) * ybuf[g, XR:, cols].astype(F32) + two(zf)))
                h_ = (x1_ - two(stat[0, g, XR:, :])) * two(stat[1, g, XR:, :]) * m(4) + m(3)
                outs[g, XR:, cols] = (x1_ + m(5) * h_).astype(BF16)

        xa, ha_ = redo(g1, b1)
        xb_, hb_ = redo(g2, b2)
        x1 = jnp.concatenate([xa, xb_], axis=0)
        h2 = jnp.concatenate([ha_, hb_], axis=0)
        h2b = h2.astype(BF16)
        row = lax.broadcasted_iota(jnp.int32, (16, 1), 0)
        grow = jnp.where(row < 8, g1 * SEG + b1 + row, g2 * SEG + b2 + row - 8)
        ks = jnp.where(grow == i1, k1, k2)
        rsel = pltpu.bitcast((ks ^ ((ks >> 31) & 0x7FFF0000)) & -65536, F32)
        acts = []
        jobs = {}
        _spread(jobs, list(range(ntail * NT // TW)), 0, T_END)
        for j in range(FF // 128):
            gt = _rb(_dot(h2b, wg_s[j]))
            for n in jobs.get(2 * j, ()):
                tail_out(n, zero_after(gt[0:8]))
            gt = _rb(gt * _rb(jax.nn.sigmoid(gt)))
            ut = _rb(_dot(h2b, wu_s[j]))
            for n in jobs.get(2 * j + 1, ()):
                tail_out(n, zero_after(ut[0:8]))
            acts.append((gt * ut).astype(BF16))
        out_copy(tail, NSEG - tail, XR, M).start()
        act = jnp.concatenate(acts, axis=1)
        y = _rb(jnp.concatenate([_dot(act, wd_s[j]) for j in range(NT)], axis=1))
        y = _rb(y * _rb(jax.nn.sigmoid(rsel)))
        sel = jnp.logical_or(grow == i1, grow == i2)
        gb2 = jnp.concatenate([modv(5)] * 2, axis=0)
        fixed = (x1 + gb2 * (h2 + jnp.where(sel, y, 0.0))).astype(BF16)

        with jax.named_scope("e_outwait"):
            out_copy(0, NSEG, 0, SEG).wait()
        outs[g1, pl.ds(b1, 8), :] = fixed[0:8]
        outs[g2, pl.ds(b2, 8), :] = fixed[8:16]
        out_copy(g1, 1, b1, 8, 0).start()

        @pl.when((i1 >> 3) != (i2 >> 3))
        def _():
            out_copy(g2, 1, b2, 8, 1).start()
            out_copy(g2, 1, b2, 8, 1).wait()

        out_copy(g1, 1, b1, 8, 0).wait()

    pl.run_scoped(
        main,
        pltpu.VMEM((FF // 128, D, 128), BF16),
        pltpu.VMEM((FF // 128, D, 128), BF16),
        pltpu.VMEM((NT, FF, 128), BF16),
        pltpu.VMEM((NSEG, SEG, D), BF16),
        pltpu.VMEM((2, NSEG, SEG, 128), F32),
        pltpu.VMEM((NSEG, SEG, D), BF16),
        pltpu.SemaphoreType.DMA((3,)),
    )


def _entry(*refs):
    pl.run_scoped(
        functools.partial(_kernel, *refs),
        pltpu.VMEM((NCHUNK, H, KQ // 2, DH), U32),
        pltpu.VMEM((NSEG + 1, NT, XR // 2, 128), U32),
        pltpu.VMEM((NT, (H * DH + H * DH // NT) // 2, 128), U32),
        pltpu.VMEM((3 * NP, NSEG, 2 * M, DH), F32),
        pltpu.VMEM((3 * H, SEG, DH), BF16),
        pltpu.VMEM((H, SEG // 2, DH), U32),
        pltpu.VMEM((H, NSEG // UNROLL, UNROLL * M // 2, DH), U32),
        pltpu.VMEM((NSEG, SEG, D), BF16),
        pltpu.VMEM((UNROLL, NT, SEG // 2, 128), U32),
        pltpu.VMEM((4, 4 * NT * UNROLL // NSEG, D, 128), BF16),
        pltpu.VMEM((8 * NT + 4, M, 128), F32),
        pltpu.VMEM((64, PR), F32),
        pltpu.VMEM((32, 128), jnp.int32),
        pltpu.VMEM((M, D), BF16),
        pltpu.VMEM((D, 128), F32),
        pltpu.VMEM((NP, SEG + M, PR), F32),
        pltpu.VMEM((8 + PAD, 128), U32),
        pltpu.SemaphoreType.DMA((4,)),
        pltpu.SemaphoreType.DMA((2,)),
    )


@functools.partial(jax.jit, static_argnames=("A_seg_len",))
def pallas_adaLN_cond__memory_aug_recurrent_mem_tr__moe_arch_mod__prompt_kernel(
    A_x: jax.Array,
    A_mem0: jax.Array,
    A_Wq: jax.Array,
    A_Wk: jax.Array,
    A_Wv: jax.Array,
    A_Wo: jax.Array,
    A_seg_len,
    B_x: jax.Array,
    B_w_r: jax.Array,
    B_w_gate: jax.Array,
    B_w_up: jax.Array,
    B_w_down: jax.Array,
    c: jax.Array,
    w_mod: jax.Array,
):
    assert A_seg_len == SEG and A_x.shape == (1, S, D)
    del B_x
    hbm = pl.BlockSpec(memory_space=pl.ANY)
    out = pl.pallas_call(
        _entry,
        out_shape=jax.ShapeDtypeStruct((NSEG, SEG, D), BF16),
        in_specs=[hbm] * 12,
        out_specs=hbm,
        compiler_params=pltpu.CompilerParams(vmem_limit_bytes=120 * 1024 * 1024,
                                             disable_bounds_checks=True),
    )(A_x.reshape(NSEG, SEG, D), A_mem0.reshape(M, D), A_Wq, A_Wk, A_Wv, A_Wo.reshape(H * DH, D),
      B_w_r, B_w_gate, B_w_up, B_w_down, c, w_mod)
    return out.reshape(1, S, D)
```

```python
import functools

import jax
import jax.numpy as jnp
from jax import lax
import jax.experimental.pallas as pl
import jax.experimental.pallas.tpu as pltpu

F32 = jnp.float32
BF16 = jnp.bfloat16
U32 = jnp.uint32

D = 1024
S = 2048
H = 32
DH = 128
M = 8
SEG = 32
NSEG = S // SEG
FF = 3584
NT = D // 128
XR = SEG - M
R0 = M * NSEG
CH = 8
KQ = D // 4
NCHUNK = 3 * D // KQ
NSLOT = 4
PR = 2 * SEG + 2 * M
NP = H // 2
EC = 128
NEC = R0 // EC
LOG2E = 1.4426950408889634
EPS = 1e-5
SCALE = DH ** -0.5
NEG_MASK = -1000000000.0

UNROLL = 4
PG = 4
LAG_S = 1
LAG_P = 4
O_PARTS = (0, 8, 12)
O_TH = (256, 256, 256, 1280)
REL_S = 3
REL_STAG = 2
G_AT = (0, 1, 2, 3, 7, 11)
GR = 32
G_LAG = 3
BLK = 32
JOB_SPAN = 40
RB = 16
RB2 = 32
FB = 32
GVR = 32
GV_FREE = 64
R_AT = ((0, 6, 16), (14, 22, 30), (30, 38, 46), (44, 52, 60))
F_AT = (0, 13)
L_AT = 6
GV_AT = (16, 56)
LNU = 16
LN_PH = (0, 10, 20)
EKH = 4
E_SPAN = 4
E_REL = 4
E_PH = (0, 10, 20)
TW = 4
T_END = 32
PAD = 24


def _schedule():
    groups = [list(range(g, g + PG)) for g in range(0, NP, PG)]
    at = {}
    for g, grp in enumerate(groups):
        at.setdefault(grp[-1] + LAG_P, []).extend(("P", q) for q in grp)
    for g, grp in enumerate(groups):
        at.setdefault(grp[-1] + LAG_S, []).extend(("S", q) for q in grp)
    ops = []
    for p in range(NP):
        ops.append(("Q", p, p == 0))
        if p in G_AT:
            ops.append(("G",))
        ops.extend(at.pop(p, []))
    bounds = list(O_PARTS) + [NP]
    t = NP
    done = 0
    for n in range(len(O_PARTS)):
        part = list(range(bounds[n], bounds[n + 1]))
        assert all(("P", q) in ops for q in part), (n, ops)
        for j in range(NT):
            ops.append(("O", j, part))
            if n == len(O_PARTS) - 1:
                ops.append(("F", j))
            done += len(part) * 16
            while t - NP < len(O_TH) and done >= O_TH[t - NP]:
                ops.extend(at.pop(t, []))
                t += 1
    assert not at
    return ops


def _rb(x):
    return x.astype(BF16).astype(F32)


def _recip(x):
    r = pl.reciprocal(x, approx=True)
    return r * (2.0 - x * r)


def _inv_std(var):
    v = _rb(_rb(var) + EPS)
    return _recip(_rb(v * lax.rsqrt(v)))


def _rstd(xc):
    return lax.rsqrt(jnp.mean(xc * xc, axis=-1, keepdims=True) + EPS)


def _dot(a, b):
    return jnp.dot(a, b, preferred_element_type=F32)


def _as_bf16(u):
    return pltpu.bitcast(u, BF16)


def _as_u32(b):
    return pltpu.bitcast(b, U32)


def _spread(jobs, fns, lo, hi):
    for n, fn in enumerate(fns):
        jobs.setdefault(lo + n * (hi - lo) // len(fns), []).append(fn)


def _kernel(x_hbm, mem0_hbm, wq_hbm, wk_hbm, wv_hbm, wo_hbm, wr_hbm, wg_hbm, wu_hbm, wd_hbm,
            c_hbm, wmod_hbm, out_hbm,
            wqkv, hs, wo_s, pre, cur_s, olhs, odef, xbuf, lhs, wm_s, mod, mk,
            top, sc_s, cb_s, ts_s, zero_s, sem_m, sem_out):
    mt = 4 * NT * UNROLL // NSEG

    def modv(j):
        return jnp.concatenate([mod[j * NT + k] for k in range(NT)], axis=1)

    def mod_store(v, t):
        v = _rb(v)
        mod[t] = jnp.where(jnp.logical_or((t >> 3) == 1, (t >> 3) == 4), _rb(1.0 + v), v)

    def mod_tile(wm, t):
        mod_store(_dot(sc_s[...], wm), t)

    def gemv_part(w, d0, acc):
        n = w.shape[1]
        p = w.astype(F32) * cb_s[d0:d0 + n, :]
        p = jnp.sum(p.reshape(w.shape[0], n // 8, 8, 128), axis=1)
        return p if acc is None else p + acc

    def gemv_finish(acc, ts):
        for u, t in enumerate(ts):
            mod_store(jnp.broadcast_to(jnp.sum(acc[u], axis=0, keepdims=True), (M, 128)), t)

    def wm_copy(it, u):
        col = pl.multiple_of((2 * NT + it * mt + u) * 128, 128)
        return pltpu.make_async_copy(wmod_hbm.at[:, pl.ds(col, 128)], wm_s.at[it & 3, u],
                                     sem_m.at[it & 3])

    def zero_after(y):
        return (y if y.dtype == U32 else pltpu.bitcast(y, U32)) & zero_s[0:8, :]

    def or_tile(u, z):
        if z is None:
            return u
        return (u.reshape(u.shape[0] // 8, 8, 128) | z).reshape(u.shape)

    def prologue(stage, wo_raw, wmod_s, nrm, ha, hb, tmp, mem0_ref, wr_ref, c_ref, sem):
        w_hbms = (wq_hbm, wk_hbm, wv_hbm)
        wob = H * DH // NT
        S_X, S_C0, S_ST, S_WO, S_MOD, S_SM = 0, 2, 6, 6 + NSLOT, 6 + NSLOT + NT, 6 + NSLOT + 2 * NT

        def x_copy(i):
            lo, n = ((XR, M), (0, XR))[i]
            return pltpu.make_async_copy(x_hbm.at[:, pl.ds(lo, n), :], xbuf.at[:, pl.ds(lo, n), :],
                                         sem.at[S_X + i])

        def mod_copies(k):
            return [pltpu.make_async_copy(wmod_hbm.at[:, pl.ds(v * D + k * 128, 128)],
                                          wmod_s.at[k, v], sem.at[S_MOD + (k if k < 2 else k & 6)])
                    for v in range(2)]

        def chunk_copy(mat, d0, g, slot, k):
            heads = pl.ds(pl.multiple_of(g * CH, CH), CH)
            return pltpu.make_async_copy(w_hbms[mat].at[pl.ds(d0, KQ), heads, :],
                                         stage.at[slot, g], sem.at[k])

        def wo_copy(j):
            return pltpu.make_async_copy(wo_hbm.at[pl.ds(pl.multiple_of(j * wob, wob), wob)],
                                         wo_raw.at[j], sem.at[S_WO + j])

        def relayout1(src, t0, z=None):
            v = src.reshape(RB * CH, 128)
            tmp[t0:t0 + RB * CH // 2, :] = or_tile(_as_u32(v), z)

        def relayout2(c, h0_, t0, d0, z=None, src=tmp):
            w = or_tile(src[pl.ds(t0, RB2, stride=CH // 2), :], z)
            rows = pl.ds(d0 // 2, RB2 // 2)
            wqkv[c, h0_, rows, :] = _as_u32(w.astype(jnp.uint16))
            wqkv[c, h0_ + 1, rows, :] = _as_u32((w >> 16).astype(jnp.uint16))

        def mod_pair(k):
            for v in range(2):
                mod_tile(wmod_s[k, v], v * NT + k)

        def fill(dst, q, t, r, z=None):
            k = 2 * q + t
            sh = mod[k] if z is None else mod[k] + pltpu.bitcast(z, F32)
            v = nrm[k, r:r + FB, :].reshape(FB // 8, 8, 128) * mod[NT + k] + sh
            dst[t, r // 2:(r + FB) // 2, :] = _as_u32(v.reshape(FB, 128).astype(BF16))

        small = [pltpu.make_async_copy(src, dst, sem.at[S_SM])
                 for src, dst in ((c_hbm, c_ref), (mem0_hbm, mem0_ref), (wr_hbm, wr_ref))]
        for cp in small:
            cp.start()
        x_copy(0).start()
        for cp in mod_copies(0) + mod_copies(1):
            cp.start()
        for g in range(4):
            chunk_copy(0, 0, g, 0, S_C0 + g).start()
        for c in range(1, NSLOT):
            for g in range(4):
                chunk_copy(c % 3, (c // 3) * KQ, g, c, S_ST + c).start()
            for cp in mod_copies(2 * c) + mod_copies(2 * c + 1):
                cp.start()

        kk = lax.broadcasted_iota(jnp.int32, (SEG + M, PR), 0)
        qq = lax.broadcasted_iota(jnp.int32, (SEG + M, PR), 1)
        k_mem = jnp.logical_and(kk >= XR, kk < SEG)
        k_pos = jnp.where(kk < SEG, kk, kk - M)
        q_mem = jnp.logical_and(qq < 2 * SEG, qq % SEG >= XR)
        q_pos = jnp.where(qq < 2 * SEG, qq % SEG, XR + qq % M)
        mk[0:SEG + M, :] = jnp.where(q_mem | k_mem | (q_pos >= k_pos), 0.0, 1.0).astype(F32)
        mod[0:2 * NT] = jnp.zeros((2 * NT, M, 128), F32)
        zero_s[...] = jnp.zeros(zero_s.shape, U32)
        top[...] = jnp.full(top.shape, jnp.iinfo(jnp.int32).min, jnp.int32)
        for cp in small:
            cp.wait()
        wr = jnp.broadcast_to(wr_ref[...].astype(F32).reshape(1, D), (M, D))
        for k in range(NT):
            mod[6 * NT + k] = wr[:, k * 128:(k + 1) * 128]
        cv = c_ref[...].astype(F32)
        sc = _rb(cv * _rb(jax.nn.sigmoid(cv)))
        sc_s[...] = jnp.broadcast_to(sc, (M, D)).astype(BF16)
        for k in range(NT):
            cb_s[k * 128:(k + 1) * 128, :] = jnp.broadcast_to(
                sc[:, k * 128:(k + 1) * 128], (128, 128)).T
        mb = mem0_ref[...]
        for k in range(NT):
            lhs[0, k, XR // 2:, :] = _as_u32(mb[:, k * 128:(k + 1) * 128])

        def zero_body(i, c):
            wo_raw[NT, pl.ds(pl.multiple_of(i * 32, 32), 32), :] = jnp.zeros((32, D), BF16)
            return c

        lax.fori_loop(0, wob // 32, zero_body, 0)
        x_copy(0).wait()

        def ln_body(i, c):
            for u in range(LNU):
                q = i * LNU + u
                x = xbuf[q, XR:, :].astype(F32)
                xc = x - jnp.mean(x, axis=-1, keepdims=True)
                v = xc * _rstd(xc)
                for k in range(NT):
                    nrm[k, pl.ds(pl.multiple_of(q * 8, 8), 8), :] = v[:, k * 128:(k + 1) * 128]
            return c

        lax.fori_loop(0, NSEG // LNU, ln_body, 0)

        def mod_body(k, c):
            pltpu.make_async_copy(wmod_s.at[k], wmod_s.at[k], sem.at[S_MOD + k]).wait()
            mod_pair(k)
            for r in range(0, R0, FB):
                fill(ha, 0, k, r)
            return c

        lax.fori_loop(0, 2, mod_body, 0)

        def hop1(g):
            chunk_copy(0, 0, g, 0, S_C0 + g).wait()

            def body(i, c):
                d0 = pl.multiple_of(i * 128, 128)
                v = stage[0, g, pl.ds(d0, 128)].reshape(128 * CH, 128)
                t0 = pl.multiple_of((g * KQ + d0) * (CH // 2), 512)
                tmp[pl.ds(t0, 128 * CH // 2), :] = _as_u32(v)
                return c

            lax.fori_loop(0, KQ // 128, body, 0)

        def hop2(c, g, j):
            src = tmp.at[pl.ds(pl.multiple_of(g * (KQ * CH // 2), 512), KQ * CH // 2 + 8)]
            for d0 in range(0, KQ, RB2):
                relayout2(c, g * CH + 2 * j, d0 * CH // 2 + j, d0, src=src)

        def bulk(units, jobs):
            due = {}
            t0 = 0
            for n, (hq, c, h0_, pi, first, r0, nrow) in enumerate(units):
                nb = nrow // BLK
                parts = []
                for u in range(nb):
                    part = hq[0, (r0 + u * BLK) // 2:(r0 + (u + 1) * BLK) // 2, :]
                    for z in due.pop(t0 + u, ()):
                        part = jnp.concatenate([part[0:8] | z, part[8:]], axis=0)
                    parts.append(part)
                hv = jnp.concatenate([_as_bf16(jnp.concatenate(parts, axis=0)),
                                      _as_bf16(hq[1, r0 // 2:(r0 + nrow) // 2, :])], axis=1)
                w = jnp.concatenate([_as_bf16(wqkv[c, h0_]), _as_bf16(wqkv[c, h0_ + 1])], axis=1)
                y = _dot(hv, w)
                segs = slice(r0 // M, (r0 + nrow) // M)
                for a in range(2):
                    old = jnp.where(first, 0.0, pre[pi, segs, a * M:(a + 1) * M, :])
                    pre[pi, segs, a * M:(a + 1) * M, :] = (
                        y[:, a * DH:(a + 1) * DH].reshape(nrow // M, M, DH) + old)
                for u in range(nb):
                    for job in jobs.get(t0 + u, ()):
                        res = job(zero_after(y[u * BLK:u * BLK + 8, 0:128]))
                        if res is not None:
                            due.setdefault(max(t0 + u + JOB_SPAN, t0 + nb), []).append(
                                zero_after(res))
                t0 += nb
            assert not due

        GP = CH // 2
        WO0 = NCHUNK - 1 - NT
        LN0 = 4
        SPI = -(-NSEG // (NCHUNK - 1 - LN0))

        def rot_body(i, c):
            slot = (i + 1) & (NSLOT - 1)
            pltpu.make_async_copy(stage.at[slot], stage.at[slot], sem.at[S_ST + slot]).wait()
            km = 2 * jnp.minimum(i, 3)

            @pl.when(jnp.logical_and(i >= 1, i <= 3))
            def _():
                wq = wmod_s.at[pl.ds(km, 2)]
                pltpu.make_async_copy(wq, wq, sem.at[S_MOD + km]).wait()

            @pl.when(i == LN0)
            def _():
                x_copy(1).wait()

            @pl.when(i >= WO0)
            def _():
                wo_copy(i - WO0).wait()

            nxt = i + NSLOT
            qn = (nxt * 43) >> 7
            for mat in range(3):
                @pl.when(jnp.logical_and(nxt < NCHUNK, nxt - 3 * qn == mat))
                def _():
                    for g in range(4):
                        chunk_copy(mat, qn * KQ, g, nxt & (NSLOT - 1),
                                   S_ST + (nxt & (NSLOT - 1))).start()

            @pl.when(i < NT)
            def _():
                wo_copy(i).start()

            @pl.when(i == 0)
            def _():
                x_copy(1).start()

            q0 = (i * 43) >> 7
            q1 = ((i + 1) * 43) >> 7
            pa = (i - 3 * q0) * NP + NP - GP
            units = ([(ha, i, H - CH + 2 * n, pa + n, q0 == 0, 0, R0) for n in range(GP)]
                     + [(hb, i + 1, 2 * n, (i + 1 - 3 * q1) * NP + n, q1 == 0, 0, R0)
                        for n in range(NP - GP)])
            jw = jnp.where(i >= WO0, i - WO0, NT)

            def wo_job(b, z):
                v = wo_raw[jw, b * 16:(b + 1) * 16, :]
                rows = pl.ds(pl.multiple_of(jw * (wob // 2) + b * 8, 8), 8)
                for j in range(NT):
                    wo_s[j, rows, :] = _as_u32(v[:, j * 128:(j + 1) * 128]) | z

            lst = {}

            def ln_job(b, ph, z):
                r = (b % 3) * 8
                seg = (i - LN0) * SPI + b // 3
                live = jnp.logical_and(i >= LN0, seg < NSEG)
                src = jnp.where(live, seg, 0) + (i >> (10 + ph))
                x = xbuf[src, pl.ds(pl.multiple_of(jnp.where(live, r, XR), 8), 8), :].astype(F32)
                zf = pltpu.bitcast(z, F32)
                if ph == 0:
                    xm = jnp.concatenate([x[:, :128] + zf, x[:, 128:]], axis=1)
                    mu = jnp.mean(xm, axis=-1, keepdims=True)
                    lst[2 * b] = jnp.broadcast_to(mu, (8, 128))
                    return None
                xc = x - jnp.concatenate([lst[2 * b] + zf] * NT, axis=1)
                if ph == 1:
                    lst[2 * b + 1] = jnp.broadcast_to(_rstd(xc), (8, 128))
                    return None
                inv = jnp.concatenate([lst[2 * b + 1]] * NT, axis=1)
                hv = (xc * inv * modv(1) + modv(0)).astype(BF16)
                u = [_as_u32(hv[:, k * 128:(k + 1) * 128]) for k in range(NT)]
                dst = jnp.where(live, seg, NSEG)
                for k in range(NT):
                    hs[dst, k, r // 2:r // 2 + 4, :] = u[k]
                res = jnp.concatenate(u[0:2], axis=0)
                for k in range(2, NT, 2):
                    res = res | jnp.concatenate(u[k:k + 2], axis=0)
                return res

            def r1_job(g, d0, z):
                relayout1(stage[slot, g, d0:d0 + RB], (g * KQ + d0) * CH // 2, z)

            def copy_job(t, r, z):
                ha[t, r:r + 32, :] = or_tile(hb[t, r:r + 32, :], z)

            P = functools.partial
            upb = R0 // BLK
            nr = NP * upb
            jobs = {}
            for g in range(4):
                lo, mid, hi = (x * upb // 4 for x in R_AT[g])
                _spread(jobs, [P(r1_job, g, d0) for d0 in range(0, KQ, RB)], lo, mid)
                _spread(jobs, [P(relayout2, i + 1, g * CH + 2 * j, (g * KQ + d0) * CH // 2 + j, d0)
                               for j in range(CH // 2) for d0 in range(0, KQ, RB2)], mid, hi)
            oz = i >> 10
            _spread(jobs, [P(fill, hb, q1, t + oz, r) for r in range(0, R0, FB) for t in range(2)],
                    F_AT[0] * upb // 4, F_AT[1] * upb // 4)
            _spread(jobs, [P(copy_job, t, r) for t in range(2) for r in range(0, R0 // 2, 32)],
                    2 * GP * upb, nr - upb)
            for ph in range(3):
                off = LN_PH[ph] - LN_PH[2]
                _spread(jobs, [P(ln_job, b, ph) for b in range(3 * SPI)],
                        L_AT * upb // 4 + LN_PH[ph], nr - max(upb, JOB_SPAN) + off)
            _spread(jobs, [P(wo_job, b) for b in range(wob // 16)], GP * upb, nr - upb)
            gv = {}

            def gv_job(d0, n, z):
                w = wmod_s[pl.ds(km, 2), :, d0:d0 + n, :].reshape(4, n, 128)
                acc = gv.get("acc")
                if z is not None:
                    zf = pltpu.bitcast(z, F32)[None]
                    acc = jnp.broadcast_to(zf, (4, 8, 128)) if acc is None else acc + zf
                gv["acc"] = gemv_part(w, d0, acc)
                if z is not None:
                    au = pltpu.bitcast(gv["acc"], U32)
                    return au[0] | au[1] | au[2] | au[3]

            _spread(jobs, [P(gv_job, d0, GVR) for d0 in range(0, D - GV_FREE, GVR)],
                    GV_AT[0] * upb // 4, min(GV_AT[1] * upb // 4, nr - JOB_SPAN))
            bulk(units, jobs)
            if GV_FREE:
                gv_job(D - GV_FREE, GV_FREE, None)
            gemv_finish(gv["acc"], [km, NT + km, km + 1, NT + km + 1])
            return c

        def outer(k, c):
            last = k == 4

            @pl.when(k < 4)
            def _():
                hop1(k)

            @pl.when(k != 3)
            def _():
                g = jnp.minimum(k, 3)
                cc = jnp.where(last, NCHUNK - 1, 0)
                for j in range(GP):
                    hop2(cc, g, j)
                bulk([(ha, cc, g * CH + 2 * n, jnp.where(last, 2 * NP, 0) + g * GP + n, k < 4,
                       0, R0) for n in range(GP)], {})

            @pl.when(k == 3)
            def _():
                for j in range(GP):
                    hop2(0, 3, j)
                lax.fori_loop(0, NCHUNK - 1, rot_body, 0)
                for it in range(2):
                    for u in range(mt):
                        wm_copy(it, u).start()

            return c

        lax.fori_loop(0, 5, outer, 0)

    pl.run_scoped(
        prologue,
        pltpu.VMEM((NSLOT, H // CH, KQ, CH, 128), BF16),
        pltpu.VMEM((NT + 1, H * DH // NT, D), BF16),
        pltpu.VMEM((NT, 2, D, 128), BF16),
        pltpu.VMEM((NT, R0, 128), F32),
        pltpu.VMEM((2, R0 // 2, 128), U32),
        pltpu.VMEM((2, R0 // 2, 128), U32),
        pltpu.VMEM((D * CH // 2 + 32, 128), U32),
        pltpu.VMEM((M, D), BF16),
        pltpu.VMEM((D,), BF16),
        pltpu.VMEM((1, D), BF16),
        pltpu.SemaphoreType.DMA((7 + NSLOT + 2 * NT,)),
    )

    def main(wg_s, wu_s, wd_s, ybuf, stat, outs, sem_f):
        def load_x_rows(slot, seg):
            for k in range(NT):
                lhs[slot, k, 0:XR // 2, :] = hs[seg, k]

        def resid(seg, r, z=None):
            rows = pl.ds(r, 8)
            t = modv(2) * ybuf[seg, rows, :].astype(F32)
            if z is not None:
                t = t + jnp.concatenate([pltpu.bitcast(z, F32)] * NT, axis=1)
            return _rb(xbuf[seg, rows, :].astype(F32) + t)

        def wide(v):
            return jnp.concatenate([v] * NT, axis=1)

        def make_key(v, row0):
            b = pltpu.bitcast(jnp.where(v != v, -jnp.inf, v + 0.0), jnp.int32)
            low = (S - 1 - row0) - lax.broadcasted_iota(jnp.int32, (8, 128), 0)
            return (b ^ ((b >> 31) & 0x7FFF0000)) | low

        def score_dot(xc, mu, seg, rows):
            mb = _rb(mu)
            stat[0, seg, rows, :] = mb
            return jnp.sum(xc * modv(7), axis=-1, keepdims=True) + (mu - mb) * mod[8 * NT + 1]

        def post(st, ph, seg, r, z):
            zf = pltpu.bitcast(z, F32)
            if ph == 0:
                st["x1"] = resid(seg, r, z)
                st["mu"] = jnp.broadcast_to(jnp.mean(st["x1"], axis=-1, keepdims=True), (8, 128))
                return None
            if ph == 1:
                mu = st["mu"] + zf
                xc = st["xc"] = st["x1"] - wide(mu)
                st["var"] = jnp.mean(xc * xc, axis=-1, keepdims=True)
                st["dot"] = score_dot(xc, mu, seg, pl.ds(r, 8))
                return None
            inv = _inv_std(st["var"]) + zf
            stat[1, seg, pl.ds(r, 8), :] = inv
            v = _rb(inv * st["dot"] + mod[8 * NT])
            key = make_key(v, seg * SEG + r)
            m1, m2 = top[0:8, :], top[8:16, :]
            top[8:16, :] = jnp.maximum(m2, jnp.minimum(m1, key))
            top[0:8, :] = jnp.maximum(m1, key)
            o = st["x1"] + modv(5) * (st["xc"] * wide(inv) * modv(4) + modv(3))
            outs[seg, pl.ds(r, 8), :] = o.astype(BF16)
            res = pltpu.bitcast(v, U32)
            for k in range(NT):
                res = res | pltpu.bitcast(o[:, k * 128:(k + 1) * 128], U32)
            return res

        def redo(seg, r):
            x1 = resid(seg, r)
            d = _rb(x1 - wide(stat[0, seg, pl.ds(r, 8), :]))
            n = _rb(d * wide(stat[1, seg, pl.ds(r, 8), :]))
            return x1, _rb(_rb(n * modv(4)) + modv(3))

        def out_copy(g0, ng, r, n, k=0):
            return pltpu.make_async_copy(outs.at[pl.ds(g0, ng), pl.ds(r, n), :],
                                         out_hbm.at[pl.ds(g0, ng), pl.ds(r, n), :], sem_out.at[k])

        late = ((wg_hbm, wg_s, FF // 128), (wu_hbm, wu_s, FF // 128), (wd_hbm, wd_s, NT))

        def col_copy(k, j):
            return pltpu.make_async_copy(
                late[k][0].at[:, pl.ds(pl.multiple_of(j * 128, 128), 128)], late[k][1].at[j],
                sem_f.at[k])

        load_x_rows(0, 0)

        def step(it, cur, state):
            s = it * UNROLL + cur
            nxt = (cur + 1) % UNROLL

            def pay(t, cost):
                now, due = state["now"], state["due"]
                for z in [z for (d, z) in due if d <= now]:
                    t = jnp.concatenate([t[0:8] | z, t[8:]], axis=0)
                state["due"] = [(d, z) for (d, z) in due if d > now]
                state["now"] = now + cost
                return t

            def release(y):
                now = state["now"]
                pend, state["pend"] = state["pend"], [e for e in state["pend"] if e[0] > now]
                for (d, f) in pend:
                    if d <= now:
                        f(zero_after(y[0:8]))

            def lv(k0, k1):
                ts = [lhs[cur, k] for k in range(k0, k1)]
                ts[0] = pay(ts[0], (k1 - k0) / NT)
                return jnp.concatenate([_as_bf16(t) for t in ts], axis=1)

            def wmat(mat, h, q0, q1):
                return _as_bf16(jnp.concatenate([wqkv[3 * q + mat, h] for q in range(q0, q1)],
                                                axis=0))

            def qkv(p, split=False):
                part = {}
                if split:
                    for mat in range(3):
                        for a in range(2):
                            part[mat, a] = _dot(lv(0, NT // 2), wmat(mat, 2 * p + a, 0, 2))
                for mat in range(3):
                    for a in range(2):
                        hm = mat * H + 2 * p + a
                        if split:
                            y = _dot(lv(NT // 2, NT), wmat(mat, 2 * p + a, 2, 4)) + part[mat, a]
                        else:
                            y = _dot(lv(0, NT), wmat(mat, 2 * p + a, 0, 4))
                        cur_s[hm] = y.astype(BF16)
                        release(y)

            def gather(mat, p):
                hm = mat * H + 2 * p
                return jnp.concatenate(
                    [cur_s[hm], cur_s[hm + 1], pre[mat * NP + p, s].astype(BF16)], axis=0)

            probs = {}

            def scores(p):
                st = lax.dot_general(gather(1, p), gather(0, p), (((1,), (1,)), ((), ())),
                                     preferred_element_type=F32)
                lane = lax.broadcasted_iota(jnp.int32, (1, PR), 1)
                is_a = jnp.logical_or(lane < SEG,
                                      jnp.logical_and(lane >= 2 * SEG, lane < 2 * SEG + M))
                ka = jnp.concatenate([st[0:SEG], st[2 * SEG:2 * SEG + M]], axis=0)
                kb = jnp.concatenate([st[SEG:2 * SEG], st[2 * SEG + M:]], axis=0)
                t = jnp.where(is_a, ka, kb) * (SCALE * LOG2E)
                ts_s[p + (it >> 10)] = jnp.where(mk[0:SEG + M, :] == 0.0, t, NEG_MASK * LOG2E)

                def softmax(z):
                    zf = pltpu.bitcast(z, F32)[:, 0:PR]
                    t = (ts_s[p].reshape(-1, 8, PR) + zf).reshape(SEG + M, PR)
                    e = jnp.exp2(t - jnp.max(t, axis=0, keepdims=True))
                    e = e * _recip(jnp.sum(e, axis=0, keepdims=True))
                    pa = jnp.where(is_a, e, 0.0)
                    pb = jnp.where(is_a, 0.0, e)
                    probs[p] = jnp.concatenate(
                        [pa[0:SEG], pb[0:SEG], pa[SEG:], pb[SEG:]], axis=0).astype(BF16)

                state["pend"].append((state["now"] + REL_S + (p % PG) * REL_STAG, softmax))

            def pv(p):
                o = lax.dot_general(probs.pop(p), gather(2, p), (((0,), (0,)), ((), ())),
                                    preferred_element_type=F32).astype(BF16)
                for a in range(2):
                    h = 2 * p + a
                    olhs[h] = _as_u32(o[a * SEG:(a + 1) * SEG])
                    odef[h, it, cur * 4:(cur + 1) * 4, :] = _as_u32(
                        o[2 * SEG + a * M:2 * SEG + (a + 1) * M])

            acc = [None] * NT

            def oproj(j, pairs):
                ts = [olhs[2 * p + a] for p in pairs for a in range(2)]
                ts[0] = pay(ts[0], len(pairs) / 4)
                ov = jnp.concatenate([_as_bf16(t) for t in ts], axis=1)
                w = wo_s[j, pairs[0] * DH:(pairs[-1] + 1) * DH, :]
                y = _dot(ov, _as_bf16(w))
                acc[j] = y if acc[j] is None else y + acc[j]
                release(acc[j])

            def fin(j):
                yb = acc[j].astype(BF16)
                ybuf[s, 0:XR, j * 128:(j + 1) * 128] = yb[0:XR]
                lhs[nxt, j, XR // 2:, :] = _as_u32(yb[XR:])

            def gemv():
                d0 = state["d0"]
                state["acc"] = gemv_part(wm_s[it & 3, :, d0:d0 + GR, :], d0, state["acc"])
                state["d0"] = d0 + GR
                au = pltpu.bitcast(state["acc"], U32)
                z = functools.reduce(lambda a, b: a | b, [au[u] for u in range(mt)])
                state["due"].append((state["now"] + G_LAG, zero_after(z)))

            load_x_rows(nxt, jnp.minimum(s + 1, NSEG - 1))
            ops = dict(Q=qkv, S=scores, P=pv, O=oproj, F=fin, G=gemv)
            for op in _schedule():
                ops[op[0]](*op[1:])

        def steps(it, carry):
            pltpu.make_async_copy(wm_s.at[it & 3], wm_s.at[it & 3], sem_m.at[it & 3]).wait()

            @pl.when(it + 2 < NSEG // UNROLL)
            def _():
                for u in range(mt):
                    wm_copy(it + 2, u).start()

            for u in range(UNROLL // 2):
                t = it * (UNROLL // 2) + u
                for k in range(3):
                    @pl.when(t < late[k][2])
                    def _():
                        col_copy(k, t).start()

            state = dict(now=0, due=[], pend=[], d0=0, acc=None)
            for u in range(UNROLL):
                step(it, u, state)
            acc = state["acc"]
            for d0 in range(state["d0"], D, 64):
                acc = gemv_part(wm_s[it & 3, :, d0:min(d0 + 64, D), :], d0, acc)
            gemv_finish(acc, [2 * NT + it * mt + u for u in range(mt)])
            return carry

        lax.fori_loop(0, NSEG // UNROLL, steps, 0)
        for k in range(3):
            for j in range(late[k][2]):
                col_copy(k, j).wait()

        ntail = EC // M
        ppi = (S // 8 - ntail) // NEC
        gpi = ppi // (XR // 8)
        nblk = EC // (UNROLL * M)

        def ep_body(i, c):
            @pl.when(i > 0)
            def _():
                out_copy((i - 1) * gpi, gpi, 0, XR).start()

            for k in range(NT):
                mod[7 * NT + k] = mod[4 * NT + k] * mod[6 * NT + k]
            mod[8 * NT] = jnp.broadcast_to(
                jnp.sum(modv(3) * modv(6), axis=-1, keepdims=True), (M, 128))
            mod[8 * NT + 1] = jnp.broadcast_to(
                jnp.sum(modv(7), axis=-1, keepdims=True), (M, 128))

            jobs = {}
            for ph in range(3):
                _spread(jobs, [(u, ph) for u in range(ppi)], E_PH[ph],
                        (NT * H // EKH - E_SPAN) * E_REL - E_PH[2] + E_PH[ph])
            sts = [{} for _ in range(ppi)]
            due = {}
            n = 0
            for j in range(NT):
                for h0_ in range(0, H, EKH):
                    ts = [odef[h, pl.ds(i * nblk, nblk)].reshape(EC // 2, DH)
                          for h in range(h0_, h0_ + EKH)]
                    for z in due.pop(n, ()):
                        ts[0] = jnp.concatenate([ts[0][0:8] | z, ts[0][8:]], axis=0)
                    w = wo_s[j, h0_ * DH // 2:(h0_ + EKH) * DH // 2, :]
                    yp = _dot(jnp.concatenate([_as_bf16(t) for t in ts], axis=1), _as_bf16(w))
                    y = yp if h0_ == 0 else yp + y
                    if h0_ + EKH == H:
                        ybuf[pl.ds(i * ntail, ntail), XR:, j * 128:(j + 1) * 128] = (
                            y.reshape(ntail, M, 128).astype(BF16))
                    for q in range(E_REL):
                        for (u, ph) in jobs.get(n * E_REL + q, ()):
                            t = i * ppi + u
                            early = t < NSEG * (XR // 8)
                            seg = jnp.where(early, t // (XR // 8), t - NSEG * (XR // 8))
                            row = pl.multiple_of(jnp.where(early, (t % (XR // 8)) * 8, XR), 8)
                            zr = q * (EC // E_REL)
                            res = post(sts[u], ph, seg, row, zero_after(y[zr:zr + 8]))
                            if res is not None:
                                due.setdefault(n + E_SPAN, []).append(zero_after(res))
                    n += 1
            return c

        lax.fori_loop(0, NEC, ep_body, 0)
        done = (NEC - 1) * gpi
        tail = NSEG - ntail
        out_copy(done, NSEG - done, 0, XR).start()
        out_copy(0, tail, XR, M).start()
        x1s = [resid(g, XR) for g in range(tail, NSEG)]
        mus = [jnp.mean(x1, axis=-1, keepdims=True) for x1 in x1s]
        pairs = [(top[0:8, :], top[8:16, :])]
        lowest = jnp.full((8, 128), jnp.iinfo(jnp.int32).min, jnp.int32)
        for g in range(tail, NSEG):
            xc = x1s[g - tail] - mus[g - tail]
            inv = _inv_std(jnp.mean(xc * xc, axis=-1, keepdims=True))
            stat[1, g, XR:, :] = jnp.broadcast_to(inv, (8, 128))
            dot = score_dot(xc, jnp.broadcast_to(mus[g - tail], (8, 128)), g, pl.ds(XR, 8))
            v = _rb(inv * dot + mod[8 * NT])
            pairs.append((make_key(v, g * SEG + XR), lowest))
        while len(pairs) > 1:
            (a1, a2), (c1, c2) = pairs.pop(0), pairs.pop(0)
            pairs.append((jnp.maximum(a1, c1),
                          jnp.maximum(jnp.minimum(a1, c1), jnp.maximum(a2, c2))))

        tk = jnp.concatenate(pairs[0], axis=0)[:, 0:1]
        k1 = jnp.max(tk[0:8], axis=0, keepdims=True)
        k2 = jnp.max(jnp.where(tk == k1, jnp.iinfo(jnp.int32).min, tk), axis=0, keepdims=True)
        i1 = (S - 1) - (k1[0, 0] & (S - 1))
        i2 = (S - 1) - (k2[0, 0] & (S - 1))
        g1, g2 = i1 >> 5, i2 >> 5
        b1 = pl.multiple_of(i1 & 24, 8)
        b2 = pl.multiple_of(i2 & 24, 8)

        def tail_out(n, z):
            g, k0 = tail + n // (NT // TW), (n % (NT // TW)) * TW
            zf = pltpu.bitcast(z, F32)
            for k in range(k0, k0 + TW, 2):
                cols = slice(k * 128, (k + 2) * 128)
                m = lambda j: jnp.concatenate([mod[j * NT + k], mod[j * NT + k + 1]], axis=1)
                two = lambda v: jnp.concatenate([v, v], axis=1)
                x1_ = (xbuf[g, XR:, cols].astype(F32)
                       + (m(2) * ybuf[g, XR:, cols].astype(F32) + two(zf)))
                h_ = (x1_ - two(stat[0, g, XR:, :])) * two(stat[1, g, XR:, :]) * m(4) + m(3)
                outs[g, XR:, cols] = (x1_ + m(5) * h_).astype(BF16)

        xa, ha_ = redo(g1, b1)
        xb_, hb_ = redo(g2, b2)
        x1 = jnp.concatenate([xa, xb_], axis=0)
        h2 = jnp.concatenate([ha_, hb_], axis=0)
        h2b = h2.astype(BF16)
        row = lax.broadcasted_iota(jnp.int32, (16, 1), 0)
        grow = jnp.where(row < 8, g1 * SEG + b1 + row, g2 * SEG + b2 + row - 8)
        ks = jnp.where(grow == i1, k1, k2)
        rsel = pltpu.bitcast((ks ^ ((ks >> 31) & 0x7FFF0000)) & -65536, F32)
        acts = []
        jobs = {}
        _spread(jobs, list(range(ntail * NT // TW)), 0, T_END)
        for j in range(FF // 128):
            gt = _rb(_dot(h2b, wg_s[j]))
            for n in jobs.get(2 * j, ()):
                tail_out(n, zero_after(gt[0:8]))
            gt = _rb(gt * _rb(jax.nn.sigmoid(gt)))
            ut = _rb(_dot(h2b, wu_s[j]))
            for n in jobs.get(2 * j + 1, ()):
                tail_out(n, zero_after(ut[0:8]))
            acts.append((gt * ut).astype(BF16))
        out_copy(tail, NSEG - tail, XR, M).start()
        act = jnp.concatenate(acts, axis=1)
        y = _rb(jnp.concatenate([_dot(act, wd_s[j]) for j in range(NT)], axis=1))
        y = _rb(y * _rb(jax.nn.sigmoid(rsel)))
        sel = jnp.logical_or(grow == i1, grow == i2)
        gb2 = jnp.concatenate([modv(5)] * 2, axis=0)
        fixed = (x1 + gb2 * (h2 + jnp.where(sel, y, 0.0))).astype(BF16)

        out_copy(0, NSEG, 0, SEG).wait()
        outs[g1, pl.ds(b1, 8), :] = fixed[0:8]
        outs[g2, pl.ds(b2, 8), :] = fixed[8:16]
        out_copy(g1, 1, b1, 8, 0).start()

        @pl.when((i1 >> 3) != (i2 >> 3))
        def _():
            out_copy(g2, 1, b2, 8, 1).start()
            out_copy(g2, 1, b2, 8, 1).wait()

        out_copy(g1, 1, b1, 8, 0).wait()

    pl.run_scoped(
        main,
        pltpu.VMEM((FF // 128, D, 128), BF16),
        pltpu.VMEM((FF // 128, D, 128), BF16),
        pltpu.VMEM((NT, FF, 128), BF16),
        pltpu.VMEM((NSEG, SEG, D), BF16),
        pltpu.VMEM((2, NSEG, SEG, 128), F32),
        pltpu.VMEM((NSEG, SEG, D), BF16),
        pltpu.SemaphoreType.DMA((3,)),
    )


def _entry(*refs):
    pl.run_scoped(
        functools.partial(_kernel, *refs),
        pltpu.VMEM((NCHUNK, H, KQ // 2, DH), U32),
        pltpu.VMEM((NSEG + 1, NT, XR // 2, 128), U32),
        pltpu.VMEM((NT, (H * DH + H * DH // NT) // 2, 128), U32),
        pltpu.VMEM((3 * NP, NSEG, 2 * M, DH), F32),
        pltpu.VMEM((3 * H, SEG, DH), BF16),
        pltpu.VMEM((H, SEG // 2, DH), U32),
        pltpu.VMEM((H, NSEG // UNROLL, UNROLL * M // 2, DH), U32),
        pltpu.VMEM((NSEG, SEG, D), BF16),
        pltpu.VMEM((UNROLL, NT, SEG // 2, 128), U32),
        pltpu.VMEM((4, 4 * NT * UNROLL // NSEG, D, 128), BF16),
        pltpu.VMEM((8 * NT + 4, M, 128), F32),
        pltpu.VMEM((64, PR), F32),
        pltpu.VMEM((32, 128), jnp.int32),
        pltpu.VMEM((M, D), BF16),
        pltpu.VMEM((D, 128), F32),
        pltpu.VMEM((NP, SEG + M, PR), F32),
        pltpu.VMEM((8 + PAD, 128), U32),
        pltpu.SemaphoreType.DMA((4,)),
        pltpu.SemaphoreType.DMA((2,)),
    )


@functools.partial(jax.jit, static_argnames=("A_seg_len",))
def pallas_adaLN_cond__memory_aug_recurrent_mem_tr__moe_arch_mod__prompt_kernel(
    A_x: jax.Array,
    A_mem0: jax.Array,
    A_Wq: jax.Array,
    A_Wk: jax.Array,
    A_Wv: jax.Array,
    A_Wo: jax.Array,
    A_seg_len,
    B_x: jax.Array,
    B_w_r: jax.Array,
    B_w_gate: jax.Array,
    B_w_up: jax.Array,
    B_w_down: jax.Array,
    c: jax.Array,
    w_mod: jax.Array,
):
    assert A_seg_len == SEG and A_x.shape == (1, S, D)
    del B_x
    hbm = pl.BlockSpec(memory_space=pl.ANY)
    out = pl.pallas_call(
        _entry,
        out_shape=jax.ShapeDtypeStruct((NSEG, SEG, D), BF16),
        in_specs=[hbm] * 12,
        out_specs=hbm,
        compiler_params=pltpu.CompilerParams(vmem_limit_bytes=120 * 1024 * 1024,
                                             disable_bounds_checks=True),
    )(A_x.reshape(NSEG, SEG, D), A_mem0.reshape(M, D), A_Wq, A_Wk, A_Wv, A_Wo.reshape(H * DH, D),
      B_w_r, B_w_gate, B_w_up, B_w_down, c, w_mod)
    return out.reshape(1, S, D)
```

```python
import functools

import jax
import jax.numpy as jnp
from jax import lax
import jax.experimental.pallas as pl
import jax.experimental.pallas.tpu as pltpu

F32 = jnp.float32
BF16 = jnp.bfloat16
U32 = jnp.uint32

D = 1024
S = 2048
H = 32
DH = 128
M = 8
SEG = 32
NSEG = S // SEG
FF = 3584
NT = D // 128
XR = SEG - M
R0 = M * NSEG
CH = 8
KQ = D // 4
NCHUNK = 3 * D // KQ
NSLOT = 4
PR = 2 * SEG + 2 * M
NP = H // 2
EC = 128
NEC = R0 // EC
LOG2E = 1.4426950408889634
EPS = 1e-5
SCALE = DH ** -0.5
NEG_MASK = -1000000000.0

UNROLL = 4
PG = 4
LAG_S = 1
LAG_P = 4
O_PARTS = (0, 8, 12)
O_TH = (256, 256, 256, 1280)
REL_S = 3
REL_STAG = 2
G_AT = (0, 1, 2, 3, 7, 11)
GR = 32
G_LAG = 3
BLK = 32
JOB_SPAN = 40
RB = 16
RB2 = 32
FB = 32
GVR = 32
GV_FREE = 64
R_AT = ((0, 6, 16), (14, 22, 30), (30, 38, 46), (44, 52, 60))
F_AT = (0, 13)
L_AT = 6
GV_AT = (16, 56)
LNU = 16
LN_PH = (0, 10, 20)
EKH = 4
E_SPAN = 20
EBLK = (64, 64)
E_PH = (0, 8, 16)
TW = 4
T_END = 32
PAD = 24


def _schedule():
    groups = [list(range(g, g + PG)) for g in range(0, NP, PG)]
    at = {}
    for g, grp in enumerate(groups):
        at.setdefault(grp[-1] + LAG_P, []).extend(("P", q) for q in grp)
    for g, grp in enumerate(groups):
        at.setdefault(grp[-1] + LAG_S, []).extend(("S", q) for q in grp)
    ops = []
    for p in range(NP):
        ops.append(("Q", p, p == 0))
        if p in G_AT:
            ops.append(("G",))
        ops.extend(at.pop(p, []))
    bounds = list(O_PARTS) + [NP]
    t = NP
    done = 0
    for n in range(len(O_PARTS)):
        part = list(range(bounds[n], bounds[n + 1]))
        assert all(("P", q) in ops for q in part), (n, ops)
        for j in range(NT):
            ops.append(("O", j, part))
            if n == len(O_PARTS) - 1:
                ops.append(("F", j))
            done += len(part) * 16
            while t - NP < len(O_TH) and done >= O_TH[t - NP]:
                ops.extend(at.pop(t, []))
                t += 1
    assert not at
    return ops


def _rb(x):
    return x.astype(BF16).astype(F32)


def _recip(x):
    r = pl.reciprocal(x, approx=True)
    return r * (2.0 - x * r)


def _inv_std(var):
    v = _rb(_rb(var) + EPS)
    return _recip(_rb(v * lax.rsqrt(v)))


def _rstd(xc):
    return lax.rsqrt(jnp.mean(xc * xc, axis=-1, keepdims=True) + EPS)


def _dot(a, b):
    return jnp.dot(a, b, preferred_element_type=F32)


def _as_bf16(u):
    return pltpu.bitcast(u, BF16)


def _as_u32(b):
    return pltpu.bitcast(b, U32)


def _spread(jobs, fns, lo, hi):
    for n, fn in enumerate(fns):
        jobs.setdefault(lo + n * (hi - lo) // len(fns), []).append(fn)


def _kernel(x_hbm, mem0_hbm, wq_hbm, wk_hbm, wv_hbm, wo_hbm, wr_hbm, wg_hbm, wu_hbm, wd_hbm,
            c_hbm, wmod_hbm, out_hbm,
            wqkv, hs, wo_s, pre, cur_s, olhs, odef, xbuf, lhs, wm_s, mod, mk,
            top, sc_s, cb_s, ts_s, zero_s, sem_m, sem_out):
    mt = 4 * NT * UNROLL // NSEG

    def modv(j):
        return jnp.concatenate([mod[j * NT + k] for k in range(NT)], axis=1)

    def mod_store(v, t):
        v = _rb(v)
        mod[t] = jnp.where(jnp.logical_or((t >> 3) == 1, (t >> 3) == 4), _rb(1.0 + v), v)

    def mod_tile(wm, t):
        mod_store(_dot(sc_s[...], wm), t)

    def gemv_part(w, d0, acc):
        n = w.shape[1]
        p = w.astype(F32) * cb_s[d0:d0 + n, :]
        p = jnp.sum(p.reshape(w.shape[0], n // 8, 8, 128), axis=1)
        return p if acc is None else p + acc

    def gemv_finish(acc, ts):
        for u, t in enumerate(ts):
            mod_store(jnp.broadcast_to(jnp.sum(acc[u], axis=0, keepdims=True), (M, 128)), t)

    def wm_copy(it, u):
        col = pl.multiple_of((2 * NT + it * mt + u) * 128, 128)
        return pltpu.make_async_copy(wmod_hbm.at[:, pl.ds(col, 128)], wm_s.at[it & 3, u],
                                     sem_m.at[it & 3])

    def zero_after(y):
        return (y if y.dtype == U32 else pltpu.bitcast(y, U32)) & zero_s[0:8, :]

    def or_tile(u, z):
        if z is None:
            return u
        return (u.reshape(u.shape[0] // 8, 8, 128) | z).reshape(u.shape)

    def prologue(stage, wo_raw, wmod_s, nrm, ha, hb, tmp, mem0_ref, wr_ref, c_ref, sem):
        w_hbms = (wq_hbm, wk_hbm, wv_hbm)
        wob = H * DH // NT
        S_X, S_C0, S_ST, S_WO, S_MOD, S_SM = 0, 2, 6, 6 + NSLOT, 6 + NSLOT + NT, 6 + NSLOT + 2 * NT

        def x_copy(i):
            lo, n = ((XR, M), (0, XR))[i]
            return pltpu.make_async_copy(x_hbm.at[:, pl.ds(lo, n), :], xbuf.at[:, pl.ds(lo, n), :],
                                         sem.at[S_X + i])

        def mod_copies(k):
            return [pltpu.make_async_copy(wmod_hbm.at[:, pl.ds(v * D + k * 128, 128)],
                                          wmod_s.at[k, v], sem.at[S_MOD + (k if k < 2 else k & 6)])
                    for v in range(2)]

        def chunk_copy(mat, d0, g, slot, k):
            heads = pl.ds(pl.multiple_of(g * CH, CH), CH)
            return pltpu.make_async_copy(w_hbms[mat].at[pl.ds(d0, KQ), heads, :],
                                         stage.at[slot, g], sem.at[k])

        def wo_copy(j):
            return pltpu.make_async_copy(wo_hbm.at[pl.ds(pl.multiple_of(j * wob, wob), wob)],
                                         wo_raw.at[j], sem.at[S_WO + j])

        def relayout1(src, t0, z=None):
            v = src.reshape(RB * CH, 128)
            tmp[t0:t0 + RB * CH // 2, :] = or_tile(_as_u32(v), z)

        def relayout2(c, h0_, t0, d0, z=None, src=tmp):
            w = or_tile(src[pl.ds(t0, RB2, stride=CH // 2), :], z)
            rows = pl.ds(d0 // 2, RB2 // 2)
            wqkv[c, h0_, rows, :] = _as_u32(w.astype(jnp.uint16))
            wqkv[c, h0_ + 1, rows, :] = _as_u32((w >> 16).astype(jnp.uint16))

        def mod_pair(k):
            for v in range(2):
                mod_tile(wmod_s[k, v], v * NT + k)

        def fill(dst, q, t, r, z=None):
            k = 2 * q + t
            sh = mod[k] if z is None else mod[k] + pltpu.bitcast(z, F32)
            v = nrm[k, r:r + FB, :].reshape(FB // 8, 8, 128) * mod[NT + k] + sh
            dst[t, r // 2:(r + FB) // 2, :] = _as_u32(v.reshape(FB, 128).astype(BF16))

        small = [pltpu.make_async_copy(src, dst, sem.at[S_SM])
                 for src, dst in ((c_hbm, c_ref), (mem0_hbm, mem0_ref), (wr_hbm, wr_ref))]
        for cp in small:
            cp.start()
        x_copy(0).start()
        for cp in mod_copies(0) + mod_copies(1):
            cp.start()
        for g in range(4):
            chunk_copy(0, 0, g, 0, S_C0 + g).start()
        for c in range(1, NSLOT):
            for g in range(4):
                chunk_copy(c % 3, (c // 3) * KQ, g, c, S_ST + c).start()
            for cp in mod_copies(2 * c) + mod_copies(2 * c + 1):
                cp.start()

        kk = lax.broadcasted_iota(jnp.int32, (SEG + M, PR), 0)
        qq = lax.broadcasted_iota(jnp.int32, (SEG + M, PR), 1)
        k_mem = jnp.logical_and(kk >= XR, kk < SEG)
        k_pos = jnp.where(kk < SEG, kk, kk - M)
        q_mem = jnp.logical_and(qq < 2 * SEG, qq % SEG >= XR)
        q_pos = jnp.where(qq < 2 * SEG, qq % SEG, XR + qq % M)
        mk[0:SEG + M, :] = jnp.where(q_mem | k_mem | (q_pos >= k_pos), 0.0, 1.0).astype(F32)
        mod[0:2 * NT] = jnp.zeros((2 * NT, M, 128), F32)
        zero_s[...] = jnp.zeros(zero_s.shape, U32)
        top[...] = jnp.full(top.shape, jnp.iinfo(jnp.int32).min, jnp.int32)
        for cp in small:
            cp.wait()
        wr = jnp.broadcast_to(wr_ref[...].astype(F32).reshape(1, D), (M, D))
        for k in range(NT):
            mod[6 * NT + k] = wr[:, k * 128:(k + 1) * 128]
        cv = c_ref[...].astype(F32)
        sc = _rb(cv * _rb(jax.nn.sigmoid(cv)))
        sc_s[...] = jnp.broadcast_to(sc, (M, D)).astype(BF16)
        for k in range(NT):
            cb_s[k * 128:(k + 1) * 128, :] = jnp.broadcast_to(
                sc[:, k * 128:(k + 1) * 128], (128, 128)).T
        mb = mem0_ref[...]
        for k in range(NT):
            lhs[0, k, XR // 2:, :] = _as_u32(mb[:, k * 128:(k + 1) * 128])

        def zero_body(i, c):
            wo_raw[NT, pl.ds(pl.multiple_of(i * 32, 32), 32), :] = jnp.zeros((32, D), BF16)
            return c

        lax.fori_loop(0, wob // 32, zero_body, 0)
        x_copy(0).wait()

        def ln_body(i, c):
            for u in range(LNU):
                q = i * LNU + u
                x = xbuf[q, XR:, :].astype(F32)
                xc = x - jnp.mean(x, axis=-1, keepdims=True)
                v = xc * _rstd(xc)
                for k in range(NT):
                    nrm[k, pl.ds(pl.multiple_of(q * 8, 8), 8), :] = v[:, k * 128:(k + 1) * 128]
            return c

        lax.fori_loop(0, NSEG // LNU, ln_body, 0)

        def mod_body(k, c):
            pltpu.make_async_copy(wmod_s.at[k], wmod_s.at[k], sem.at[S_MOD + k]).wait()
            mod_pair(k)
            for r in range(0, R0, FB):
                fill(ha, 0, k, r)
            return c

        lax.fori_loop(0, 2, mod_body, 0)

        def hop1(g):
            chunk_copy(0, 0, g, 0, S_C0 + g).wait()

            def body(i, c):
                d0 = pl.multiple_of(i * 128, 128)
                v = stage[0, g, pl.ds(d0, 128)].reshape(128 * CH, 128)
                t0 = pl.multiple_of((g * KQ + d0) * (CH // 2), 512)
                tmp[pl.ds(t0, 128 * CH // 2), :] = _as_u32(v)
                return c

            lax.fori_loop(0, KQ // 128, body, 0)

        def hop2(c, g, j):
            src = tmp.at[pl.ds(pl.multiple_of(g * (KQ * CH // 2), 512), KQ * CH // 2 + 8)]
            for d0 in range(0, KQ, RB2):
                relayout2(c, g * CH + 2 * j, d0 * CH // 2 + j, d0, src=src)

        def bulk(units, jobs):
            due = {}
            t0 = 0
            for n, (hq, c, h0_, pi, first, r0, nrow) in enumerate(units):
                nb = nrow // BLK
                parts = []
                for u in range(nb):
                    part = hq[0, (r0 + u * BLK) // 2:(r0 + (u + 1) * BLK) // 2, :]
                    for z in due.pop(t0 + u, ()):
                        part = jnp.concatenate([part[0:8] | z, part[8:]], axis=0)
                    parts.append(part)
                hv = jnp.concatenate([_as_bf16(jnp.concatenate(parts, axis=0)),
                                      _as_bf16(hq[1, r0 // 2:(r0 + nrow) // 2, :])], axis=1)
                w = jnp.concatenate([_as_bf16(wqkv[c, h0_]), _as_bf16(wqkv[c, h0_ + 1])], axis=1)
                y = _dot(hv, w)
                segs = slice(r0 // M, (r0 + nrow) // M)
                for a in range(2):
                    old = jnp.where(first, 0.0, pre[pi, segs, a * M:(a + 1) * M, :])
                    pre[pi, segs, a * M:(a + 1) * M, :] = (
                        y[:, a * DH:(a + 1) * DH].reshape(nrow // M, M, DH) + old)
                for u in range(nb):
                    for job in jobs.get(t0 + u, ()):
                        res = job(zero_after(y[u * BLK:u * BLK + 8, 0:128]))
                        if res is not None:
                            due.setdefault(max(t0 + u + JOB_SPAN, t0 + nb), []).append(
                                zero_after(res))
                t0 += nb
            assert not due

        GP = CH // 2
        WO0 = NCHUNK - 1 - NT
        LN0 = 4
        SPI = -(-NSEG // (NCHUNK - 1 - LN0))

        def rot_body(i, c):
            slot = (i + 1) & (NSLOT - 1)
            pltpu.make_async_copy(stage.at[slot], stage.at[slot], sem.at[S_ST + slot]).wait()
            km = 2 * jnp.minimum(i, 3)

            @pl.when(jnp.logical_and(i >= 1, i <= 3))
            def _():
                wq = wmod_s.at[pl.ds(km, 2)]
                pltpu.make_async_copy(wq, wq, sem.at[S_MOD + km]).wait()

            @pl.when(i == LN0)
            def _():
                x_copy(1).wait()

            @pl.when(i >= WO0)
            def _():
                wo_copy(i - WO0).wait()

            nxt = i + NSLOT
            qn = (nxt * 43) >> 7
            for mat in range(3):
                @pl.when(jnp.logical_and(nxt < NCHUNK, nxt - 3 * qn == mat))
                def _():
                    for g in range(4):
                        chunk_copy(mat, qn * KQ, g, nxt & (NSLOT - 1),
                                   S_ST + (nxt & (NSLOT - 1))).start()

            @pl.when(i < NT)
            def _():
                wo_copy(i).start()

            @pl.when(i == 0)
            def _():
                x_copy(1).start()

            q0 = (i * 43) >> 7
            q1 = ((i + 1) * 43) >> 7
            pa = (i - 3 * q0) * NP + NP - GP
            units = ([(ha, i, H - CH + 2 * n, pa + n, q0 == 0, 0, R0) for n in range(GP)]
                     + [(hb, i + 1, 2 * n, (i + 1 - 3 * q1) * NP + n, q1 == 0, 0, R0)
                        for n in range(NP - GP)])
            jw = jnp.where(i >= WO0, i - WO0, NT)

            def wo_job(b, z):
                v = wo_raw[jw, b * 16:(b + 1) * 16, :]
                rows = pl.ds(pl.multiple_of(jw * (wob // 2) + b * 8, 8), 8)
                for j in range(NT):
                    wo_s[j, rows, :] = _as_u32(v[:, j * 128:(j + 1) * 128]) | z

            lst = {}

            def ln_job(b, ph, z):
                r = (b % 3) * 8
                seg = (i - LN0) * SPI + b // 3
                live = jnp.logical_and(i >= LN0, seg < NSEG)
                src = jnp.where(live, seg, 0) + (i >> (10 + ph))
                x = xbuf[src, pl.ds(pl.multiple_of(jnp.where(live, r, XR), 8), 8), :].astype(F32)
                zf = pltpu.bitcast(z, F32)
                if ph == 0:
                    xm = jnp.concatenate([x[:, :128] + zf, x[:, 128:]], axis=1)
                    mu = jnp.mean(xm, axis=-1, keepdims=True)
                    lst[2 * b] = jnp.broadcast_to(mu, (8, 128))
                    return None
                xc = x - jnp.concatenate([lst[2 * b] + zf] * NT, axis=1)
                if ph == 1:
                    lst[2 * b + 1] = jnp.broadcast_to(_rstd(xc), (8, 128))
                    return None
                inv = jnp.concatenate([lst[2 * b + 1]] * NT, axis=1)
                hv = (xc * inv * modv(1) + modv(0)).astype(BF16)
                u = [_as_u32(hv[:, k * 128:(k + 1) * 128]) for k in range(NT)]
                dst = jnp.where(live, seg, NSEG)
                for k in range(NT):
                    hs[dst, k, r // 2:r // 2 + 4, :] = u[k]
                res = jnp.concatenate(u[0:2], axis=0)
                for k in range(2, NT, 2):
                    res = res | jnp.concatenate(u[k:k + 2], axis=0)
                return res

            def r1_job(g, d0, z):
                relayout1(stage[slot, g, d0:d0 + RB], (g * KQ + d0) * CH // 2, z)

            def copy_job(t, r, z):
                ha[t, r:r + 32, :] = or_tile(hb[t, r:r + 32, :], z)

            P = functools.partial
            upb = R0 // BLK
            nr = NP * upb
            jobs = {}
            for g in range(4):
                lo, mid, hi = (x * upb // 4 for x in R_AT[g])
                _spread(jobs, [P(r1_job, g, d0) for d0 in range(0, KQ, RB)], lo, mid)
                _spread(jobs, [P(relayout2, i + 1, g * CH + 2 * j, (g * KQ + d0) * CH // 2 + j, d0)
                               for j in range(CH // 2) for d0 in range(0, KQ, RB2)], mid, hi)
            oz = i >> 10
            _spread(jobs, [P(fill, hb, q1, t + oz, r) for r in range(0, R0, FB) for t in range(2)],
                    F_AT[0] * upb // 4, F_AT[1] * upb // 4)
            _spread(jobs, [P(copy_job, t, r) for t in range(2) for r in range(0, R0 // 2, 32)],
                    2 * GP * upb, nr - upb)
            for ph in range(3):
                off = LN_PH[ph] - LN_PH[2]
                _spread(jobs, [P(ln_job, b, ph) for b in range(3 * SPI)],
                        L_AT * upb // 4 + LN_PH[ph], nr - max(upb, JOB_SPAN) + off)
            _spread(jobs, [P(wo_job, b) for b in range(wob // 16)], GP * upb, nr - upb)
            gv = {}

            def gv_job(d0, n, z):
                w = wmod_s[pl.ds(km, 2), :, d0:d0 + n, :].reshape(4, n, 128)
                acc = gv.get("acc")
                if z is not None:
                    zf = pltpu.bitcast(z, F32)[None]
                    acc = jnp.broadcast_to(zf, (4, 8, 128)) if acc is None else acc + zf
                gv["acc"] = gemv_part(w, d0, acc)
                if z is not None:
                    au = pltpu.bitcast(gv["acc"], U32)
                    return au[0] | au[1] | au[2] | au[3]

            _spread(jobs, [P(gv_job, d0, GVR) for d0 in range(0, D - GV_FREE, GVR)],
                    GV_AT[0] * upb // 4, min(GV_AT[1] * upb // 4, nr - JOB_SPAN))
            bulk(units, jobs)
            if GV_FREE:
                gv_job(D - GV_FREE, GV_FREE, None)
            gemv_finish(gv["acc"], [km, NT + km, km + 1, NT + km + 1])
            return c

        def outer(k, c):
            last = k == 4

            @pl.when(k < 4)
            def _():
                hop1(k)

            @pl.when(k != 3)
            def _():
                g = jnp.minimum(k, 3)
                cc = jnp.where(last, NCHUNK - 1, 0)
                for j in range(GP):
                    hop2(cc, g, j)
                bulk([(ha, cc, g * CH + 2 * n, jnp.where(last, 2 * NP, 0) + g * GP + n, k < 4,
                       0, R0) for n in range(GP)], {})

            @pl.when(k == 3)
            def _():
                for j in range(GP):
                    hop2(0, 3, j)
                lax.fori_loop(0, NCHUNK - 1, rot_body, 0)
                for it in range(2):
                    for u in range(mt):
                        wm_copy(it, u).start()

            return c

        lax.fori_loop(0, 5, outer, 0)

    pl.run_scoped(
        prologue,
        pltpu.VMEM((NSLOT, H // CH, KQ, CH, 128), BF16),
        pltpu.VMEM((NT + 1, H * DH // NT, D), BF16),
        pltpu.VMEM((NT, 2, D, 128), BF16),
        pltpu.VMEM((NT, R0, 128), F32),
        pltpu.VMEM((2, R0 // 2, 128), U32),
        pltpu.VMEM((2, R0 // 2, 128), U32),
        pltpu.VMEM((D * CH // 2 + 32, 128), U32),
        pltpu.VMEM((M, D), BF16),
        pltpu.VMEM((D,), BF16),
        pltpu.VMEM((1, D), BF16),
        pltpu.SemaphoreType.DMA((7 + NSLOT + 2 * NT,)),
    )

    def main(wg_s, wu_s, wd_s, ybuf, stat, outs, sem_f):
        def load_x_rows(slot, seg):
            for k in range(NT):
                lhs[slot, k, 0:XR // 2, :] = hs[seg, k]

        def resid(seg, r, z=None):
            rows = pl.ds(r, 8)
            t = modv(2) * ybuf[seg, rows, :].astype(F32)
            if z is not None:
                t = t + jnp.concatenate([pltpu.bitcast(z, F32)] * NT, axis=1)
            return _rb(xbuf[seg, rows, :].astype(F32) + t)

        def wide(v):
            return jnp.concatenate([v] * NT, axis=1)

        def make_key(v, row0):
            b = pltpu.bitcast(jnp.where(v != v, -jnp.inf, v + 0.0), jnp.int32)
            low = (S - 1 - row0) - lax.broadcasted_iota(jnp.int32, (8, 128), 0)
            return (b ^ ((b >> 31) & 0x7FFF0000)) | low

        def score_dot(xc, mu, seg, rows):
            mb = _rb(mu)
            stat[0, seg, rows, :] = mb
            return jnp.sum(xc * modv(7), axis=-1, keepdims=True) + (mu - mb) * mod[8 * NT + 1]

        def post(st, ph, seg, r, z):
            zf = pltpu.bitcast(z, F32)
            if ph == 0:
                st["x1"] = resid(seg, r, z)
                st["mu"] = jnp.broadcast_to(jnp.mean(st["x1"], axis=-1, keepdims=True), (8, 128))
                return None
            if ph == 1:
                mu = st["mu"] + zf
                xc = st["xc"] = st["x1"] - wide(mu)
                st["var"] = jnp.mean(xc * xc, axis=-1, keepdims=True)
                st["dot"] = score_dot(xc, mu, seg, pl.ds(r, 8))
                return None
            inv = _inv_std(st["var"]) + zf
            stat[1, seg, pl.ds(r, 8), :] = inv
            v = _rb(inv * st["dot"] + mod[8 * NT])
            key = make_key(v, seg * SEG + r)
            m1, m2 = top[0:8, :], top[8:16, :]
            top[8:16, :] = jnp.maximum(m2, jnp.minimum(m1, key))
            top[0:8, :] = jnp.maximum(m1, key)
            o = st["x1"] + modv(5) * (st["xc"] * wide(inv) * modv(4) + modv(3))
            outs[seg, pl.ds(r, 8), :] = o.astype(BF16)
            res = pltpu.bitcast(v, U32)
            for k in range(NT):
                res = res | pltpu.bitcast(o[:, k * 128:(k + 1) * 128], U32)
            return res

        def redo(seg, r):
            x1 = resid(seg, r)
            d = _rb(x1 - wide(stat[0, seg, pl.ds(r, 8), :]))
            n = _rb(d * wide(stat[1, seg, pl.ds(r, 8), :]))
            return x1, _rb(_rb(n * modv(4)) + modv(3))

        def out_copy(g0, ng, r, n, k=0):
            return pltpu.make_async_copy(outs.at[pl.ds(g0, ng), pl.ds(r, n), :],
                                         out_hbm.at[pl.ds(g0, ng), pl.ds(r, n), :], sem_out.at[k])

        late = ((wg_hbm, wg_s, FF // 128), (wu_hbm, wu_s, FF // 128), (wd_hbm, wd_s, NT))

        def col_copy(k, j):
            return pltpu.make_async_copy(
                late[k][0].at[:, pl.ds(pl.multiple_of(j * 128, 128), 128)], late[k][1].at[j],
                sem_f.at[k])

        load_x_rows(0, 0)

        def step(it, cur, state):
            s = it * UNROLL + cur
            nxt = (cur + 1) % UNROLL

            def pay(t, cost):
                now, due = state["now"], state["due"]
                for z in [z for (d, z) in due if d <= now]:
                    t = jnp.concatenate([t[0:8] | z, t[8:]], axis=0)
                state["due"] = [(d, z) for (d, z) in due if d > now]
                state["now"] = now + cost
                return t

            def release(y):
                now = state["now"]
                pend, state["pend"] = state["pend"], [e for e in state["pend"] if e[0] > now]
                for (d, f) in pend:
                    if d <= now:
                        f(zero_after(y[0:8]))

            def lv(k0, k1):
                ts = [lhs[cur, k] for k in range(k0, k1)]
                ts[0] = pay(ts[0], (k1 - k0) / NT)
                return jnp.concatenate([_as_bf16(t) for t in ts], axis=1)

            def wmat(mat, h, q0, q1):
                return _as_bf16(jnp.concatenate([wqkv[3 * q + mat, h] for q in range(q0, q1)],
                                                axis=0))

            def qkv(p, split=False):
                part = {}
                if split:
                    for mat in range(3):
                        for a in range(2):
                            part[mat, a] = _dot(lv(0, NT // 2), wmat(mat, 2 * p + a, 0, 2))
                for mat in range(3):
                    for a in range(2):
                        hm = mat * H + 2 * p + a
                        if split:
                            y = _dot(lv(NT // 2, NT), wmat(mat, 2 * p + a, 2, 4)) + part[mat, a]
                        else:
                            y = _dot(lv(0, NT), wmat(mat, 2 * p + a, 0, 4))
                        cur_s[hm] = y.astype(BF16)
                        release(y)

            def gather(mat, p):
                hm = mat * H + 2 * p
                return jnp.concatenate(
                    [cur_s[hm], cur_s[hm + 1], pre[mat * NP + p, s].astype(BF16)], axis=0)

            probs = {}

            def scores(p):
                st = lax.dot_general(gather(1, p), gather(0, p), (((1,), (1,)), ((), ())),
                                     preferred_element_type=F32)
                lane = lax.broadcasted_iota(jnp.int32, (1, PR), 1)
                is_a = jnp.logical_or(lane < SEG,
                                      jnp.logical_and(lane >= 2 * SEG, lane < 2 * SEG + M))
                ka = jnp.concatenate([st[0:SEG], st[2 * SEG:2 * SEG + M]], axis=0)
                kb = jnp.concatenate([st[SEG:2 * SEG], st[2 * SEG + M:]], axis=0)
                t = jnp.where(is_a, ka, kb) * (SCALE * LOG2E)
                ts_s[p + (it >> 10)] = jnp.where(mk[0:SEG + M, :] == 0.0, t, NEG_MASK * LOG2E)

                def softmax(z):
                    zf = pltpu.bitcast(z, F32)[:, 0:PR]
                    t = (ts_s[p].reshape(-1, 8, PR) + zf).reshape(SEG + M, PR)
                    e = jnp.exp2(t - jnp.max(t, axis=0, keepdims=True))
                    e = e * _recip(jnp.sum(e, axis=0, keepdims=True))
                    pa = jnp.where(is_a, e, 0.0)
                    pb = jnp.where(is_a, 0.0, e)
                    probs[p] = jnp.concatenate(
                        [pa[0:SEG], pb[0:SEG], pa[SEG:], pb[SEG:]], axis=0).astype(BF16)

                state["pend"].append((state["now"] + REL_S + (p % PG) * REL_STAG, softmax))

            def pv(p):
                o = lax.dot_general(probs.pop(p), gather(2, p), (((0,), (0,)), ((), ())),
                                    preferred_element_type=F32).astype(BF16)
                for a in range(2):
                    h = 2 * p + a
                    olhs[h] = _as_u32(o[a * SEG:(a + 1) * SEG])
                    odef[h, it, cur * 4:(cur + 1) * 4, :] = _as_u32(
                        o[2 * SEG + a * M:2 * SEG + (a + 1) * M])

            acc = [None] * NT

            def oproj(j, pairs):
                ts = [olhs[2 * p + a] for p in pairs for a in range(2)]
                ts[0] = pay(ts[0], len(pairs) / 4)
                ov = jnp.concatenate([_as_bf16(t) for t in ts], axis=1)
                w = wo_s[j, pairs[0] * DH:(pairs[-1] + 1) * DH, :]
                y = _dot(ov, _as_bf16(w))
                acc[j] = y if acc[j] is None else y + acc[j]
                release(acc[j])

            def fin(j):
                yb = acc[j].astype(BF16)
                ybuf[s, 0:XR, j * 128:(j + 1) * 128] = yb[0:XR]
                lhs[nxt, j, XR // 2:, :] = _as_u32(yb[XR:])

            def gemv():
                d0 = state["d0"]
                state["acc"] = gemv_part(wm_s[it & 3, :, d0:d0 + GR, :], d0, state["acc"])
                state["d0"] = d0 + GR
                au = pltpu.bitcast(state["acc"], U32)
                z = functools.reduce(lambda a, b: a | b, [au[u] for u in range(mt)])
                state["due"].append((state["now"] + G_LAG, zero_after(z)))

            load_x_rows(nxt, jnp.minimum(s + 1, NSEG - 1))
            ops = dict(Q=qkv, S=scores, P=pv, O=oproj, F=fin, G=gemv)
            for op in _schedule():
                ops[op[0]](*op[1:])

        def steps(it, carry):
            pltpu.make_async_copy(wm_s.at[it & 3], wm_s.at[it & 3], sem_m.at[it & 3]).wait()

            @pl.when(it + 2 < NSEG // UNROLL)
            def _():
                for u in range(mt):
                    wm_copy(it + 2, u).start()

            for u in range(UNROLL // 2):
                t = it * (UNROLL // 2) + u
                for k in range(3):
                    @pl.when(t < late[k][2])
                    def _():
                        col_copy(k, t).start()

            state = dict(now=0, due=[], pend=[], d0=0, acc=None)
            for u in range(UNROLL):
                step(it, u, state)
            acc = state["acc"]
            for d0 in range(state["d0"], D, 64):
                acc = gemv_part(wm_s[it & 3, :, d0:min(d0 + 64, D), :], d0, acc)
            gemv_finish(acc, [2 * NT + it * mt + u for u in range(mt)])
            return carry

        lax.fori_loop(0, NSEG // UNROLL, steps, 0)
        for k in range(3):
            for j in range(late[k][2]):
                col_copy(k, j).wait()

        ntail = EBLK[-1] // M
        ppi = (S // 8 - ntail) // NEC
        gpi = ppi // (XR // 8)
        gb_ = UNROLL * M

        def ep_body(i, c):
            @pl.when(i > 0)
            def _():
                out_copy((i - 1) * gpi, gpi, 0, XR).start()

            for k in range(NT):
                mod[7 * NT + k] = mod[4 * NT + k] * mod[6 * NT + k]
            mod[8 * NT] = jnp.broadcast_to(
                jnp.sum(modv(3) * modv(6), axis=-1, keepdims=True), (M, 128))
            mod[8 * NT + 1] = jnp.broadcast_to(
                jnp.sum(modv(7), axis=-1, keepdims=True), (M, 128))

            nrel = NT * H // EKH * EC // 32
            jobs = {}
            for ph in range(3):
                _spread(jobs, [(u, ph) for u in range(ppi)], E_PH[ph],
                        nrel - E_SPAN - E_PH[2] + E_PH[ph])
            sts = [{} for _ in range(ppi)]
            due = []
            n = 0
            r0 = 0
            for nr in EBLK:
                for j in range(NT):
                    for h0_ in range(0, H, EKH):
                        blk = pl.ds(i * (EC // gb_) + r0 // gb_, nr // gb_)
                        ts = [odef[h, blk].reshape(nr // 2, DH) for h in range(h0_, h0_ + EKH)]
                        for z in [z for (d, z) in due if d <= n]:
                            ts[0] = jnp.concatenate([ts[0][0:8] | z, ts[0][8:]], axis=0)
                        due = [(d, z) for (d, z) in due if d > n]
                        w = wo_s[j, h0_ * DH // 2:(h0_ + EKH) * DH // 2, :]
                        yp = _dot(jnp.concatenate([_as_bf16(t) for t in ts], axis=1), _as_bf16(w))
                        y = yp if h0_ == 0 else yp + y
                        if h0_ + EKH == H:
                            segs = pl.ds(i * (EC // M) + r0 // M, nr // M)
                            ybuf[segs, XR:, j * 128:(j + 1) * 128] = (
                                y.reshape(nr // M, M, 128).astype(BF16))
                        for q in range(nr // 32):
                            for (u, ph) in jobs.get(n + q, ()):
                                assert (u - ppi + (EC - EBLK[-1]) // M) * M < r0
                                t = i * ppi + u
                                early = t < NSEG * (XR // 8)
                                seg = jnp.where(early, t // (XR // 8), t - NSEG * (XR // 8))
                                row = pl.multiple_of(
                                    jnp.where(early, (t % (XR // 8)) * 8, XR), 8)
                                res = post(sts[u], ph, seg, row, zero_after(y[q * 32:q * 32 + 8]))
                                if res is not None:
                                    due.append((n + E_SPAN, zero_after(res)))
                        n += nr // 32
                r0 += nr
            return c

        lax.fori_loop(0, NEC, ep_body, 0)
        done = (NEC - 1) * gpi
        tail = NSEG - ntail
        out_copy(done, NSEG - done, 0, XR).start()
        out_copy(0, tail, XR, M).start()
        x1s = [resid(g, XR) for g in range(tail, NSEG)]
        mus = [jnp.mean(x1, axis=-1, keepdims=True) for x1 in x1s]
        pairs = [(top[0:8, :], top[8:16, :])]
        lowest = jnp.full((8, 128), jnp.iinfo(jnp.int32).min, jnp.int32)
        for g in range(tail, NSEG):
            xc = x1s[g - tail] - mus[g - tail]
            inv = _inv_std(jnp.mean(xc * xc, axis=-1, keepdims=True))
            stat[1, g, XR:, :] = jnp.broadcast_to(inv, (8, 128))
            dot = score_dot(xc, jnp.broadcast_to(mus[g - tail], (8, 128)), g, pl.ds(XR, 8))
            v = _rb(inv * dot + mod[8 * NT])
            pairs.append((make_key(v, g * SEG + XR), lowest))
        while len(pairs) > 1:
            (a1, a2), (c1, c2) = pairs.pop(0), pairs.pop(0)
            pairs.append((jnp.maximum(a1, c1),
                          jnp.maximum(jnp.minimum(a1, c1), jnp.maximum(a2, c2))))

        tk = jnp.concatenate(pairs[0], axis=0)[:, 0:1]
        k1 = jnp.max(tk[0:8], axis=0, keepdims=True)
        k2 = jnp.max(jnp.where(tk == k1, jnp.iinfo(jnp.int32).min, tk), axis=0, keepdims=True)
        i1 = (S - 1) - (k1[0, 0] & (S - 1))
        i2 = (S - 1) - (k2[0, 0] & (S - 1))
        g1, g2 = i1 >> 5, i2 >> 5
        b1 = pl.multiple_of(i1 & 24, 8)
        b2 = pl.multiple_of(i2 & 24, 8)

        def tail_out(n, z):
            g, k0 = tail + n // (NT // TW), (n % (NT // TW)) * TW
            zf = pltpu.bitcast(z, F32)
            for k in range(k0, k0 + TW, 2):
                cols = slice(k * 128, (k + 2) * 128)
                m = lambda j: jnp.concatenate([mod[j * NT + k], mod[j * NT + k + 1]], axis=1)
                two = lambda v: jnp.concatenate([v, v], axis=1)
                x1_ = (xbuf[g, XR:, cols].astype(F32)
                       + (m(2) * ybuf[g, XR:, cols].astype(F32) + two(zf)))
                h_ = (x1_ - two(stat[0, g, XR:, :])) * two(stat[1, g, XR:, :]) * m(4) + m(3)
                outs[g, XR:, cols] = (x1_ + m(5) * h_).astype(BF16)

        xa, ha_ = redo(g1, b1)
        xb_, hb_ = redo(g2, b2)
        x1 = jnp.concatenate([xa, xb_], axis=0)
        h2 = jnp.concatenate([ha_, hb_], axis=0)
        h2b = h2.astype(BF16)
        row = lax.broadcasted_iota(jnp.int32, (16, 1), 0)
        grow = jnp.where(row < 8, g1 * SEG + b1 + row, g2 * SEG + b2 + row - 8)
        ks = jnp.where(grow == i1, k1, k2)
        rsel = pltpu.bitcast((ks ^ ((ks >> 31) & 0x7FFF0000)) & -65536, F32)
        acts = []
        jobs = {}
        _spread(jobs, list(range(ntail * NT // TW)), 0, T_END)
        for j in range(FF // 128):
            gt = _rb(_dot(h2b, wg_s[j]))
            for n in jobs.get(2 * j, ()):
                tail_out(n, zero_after(gt[0:8]))
            gt = _rb(gt * _rb(jax.nn.sigmoid(gt)))
            ut = _rb(_dot(h2b, wu_s[j]))
            for n in jobs.get(2 * j + 1, ()):
                tail_out(n, zero_after(ut[0:8]))
            acts.append((gt * ut).astype(BF16))
        out_copy(tail, NSEG - tail, XR, M).start()
        act = jnp.concatenate(acts, axis=1)
        y = _rb(jnp.concatenate([_dot(act, wd_s[j]) for j in range(NT)], axis=1))
        y = _rb(y * _rb(jax.nn.sigmoid(rsel)))
        sel = jnp.logical_or(grow == i1, grow == i2)
        gb2 = jnp.concatenate([modv(5)] * 2, axis=0)
        fixed = (x1 + gb2 * (h2 + jnp.where(sel, y, 0.0))).astype(BF16)

        out_copy(0, NSEG, 0, SEG).wait()
        outs[g1, pl.ds(b1, 8), :] = fixed[0:8]
        outs[g2, pl.ds(b2, 8), :] = fixed[8:16]
        out_copy(g1, 1, b1, 8, 0).start()

        @pl.when((i1 >> 3) != (i2 >> 3))
        def _():
            out_copy(g2, 1, b2, 8, 1).start()
            out_copy(g2, 1, b2, 8, 1).wait()

        out_copy(g1, 1, b1, 8, 0).wait()

    pl.run_scoped(
        main,
        pltpu.VMEM((FF // 128, D, 128), BF16),
        pltpu.VMEM((FF // 128, D, 128), BF16),
        pltpu.VMEM((NT, FF, 128), BF16),
        pltpu.VMEM((NSEG, SEG, D), BF16),
        pltpu.VMEM((2, NSEG, SEG, 128), F32),
        pltpu.VMEM((NSEG, SEG, D), BF16),
        pltpu.SemaphoreType.DMA((3,)),
    )


def _entry(*refs):
    pl.run_scoped(
        functools.partial(_kernel, *refs),
        pltpu.VMEM((NCHUNK, H, KQ // 2, DH), U32),
        pltpu.VMEM((NSEG + 1, NT, XR // 2, 128), U32),
        pltpu.VMEM((NT, (H * DH + H * DH // NT) // 2, 128), U32),
        pltpu.VMEM((3 * NP, NSEG, 2 * M, DH), F32),
        pltpu.VMEM((3 * H, SEG, DH), BF16),
        pltpu.VMEM((H, SEG // 2, DH), U32),
        pltpu.VMEM((H, NSEG // UNROLL, UNROLL * M // 2, DH), U32),
        pltpu.VMEM((NSEG, SEG, D), BF16),
        pltpu.VMEM((UNROLL, NT, SEG // 2, 128), U32),
        pltpu.VMEM((4, 4 * NT * UNROLL // NSEG, D, 128), BF16),
        pltpu.VMEM((8 * NT + 4, M, 128), F32),
        pltpu.VMEM((64, PR), F32),
        pltpu.VMEM((32, 128), jnp.int32),
        pltpu.VMEM((M, D), BF16),
        pltpu.VMEM((D, 128), F32),
        pltpu.VMEM((NP, SEG + M, PR), F32),
        pltpu.VMEM((8 + PAD, 128), U32),
        pltpu.SemaphoreType.DMA((4,)),
        pltpu.SemaphoreType.DMA((2,)),
    )


@functools.partial(jax.jit, static_argnames=("A_seg_len",))
def pallas_adaLN_cond__memory_aug_recurrent_mem_tr__moe_arch_mod__prompt_kernel(
    A_x: jax.Array,
    A_mem0: jax.Array,
    A_Wq: jax.Array,
    A_Wk: jax.Array,
    A_Wv: jax.Array,
    A_Wo: jax.Array,
    A_seg_len,
    B_x: jax.Array,
    B_w_r: jax.Array,
    B_w_gate: jax.Array,
    B_w_up: jax.Array,
    B_w_down: jax.Array,
    c: jax.Array,
    w_mod: jax.Array,
):
    assert A_seg_len == SEG and A_x.shape == (1, S, D)
    del B_x
    hbm = pl.BlockSpec(memory_space=pl.ANY)
    out = pl.pallas_call(
        _entry,
        out_shape=jax.ShapeDtypeStruct((NSEG, SEG, D), BF16),
        in_specs=[hbm] * 12,
        out_specs=hbm,
        compiler_params=pltpu.CompilerParams(vmem_limit_bytes=120 * 1024 * 1024,
                                             disable_bounds_checks=True),
    )(A_x.reshape(NSEG, SEG, D), A_mem0.reshape(M, D), A_Wq, A_Wk, A_Wv, A_Wo.reshape(H * DH, D),
      B_w_r, B_w_gate, B_w_up, B_w_down, c, w_mod)
    return out.reshape(1, S, D)
```
